```python
import jax
import jax.numpy as jnp

def _softmax(x, axis=-1):
    return jax.nn.softmax(x, axis=axis)
def _gelu(x):
    return jax.nn.gelu(x, approximate=True)
def _silu(x):
    return jax.nn.silu(x)
def _sigmoid(x):
    return jax.nn.sigmoid(x)
def _layernorm(x, axis=-1, eps=1e-5):
    m = jnp.mean(x, axis=axis, keepdims=True)
    v = jnp.var(x, axis=axis, keepdims=True)
    return (x - m) / jnp.sqrt(v + eps)
def _scatter_add(tgt, idx, src, axis=0):
    return tgt.at[idx].add(src)
def _segment_sum(src, seg, n):
    return jax.ops.segment_sum(src, seg, n)
class _Rng:
    def __init__(self, key):
        self._k = key
    def _next(self):
        self._k, sub = jax.random.split(self._k)
        return sub
    def normal(self, shape):
        return jax.random.normal(self._next(), shape, dtype=jnp.bfloat16)
    def randint(self, lo, hi, shape):
        return jax.random.randint(self._next(), shape, lo, hi, dtype=jnp.int32)
    def uniform(self, shape, lo=0.0, hi=1.0):
        return jax.random.uniform(self._next(), shape, jnp.bfloat16, lo, hi)
    def permutation(self, n):
        return jax.random.permutation(self._next(), n)


kernel_name = 'concat_heads__sliding_local_dilated__compressed_kv_cla__prompt'

def setup_inputs():
    _rng = _Rng(jax.random.key(int.from_bytes(__import__("os").urandom(4), "little")))
    _w = (lambda a: (lambda t: t.astype(jnp.bfloat16) if jnp.issubdtype(t.dtype, jnp.floating) else t)(jnp.asarray(a)))
    def _A_setup():
        B, S, D = 1, 2048, 1024
        return {
            "x": _w((lambda *s: _rng.normal(s) * 0.05)(B, S, D)),
            "wqkv": _w((lambda *s: _rng.normal(s) * 0.05)(D, 3 * D)),
            "wo": _w((lambda *s: _rng.normal(s) * 0.05)(D, D)),
        }
    _A_in = _A_setup()

    def _B_setup():
        B, H, Sq, Sk, D, M = 1, 32, 2048, 2048, 128, 1024
        Dc = 4 * D
        return {
            "x": _w((lambda *s: _rng.normal(s) * 0.05)(B, Sq, M)),
            "c_kv": _w((lambda *s: _rng.normal(s) * 0.05)(B, Sk, Dc)),
            "w_q": _w((lambda *s: _rng.normal(s) * 0.05)(M, H, D) * (M ** -0.5)),
            "w_uk": _w((lambda *s: _rng.normal(s) * 0.05)(Dc, H, D) * (Dc ** -0.5)),
            "w_uv": _w((lambda *s: _rng.normal(s) * 0.05)(Dc, H, D) * (Dc ** -0.5)),
            "w_o": _w((lambda *s: _rng.normal(s) * 0.05)(H, D, M) * ((H * D) ** -0.5)),
        }
    _B_in = _B_setup()

    return {
        "A_x": _A_in["x"],
        "A_wqkv": _A_in["wqkv"],
        "A_wo": _A_in["wo"],
        "B_x": _B_in["x"],
        "B_c_kv": _B_in["c_kv"],
        "B_w_q": _B_in["w_q"],
        "B_w_uk": _B_in["w_uk"],
        "B_w_uv": _B_in["w_uv"],
        "B_w_o": _B_in["w_o"],
    }

def reference(A_x, A_wqkv, A_wo, B_x, B_c_kv, B_w_q, B_w_uk, B_w_uv, B_w_o):
    def _A_ref(x, wqkv, wo):
        B, S, D = x.shape
        H = 32; Dh = D // H
        W, dil = 8, 2
        qkv = (lambda x, *d: x.transpose(*d))((x @ wqkv).reshape(B, S, 3, H, Dh), 2, 0, 3, 1, 4)
        q, k, v = qkv[0], qkv[1], qkv[2]
        scale = Dh ** -0.5
        pos = jnp.arange(S)
        off = jnp.arange(W) * dil
        idx = pos[:, None] - off[None, :]
        mask = idx >= 0
        idx_c = jnp.where(mask, idx, 0).reshape(-1)
        kg = k[:, :, idx_c, :].reshape(B, H, S, W, Dh)
        vg = v[:, :, idx_c, :].reshape(B, H, S, W, Dh)
        logits = jnp.einsum("bhsd,bhswd->bhsw", q, kg) * scale
        logits = jnp.where(mask[None, None, :, :], logits, -1e9)
        attn = _softmax(logits, axis=-1)
        o = jnp.einsum("bhsw,bhswd->bhsd", attn, vg)
        return (lambda x, *d: x.transpose(*d))(o, 0, 2, 1, 3).reshape(B, S, D) @ wo

    def _B_ref(x, c_kv, w_q, w_uk, w_uv, w_o):
        B, Sq, M = x.shape[0], x.shape[1], x.shape[2]
        Sk = c_kv.shape[1]
        H, D = w_q.shape[1], w_q.shape[2]
        q = jnp.einsum("bqm,mhd->bhqd", x, w_q)
        k = jnp.einsum("bkc,chd->bhkd", c_kv, w_uk)
        v = jnp.einsum("bkc,chd->bhkd", c_kv, w_uv)
        scores = jnp.einsum("bhqd,bhkd->bhqk", q, k) * (D ** -0.5)
        off = Sk - Sq
        qi = jnp.arange(Sq)[:, None]
        kj = jnp.arange(Sk)[None, :]
        cmask = kj <= (qi + off)
        scores = jnp.where(cmask[None, None], scores, -1e9)
        p = _softmax(scores, axis=-1)
        ctx = jnp.einsum("bhqk,bhkd->bhqd", p, v)
        return jnp.einsum("bhqd,hdm->bqm", ctx, w_o)

    a = _A_ref(A_x, A_wqkv, A_wo)
    b = _B_ref(B_x, B_c_kv, B_w_q, B_w_uk, B_w_uv, B_w_o)
    return jnp.concatenate([a, b], axis=-1)
```

```python
import math

import jax
import jax.numpy as jnp
from jax import lax
import jax.experimental.pallas as pl
import jax.experimental.pallas.tpu as pltpu

F32, BF16, U32 = jnp.float32, jnp.bfloat16, jnp.uint32

S = 2048
DM = 1024
DC = 512
NH = 32
HD = 128
AD = 32
WIN, DIL = 8, 2

R = 128
CH = 2 * R
NC = S // CH
NP = NH // 2
HALO = 16
PITCH = 33

LOG2E = math.log2(math.e)
MASKED = -1e9 * LOG2E

NN = (((1,), (0,)), ((), ()))
NT = (((1,), (1,)), ((), ()))


_STRASSEN = dict(
    lhs=(((0, 1), (3, 1)), ((2, 1), (3, 1)), ((0, 1),), ((3, 1),),
         ((0, 1), (1, 1)), ((2, 1), (0, -1)), ((1, 1), (3, -1))),
    rhs=(((0, 1), (3, 1)), ((0, 1),), ((1, 1), (3, -1)), ((2, 1), (0, -1)),
         ((3, 1),), ((0, 1), (1, 1)), ((2, 1), (3, 1))),
    prods=((0, 0, ((0, 1), (3, 1))), (1, 1, ((2, 1), (3, -1))),
           (2, 2, ((1, 1), (3, 1))), (3, 3, ((0, 1), (2, 1))),
           (4, 4, ((0, -1), (1, 1))), (5, 5, ((3, 1),)), (6, 6, ((0, 1),))),
)
_PLAIN = dict(
    lhs=(((0, 1),), ((1, 1),), ((2, 1),), ((3, 1),)),
    rhs=(((0, 1),), ((1, 1),), ((2, 1),), ((3, 1),)),
    prods=((0, 0, ((0, 1),)), (1, 2, ((0, 1),)), (0, 1, ((1, 1),)),
           (1, 3, ((1, 1),)), (2, 0, ((2, 1),)), (3, 2, ((2, 1),)),
           (2, 1, ((3, 1),)), (3, 3, ((3, 1),))),
)
SCHEME = _STRASSEN
NOPS = len(SCHEME["lhs"])
NPROD = len(SCHEME["prods"])


def _combine(blocks, terms):
    out = None
    for i, sign in terms:
        if out is None:
            out = blocks[i] if sign > 0 else -blocks[i]
        else:
            out = out + blocks[i] if sign > 0 else out - blocks[i]
    return out


def _pack(x):
    return pltpu.bitcast(x.astype(BF16), U32)


def _bf16(words):
    return pltpu.bitcast(words, BF16)


def _halves(words):
    lo = pltpu.bitcast(words << 16, F32)
    hi = pltpu.bitcast(words & jnp.uint32(0xFFFF0000), F32)
    return lo, hi


def _recip(x):
    r = pltpu.reciprocal(x, approx=True)
    return r * (2.0 - x * r)


class _BlockProduct:
    def __init__(self, lhs, rhs, done, dims=NN, init=None):
        self.lhs, self.rhs, self.done, self.dims = lhs, rhs, done, dims
        self.init = init
        self.c = [None] * 4
        self.n = 0

    def step(self):
        ia, ib, outs = SCHEME["prods"][self.n]
        m = lax.dot_general(self.lhs(ia), self.rhs(ib), self.dims,
                            preferred_element_type=F32)
        for o, sign in outs:
            if self.c[o] is None and self.init is not None:
                self.c[o] = self.init(o)
            if self.c[o] is None:
                self.c[o] = m if sign > 0 else -m
            else:
                self.c[o] = self.c[o] + m if sign > 0 else self.c[o] - m
        self.n += 1
        later = {o for _, _, os in SCHEME["prods"][self.n:] for o, _ in os}
        for o, _ in outs:
            if o not in later:
                self.done(o, self.c[o])

    def steps(self):
        return [self.step] * NPROD


def _kernel(ax_hbm, awqkv_hbm, awo_hbm, bx_hbm, c_hbm, wq_hbm, wuk_hbm, wuv_hbm,
            wo_hbm, out_hbm,
            xs, cs, xop, cop, wq_raw, wuk_raw, wuv_raw, wo_raw,
            wqop, wkvop, woop, q_s, k_s, v_s, acc,
            aw_raw, shuf, awop, xa, awo_raw, awoop, xaop, aq, ak, av, ao,
            aoop, a_out,
            sem_x, sem_c, sem_w, sem_aw, sem_a, sem_out):
    wq32 = wq_hbm.bitcast(U32)
    wuk32 = wuk_hbm.bitcast(U32)
    wuv32 = wuv_hbm.bitcast(U32)

    def cp_x(c):
        rows = pl.ds(c * CH, CH)
        return pltpu.make_async_copy(bx_hbm.at[rows], xs.at[rows], sem_x.at[c])

    def cp_c(c):
        rows = pl.ds(c * CH, CH)
        return pltpu.make_async_copy(c_hbm.at[rows], cs.at[rows], sem_c.at[c])

    def cp_proj_w(j):
        s = j % 2
        return [
            pltpu.make_async_copy(wuk32.at[:, j, :], wuk_raw.at[s], sem_w.at[s]),
            pltpu.make_async_copy(wuv32.at[:, j, :], wuv_raw.at[s], sem_w.at[2 + s]),
            pltpu.make_async_copy(wq32.at[:, j, :], wq_raw.at[s], sem_w.at[4 + s]),
        ]

    def cp_wo(j):
        s = j % 2
        rows = pl.ds(pl.multiple_of(j * 2 * HD, 2 * HD), 2 * HD)
        return pltpu.make_async_copy(wo_hbm.at[rows], wo_raw.at[s], sem_w.at[6 + s])

    def cp_aw(u):
        s = u % 2
        cols = pl.ds(pl.multiple_of((u // 4) * DM, DM), DM)
        return [
            pltpu.make_async_copy(
                awqkv_hbm.at[pl.ds(pl.multiple_of((u % 4) * 128 + half * (DM // 2), 128), 128), cols],
                aw_raw.at[s, half], sem_aw.at[2 * s + half])
            for half in range(2)
        ]

    def cp_xa():
        return pltpu.make_async_copy(ax_hbm, xa, sem_a.at[0])

    def cp_awo():
        return pltpu.make_async_copy(awo_hbm, awo_raw, sem_a.at[1])

    def cp_out_b(c):
        rows = pl.ds(c * CH, CH)
        return pltpu.make_async_copy(
            xs.at[rows], out_hbm.at[rows, pl.ds(DM, DM)], sem_out.at[c])

    def cp_out_a(c):
        rows = pl.ds(pl.multiple_of(c * CH, CH), CH)
        return pltpu.make_async_copy(
            a_out.at[rows], out_hbm.at[rows, pl.ds(0, DM)], sem_out.at[NC + c])

    def lhs_ops(x, store):
        m = x.shape[1] // 2
        blocks = [x[:R, :m], x[:R, m:], x[R:, :m], x[R:, m:]]
        for i, terms in enumerate(SCHEME["lhs"]):
            store(i, _pack(_combine(blocks, terms)))

    def prep_x(c):
        def store(i, v):
            xop[i, c] = v
        lhs_ops(xs[pl.ds(c * CH, CH), :].astype(F32), store)

    def prep_c(c):
        def store(i, v):
            cop[i, c] = v
        lhs_ops(cs[pl.ds(c * CH, CH), :].astype(F32), store)

    def prep_wq(s):
        top, bot = _halves(wq_raw[s, :DM // 2]), _halves(wq_raw[s, DM // 2:])
        blocks = [*top, *bot]
        for i, terms in enumerate(SCHEME["rhs"]):
            wqop[i] = _pack(_combine(blocks, terms))

    def prep_wkv(s):
        for n, raw in enumerate((wuk_raw, wuv_raw)):
            top, bot = _halves(raw[s, :DC // 2]), _halves(raw[s, DC // 2:])
            blocks = [*top, *bot]
            for i, terms in enumerate(SCHEME["rhs"]):
                wkvop[i, :, n * HD:(n + 1) * HD] = _pack(_combine(blocks, terms))

    def prep_wo(s):
        w = wo_raw[s].astype(F32)
        m = DM // 2
        blocks = [w[:HD, :m], w[:HD, m:], w[HD:, :m], w[HD:, m:]]
        for i, terms in enumerate(SCHEME["rhs"]):
            woop[i] = _pack(_combine(blocks, terms))

    def dim_major(piece):
        for u in range(NH * AD // 128):
            t = piece(u)
            for h in range(128 // AD):
                shuf[pl.ds((4 * u + h) * PITCH, AD), :] = t[h * AD:(h + 1) * AD]
        rows = [shuf[pl.ds(d, NH, stride=PITCH), :] for d in range(AD)]
        return (jnp.concatenate(rows[:AD // 2], axis=0),
                jnp.concatenate(rows[AD // 2:], axis=0))

    def prep_aw(u, s):
        blocks = []
        for half in range(2):
            w = aw_raw[s, half].astype(F32)
            blocks += dim_major(lambda t: w[:, 128 * t:128 * (t + 1)].T)
        for i, terms in enumerate(SCHEME["rhs"]):
            awop[u, i] = _pack(_combine(blocks, terms))

    def prep_awo(n):
        cols = [dim_major(
            lambda t: awo_raw[128 * t:128 * (t + 1), c0:c0 + 128].astype(F32))
            for c0 in (128 * n, DM // 2 + 128 * n)]
        blocks = [cols[0][0], cols[1][0], cols[0][1], cols[1][1]]
        for i, terms in enumerate(SCHEME["rhs"]):
            awoop[i, :, 128 * n:128 * (n + 1)] = _pack(_combine(blocks, terms))

    def prep_xa(c):
        def store(i, v):
            xaop[i] = v
        rows = pl.ds(pl.multiple_of(c * CH, CH), CH)
        lhs_ops(xa[rows, :].astype(F32), store)

    def words(blk):
        return pl.ds(blk * (R // 2), R // 2)

    def q_proj(c):
        def done(o, val):
            q_s[o % 2, words(2 * c + o // 2), :] = _pack(val * (HD ** -0.5 * LOG2E))
        return _BlockProduct(lambda i: _bf16(xop[i, c]),
                             lambda i: _bf16(wqop[i]), done).steps()

    def kv_proj(c):
        def done(o, val):
            k_s[o % 2, words(2 * c + o // 2), :] = _pack(val[:, :HD])
            v_s[o % 2, words(2 * c + o // 2), :] = _pack(val[:, HD:])
        return _BlockProduct(lambda i: _bf16(cop[i, c]),
                             lambda i: _bf16(wkvop[i]), done).steps()

    def o_proj(c, ctx, last):
        def where(o):
            return (pl.ds((2 * c + o // 2) * R, R), pl.ds((o % 2) * (DM // 2), DM // 2))

        def done(o, val):
            if last:
                xs[where(o)] = val.astype(BF16)
            else:
                acc[where(o)] = val
        steps = _BlockProduct(
            lambda i: _combine(ctx, SCHEME["lhs"][i]).astype(BF16),
            lambda i: _bf16(woop[i]), done, init=lambda o: acc[where(o)]).steps()
        if last:
            steps = steps + [lambda: cp_out_b(c).start()]
        return steps

    def scores(h, blk):
        n = (blk + 1) * R
        s = lax.dot_general(_bf16(q_s[h, words(blk), :]), _bf16(k_s[h, :n // 2, :]),
                            NT, preferred_element_type=F32)
        row = lax.broadcasted_iota(jnp.int32, (R, R), 0)
        col = lax.broadcasted_iota(jnp.int32, (R, R), 1)
        diag = jnp.where(col <= row, s[:, n - R:], MASKED)
        return diag if blk == 0 else jnp.concatenate([s[:, :n - R], diag], axis=1)

    def attend(h, blk, s):
        n = (blk + 1) * R
        p = jnp.exp2(s - jnp.max(s, axis=1, keepdims=True))
        inv = _recip(jnp.sum(p, axis=1, keepdims=True))
        o = lax.dot_general(p.astype(BF16), _bf16(v_s[h, :n // 2, :]), NN,
                            preferred_element_type=F32)
        return o * inv

    def run(steps, n):
        for _ in range(min(n, len(steps))):
            steps.pop(0)()

    def pair_attention(last, filler):
        todo = []
        for c in reversed(range(NC)):
            hi, lo = 2 * c + 1, 2 * c
            per = -(-len(todo) // 5)
            s0 = scores(0, hi)
            run(todo, per)
            s1 = scores(1, hi)
            run(todo, per)
            o0h = attend(0, hi, s0)
            s2 = scores(0, lo)
            run(todo, per)
            o1h = attend(1, hi, s1)
            s3 = scores(1, lo)
            run(todo, per)
            o0l = attend(0, lo, s2)
            run(todo, len(todo))
            o1l = attend(1, lo, s3)
            extra = filler(c)
            todo = extra[:NPROD] + o_proj(c, [o0l, o1l, o0h, o1h], last) + extra[NPROD:]
        run(todo, len(todo))

    def a_proj(part):
        steps = []
        for t in range(4):
            def done(o, val, t=t):
                tile, r0 = t + 4 * (o % 2), (o // 2) * R
                if part == 0:
                    aq[tile, pl.ds(r0, R), :] = val * (AD ** -0.5 * LOG2E)
                else:
                    (ak, av)[part - 1][tile, pl.ds(HALO + r0, R), :] = val

            def rhs(i, t=t):
                return _bf16(jnp.concatenate(
                    [awop[4 * part + m, i, pl.ds(64 * t, 64), :] for m in range(4)],
                    axis=1))
            steps += _BlockProduct(lambda i: _bf16(xaop[i]), rhs, done, dims=NT).steps()
        return steps

    SLAB = 32

    def a_weights(c, r0):
        logits = []
        for w in range(WIN):
            tot = None
            for t in range(8):
                pr = aq[t, pl.ds(r0, SLAB), :] * ak[t, pl.ds(HALO + r0 - DIL * w, SLAB), :]
                tot = pr if tot is None else tot + pr
            logits.append(tot)
        logits = [x + pltpu.roll(x, 64, 1) for x in logits]
        logits = [x + pltpu.roll(x, 32, 1) for x in logits]
        if r0 < (WIN - 1) * DIL:
            pos = c * CH + r0 + lax.broadcasted_iota(jnp.int32, (SLAB, 128), 0)
            logits = [x if w == 0 else jnp.where(pos >= DIL * w, x, MASKED)
                      for w, x in enumerate(logits)]
        top = logits[0]
        for x in logits[1:]:
            top = jnp.maximum(top, x)
        e = [jnp.exp2(x - top) for x in logits]
        tot = e[0]
        for x in e[1:]:
            tot = tot + x
        inv = _recip(tot)
        return [x * inv for x in e]

    def a_mix(r0, p):
        for t in range(8):
            tot = None
            for w in range(WIN):
                pr = p[w] * av[t, pl.ds(HALO + r0 - DIL * w, SLAB), :]
                tot = pr if tot is None else tot + pr
            ao[t, pl.ds(r0, SLAB), :] = tot

    def prep_ao():
        def store(i, v):
            aoop[i] = v
        lhs_ops(jnp.concatenate([ao[t] for t in range(8)], axis=1), store)

    def a_out_proj(c):
        def done(o, val):
            rows = pl.ds(pl.multiple_of(c * CH + (o // 2) * R, R), R)
            a_out[rows, pl.ds((o % 2) * (DM // 2), DM // 2)] = val.astype(BF16)
        return _BlockProduct(lambda i: _bf16(aoop[i]),
                             lambda i: _bf16(awoop[i]), done).steps()

    def a_attention(c, v_steps, out_steps):
        slabs = list(range(0, CH, SLAB))
        ps = []
        per = -(-len(v_steps) // len(slabs))
        for r0 in slabs:
            run(v_steps, per)
            ps.append(a_weights(c, r0))
        per = -(-len(out_steps) // len(slabs))
        for r0, p in zip(slabs, ps):
            run(out_steps, per)
            a_mix(r0, p)
        for buf in (ak, av):
            buf[:, :HALO, :] = buf[:, CH:, :]

    order = list(reversed(range(NC)))
    first_w = cp_proj_w(0)
    cp_c(order[0]).start()
    first_w[0].start()
    first_w[1].start()
    for c in order[1:]:
        cp_c(c).start()
    first_w[2].start()
    for c in order:
        cp_x(c).start()
    cp_wo(0).start()
    for cp in cp_proj_w(1) + cp_aw(0):
        cp.start()
    cp_xa().start()
    cp_awo().start()

    acc[...] = jnp.zeros(acc.shape, F32)
    for buf in (ak, av):
        buf[:, :HALO, :] = jnp.zeros((8, HALO, 128), F32)
    first_w[0].wait()
    first_w[1].wait()
    prep_wkv(0)
    for c in order:
        cp_c(c).wait()
        prep_c(c)
        run(kv_proj(c), NPROD)
    first_w[2].wait()
    prep_wq(0)
    for c in order:
        cp_x(c).wait()
        prep_x(c)
        run(q_proj(c), NPROD)

    n_units = 12

    def pair_step(j, carry):
        for cp in cp_proj_w(j + 1):
            cp.wait()
        cp_wo(j).wait()
        cp_wo(j + 1).start()

        @pl.when(j + 2 < NP)
        def _():
            for cp in cp_proj_w(j + 2):
                cp.start()

        @pl.when(j < n_units)
        def _():
            for cp in cp_aw(j):
                cp.wait()

        @pl.when(j + 1 < n_units)
        def _():
            for cp in cp_aw(j + 1):
                cp.start()

        prep_wo(j % 2)
        prep_wq((j + 1) % 2)
        prep_wkv((j + 1) % 2)
        u = jnp.minimum(j, n_units - 1)
        prep_aw(u, u % 2)
        pair_attention(False, lambda c: q_proj(c) + kv_proj(c))
        return carry

    lax.fori_loop(0, NP - 1, pair_step, 0)

    cp_wo(NP - 1).wait()
    cp_xa().wait()
    cp_awo().wait()
    prep_wo((NP - 1) % 2)
    prep_xa(0)
    for n in range(4):
        prep_awo(n)
    qk_steps = a_proj(0) + a_proj(1)
    per_chunk = len(qk_steps) // NC

    def take(_):
        taken = qk_steps[:per_chunk]
        del qk_steps[:per_chunk]
        return taken

    pair_attention(True, take)
    a_attention(0, a_proj(2), [])

    def chunk_step(c, carry):
        prep_xa(c)
        prep_ao()
        run(a_proj(0) + a_proj(1), 8 * NPROD)
        a_attention(c, a_proj(2), a_out_proj(c - 1))
        cp_out_a(c - 1).start()
        return carry

    lax.fori_loop(1, NC, chunk_step, 0)
    prep_ao()
    run(a_out_proj(NC - 1), NPROD)
    cp_out_a(NC - 1).start()
    for c in range(NC):
        cp_out_b(c).wait()
        cp_out_a(c).wait()


@jax.jit
def pallas_concat_heads__sliding_local_dilated__compressed_kv_cla__prompt_kernel(
    A_x: jax.Array,
    A_wqkv: jax.Array,
    A_wo: jax.Array,
    B_x: jax.Array,
    B_c_kv: jax.Array,
    B_w_q: jax.Array,
    B_w_uk: jax.Array,
    B_w_uv: jax.Array,
    B_w_o: jax.Array,
):
    vmem = pltpu.VMEM
    dma = pltpu.SemaphoreType.DMA
    scratch = [
        vmem((S, DM), BF16),
        vmem((S, DC), BF16),
        vmem((NOPS, NC, R // 2, DM // 2), U32),
        vmem((NOPS, NC, R // 2, DC // 2), U32),
        vmem((2, DM, HD), U32),
        vmem((2, DC, HD), U32),
        vmem((2, DC, HD), U32),
        vmem((2, 2 * HD, DM), BF16),
        vmem((NOPS, DM // 4, HD), U32),
        vmem((NOPS, DC // 4, 2 * HD), U32),
        vmem((NOPS, HD // 2, DM // 2), U32),
        vmem((2, S // 2, HD), U32),
        vmem((2, S // 2, HD), U32),
        vmem((2, S // 2, HD), U32),
        vmem((S, DM), F32),
        vmem((2, 2, 128, DM), BF16),
        vmem((NH * PITCH, 128), F32),
        vmem((12, NOPS, DM // 4, 128), U32),
        vmem((S, DM), BF16),
        vmem((DM, DM), BF16),
        vmem((NOPS, DM // 4, DM // 2), U32),
        vmem((NOPS, R // 2, DM // 2), U32),
        vmem((8, CH, 128), F32),
        vmem((8, HALO + CH, 128), F32),
        vmem((8, HALO + CH, 128), F32),
        vmem((8, CH, 128), F32),
        vmem((NOPS, R // 2, DM // 2), U32),
        vmem((S, DM), BF16),
        dma((NC,)), dma((NC,)), dma((8,)), dma((4,)), dma((2,)), dma((2 * NC,)),
    ]
    out = pl.pallas_call(
        _kernel,
        out_shape=jax.ShapeDtypeStruct((S, 2 * DM), BF16),
        in_specs=[pl.BlockSpec(memory_space=pl.ANY)] * 9,
        out_specs=pl.BlockSpec(memory_space=pl.ANY),
        scratch_shapes=scratch,
        compiler_params=pltpu.CompilerParams(vmem_limit_bytes=110 * 2**20),
        name="fused_local_and_latent_attention",
    )(
        A_x.reshape(S, DM), A_wqkv, A_wo,
        B_x.reshape(S, DM), B_c_kv.reshape(S, DC),
        B_w_q, B_w_uk, B_w_uv, B_w_o.reshape(NH * HD, DM),
    )
    return out.reshape(1, S, 2 * DM)
```

```python
import math

import jax
import jax.numpy as jnp
from jax import lax
import jax.experimental.pallas as pl
import jax.experimental.pallas.tpu as pltpu

F32, BF16, U32 = jnp.float32, jnp.bfloat16, jnp.uint32

S = 2048
DM = 1024
DC = 512
NH = 32
HD = 128
AD = 32
WIN, DIL = 8, 2

R = 128
CH = 2 * R
NC = S // CH
NP = NH // 2
HALO = 16
PITCH = 33

_PARTS = ("pro", "bloop", "q0", "aloop", "epi")
_FLAGS = {}
_X = ""
_FIRST = 5
_NK = 2
_NA = 2
_LAG = 3
_AT = 3
_NB = 32
LOG2E = math.log2(math.e)
MASKED = -1e9 * LOG2E

NN = (((1,), (0,)), ((), ()))
NT = (((1,), (1,)), ((), ()))

_STRASSEN = dict(
    lhs=(((0, 1), (3, 1)), ((2, 1), (3, 1)), ((0, 1),), ((3, 1),),
         ((0, 1), (1, 1)), ((2, 1), (0, -1)), ((1, 1), (3, -1))),
    rhs=(((0, 1), (3, 1)), ((0, 1),), ((1, 1), (3, -1)), ((2, 1), (0, -1)),
         ((3, 1),), ((0, 1), (1, 1)), ((2, 1), (3, 1))),
    prods=((2, 2, ((1, 1), (3, 1))), (4, 4, ((0, -1), (1, 1))),
           (3, 3, ((0, 1), (2, 1))), (1, 1, ((2, 1), (3, -1))),
           (5, 5, ((3, 1),)), (0, 0, ((0, 1), (3, 1))), (6, 6, ((0, 1),))),
)
SCHEME = _STRASSEN
NOPS = len(SCHEME["lhs"])
NPROD = len(SCHEME["prods"])

OPROWS = 256
N_UNITS = 12
W_Q, W_KV, W_O = range(3)
RING = 8


def _combine(blocks, terms):
    out = None
    for i, sign in terms:
        if out is None:
            assert sign > 0
            out = blocks[i]
        else:
            out = out + blocks[i] if sign > 0 else out - blocks[i]
    return out


def _pack(x):
    return pltpu.bitcast(x.astype(BF16), U32)


def _bf16(words):
    return pltpu.bitcast(words, BF16)


def _halves(words):
    lo = pltpu.bitcast(words << 16, F32)
    hi = pltpu.bitcast(words & jnp.uint32(0xFFFF0000), F32)
    return lo, hi


def _recip(x):
    r = pltpu.reciprocal(x, approx=True)
    return r * (2.0 - x * r)


def _operands(blocks, side):
    return [_pack(_combine(blocks, terms)) for terms in SCHEME[side]]


def _block_product(lhs, rhs, done, dims=NN, init=None):
    c, signs = [None] * 4, [1] * 4

    def step(n):
        ia, ib, outs = SCHEME["prods"][n]
        m = lax.dot_general(lhs(ia), rhs(ib), dims, preferred_element_type=F32)
        later = {o for _, _, os in SCHEME["prods"][n + 1:] for o, _ in os}
        for o, sign in outs:
            if c[o] is None and init is not None:
                c[o] = init(o)
            if c[o] is None:
                c[o], signs[o] = m, sign
            elif signs[o] > 0:
                c[o] = c[o] + m if sign > 0 else c[o] - m
            else:
                assert sign > 0
                c[o], signs[o] = m - c[o], 1
            if o not in later:
                assert signs[o] > 0
                done(o, c[o])
        return m

    return [lambda n=n: step(n) for n in range(NPROD)]


def _run(steps, n=None):
    out = None
    for _ in range(len(steps) if n is None else min(n, len(steps))):
        out = steps.pop(0)()
    return out


def _group(steps, n):
    return [lambda g=steps[i:i + n]: _run(g) for i in range(0, len(steps), n)]


def _share(items, k, n):
    return items[k * len(items) // n:(k + 1) * len(items) // n]


def _witness(values):
    out = None
    for v in values:
        v = pltpu.bitcast(v, U32)
        for r in range(0, v.shape[0], 8):
            for c in range(0, v.shape[1], 128):
                out = v[r:r + 8, c:c + 128] if out is None else out | v[r:r + 8, c:c + 128]
    return out


def _mingle(steps, pieces):
    history = []

    def both(step, mine):
        history.append(step())
        for i, (pace, work, *lag) in enumerate(mine):
            seen = work()
            m = history[max(0, len(history) - 1 - sum(lag))]
            if m is not None:
                r = 8 * (i * (m.shape[0] // 8) // len(mine))
                pace(_witness([m[r:r + 8, :128]] + list(seen)))
        return history[-1]

    return [lambda step=step, mine=_share(pieces, i, len(steps)): both(step, mine)
            for i, step in enumerate(steps)]


def _now(pieces):
    for _, work, *_ in pieces:
        work()


def _kernel(ax_hbm, awqkv_hbm, awo_hbm, bx_hbm, c_hbm, wq_hbm, wuk_hbm, wuv_hbm,
            wo_hbm, out_hbm,
            xs, cs, blop, wq_raw, wuk_raw, wuv_raw, wo_raw, bwop,
            q_s, k_s, v_s, acc, aw_raw, shuf, awop, xa, awo_raw, xaop, aoop, aqkv, a_out,
            sem_x, sem_c, sem_w, sem_aw, sem_a, sem_out):
    wq32 = wq_hbm.bitcast(U32)
    wuk32 = wuk_hbm.bitcast(U32)
    wuv32 = wuv_hbm.bitcast(U32)

    def cp_x(c):
        rows = pl.ds(c * CH, CH)
        return pltpu.make_async_copy(bx_hbm.at[rows], xs.at[rows], sem_x.at[c])

    def cp_c(c):
        rows = pl.ds(c * CH, CH)
        return pltpu.make_async_copy(c_hbm.at[rows], cs.at[rows], sem_c.at[c])

    def cp_proj_w(j, s):
        return [
            pltpu.make_async_copy(wuk32.at[:, j, :], wuk_raw.at[s], sem_w.at[s]),
            pltpu.make_async_copy(wuv32.at[:, j, :], wuv_raw.at[s], sem_w.at[2 + s]),
            pltpu.make_async_copy(wq32.at[:, j, :], wq_raw.at[s], sem_w.at[4 + s]),
        ]

    def cp_wo(j, s):
        rows = pl.ds(pl.multiple_of(j * 2 * HD, 2 * HD), 2 * HD)
        return [pltpu.make_async_copy(wo_hbm.at[rows], wo_raw.at[s], sem_w.at[6 + s])]

    def cp_aw(u, s):
        cols = pl.ds(pl.multiple_of((u // 4) * DM, DM), DM)
        return [
            pltpu.make_async_copy(
                awqkv_hbm.at[pl.ds(pl.multiple_of((u % 4) * 128 + half * (DM // 2), 128), 128), cols],
                aw_raw.at[s, half], sem_aw.at[2 * s + half])
            for half in range(2)
        ]

    def cp_step(j):
        return (cp_proj_w(jnp.minimum(j + 2, NP - 1), j % 2)
                + cp_wo(jnp.minimum(j + 1, NP - 1), j % 2)
                + cp_aw(jnp.minimum(j, N_UNITS - 1), j % 2))

    def cp_xa():
        return [pltpu.make_async_copy(ax_hbm.at[pl.ds(c * CH, CH)], xa.at[c], sem_a.at[0])
                for c in range(NC)]

    def cp_awo():
        return [pltpu.make_async_copy(awo_hbm.at[pl.ds(128 * t, 128)], awo_raw.at[t], sem_a.at[1])
                for t in range(8)]

    def cp_out_b(c):
        rows = pl.ds(c * CH, CH)
        return pltpu.make_async_copy(
            xs.at[rows], out_hbm.at[rows, pl.ds(DM, DM)], sem_out.at[c])

    def cp_out_a(c):
        rows = pl.ds(pl.multiple_of(c * CH, CH), CH)
        return pltpu.make_async_copy(
            a_out.at[rows], out_hbm.at[rows, pl.ds(0, DM)], sem_out.at[NC + c])

    def tiles(ref, page, i, n):
        h = OPROWS // n
        return _bf16(jnp.concatenate(
            [ref[page, i, pl.ds(t * h, h), :] for t in range(n)], axis=1))

    def put(ref, page, blocks, row):
        ops = _operands(blocks, "rhs")
        for i, v in enumerate(ops):
            ref[page, i, pl.ds(row, v.shape[0]), :] = v
        return ops

    def pacer(ref, *index):
        def pace(v):
            if ref.dtype == BF16:
                ref[(*index, pl.ds(0, 16), pl.ds(0, 128))] = _bf16(v)
            else:
                ref[(*index, pl.ds(0, 8), pl.ds(0, 128))] = pltpu.bitcast(v, ref.dtype)
        return pace

    def prep_rows(src, c, col):
        x = src[pl.ds(c * CH, CH), :].astype(F32)
        m = x.shape[1] // 2
        blocks = [x[:R, :m], x[:R, m:], x[R:, :m], x[R:, m:]]
        for i, v in enumerate(_operands(blocks, "lhs")):
            blop[c, i, :, pl.ds(col, m)] = v

    def prep_pair_w(raw, s, page, row0, zero, n=_NB):
        half = raw.shape[1] // 2

        def piece(r):
            blocks = [*_halves(raw[s, pl.ds(r, n)]), *_halves(raw[s, pl.ds(half + r, n)])]
            return put(bwop, page, blocks, row0 + r // 2)
        return [(pacer(raw, 2 + zero), lambda r=r: piece(r)) for r in range(0, half, n)]

    def prep_proj_w(s, page, zero):
        return (prep_pair_w(wuk_raw, s, page + W_KV, 0, zero)
                + prep_pair_w(wuv_raw, s, page + W_KV, OPROWS // 2, zero)
                + prep_pair_w(wq_raw, s, page + W_Q, 0, zero))

    def prep_wo(s, page, zero, n=_NB):
        def piece(t, r):
            blocks = [wo_raw[s, pl.ds(k * HD + r, n), pl.ds(h * (DM // 2) + 128 * t, 128)].astype(F32)
                      for k in range(2) for h in range(2)]
            return put(bwop, page + W_O, blocks, t * (HD // 2) + r // 2)
        return [(pacer(wo_raw, 2 + zero), lambda t=t, r=r: piece(t, r))
                for t in range(4) for r in range(0, HD, n)]

    def dim_major(src, pace, page, swap, zero):
        def scatter(k, u):
            t = src(k, u)
            for h in range(128 // AD):
                shuf[k, pl.ds((4 * u + h) * PITCH, AD), :] = t[h * AD:(h + 1) * AD]
            return [t]

        def gather(d, h):
            x = [[shuf[k, pl.ds(h * PITCH + a * AD // 2 + d, 16, stride=PITCH), :]
                  for k in range(2)] for a in range(2)]
            blocks = ([x[0][0], x[1][0], x[0][1], x[1][1]] if swap
                      else [x[0][0], x[0][1], x[1][0], x[1][1]])
            return put(awop, page, blocks, (d * NH + h) // 2)

        return ([(pace, lambda k=k, u=u: scatter(k, u), _LAG)
                 for k in range(2) for u in range(NH * AD // 128)]
                + [(pacer(shuf, 2 + zero), lambda d=d, h=h: gather(d, h))
                   for d in range(AD // 2) for h in range(0, NH, 16)])

    def prep_aw(u, s, zero):
        return dim_major(
            lambda k, t: aw_raw[s, k, :, 128 * t:128 * (t + 1)].astype(F32).T,
            pacer(blop, NC + zero, 0), u, True, zero)

    def prep_awo(n, zero):
        return dim_major(
            lambda k, t: awo_raw[t, :, pl.ds(k * (DM // 2) + 128 * n, 128)].astype(F32),
            pacer(awo_raw, 8 + zero), N_UNITS + n, False, zero)

    def put_a(ref, blocks, t, r):
        ops = _operands(blocks, "lhs")
        for i, v in enumerate(ops):
            ref[0, i, pl.ds(r // 2, v.shape[0]), pl.ds(128 * t, 128)] = v
        return ops

    def prep_xa(c, zero, n=_NB):
        def piece(t, r):
            blocks = [xa[c, pl.ds(k * R + r, n), pl.ds(h * (DM // 2) + 128 * t, 128)].astype(F32)
                      for k in range(2) for h in range(2)]
            return put_a(xaop, blocks, t, r)
        return [(pacer(xa, NC + zero), lambda t=t, r=r: piece(t, r))
                for t in range(4) for r in range(0, R, n)]

    def words(blk):
        return pl.ds(blk * (R // 2), R // 2)

    def q_proj(c, page):
        def done(o, val):
            q_s[o % 2, words(2 * c + o // 2), :] = _pack(val * (HD ** -0.5 * LOG2E))
        return _block_product(lambda i: _bf16(blop[c, i, :, :DM // 2]),
                              lambda i: tiles(bwop, page + W_Q, i, 1), done)

    def kv_proj(c, page):
        lhs = lambda i: _bf16(blop[c, i, :, DM // 2:])
        if _NK == 1:
            def done(o, val):
                k_s[o % 2, words(2 * c + o // 2), :] = _pack(val[:, :HD])
                v_s[o % 2, words(2 * c + o // 2), :] = _pack(val[:, HD:])
            return _block_product(lhs, lambda i: tiles(bwop, page + W_KV, i, 2), done)
        steps = []
        for n, dst in enumerate((k_s, v_s)):
            def done(o, val, dst=dst):
                dst[o % 2, words(2 * c + o // 2), :] = _pack(val)
            steps += _block_product(
                lhs, lambda i, n=n: _bf16(bwop[page + W_KV, i, pl.ds(n * OPROWS // 2, OPROWS // 2), :]),
                done)
        return _group(steps, 2)

    def o_proj(c, ctx, page, last):
        lhs = [_combine(ctx, terms).astype(BF16) for terms in SCHEME["lhs"]]
        steps = []
        for n in range(4):
            def where(o, n=n):
                return (pl.ds((2 * c + o // 2) * R, R), pl.ds((o % 2) * (DM // 2) + 128 * n, 128))

            def done(o, val, where=where):
                if last:
                    xs[where(o)] = val.astype(BF16)
                else:
                    acc[where(o)] = val
            steps += _block_product(
                lambda i: lhs[i],
                lambda i, n=n: _bf16(bwop[page + W_O, i, pl.ds(n * HD // 2, HD // 2), :]),
                done, init=lambda o, where=where: acc[where(o)])
        steps = _group(steps, 4)
        if last:
            steps = steps + [lambda: cp_out_b(c).start()]
        return steps

    def scores(h, blk):
        n = (blk + 1) * R
        s = lax.dot_general(_bf16(q_s[h, words(blk), :]), _bf16(k_s[h, :n // 2, :]),
                            NT, preferred_element_type=F32)
        row = lax.broadcasted_iota(jnp.int32, (R, R), 0)
        col = lax.broadcasted_iota(jnp.int32, (R, R), 1)
        diag = jnp.where(col <= row, s[:, n - R:], MASKED)
        return diag if blk == 0 else jnp.concatenate([s[:, :n - R], diag], axis=1)

    def attend(h, blk, s):
        n = (blk + 1) * R
        p = jnp.exp2(s - jnp.max(s, axis=1, keepdims=True))
        if "u" in _X:
            p = p.astype(BF16).astype(F32)
        inv = _recip(jnp.sum(p, axis=1, keepdims=True))
        o = lax.dot_general(p.astype(BF16), _bf16(v_s[h, :n // 2, :]), NN,
                            preferred_element_type=F32)
        return o * inv

    def pair_attention(filler):
        blocks = [(h, 2 * c + u) for c in reversed(range(NC)) for u in (1, 0) for h in (0, 1)]
        todo, ctx = [], {}
        s = scores(*blocks[0])
        for n, (h, blk) in enumerate(blocks):
            ahead = scores(*blocks[n + 1]) if n + 1 < len(blocks) else None
            _run(todo, -(-len(todo) // (4 - n % 4)))
            ctx[h, blk] = attend(h, blk, s)
            s = ahead
            if n % 4 == 3:
                todo = filler(blk // 2, [ctx[0, blk], ctx[1, blk], ctx[0, blk + 1], ctx[1, blk + 1]])
        _run(todo)

    def window(c):
        return pl.multiple_of(c * CH, CH)

    def a_proj(row0):
        steps = []
        for part in range(3):
            for t in range(4):
                def done(o, val, part=part, t=t):
                    if part == 0:
                        val = val * (AD ** -0.5 * LOG2E)
                    aqkv[8 * part + t + 4 * (o % 2), pl.ds(row0 + (HALO + (o // 2) * R), R), :] = val

                def rhs(i, part=part, t=t):
                    return _bf16(jnp.concatenate(
                        [awop[4 * part + m, i, pl.ds(64 * t, 64), :] for m in range(4)], axis=1))
                steps += _block_product(lambda i: _bf16(xaop[0, i]), rhs, done, dims=NT)
        return steps

    def a_attention(c, row0, zero):
        logit, prob, mixed = {}, {}, {}

        def dot(r, w):
            tot = None
            for t in range(8):
                if (r, t) not in logit:
                    logit[r, t] = aqkv[t, pl.ds(row0 + (HALO + r), 8), :]
                pr = logit[r, t] * aqkv[8 + t, pl.ds(row0 + (HALO + r - DIL * w), 8), :]
                tot = pr if tot is None else tot + pr
            logit[r, "w", w] = tot
            if w == WIN - 1:
                weights(r)
            return [tot]

        def weights(r):
            logits = [logit[r, "w", w] for w in range(WIN)]
            logits = [x + pltpu.roll(x, 64, 1) for x in logits]
            logits = [x + pltpu.roll(x, 32, 1) for x in logits]
            if r < (WIN - 1) * DIL:
                pos = c * CH + r + lax.broadcasted_iota(jnp.int32, (8, 128), 0)
                logits = [x if w == 0 else jnp.where(pos >= DIL * w, x, MASKED)
                          for w, x in enumerate(logits)]
            top = logits[0]
            for x in logits[1:]:
                top = jnp.maximum(top, x)
            e = [jnp.exp2(x - top) for x in logits]
            tot = e[0]
            for x in e[1:]:
                tot = tot + x
            inv = _recip(tot)
            prob[r] = [x * inv for x in e]

        def mix(r, t, d, h):
            tot = None
            for w in range(WIN):
                pr = prob[r + d][w] * aqkv[16 + t + 4 * h, pl.ds(row0 + (HALO + r + d - DIL * w), 8), :]
                tot = pr if tot is None else tot + pr
            mixed[d, h] = tot
            if (d, h) == (R + 8, 1):
                return put_a(aoop, [jnp.concatenate([mixed[k, h], mixed[k + 8, h]], axis=0)
                                    for k in (0, R) for h in range(2)], t, r)
            return [tot]

        def dots(r):
            return [lambda d=d, w=w: dot(r + d, w) for d in (0, 8, R, R + 8) for w in range(WIN)]

        def mixes(r):
            return [lambda t=t, d=d, h=h: mix(r, t, d, h)
                    for t in range(4) for d in (0, 8, R, R + 8) for h in range(2)]

        work = dots(0)
        for r in range(16, R, 16):
            work += [w for pair in zip(dots(r), mixes(r - 16)) for w in pair]
        work += mixes(R - 16)
        return [(pacer(aqkv, 24 + zero), lambda g=work[i:i + _NA]: sum((w() for w in g), []))
                for i in range(0, len(work), _NA)]

    def a_out_proj(c, zero):
        steps = []
        for n in range(4):
            def done(o, val, n=n):
                rows = pl.ds(pl.multiple_of(c * CH + (o // 2) * R, R), R)
                a_out[rows, pl.ds((o % 2) * (DM // 2) + 128 * n, 128)] = val.astype(BF16)
            steps += _block_product(lambda i: _bf16(aoop[zero, i]),
                                    lambda i, n=n: tiles(awop, N_UNITS + n, i, 1), done)
        return steps + [lambda: cp_out_a(c).start()]

    order = list(reversed(range(NC)))
    if "pro" in _PARTS:
        first_w = cp_proj_w(0, 0)
        for cp in (cp_c(order[0]), first_w[0], first_w[1]):
            cp.start()
        for c in order[1:]:
            cp_c(c).start()
        acc[...] = jnp.zeros(acc.shape, F32)
        aqkv[8:24, :HALO, :] = jnp.zeros((16, HALO, 128), F32)
        for cp in (cp_c(order[0]), first_w[0], first_w[1]):
            cp.wait()
        first_w[2].start()
        for c in order:
            cp_x(c).start()
        prep = prep_proj_w(0, 3, 0)
        _now(prep[:len(prep) // 2])
        prep_rows(cs, order[0], DM // 2)
        for n, c in enumerate(order):
            if n + 1 < NC:
                cp_c(order[n + 1]).wait()
                prep_rows(cs, order[n + 1], DM // 2)
            else:
                first_w[2].wait()
                cp_x(order[0]).wait()
                _now(prep[len(prep) // 2:])
                prep_rows(xs, order[0], 0)
            _run(kv_proj(c, 3))
        second = cp_proj_w(1, 1) + cp_wo(0, 1)
        for n, c in enumerate(order):
            if n == 2:
                for cp in second + cp_step(0):
                    cp.start()
            if n + 1 < NC:
                cp_x(order[n + 1]).wait()
                prep_rows(xs, order[n + 1], 0)
            else:
                for cp in second:
                    cp.wait()
                _now(prep_proj_w(1, 0, 0) + prep_wo(1, 0, 0))
            _run(q_proj(c, 3))

    def pair_step(j, zero):
        if "c" not in _X:
            @pl.when(j == RING)
            def _():
                bwop[:3] = bwop[3 * RING:]

        @pl.when(j == 0)
        def _():
            for cp in cp_xa() + cp_awo():
                cp.start()

        for cp in cp_step(j):
            cp.wait()
        for cp in cp_step(j + 1):
            cp.start()
        page = 3 * (j % RING)
        aw = prep_aw(jnp.minimum(j, N_UNITS - 1), j % 2, zero)
        bw = prep_proj_w(j % 2, page + 3, zero) + prep_wo(j % 2, page + 3, zero)
        side = [p for k in range(8) for p in _share(aw, k, 8) + _share(bw, k, 8)]

        def filler(c, ctx):
            mine = _share(side, _FIRST - c, _FIRST + 1) if c <= _FIRST else []
            return _mingle(q_proj(c, page) + o_proj(c, ctx, page, False) + kv_proj(c, page), mine)

        pair_attention(filler)
        return zero + j // NP

    zero = jnp.int32(0)
    if "bloop" in _PARTS:
        zero = lax.fori_loop(0, NP - 1, pair_step, zero)
    else:
        zero = lax.fori_loop(0, NP - 1, lambda j, z: z + j // NP, zero)

    if "q0" in _PARTS:
        for cp in cp_step(NP - 1) + cp_xa() + cp_awo():
            cp.wait()
        _now(prep_xa(zero, zero))
        _run(_mingle(a_proj(0), sum((prep_awo(n, zero) for n in range(4)), [])))
        _now(prep_xa(1 + zero, zero))

    def chunk_step(c, zero):
        row0 = window(c - 1)
        steps = a_proj(row0 + CH)
        _run(_mingle(steps[:-_AT], a_attention(c - 1, row0, zero)) + steps[-_AT:])
        _run(_mingle(a_out_proj(c - 1, c // NC), prep_xa(jnp.minimum(c + 1, NC - 1), zero)))
        return zero + c // NC

    if "aloop" in _PARTS:
        zero = lax.fori_loop(1, NC, chunk_step, zero)

    if "epi" in _PARTS:
        page = 3 * ((NP - 1) % RING)
        side = a_attention(NC - 1, (NC - 1) * CH, zero)
        tail = a_out_proj(NC - 1, zero)

        def filler(c, ctx):
            steps = o_proj(c, ctx, page, True)
            if c >= 3:
                return _mingle(steps, _share(side, NC - 1 - c, NC - 3))
            return steps + _share(tail, 2 - c, 3)

        pair_attention(filler)
        for c in range(NC):
            cp_out_b(c).wait()
            cp_out_a(c).wait()
    else:
        a_out[:16, :128] = (aqkv[3, :16, :] + acc[:16, :128]).astype(BF16)
        a_out[16:32, :128] = _bf16(awop[0, 0, :8, :] + q_s[0, :8, :] + k_s[0, :8, :] + v_s[0, :8, :])
        cp_out_a(0).start()
        cp_out_a(0).wait()


@jax.jit
def pallas_concat_heads__sliding_local_dilated__compressed_kv_cla__prompt_kernel(
    A_x: jax.Array,
    A_wqkv: jax.Array,
    A_wo: jax.Array,
    B_x: jax.Array,
    B_c_kv: jax.Array,
    B_w_q: jax.Array,
    B_w_uk: jax.Array,
    B_w_uv: jax.Array,
    B_w_o: jax.Array,
):
    vmem = pltpu.VMEM
    dma = pltpu.SemaphoreType.DMA
    scratch = [
        vmem((S, DM), BF16),
        vmem((S, DC), BF16),
        vmem((NC + 1, NOPS, R // 2, (DM + DC) // 2), U32),
        vmem((3, DM, HD), U32),
        vmem((3, DC, HD), U32),
        vmem((3, DC, HD), U32),
        vmem((3, 2 * HD, DM), BF16),
        vmem((3 * (RING + 1), NOPS, OPROWS, 128), U32),
        vmem((2, S // 2, HD), U32),
        vmem((2, S // 2, HD), U32),
        vmem((2, S // 2, HD), U32),
        vmem((S, DM), F32),
        vmem((3, 2, 128, DM), BF16),
        vmem((3, NH * PITCH, 128), F32),
        vmem((N_UNITS + 4, NOPS, OPROWS, 128), U32),
        vmem((NC + 1, CH, DM), BF16),
        vmem((9, 128, DM), BF16),
        vmem((1, NOPS, R // 2, DM // 2), U32),
        vmem((1, NOPS, R // 2, DM // 2), U32),
        vmem((25, HALO + S, 128), F32),
        vmem((S, DM), BF16),
        dma((NC,)), dma((NC,)), dma((8,)), dma((4,)), dma((2,)), dma((2 * NC,)),
    ]
    out = pl.pallas_call(
        _kernel,
        out_shape=jax.ShapeDtypeStruct((S, 2 * DM), BF16),
        in_specs=[pl.BlockSpec(memory_space=pl.ANY)] * 9,
        out_specs=pl.BlockSpec(memory_space=pl.ANY),
        scratch_shapes=scratch,
        compiler_params=pltpu.CompilerParams(vmem_limit_bytes=120 * 2**20, flags=_FLAGS or None),
        name="fused_local_and_latent_attention",
    )(
        A_x.reshape(S, DM), A_wqkv, A_wo,
        B_x.reshape(S, DM), B_c_kv.reshape(S, DC),
        B_w_q, B_w_uk, B_w_uv, B_w_o.reshape(NH * HD, DM),
    )
    return out.reshape(1, S, 2 * DM)
```

```python
import math

import jax
import jax.numpy as jnp
from jax import lax
import jax.experimental.pallas as pl
import jax.experimental.pallas.tpu as pltpu

F32, BF16, U32 = jnp.float32, jnp.bfloat16, jnp.uint32

S = 2048
DM = 1024
DC = 512
NH = 32
HD = 128
AD = 32
WIN, DIL = 8, 2

R = 128
CH = 2 * R
NC = S // CH
NP = NH // 2
HALO = 16
PITCH = 33

_PARTS = ("pro", "bloop", "q0", "aloop", "epi")
_FLAGS = {}
_X = "u"
_FIRST = 5
_NK = 2
_NA = 2
_CUT = 5
_SPLIT = 2
_ET = 12
_LAG = 3
_AT = 3
_NB = 32
LOG2E = math.log2(math.e)
MASKED = -1e9 * LOG2E

NN = (((1,), (0,)), ((), ()))
NT = (((1,), (1,)), ((), ()))

_STRASSEN = dict(
    lhs=(((0, 1), (3, 1)), ((2, 1), (3, 1)), ((0, 1),), ((3, 1),),
         ((0, 1), (1, 1)), ((2, 1), (0, -1)), ((1, 1), (3, -1))),
    rhs=(((0, 1), (3, 1)), ((0, 1),), ((1, 1), (3, -1)), ((2, 1), (0, -1)),
         ((3, 1),), ((0, 1), (1, 1)), ((2, 1), (3, 1))),
    prods=((2, 2, ((1, 1), (3, 1))), (4, 4, ((0, -1), (1, 1))),
           (3, 3, ((0, 1), (2, 1))), (1, 1, ((2, 1), (3, -1))),
           (5, 5, ((3, 1),)), (0, 0, ((0, 1), (3, 1))), (6, 6, ((0, 1),))),
)
SCHEME = _STRASSEN
NOPS = len(SCHEME["lhs"])
NPROD = len(SCHEME["prods"])

OPROWS = 256
N_UNITS = 12
W_Q, W_KV, W_O = range(3)
RING = 5


def _combine(blocks, terms):
    out = None
    for i, sign in terms:
        if out is None:
            assert sign > 0
            out = blocks[i]
        else:
            out = out + blocks[i] if sign > 0 else out - blocks[i]
    return out


def _pack(x):
    return pltpu.bitcast(x.astype(BF16), U32)


def _bf16(words):
    return pltpu.bitcast(words, BF16)


def _halves(words):
    lo = pltpu.bitcast(words << 16, F32)
    hi = pltpu.bitcast(words & jnp.uint32(0xFFFF0000), F32)
    return lo, hi


def _recip(x):
    r = pltpu.reciprocal(x, approx=True)
    return r * (2.0 - x * r)


def _operands(blocks, side):
    return [_pack(_combine(blocks, terms)) for terms in SCHEME[side]]


def _block_product(lhs, rhs, done, dims=NN, init=None):
    c, signs = [None] * 4, [1] * 4

    def step(n):
        ia, ib, outs = SCHEME["prods"][n]
        m = lax.dot_general(lhs(ia), rhs(ib), dims, preferred_element_type=F32)
        later = {o for _, _, os in SCHEME["prods"][n + 1:] for o, _ in os}
        for o, sign in outs:
            if c[o] is None and init is not None:
                c[o] = init(o)
            if c[o] is None:
                c[o], signs[o] = m, sign
            elif signs[o] > 0:
                c[o] = c[o] + m if sign > 0 else c[o] - m
            else:
                assert sign > 0
                c[o], signs[o] = m - c[o], 1
            if o not in later:
                assert signs[o] > 0
                done(o, c[o])
        return m

    return [lambda n=n: step(n) for n in range(NPROD)]


def _run(steps, n=None):
    out = None
    for _ in range(len(steps) if n is None else min(n, len(steps))):
        out = steps.pop(0)()
    return out


def _group(steps, n):
    return [lambda g=steps[i:i + n]: _run(g) for i in range(0, len(steps), n)]


def _share(items, k, n):
    return items[k * len(items) // n:(k + 1) * len(items) // n]


def _witness(values):
    out = None
    for v in values:
        v = pltpu.bitcast(v, U32)
        for r in range(0, v.shape[0], 8):
            for c in range(0, v.shape[1], 128):
                out = v[r:r + 8, c:c + 128] if out is None else out | v[r:r + 8, c:c + 128]
    return out


def _mingle(steps, pieces):
    history = []

    def both(step, mine):
        history.append(step())
        for i, (pace, work, *lag) in enumerate(mine):
            seen = work()
            m = history[max(0, len(history) - 1 - sum(lag))]
            if m is not None:
                r = 8 * (i * (m.shape[0] // 8) // len(mine))
                pace(_witness([m[r:r + 8, :128]] + list(seen)))
        return history[-1]

    return [lambda step=step, mine=_share(pieces, i, len(steps)): both(step, mine)
            for i, step in enumerate(steps)]


def _now(pieces):
    for _, work, *_ in pieces:
        work()


def _kernel(ax_hbm, awqkv_hbm, awo_hbm, bx_hbm, c_hbm, wq_hbm, wuk_hbm, wuv_hbm,
            wo_hbm, out_hbm,
            xs, cs, blop, wq_raw, wuk_raw, wuv_raw, wo_raw, bwop,
            q_s, k_s, v_s, acc, aw_raw, shuf, awop, xa, awo_raw, xaop, aoop, aqkv, a_out,
            sem_x, sem_c, sem_w, sem_aw, sem_a, sem_out):
    wq32 = wq_hbm.bitcast(U32)
    wuk32 = wuk_hbm.bitcast(U32)
    wuv32 = wuv_hbm.bitcast(U32)

    def cp_x(c):
        return pltpu.make_async_copy(bx_hbm.at[pl.ds(c * CH, CH)], xs.at[c], sem_x.at[c])

    def cp_c(c):
        return pltpu.make_async_copy(c_hbm.at[pl.ds(c * CH, CH)], cs.at[c], sem_c.at[c])

    def cp_proj_w(j, s):
        return [
            pltpu.make_async_copy(wuk32.at[:, j, :], wuk_raw.at[s], sem_w.at[s]),
            pltpu.make_async_copy(wuv32.at[:, j, :], wuv_raw.at[s], sem_w.at[2 + s]),
            pltpu.make_async_copy(wq32.at[:, j, :], wq_raw.at[s], sem_w.at[4 + s]),
        ]

    def cp_wo(j, s):
        rows = pl.ds(pl.multiple_of(j * 2 * HD, 2 * HD), 2 * HD)
        return [pltpu.make_async_copy(wo_hbm.at[rows], wo_raw.at[s], sem_w.at[6 + s])]

    def cp_aw(u, s):
        cols = pl.ds(pl.multiple_of((u // 4) * DM, DM), DM)
        return [
            pltpu.make_async_copy(
                awqkv_hbm.at[pl.ds(pl.multiple_of((u % 4) * 128 + half * (DM // 2), 128), 128), cols],
                aw_raw.at[s, half], sem_aw.at[2 * s + half])
            for half in range(2)
        ]

    def cp_step(j):
        return (cp_proj_w(jnp.minimum(j + 2, NP - 1), j % 2)
                + cp_wo(jnp.minimum(j + 1, NP - 1), j % 2)
                + cp_aw(jnp.minimum(j, N_UNITS - 1), j % 2))

    def cp_xa():
        return [pltpu.make_async_copy(ax_hbm.at[pl.ds(c * CH, CH)], xa.at[c], sem_a.at[0])
                for c in range(NC)]

    def cp_awo():
        return [pltpu.make_async_copy(awo_hbm.at[pl.ds(128 * t, 128)], awo_raw.at[t], sem_a.at[1])
                for t in range(8)]

    def cp_out_b(c):
        rows = pl.ds(c * CH, CH)
        return pltpu.make_async_copy(
            xs.at[c], out_hbm.at[rows, pl.ds(DM, DM)], sem_out.at[c])

    def cp_out_a(c):
        rows = pl.ds(pl.multiple_of(c * CH, CH), CH)
        return pltpu.make_async_copy(
            a_out.at[rows], out_hbm.at[rows, pl.ds(0, DM)], sem_out.at[NC + c])

    def tiles(ref, page, i, n):
        h = OPROWS // n
        return _bf16(jnp.concatenate(
            [ref[page, i, pl.ds(t * h, h), :] for t in range(n)], axis=1))

    def put(ref, page, blocks, row):
        ops = _operands(blocks, "rhs")
        for i, v in enumerate(ops):
            ref[page, i, pl.ds(row, v.shape[0]), :] = v
        return ops

    def pacer(ref, *index):
        def pace(v):
            if ref.dtype == BF16:
                ref[(*index, pl.ds(0, 16), pl.ds(0, 128))] = _bf16(v)
            else:
                ref[(*index, pl.ds(0, 8), pl.ds(0, 128))] = pltpu.bitcast(v, ref.dtype)
        return pace

    def prep_rows(src, c, col, zero, n=_NB):
        m = src.shape[2] // 2

        def piece(t, r):
            blocks = [src[c, pl.ds(k * R + r, n), pl.ds(h * m + 128 * t, 128)].astype(F32)
                      for k in range(2) for h in range(2)]
            ops = _operands(blocks, "lhs")
            for i, v in enumerate(ops):
                blop[c, i, pl.ds(r // 2, n // 2), pl.ds(col + 128 * t, 128)] = v
            return ops
        return [(pacer(src, NC + zero), lambda t=t, r=r: piece(t, r))
                for t in range(m // 128) for r in range(0, R, n)]

    def prep_pair_w(raw, s, page, row0, zero, n=_NB):
        half = raw.shape[1] // 2

        def piece(r):
            blocks = [*_halves(raw[s, pl.ds(r, n)]), *_halves(raw[s, pl.ds(half + r, n)])]
            return put(bwop, page, blocks, row0 + r // 2)
        return [(pacer(raw, 2 + zero), lambda r=r: piece(r)) for r in range(0, half, n)]

    def prep_kv_w(s, page, zero):
        return (prep_pair_w(wuk_raw, s, page + W_KV, 0, zero)
                + prep_pair_w(wuv_raw, s, page + W_KV, OPROWS // 2, zero))

    def prep_q_w(s, page, zero):
        return prep_pair_w(wq_raw, s, page + W_Q, 0, zero)

    def prep_wo(s, page, zero, n=_NB):
        def piece(t, r):
            blocks = [wo_raw[s, pl.ds(k * HD + r, n), pl.ds(h * (DM // 2) + 128 * t, 128)].astype(F32)
                      for k in range(2) for h in range(2)]
            return put(bwop, page + W_O, blocks, t * (HD // 2) + r // 2)
        return [(pacer(wo_raw, 2 + zero), lambda t=t, r=r: piece(t, r))
                for t in range(4) for r in range(0, HD, n)]

    def dim_major(src, pace, page, swap, zero):
        def scatter(k, u):
            t = src(k, u)
            for h in range(128 // AD):
                shuf[k, pl.ds((4 * u + h) * PITCH, AD), :] = t[h * AD:(h + 1) * AD]
            return [t]

        def gather(d, h):
            x = [[shuf[k, pl.ds(h * PITCH + a * AD // 2 + d, 16, stride=PITCH), :]
                  for k in range(2)] for a in range(2)]
            blocks = ([x[0][0], x[1][0], x[0][1], x[1][1]] if swap
                      else [x[0][0], x[0][1], x[1][0], x[1][1]])
            return put(awop, page, blocks, (d * NH + h) // 2)

        return ([(pace, lambda k=k, u=u: scatter(k, u), _LAG)
                 for k in range(2) for u in range(NH * AD // 128)]
                + [(pacer(shuf, 2 + zero), lambda d=d, h=h: gather(d, h))
                   for d in range(AD // 2) for h in range(0, NH, 16)])

    def prep_aw(u, s, zero):
        return dim_major(
            lambda k, t: aw_raw[s, k, :, 128 * t:128 * (t + 1)].astype(F32).T,
            pacer(blop, NC + zero, 0), u, True, zero)

    def prep_awo(n, zero):
        return dim_major(
            lambda k, t: awo_raw[t, :, pl.ds(k * (DM // 2) + 128 * n, 128)].astype(F32),
            pacer(awo_raw, 8 + zero), N_UNITS + n, False, zero)

    def put_a(ref, blocks, t, r):
        ops = _operands(blocks, "lhs")
        for i, v in enumerate(ops):
            ref[0, i, pl.ds(r // 2, v.shape[0]), pl.ds(128 * t, 128)] = v
        return ops

    def prep_xa(c, zero, n=_NB):
        def piece(t, r):
            blocks = [xa[c, pl.ds(k * R + r, n), pl.ds(h * (DM // 2) + 128 * t, 128)].astype(F32)
                      for k in range(2) for h in range(2)]
            return put_a(xaop, blocks, t, r)
        return [(pacer(xa, NC + zero), lambda t=t, r=r: piece(t, r))
                for t in range(4) for r in range(0, R, n)]

    def words(blk):
        return pl.ds(blk * (R // 2), R // 2)

    def q_proj(c, page):
        def done(o, val):
            q_s[o % 2, words(2 * c + o // 2), :] = _pack(val * (HD ** -0.5 * LOG2E))
        return _block_product(lambda i: _bf16(blop[c, i, :, :DM // 2]),
                              lambda i: tiles(bwop, page + W_Q, i, 1), done)

    def kv_proj(c, page):
        lhs = lambda i: _bf16(blop[c, i, :, DM // 2:])
        if _NK == 1:
            def done(o, val):
                k_s[o % 2, words(2 * c + o // 2), :] = _pack(val[:, :HD])
                v_s[o % 2, words(2 * c + o // 2), :] = _pack(val[:, HD:])
            return _block_product(lhs, lambda i: tiles(bwop, page + W_KV, i, 2), done)
        steps = []
        for n, dst in enumerate((k_s, v_s)):
            def done(o, val, dst=dst):
                dst[o % 2, words(2 * c + o // 2), :] = _pack(val)
            steps += _block_product(
                lhs, lambda i, n=n: _bf16(bwop[page + W_KV, i, pl.ds(n * OPROWS // 2, OPROWS // 2), :]),
                done)
        return _group(steps, 2)

    def o_proj(c, lhs, page, last):
        steps = []
        for n in range(4):
            def cols(o, n=n):
                return pl.ds((o % 2) * (DM // 2) + 128 * n, 128)

            def rows(o):
                return pl.ds((2 * c + o // 2) * R, R)

            def done(o, val, cols=cols):
                if last:
                    xs[c, pl.ds((o // 2) * R, R), cols(o)] = val.astype(BF16)
                else:
                    acc[rows(o), cols(o)] = val
            steps += _block_product(
                lambda i: _bf16(lhs[i]),
                lambda i, n=n: _bf16(bwop[page + W_O, i, pl.ds(n * HD // 2, HD // 2), :]),
                done, init=lambda o, cols=cols: acc[rows(o), cols(o)])
        return steps + [lambda: cp_out_b(c).start()] if last else _group(steps, 4)

    def scores(h, blk):
        n = (blk + 1) * R
        s = lax.dot_general(_bf16(q_s[h, words(blk), :]), _bf16(k_s[h, :n // 2, :]),
                            NT, preferred_element_type=F32)
        row = lax.broadcasted_iota(jnp.int32, (R, R), 0)
        col = lax.broadcasted_iota(jnp.int32, (R, R), 1)
        diag = jnp.where(col <= row, s[:, n - R:], MASKED)
        return diag if blk == 0 else jnp.concatenate([s[:, :n - R], diag], axis=1)

    def attend(h, blk, s):
        n = (blk + 1) * R
        p = jnp.exp2(s - jnp.max(s, axis=1, keepdims=True))
        if "u" in _X:
            p = p.astype(BF16).astype(F32)
        if "m" in _X and blk >= 8:
            tot, cols = p[:, :R], [p[:, :R]]
            for t in range(1, blk + 1):
                x = p[:, t * R:(t + 1) * R]
                tot = tot + x
                cols.append(jnp.minimum(x, tot))
            o = lax.dot_general(jnp.concatenate(cols, axis=1).astype(BF16), _bf16(v_s[h, :n // 2, :]), NN,
                                preferred_element_type=F32)
            return o * _recip(jnp.sum(tot, axis=1, keepdims=True))
        inv = _recip(jnp.sum(p, axis=1, keepdims=True))
        o = lax.dot_general(p.astype(BF16), _bf16(v_s[h, :n // 2, :]), NN,
                            preferred_element_type=F32)
        return o * inv

    def pair_attention(filler, chunks=tuple(reversed(range(NC))), todo=()):
        blocks = [(h, 2 * c + u) for c in chunks for u in (1, 0) for h in (0, 1)]
        todo, ctx = list(todo), {}
        s = scores(*blocks[0])
        for n, (h, blk) in enumerate(blocks):
            ahead = scores(*blocks[n + 1]) if n + 1 < len(blocks) else None
            cnt = -(-len(todo) // (4 - n % 4))
            _run(todo, cnt - cnt // 2)
            ctx[h, blk] = attend(h, blk, s)
            _run(todo, cnt // 2)
            s = ahead
            if n % 4 == 3:
                todo = filler(blk // 2, [ctx[0, blk], ctx[1, blk], ctx[0, blk + 1], ctx[1, blk + 1]])
        _run(todo)

    def window(c):
        return pl.multiple_of(c * CH, CH)

    def a_proj(row0):
        steps = []
        for part in range(3):
            for t in range(4):
                def done(o, val, part=part, t=t):
                    if part == 0:
                        val = val * (AD ** -0.5 * LOG2E)
                    aqkv[8 * part + t + 4 * (o % 2), pl.ds(row0 + (HALO + (o // 2) * R), R), :] = val

                def rhs(i, part=part, t=t):
                    return _bf16(jnp.concatenate(
                        [awop[4 * part + m, i, pl.ds(64 * t, 64), :] for m in range(4)], axis=1))
                steps += _block_product(lambda i: _bf16(xaop[0, i]), rhs, done, dims=NT)
        return steps

    def a_attention(c, row0, zero):
        logit, prob, mixed = {}, {}, {}

        def dot(r, w):
            tot = None
            for t in range(8):
                if (r, t) not in logit:
                    logit[r, t] = aqkv[t, pl.ds(row0 + (HALO + r), 8), :]
                pr = logit[r, t] * aqkv[8 + t, pl.ds(row0 + (HALO + r - DIL * w), 8), :]
                tot = pr if tot is None else tot + pr
            logit[r, "w", w] = tot
            if w == WIN - 1:
                weights(r)
            return [tot]

        def weights(r):
            logits = [logit[r, "w", w] for w in range(WIN)]
            logits = [x + pltpu.roll(x, 64, 1) for x in logits]
            logits = [x + pltpu.roll(x, 32, 1) for x in logits]
            if r < (WIN - 1) * DIL:
                pos = c * CH + r + lax.broadcasted_iota(jnp.int32, (8, 128), 0)
                logits = [x if w == 0 else jnp.where(pos >= DIL * w, x, MASKED)
                          for w, x in enumerate(logits)]
            top = logits[0]
            for x in logits[1:]:
                top = jnp.maximum(top, x)
            e = [jnp.exp2(x - top) for x in logits]
            tot = e[0]
            for x in e[1:]:
                tot = tot + x
            inv = _recip(tot)
            prob[r] = [x * inv for x in e]

        def mix(r, t, d, h):
            tot = None
            for w in range(WIN):
                pr = prob[r + d][w] * aqkv[16 + t + 4 * h, pl.ds(row0 + (HALO + r + d - DIL * w), 8), :]
                tot = pr if tot is None else tot + pr
            mixed[d, h] = tot
            if (d, h) == (R + 8, 1):
                return put_a(aoop, [jnp.concatenate([mixed[k, h], mixed[k + 8, h]], axis=0)
                                    for k in (0, R) for h in range(2)], t, r)
            return [tot]

        def dots(r):
            return [lambda d=d, w=w: dot(r + d, w) for d in (0, 8, R, R + 8) for w in range(WIN)]

        def mixes(r):
            return [lambda t=t, d=d, h=h: mix(r, t, d, h)
                    for t in range(4) for d in (0, 8, R, R + 8) for h in range(2)]

        work = dots(0)
        for r in range(16, R, 16):
            work += [w for pair in zip(dots(r), mixes(r - 16)) for w in pair]
        work += mixes(R - 16)
        return [(pacer(aqkv, 24 + zero), lambda g=work[i:i + _NA]: sum((w() for w in g), []))
                for i in range(0, len(work), _NA)]

    def a_out_proj(c, zero):
        steps = []
        for n in range(4):
            def done(o, val, n=n):
                rows = pl.ds(pl.multiple_of(c * CH + (o // 2) * R, R), R)
                a_out[rows, pl.ds((o % 2) * (DM // 2) + 128 * n, 128)] = val.astype(BF16)
            steps += _block_product(lambda i: _bf16(aoop[zero, i]),
                                    lambda i, n=n: tiles(awop, N_UNITS + n, i, 1), done)
        return steps + [lambda: cp_out_a(c).start()]

    zero = lax.fori_loop(0, NP - 1, lambda i, z: z + i // NP, jnp.int32(0))
    if "pro" in _PARTS:
        w0 = cp_proj_w(0, 0)
        w1 = cp_proj_w(1, 1) + cp_wo(0, 1)
        stages = [w0[:2] + [cp_c(c) for c in (7, 6, 5)],
                  [cp_c(c) for c in (4, 3, 2, 1, 0)] + w0[2:],
                  [cp_x(c) for c in (7, 6, 5, 4)],
                  [cp_x(c) for c in (3, 2, 1, 0)],
                  w1, cp_step(0)]

        def issue(i, zero):
            for k, stage in enumerate(stages):
                @pl.when(i == k)
                def _(stage=stage):
                    for cp in stage:
                        cp.start()
            return zero + i // NP

        zero = lax.fori_loop(0, len(stages), issue, jnp.int32(0))
        acc[...] = jnp.zeros(acc.shape, F32)
        aqkv[8:24, :HALO, :] = jnp.zeros((16, HALO, 128), F32)

        def project(steps, src, col, chunks, side):
            _now(prep_rows(src, chunks[0], col, zero))
            for n, c in enumerate(chunks):
                ahead = prep_rows(src, chunks[n + 1], col, zero) if n + 1 < len(chunks) else []
                _run(_mingle(steps(c, 3), ahead + _share(side, n, len(chunks))))

        for cp in stages[0]:
            cp.wait()
        _now(prep_kv_w(0, 3, zero))
        project(kv_proj, cs, DM // 2, (7, 6, 5), [])
        for cp in stages[1]:
            cp.wait()
        project(kv_proj, cs, DM // 2, (4, 3, 2, 1, 0), prep_q_w(0, 3, zero))
        for cp in stages[2]:
            cp.wait()
        project(q_proj, xs, 0, (7, 6, 5, 4), [])
        for cp in stages[3]:
            cp.wait()
        project(q_proj, xs, 0, (3, 2), [])
        for cp in w1:
            cp.wait()
        project(q_proj, xs, 0, (1, 0),
                prep_q_w(1, 0, zero) + prep_wo(1, 0, zero) + prep_kv_w(1, 0, zero))

    def pair_step(j, zero):
        if "c" not in _X:
            @pl.when((j == RING) | (j == 2 * RING))
            def _():
                bwop[:3] = bwop[3 * RING:]

        @pl.when(j == 0)
        def _():
            for cp in cp_xa() + cp_awo():
                cp.start()

        for cp in cp_step(j):
            cp.wait()
        for cp in cp_step(j + 1):
            cp.start()
        page = 3 * (j % RING)
        aw = prep_aw(jnp.minimum(j, N_UNITS - 1), j % 2, zero)
        bw = (prep_kv_w(j % 2, page + 3, zero) + prep_q_w(j % 2, page + 3, zero)
              + prep_wo(j % 2, page + 3, zero))
        side = [p for k in range(8) for p in _share(aw, k, 8) + _share(bw, k, 8)]

        def filler(c, ctx):
            mine = _share(side, _FIRST - c, _FIRST + 1) if c <= _FIRST else []
            return _mingle(q_proj(c, page) + o_proj(c, _operands(ctx, "lhs"), page, False) + kv_proj(c, page), mine)

        pair_attention(filler)
        return zero + j // NP

    if "bloop" in _PARTS:
        zero = lax.fori_loop(0, NP - 1, pair_step, zero)

    if "q0" in _PARTS:
        for cp in cp_step(NP - 1) + cp_xa() + cp_awo():
            cp.wait()
        _now(prep_xa(zero, zero))
        steps = _mingle(a_proj(0), sum((prep_awo(n, zero) for n in range(4)), []))

        def keep(c, ctx):
            for i, v in enumerate(_operands(ctx, "lhs")):
                blop[c, i, :, :HD] = v
            return _share(steps, NC - c + (c < _CUT), NC + 2)

        pair_attention(keep, tuple(reversed(range(_CUT, NC))), _share(steps, 0, NC + 2))

        @pl.loop(0, 2)
        def _(i):
            pacer(xa, NC + zero * i)(jnp.zeros((8, 128), U32))

        pair_attention(keep, tuple(reversed(range(_CUT))), _share(steps, NC - _CUT + 1, NC + 2))
        _now(prep_xa(1 + zero, zero))

    def chunk_step(c, zero):
        row0 = window(c - 1)
        steps = a_proj(row0 + CH)
        _run(_mingle(steps[:-_AT], a_attention(c - 1, row0, zero)) + steps[-_AT:])
        _run(_mingle(a_out_proj(c - 1, c // NC), prep_xa(jnp.minimum(c + 1, NC - 1), zero)))
        return zero + c // NC

    if "aloop" in _PARTS:
        zero = lax.fori_loop(1, NC, chunk_step, zero)

    if "epi" in _PARTS:
        page = 3 * ((NP - 2) % RING + 1)
        steps = []
        for c in range(NC):
            steps += o_proj(c, [blop[c, i, :, :HD] for i in range(NOPS)], page, True)
        _run(_mingle(steps[:-_ET], a_attention(NC - 1, (NC - 1) * CH, zero)) + steps[-_ET:])
        _run(a_out_proj(NC - 1, zero))
        for c in range(NC):
            cp_out_b(c).wait()
            cp_out_a(c).wait()
    else:
        a_out[:16, :128] = (aqkv[3, :16, :] + acc[:16, :128]).astype(BF16)
        a_out[16:32, :128] = _bf16(awop[0, 0, :8, :] + q_s[0, :8, :] + k_s[0, :8, :] + v_s[0, :8, :])
        cp_out_a(0).start()
        cp_out_a(0).wait()


@jax.jit
def pallas_concat_heads__sliding_local_dilated__compressed_kv_cla__prompt_kernel(
    A_x: jax.Array,
    A_wqkv: jax.Array,
    A_wo: jax.Array,
    B_x: jax.Array,
    B_c_kv: jax.Array,
    B_w_q: jax.Array,
    B_w_uk: jax.Array,
    B_w_uv: jax.Array,
    B_w_o: jax.Array,
):
    vmem = pltpu.VMEM
    dma = pltpu.SemaphoreType.DMA
    scratch = [
        vmem((NC + 1, CH, DM), BF16),
        vmem((NC + 1, CH, DC), BF16),
        vmem((NC + 1, NOPS, R // 2, (DM + DC) // 2), U32),
        vmem((3, DM, HD), U32),
        vmem((3, DC, HD), U32),
        vmem((3, DC, HD), U32),
        vmem((3, 2 * HD, DM), BF16),
        vmem((3 * (RING + 1), NOPS, OPROWS, 128), U32),
        vmem((2, S // 2, HD), U32),
        vmem((2, S // 2, HD), U32),
        vmem((2, S // 2, HD), U32),
        vmem((S, DM), F32),
        vmem((3, 2, 128, DM), BF16),
        vmem((3, NH * PITCH, 128), F32),
        vmem((N_UNITS + 4, NOPS, OPROWS, 128), U32),
        vmem((NC + 1, CH, DM), BF16),
        vmem((9, 128, DM), BF16),
        vmem((1, NOPS, R // 2, DM // 2), U32),
        vmem((1, NOPS, R // 2, DM // 2), U32),
        vmem((25, HALO + S, 128), F32),
        vmem((S, DM), BF16),
        dma((NC,)), dma((NC,)), dma((8,)), dma((4,)), dma((2,)), dma((2 * NC,)),
    ]
    out = pl.pallas_call(
        _kernel,
        out_shape=jax.ShapeDtypeStruct((S, 2 * DM), BF16),
        in_specs=[pl.BlockSpec(memory_space=pl.ANY)] * 9,
        out_specs=pl.BlockSpec(memory_space=pl.ANY),
        scratch_shapes=scratch,
        compiler_params=pltpu.CompilerParams(vmem_limit_bytes=120 * 2**20, flags=_FLAGS or None),
        name="fused_local_and_latent_attention",
    )(
        A_x.reshape(S, DM), A_wqkv, A_wo,
        B_x.reshape(S, DM), B_c_kv.reshape(S, DC),
        B_w_q, B_w_uk, B_w_uv, B_w_o.reshape(NH * HD, DM),
    )
    return out.reshape(1, S, 2 * DM)
```

```python
import math

import jax
import jax.numpy as jnp
from jax import lax
import jax.experimental.pallas as pl
import jax.experimental.pallas.tpu as pltpu

F32, BF16, U32 = jnp.float32, jnp.bfloat16, jnp.uint32

S = 2048
DM = 1024
DC = 512
NH = 32
HD = 128
AD = 32
WIN, DIL = 8, 2

R = 128
CH = 2 * R
NC = S // CH
NP = NH // 2
HALO = 16
PITCH = 33

_PARTS = ("pro", "bloop", "last", "s0", "aloop", "epi")
_X = "u"
_FIRST = 7
_NA = 2
_NB = 32
_LAG = 3
_AT = 3
_PRIO = 0
_DUM = 24
_QP = 16
_AP = 16
_PA = 0
_PB = 0
_CL = 4
_DEPTH = 2
LOG2E = math.log2(math.e)
MASKED = -1e9 * LOG2E

NN = (((1,), (0,)), ((), ()))
NT = (((1,), (1,)), ((), ()))

LHS = (((0, 1), (3, 1)), ((2, 1), (3, 1)), ((0, 1),), ((3, 1),),
       ((0, 1), (1, 1)), ((2, 1), (0, -1)), ((1, 1), (3, -1)))
RHS = (((0, 1), (3, 1)), ((0, 1),), ((1, 1), (3, -1)), ((2, 1), (0, -1)),
       ((3, 1),), ((0, 1), (1, 1)), ((2, 1), (3, 1)))
PRODUCTS = ((2, ((1, 1), (3, 1))), (4, ((0, -1), (1, 1))), (3, ((0, 1), (2, 1))),
            (1, ((2, 1), (3, -1))), (5, ((3, 1),)), (0, ((0, 1), (3, 1))),
            (6, ((0, 1),)))
NOPS = len(PRODUCTS)

OPROWS = 256
N_UNITS = 12
W_KV, W_Q = range(2)
RING = 5


def _combine(blocks, terms):
    if isinstance(blocks[terms[0][0]], list):
        return [_combine({b: blocks[b][i] for b, _ in terms}, terms) for i in range(4)]
    out = None
    for i, sign in terms:
        if out is None:
            assert sign > 0
            out = blocks[i]
        else:
            out = out + blocks[i] if sign > 0 else out - blocks[i]
    return out


def _store(words, index, row, col, x):
    matrix = words.bitcast(BF16).at[index]
    matrix[pl.ds(2 * row, x.shape[0]), pl.ds(col, x.shape[1])] = x.astype(BF16)


def _bf16(words):
    return pltpu.bitcast(words, BF16)


def _halves(words):
    lo = pltpu.bitcast(words << 16, F32)
    hi = pltpu.bitcast(words & jnp.uint32(0xFFFF0000), F32)
    return lo, hi


def _split(words):
    return jnp.concatenate(_halves(words), axis=0)


def _join(x):
    n = x.shape[0] // 2
    return pltpu.pack_elementwise([x[:n], x[n:]], packed_dtype=BF16)


def _recip(x):
    r = pltpu.reciprocal(x, approx=True)
    return r * (2.0 - x * r)


def _operands(blocks, side):
    return [_combine(blocks, terms) for terms in side]


def _block_product(lhs, rhs, done, dims=NN, levels=1):
    if levels == 0:
        def step():
            m = lax.dot_general(lhs(0), rhs(0), dims, preferred_element_type=F32)
            done((), m)
            return m
        return [step]

    held, steps = {}, []
    inner = NOPS ** (levels - 1)
    for n, (i, outs) in enumerate(PRODUCTS):
        later = {o for _, others in PRODUCTS[n + 1:] for o, _ in others}

        def add(sub, m, outs=outs, later=later):
            for o, sign in outs:
                if (o, sub) not in held:
                    held[o, sub] = m, sign
                else:
                    c, s = held[o, sub]
                    assert s > 0 or sign > 0
                    held[o, sub] = (m - c if s < 0 else c + m if sign > 0 else c - m), 1
                if o not in later:
                    done((o, *sub), held.pop((o, sub))[0])

        steps += _block_product(lambda k, i=i: lhs(i * inner + k),
                                lambda k, i=i: rhs(i * inner + k), add, dims, levels - 1)
    return steps


def _run(steps, n=None):
    out = None
    for _ in range(len(steps) if n is None else min(n, len(steps))):
        out = steps.pop(0)()
    return out


def _group(steps, n):
    return [lambda g=steps[i:i + n]: _run(g) for i in range(0, len(steps), n)]


def _share(items, k, n):
    return items[k * len(items) // n:(k + 1) * len(items) // n]


def _witness(values):
    out = None
    for v in values:
        v = pltpu.bitcast(v, U32)
        for r in range(0, v.shape[0], 8):
            for c in range(0, v.shape[1], 128):
                out = v[r:r + 8, c:c + 128] if out is None else out | v[r:r + 8, c:c + 128]
    return out


def _mingle(steps, pieces):
    history = []

    def both(step, mine):
        history.append(step())
        for i, (pace, work, *lag) in enumerate(mine):
            seen = work()
            m = history[max(0, len(history) - 1 - sum(lag))]
            if m is not None:
                r = 8 * (i * (m.shape[0] // 8) // len(mine))
                pace(_witness([m[r:r + 8, :128]] + list(seen)))
        return history[-1]

    return [lambda step=step, mine=_share(pieces, i, len(steps)): both(step, mine)
            for i, step in enumerate(steps)]


def _now(pieces):
    for _, work, *_ in pieces:
        work()


def _pacer(ref, *index):
    def pace(v):
        if ref.dtype == BF16:
            ref[(*index, pl.ds(0, 16), pl.ds(0, 128))] = _bf16(v)
        else:
            ref[(*index, pl.ds(0, 8), pl.ds(0, 128))] = pltpu.bitcast(v, ref.dtype)
    return pace


def _dim_major(src, pace, shuf, dst, page, swap, zero):
    def start(head):
        return ((head % 2) * NH // 2 + head // 2) * PITCH

    def scatter(k, u):
        t = src(k, u)
        for h in range(128 // AD):
            shuf[k, pl.ds(start(4 * u + h), AD), :] = t[h * AD:(h + 1) * AD]
        return [t]

    def gather(d, h):
        x = [[jnp.concatenate([shuf[k, pl.ds(start(h + p) + a * AD // 2 + d, 8, stride=PITCH), :]
                               for p in range(2)], axis=0)
              for k in range(2)] for a in range(2)]
        blocks = ([x[0][0], x[1][0], x[0][1], x[1][1]] if swap
                  else [x[0][0], x[0][1], x[1][0], x[1][1]])
        ops = [_join(v) for v in _operands(blocks, RHS)]
        for i, v in enumerate(ops):
            dst[page, i, pl.ds((d * NH + h) // 2, 8), :] = v
        return ops

    return ([(pace, lambda k=k, u=u: scatter(k, u), _LAG if swap else 0)
             for k in range(2) for u in range(NH * AD // 128)]
            + [(_pacer(shuf, 2 + zero), lambda d=d, h=h: gather(d, h))
               for d in range(AD // 2) for h in range(0, NH, 16)])


def _kernel(ax_hbm, awqkv_hbm, awo_hbm, bx_hbm, c_hbm, wq_hbm, wuk_hbm, wuv_hbm,
            wo_hbm, out_hbm,
            dummy, ctx, wo_raw, woop, awop, xa, awo_raw, shuf,
            sem_x, sem_c, sem_w, sem_aw, sem_a, sem_out):

    def cp_wo(u, s):
        rows = pl.ds(pl.multiple_of((u // 2) * 4 * HD, 4 * HD), 4 * HD)
        return [pltpu.make_async_copy(
            wo_hbm.at[rows, pl.ds(pl.multiple_of(q * 256 + (u % 2) * 128, 128), 128)],
            wo_raw.at[s, q].bitcast(BF16), sem_w.at[6 + s]) for q in range(4)]

    def prep_wo(u, s, zero):
        def piece(r, i):
            outer = {b: [_split(wo_raw[s, 2 * (b % 2) + b2,
                                       pl.ds((2 * a2 + b // 2) * (HD // 2) + r, 8), :])
                         for a2 in range(2) for b2 in range(2)] for b, _ in RHS[i]}
            ops = [_join(v) for v in _operands(_combine(outer, RHS[i]), RHS)]
            row = pl.multiple_of((u // 2) * (HD // 2) + r, 8)
            for k, v in enumerate(ops):
                woop[u % 2, NOPS * i + k, pl.ds(row, 8), :] = v
            return ops
        return [(_pacer(wo_raw, 2 + zero, 0), lambda r=r, i=i: piece(r, i))
                for r in range(0, HD // 2, 8) for i in range(NOPS)]

    def gap(flag, zero):
        if flag in _X:
            @pl.loop(0, 2)
            def _(i):
                _pacer(shuf, 2 + zero * i)(jnp.zeros((8, 128), U32))

    def pad(n, zero):
        if n:
            @pl.when(zero != 0)
            def _():
                v = shuf[0, :128]
                for _ in range(n * 95):
                    v = v * 1.0001 + 0.5
                shuf[0, :128] = v

    dummy[:8] = jnp.zeros((8, 128), F32)
    shuf[0, :8] = dummy[pl.ds(1, 8)]

    def cp_a():
        return ([pltpu.make_async_copy(ax_hbm.at[pl.ds(c * CH, CH)], xa.at[c], sem_a.at[0])
                 for c in range(NC)]
                + [pltpu.make_async_copy(awo_hbm.at[pl.ds(128 * t, 128)], awo_raw.at[t], sem_a.at[1])
                   for t in range(8)])

    def heads(xs, cs, blop, wq_raw, wuk_raw, wuv_raw, bwop, q_s, k_s, v_s, aw_raw):
        wq32 = wq_hbm.bitcast(U32)
        wuk32 = wuk_hbm.bitcast(U32)
        wuv32 = wuv_hbm.bitcast(U32)

        def cp_x(c):
            return pltpu.make_async_copy(bx_hbm.at[pl.ds(c * CH, CH)], xs.at[c], sem_x.at[c])

        def cp_c(c):
            return pltpu.make_async_copy(c_hbm.at[pl.ds(c * CH, CH)], cs.at[c], sem_c.at[c])

        def cp_proj_w(j, s):
            return [
                pltpu.make_async_copy(wuk32.at[:, j, :], wuk_raw.at[s], sem_w.at[s]),
                pltpu.make_async_copy(wuv32.at[:, j, :], wuv_raw.at[s], sem_w.at[2 + s]),
                pltpu.make_async_copy(wq32.at[:, j, :], wq_raw.at[s], sem_w.at[4 + s]),
            ]

        def cp_aw(u, s):
            cols = pl.ds(pl.multiple_of((u // 4) * DM, DM), DM)
            return [pltpu.make_async_copy(
                awqkv_hbm.at[pl.ds(pl.multiple_of((u % 4) * 128 + half * (DM // 2), 128), 128), cols],
                aw_raw.at[s, half], sem_aw.at[2 * s + half]) for half in range(2)]

        def cp_step(j):
            return (cp_proj_w(jnp.minimum(j + 2, NP - 1), j % 2) + cp_wo(j, j % 2)
                    + cp_aw(jnp.minimum(j, N_UNITS - 1), j % 2))

        def prep_rows(src, c, col, zero, n=_NB):
            m = src.shape[2] // 2

            def piece(t, r):
                blocks = [_split(pltpu.bitcast(
                    src[c, pl.ds(k * R + r, n), pl.ds(h * m + 128 * t, 128)], U32))
                    for k in range(2) for h in range(2)]
                ops = [_join(v) for v in _operands(blocks, LHS)]
                for i, v in enumerate(ops):
                    blop[c, i, pl.ds(r // 2, n // 2), pl.ds(col + 128 * t, 128)] = v
                return ops
            return [(_pacer(src, NC + zero), lambda t=t, r=r: piece(t, r))
                    for t in range(m // 128) for r in range(0, R, n)]

        def prep_pair_w(raw, s, page, row0, zero, n=_NB):
            half = raw.shape[1] // 2

            def piece(r):
                blocks = []
                for k in range(2):
                    even, odd = (_halves(raw[s, pl.ds(k * half + r + p, n // 2, stride=2), :])
                                 for p in range(2))
                    blocks += [jnp.concatenate([even[h], odd[h]], axis=0) for h in range(2)]
                ops = [_join(v) for v in _operands(blocks, RHS)]
                for i, v in enumerate(ops):
                    bwop[page, i, pl.ds(row0 + r // 2, n // 2), :] = v
                return ops
            return [(_pacer(raw, 2 + zero), lambda r=r: piece(r)) for r in range(0, half, n)]

        def prep_kv_w(s, page, zero):
            return (prep_pair_w(wuk_raw, s, page + W_KV, 0, zero)
                    + prep_pair_w(wuv_raw, s, page + W_KV, OPROWS // 2, zero))

        def prep_q_w(s, page, zero):
            return prep_pair_w(wq_raw, s, page + W_Q, 0, zero)

        def prep_aw(u, s, zero):
            return _dim_major(
                lambda k, t: aw_raw[s, k, :, 128 * t:128 * (t + 1)].astype(F32).T,
                _pacer(blop, NC + zero, 0), shuf, awop, u, True, zero)

        def words(blk):
            return pl.ds(blk * (R // 2), R // 2)

        def q_proj(c, page):
            def done(o, val):
                _store(q_s, 0, (2 * c + o[0] // 2) * (R // 2), (o[0] % 2) * HD,
                       val * (HD ** -0.5 * LOG2E))
            return _block_product(lambda i: _bf16(blop[c, i, :, :DM // 2]),
                                  lambda i: _bf16(bwop[page + W_Q, i]), done)

        def kv_proj(c, page):
            steps = []
            for n, dst in enumerate((k_s, v_s)):
                def done(o, val, dst=dst):
                    _store(dst, 0, (2 * c + o[0] // 2) * (R // 2), (o[0] % 2) * HD, val)
                steps += _block_product(
                    lambda i: _bf16(blop[c, i, :, DM // 2:]),
                    lambda i, n=n: _bf16(bwop[page + W_KV, i, pl.ds(n * OPROWS // 2, OPROWS // 2), :]),
                    done)
            return _group(steps, 2)

        def scores(h, blk):
            n = (blk + 1) * R
            s = lax.dot_general(_bf16(q_s[0, words(blk), pl.ds(h * HD, HD)]),
                                _bf16(k_s[0, :n // 2, pl.ds(h * HD, HD)]),
                                NT, preferred_element_type=F32)
            row = lax.broadcasted_iota(jnp.int32, (R, R), 0)
            col = lax.broadcasted_iota(jnp.int32, (R, R), 1)
            diag = jnp.where(col <= row, s[:, n - R:], MASKED)
            return diag if blk == 0 else jnp.concatenate([s[:, :n - R], diag], axis=1)

        def attend(h, blk, s):
            n = (blk + 1) * R
            p = jnp.exp2(s - jnp.max(s, axis=1, keepdims=True))
            if "u" in _X:
                p = p.astype(BF16).astype(F32)
            inv = _recip(jnp.sum(p, axis=1, keepdims=True))
            o = lax.dot_general(p.astype(BF16), _bf16(v_s[0, :n // 2, pl.ds(h * HD, HD)]), NN,
                                preferred_element_type=F32)
            return o * inv

        def pair_attention(j, zero, filler, depth=1):
            blocks = [(h, 2 * c + u) for c in reversed(range(NC)) for u in (1, 0) for h in (0, 1)]
            todo, done = [], []
            ahead = [scores(*b) for b in blocks[:depth]]
            for n, (h, blk) in enumerate(blocks):
                ahead += [scores(*b) for b in blocks[n + depth:n + depth + 1]]
                cnt = -(-len(todo) // (4 - n % 4))
                _run(todo, cnt - cnt // 2)
                done.append(attend(h, blk, ahead.pop(0)))
                _store(ctx, j, blk * (R // 2), h * HD, done[-1])
                if len(done) > _CL:
                    q_s[zero, pl.ds(S // 2, 8), :128] = _witness([done.pop(0)])
                _run(todo, cnt // 2)
                if n % 4 == 3:
                    todo = filler(blk // 2)
            _run(todo)

        w0, w1 = cp_proj_w(0, 0), cp_proj_w(1, 1)
        stages = [w0[:2] + [cp_c(c) for c in (7, 6, 5)],
                  [cp_c(c) for c in (4, 3, 2, 1, 0)] + w0[2:],
                  [cp_x(c) for c in (7, 6, 5, 4)],
                  [cp_x(c) for c in (3, 2, 1, 0)] + w1,
                  cp_step(0)]

        def issue(i, zero):
            for k, stage in enumerate(stages):
                @pl.when(i == k)
                def _(stage=stage):
                    for cp in stage:
                        cp.start()
            return zero + i // NP

        zero = lax.fori_loop(0, len(stages), issue, jnp.int32(0)) if 'pro' in _PARTS else lax.fori_loop(0, 15, lambda i, z: z + i // NP, jnp.int32(0))

        def project(steps, src, col, chunks, side):
            _now(prep_rows(src, chunks[0], col, zero))
            for n, c in enumerate(chunks):
                ahead = prep_rows(src, chunks[n + 1], col, zero) if n + 1 < len(chunks) else []
                _run(_mingle(steps(c, 2), ahead + _share(side, n, len(chunks))))

        if "pro" in _PARTS:
            for cp in stages[0]:
                cp.wait()
            _now(prep_kv_w(0, 2, zero))
            project(kv_proj, cs, DM // 2, (7, 6, 5), [])
            for cp in stages[1]:
                cp.wait()
            project(kv_proj, cs, DM // 2, (4, 3, 2, 1, 0), prep_q_w(0, 2, zero))
            for cp in stages[2]:
                cp.wait()
            project(q_proj, xs, 0, (7, 6, 5, 4), [])
            for cp in stages[3]:
                cp.wait()
            project(q_proj, xs, 0, (3, 2, 1, 0), prep_q_w(1, 0, zero) + prep_kv_w(1, 0, zero))

        def pair_step(j, zero):
            for cp in cp_step(j):
                cp.wait()
            for cp in cp_step(j + 1):
                cp.start(priority=_PRIO)
            page = 2 * (j % RING)
            aw = prep_aw(jnp.minimum(j, N_UNITS - 1), j % 2, zero)
            bw = prep_kv_w(j % 2, page + 2, zero) + prep_q_w(j % 2, page + 2, zero)
            wo = prep_wo(j, j % 2, zero)
            side = [p for k in range(8)
                    for p in _share(aw, k, 8) + _share(wo, k, 8) + _share(bw, k, 8)]

            def filler(c):
                mine = _share(side, _FIRST - c, _FIRST + 1) if c <= _FIRST else []
                return _mingle(q_proj(c, page) + kv_proj(c, page), mine)

            pair_attention(j, zero, filler)
            return zero + j // NP

        def lap(k, zero):
            @pl.when(k == 0)
            def _():
                for cp in cp_a():
                    cp.start()

            @pl.when(k > 0)
            def _():
                bwop[:2] = bwop[2 * RING:]

            return lax.fori_loop(k * RING, (k + 1) * RING, pair_step, zero)

        pad(_PB, zero)
        if "bloop" in _PARTS:
            zero = lax.fori_loop(0, (NP - 1) // RING, lap, zero)
        gap("4", zero)
        if "last" in _PARTS:
            for cp in cp_step(NP - 1) + cp_a():
                cp.wait()
            pair_attention(NP - 1, zero, lambda c: [], _DEPTH)
        else:
            ctx[0, :8, :128] = q_s[0, :8, :128] + k_s[0, :8, :128] + v_s[0, :8, :128] + bwop[0, 0, :8, :]

    def rows(xaop, aoop, aqkv, oop, out_s):
        @pl.loop(0, 2)
        def _(i):
            aqkv[pl.ds(8 + 8 * i, 8), :HALO, :] = jnp.zeros((8, HALO, 128), F32)

        zero = lax.fori_loop(0, NP - 1, lambda i, z: z + i // NP, jnp.int32(0))

        def cp_out(c, half):
            cols = pl.ds(half * DM, DM)
            return pltpu.make_async_copy(
                out_s.at[half, c], out_hbm.at[pl.ds(pl.multiple_of(c * CH, CH), CH), cols],
                sem_out.at[half * NC + c])

        def prep_xa(c, zero, n=_NB):
            def piece(t, r):
                blocks = [_split(pltpu.bitcast(
                    xa[c, pl.ds(k * R + r, n), pl.ds(h * (DM // 2) + 128 * t, 128)], U32))
                    for k in range(2) for h in range(2)]
                ops = [_join(v) for v in _operands(blocks, LHS)]
                for i, v in enumerate(ops):
                    xaop[0, i, pl.ds(r // 2, n // 2), pl.ds(128 * t, 128)] = v
                return ops
            return [(_pacer(xa, NC + zero), lambda t=t, r=r: piece(t, r))
                    for t in range(4) for r in range(0, R, n)]

        def prep_awo(n, zero):
            return _dim_major(
                lambda k, t: awo_raw[t, :, pl.ds(k * (DM // 2) + 128 * n, 128)].astype(F32),
                _pacer(awo_raw, 8 + zero), shuf, awop, N_UNITS + n, False, zero)

        def prep_ctx(c, zero):
            base = pl.multiple_of(c * (CH // 2), CH // 2)

            def piece(m, r, i):
                outer = {b: [_split(ctx[2 * m + a2, pl.ds(base + ((b // 2) * 64 + r2 * 32 + r), 8),
                                        pl.ds((b % 2) * HD, HD)])
                             for r2 in range(2) for a2 in range(2)] for b, _ in LHS[i]}
                ops = [_join(v) for v in _operands(_combine(outer, LHS[i]), LHS)]
                for k, v in enumerate(ops):
                    oop[NOPS * i + k, pl.ds(r, 8), pl.ds(HD * m, HD)] = v
                return ops
            return [(_pacer(ctx, NP + zero), lambda m=m, r=r, i=i: piece(m, r, i))
                    for m in range(NP // 2) for r in range(0, 32, 8) for i in range(NOPS)]

        def o_proj(c):
            steps = []
            for t in range(2):
                def done(o, val, t=t):
                    r0 = (o[0] // 2) * R + (o[1] // 2) * (R // 2)
                    n0 = (o[0] % 2) * 512 + (o[1] % 2) * 256 + 128 * t
                    out_s[1, c, pl.ds(r0, R // 2), pl.ds(n0, 128)] = val.astype(BF16)
                steps += _block_product(lambda i: _bf16(oop[i]),
                                        lambda i, t=t: _bf16(woop[t, i]), done, levels=2)
            return steps + ([lambda: cp_out(c, 1).start(priority=_PRIO)] if 'D' not in _X else [])

        def a_proj(row0):
            steps = []
            for part in range(3):
                for t in range(4):
                    def done(o, val, part=part, t=t):
                        if part == 0:
                            val = val * (AD ** -0.5 * LOG2E)
                        aqkv[8 * part + t + 4 * (o[0] % 2),
                             pl.ds(row0 + (HALO + (o[0] // 2) * R), R), :] = val

                    def rhs(i, part=part, t=t):
                        return _bf16(jnp.concatenate(
                            [awop[4 * part + m, i, pl.ds(64 * t, 64), :] for m in range(4)], axis=1))
                    steps += _block_product(lambda i: _bf16(xaop[0, i]), rhs, done, dims=NT)
            return steps

        def a_attention(c, row0, zero):
            logit, prob, mixed = {}, {}, {}

            def dot(r, w):
                tot = None
                for t in range(8):
                    if (r, t) not in logit:
                        logit[r, t] = aqkv[t, pl.ds(row0 + (HALO + r), 8), :]
                    pr = logit[r, t] * aqkv[8 + t, pl.ds(row0 + (HALO + r - DIL * w), 8), :]
                    tot = pr if tot is None else tot + pr
                logit[r, "w", w] = tot
                if w == WIN - 1:
                    weights(r)
                return [tot]

            def weights(r):
                logits = [logit[r, "w", w] for w in range(WIN)]
                logits = [x + pltpu.roll(x, 64, 1) for x in logits]
                logits = [x + pltpu.roll(x, 32, 1) for x in logits]
                if r < (WIN - 1) * DIL:
                    pos = c * CH + r + lax.broadcasted_iota(jnp.int32, (8, 128), 0)
                    logits = [x if w == 0 else jnp.where(pos >= DIL * w, x, MASKED)
                              for w, x in enumerate(logits)]
                top = logits[0]
                for x in logits[1:]:
                    top = jnp.maximum(top, x)
                e = [jnp.exp2(x - top) for x in logits]
                tot = e[0]
                for x in e[1:]:
                    tot = tot + x
                inv = _recip(tot)
                prob[r] = [x * inv for x in e]

            def mix(r, t, d, h):
                tot = None
                for w in range(WIN):
                    pr = prob[r + d][w] * aqkv[16 + t + 4 * h,
                                               pl.ds(row0 + (HALO + r + d - DIL * w), 8), :]
                    tot = pr if tot is None else tot + pr
                mixed[d, h] = tot
                if (d, h) == (R + 8, 1):
                    ops = _operands([jnp.concatenate([mixed[k, h], mixed[k + 8, h]], axis=0)
                                     for k in (0, R) for h in range(2)], LHS)
                    for i, v in enumerate(ops):
                        _store(aoop, (0, i), r // 2, 128 * t, v)
                    return ops
                return [tot]

            def dots(r):
                return [lambda d=d, w=w: dot(r + d, w) for d in (0, 8, R, R + 8) for w in range(WIN)]

            def mixes(r):
                return [lambda t=t, d=d, h=h: mix(r, t, d, h)
                        for t in range(4) for d in (0, 8, R, R + 8) for h in range(2)]

            work = dots(0)
            for r in range(16, R, 16):
                work += [w for pair in zip(dots(r), mixes(r - 16)) for w in pair]
            work += mixes(R - 16)
            return [(_pacer(aqkv, 24 + zero), lambda g=work[i:i + _NA]: sum((w() for w in g), []))
                    for i in range(0, len(work), _NA)]

        def a_out_proj(c, zero):
            steps = []
            for n in range(4):
                def done(o, val, n=n):
                    out_s[0, c, pl.ds((o[0] // 2) * R, R),
                          pl.ds((o[0] % 2) * (DM // 2) + 128 * n, 128)] = val.astype(BF16)
                steps += _block_product(lambda i: _bf16(aoop[zero, i]),
                                        lambda i, n=n: _bf16(awop[N_UNITS + n, i]), done)
            return steps + ([lambda: cp_out(c, 0).start(priority=_PRIO)] if 'D' not in _X else [])

        if "s0" in _PARTS:
            _now(prep_xa(zero, zero))
            side = (prep_wo(NP - 1, (NP - 1) % 2, zero) + prep_ctx(0, zero)
                    + sum((prep_awo(n, zero) for n in range(4)), []))
            _run(_mingle(a_proj(0), side))

        def chunk_step(c, zero):
            row0 = pl.multiple_of((c - 1) * CH, CH)
            first, second = o_proj(c - 1), a_proj(row0 + CH)
            att = a_attention(c - 1, row0, zero) if 'A' not in _X else []
            cut = len(att) * 3 // 5
            xap, ctxp = prep_xa(c, zero), prep_ctx(c, zero) if 'C' not in _X else []
            _run(_mingle(first[:-_AT], [p for k in range(16)
                                        for p in _share(att[:cut], k, 16) + _share(xap, k, 16)])
                 + first[-_AT:])
            _run(_mingle(second[:-_AT], [p for k in range(32)
                                         for p in _share(att[cut:], k, 32) + _share(ctxp, k, 32)])
                 + second[-_AT:])
            _run(a_out_proj(c - 1, zero))
            return zero + c // NC

        pad(_PA, zero)
        if "aloop" in _PARTS:
            zero = lax.fori_loop(1, NC, chunk_step, zero)
        gap("2", zero)

        if "epi" in _PARTS:
            steps = o_proj(NC - 1)
            _run(_mingle(steps[:-_AT], a_attention(NC - 1, (NC - 1) * CH, zero)) + steps[-_AT:])
            _run(a_out_proj(NC - 1, zero))
            for c in range(NC):
                cp_out(c, 1).wait()
                cp_out(c, 0).wait()
        else:
            out_s[0, 0, :16, :128] = aqkv[3, :16, :].astype(BF16)
            out_s[0, 0, 16:32, :128] = _bf16(awop[0, 0, :8, :] + ctx[0, :8, :128] + woop[0, 0, :8, :]
                                             + oop[0, :8, :128])
            cp_out(0, 0).start()
            cp_out(0, 0).wait()

    vmem = pltpu.VMEM
    pl.run_scoped(
        heads,
        vmem((NC + 1, CH, DM), BF16),
        vmem((NC + 1, CH, DC), BF16),
        vmem((NC + 1, NOPS, R // 2, (DM + DC) // 2), U32),
        vmem((3, DM, HD), U32),
        vmem((3, DC, HD), U32),
        vmem((3, DC, HD), U32),
        vmem((2 * (RING + 1), NOPS, OPROWS, 128), U32),
        vmem((1, S // 2 + _QP, 2 * HD), U32),
        vmem((1, S // 2, 2 * HD), U32),
        vmem((1, S // 2, 2 * HD), U32),
        vmem((3, 2, 128, DM), BF16),
    )
    pl.run_scoped(
        rows,
        vmem((1, NOPS, R // 2, DM // 2), U32),
        vmem((1, NOPS, R // 2, DM // 2), U32),
        vmem((25, HALO + S + _AP, 128), F32),
        vmem((NOPS * NOPS, R // 4, NP * HD // 2), U32),
        vmem((2, NC, CH, DM), BF16),
    )


@jax.jit
def pallas_concat_heads__sliding_local_dilated__compressed_kv_cla__prompt_kernel(
    A_x: jax.Array,
    A_wqkv: jax.Array,
    A_wo: jax.Array,
    B_x: jax.Array,
    B_c_kv: jax.Array,
    B_w_q: jax.Array,
    B_w_uk: jax.Array,
    B_w_uv: jax.Array,
    B_w_o: jax.Array,
):
    vmem = pltpu.VMEM
    dma = pltpu.SemaphoreType.DMA
    scratch = [
        vmem((_DUM, 128), F32),
        vmem((NP + 1, S // 2, 2 * HD), U32),
        vmem((3, 4, 2 * HD, 128), U32),
        vmem((2, NOPS * NOPS, NP * HD // 4, 128), U32),
        vmem((N_UNITS + 4, NOPS, OPROWS, 128), U32),
        vmem((NC + 1, CH, DM), BF16),
        vmem((9, 128, DM), BF16),
        vmem((3, NH * PITCH, 128), F32),
        dma((NC,)), dma((NC,)), dma((8,)), dma((4,)), dma((2,)), dma((2 * NC,)),
    ]
    out = pl.pallas_call(
        _kernel,
        out_shape=jax.ShapeDtypeStruct((S, 2 * DM), BF16),
        in_specs=[pl.BlockSpec(memory_space=pl.ANY)] * 9,
        out_specs=pl.BlockSpec(memory_space=pl.ANY),
        scratch_shapes=scratch,
        compiler_params=pltpu.CompilerParams(vmem_limit_bytes=124 * 2**20),
        name="fused_local_and_latent_attention",
    )(
        A_x.reshape(S, DM), A_wqkv, A_wo,
        B_x.reshape(S, DM), B_c_kv.reshape(S, DC),
        B_w_q, B_w_uk, B_w_uv, B_w_o.reshape(NH * HD, DM),
    )
    return out.reshape(1, S, 2 * DM)
```

```python
import math

import jax
import jax.numpy as jnp
from jax import lax
import jax.experimental.pallas as pl
import jax.experimental.pallas.tpu as pltpu

F32, BF16, U32 = jnp.float32, jnp.bfloat16, jnp.uint32

S = 2048
DM = 1024
DC = 512
NH = 32
HD = 128
AD = 32
WIN, DIL = 8, 2

R = 128
CH = 2 * R
NC = S // CH
NP = NH // 2
HALO = 16
PITCH = 33

_PARTS = ("pro", "bloop", "last", "s0", "aloop", "epi")
_X = ""
_FIRST = 6
_NA = 2
_NB = 16
_LAG = 3
_AT = 3
_PRIO = 0
_QS = 'ob'
_Q0 = 4
_SP = 1
_KG = 4
_CT = 4
_CU = 10
_DUM = 24
_QP = 16
_AP = 16
_PA = 0
_PB = 0
_CL = 4
_DEPTH = 2
LOG2E = math.log2(math.e)
MASKED = -1e9 * LOG2E

NN = (((1,), (0,)), ((), ()))
NT = (((1,), (1,)), ((), ()))

LHS = (((0, 1), (3, 1)), ((2, 1), (3, 1)), ((0, 1),), ((3, 1),),
       ((0, 1), (1, 1)), ((2, 1), (0, -1)), ((1, 1), (3, -1)))
RHS = (((0, 1), (3, 1)), ((0, 1),), ((1, 1), (3, -1)), ((2, 1), (0, -1)),
       ((3, 1),), ((0, 1), (1, 1)), ((2, 1), (3, 1)))
PRODUCTS = ((2, ((1, 1), (3, 1))), (4, ((0, -1), (1, 1))), (3, ((0, 1), (2, 1))),
            (1, ((2, 1), (3, -1))), (5, ((3, 1),)), (0, ((0, 1), (3, 1))),
            (6, ((0, 1),)))
NOPS = len(PRODUCTS)

OPROWS = 256
N_UNITS = 12
KVROWS = 64
W_KV = NOPS * OPROWS
SLOT = W_KV + NOPS * NOPS * KVROWS
RING = 5


def _combine(blocks, terms):
    if isinstance(blocks[terms[0][0]], list):
        return [_combine({b: blocks[b][i] for b, _ in terms}, terms) for i in range(4)]
    out = None
    for i, sign in terms:
        if out is None:
            assert sign > 0
            out = blocks[i]
        else:
            out = out + blocks[i] if sign > 0 else out - blocks[i]
    return out


def _store(words, index, row, col, x):
    matrix = words.bitcast(BF16).at[index]
    matrix[pl.ds(2 * row, x.shape[0]), pl.ds(col, x.shape[1])] = x.astype(BF16)


def _bf16(words):
    return pltpu.bitcast(words, BF16)


def _halves(words):
    lo = pltpu.bitcast(words << 16, F32)
    hi = pltpu.bitcast(words & jnp.uint32(0xFFFF0000), F32)
    return lo, hi


def _split(words):
    return jnp.concatenate(_halves(words), axis=0)


def _join(x):
    n = x.shape[0] // 2
    return pltpu.pack_elementwise([x[:n], x[n:]], packed_dtype=BF16)


def _recip(x):
    r = pltpu.reciprocal(x, approx=True)
    return r * (2.0 - x * r)


def _operands(blocks, side):
    return [_combine(blocks, terms) for terms in side]


def _block_product(lhs, rhs, done, dims=NN, levels=1):
    if levels == 0:
        def step():
            m = lax.dot_general(lhs(0), rhs(0), dims, preferred_element_type=F32)
            done((), m)
            return m
        return [step]

    held, steps = {}, []
    inner = NOPS ** (levels - 1)
    for n, (i, outs) in enumerate(PRODUCTS):
        later = {o for _, others in PRODUCTS[n + 1:] for o, _ in others}

        def add(sub, m, outs=outs, later=later):
            for o, sign in outs:
                if (o, sub) not in held:
                    held[o, sub] = m, sign
                else:
                    c, s = held[o, sub]
                    assert s > 0 or sign > 0
                    held[o, sub] = (m - c if s < 0 else c + m if sign > 0 else c - m), 1
                if o not in later:
                    done((o, *sub), held.pop((o, sub))[0])

        steps += _block_product(lambda k, i=i: lhs(i * inner + k),
                                lambda k, i=i: rhs(i * inner + k), add, dims, levels - 1)
    return steps


def _run(steps, n=None):
    out = None
    for _ in range(len(steps) if n is None else min(n, len(steps))):
        out = steps.pop(0)()
    return out


def _group(steps, n):
    return [lambda g=steps[i:i + n]: _run(g) for i in range(0, len(steps), n)]


def _share(items, k, n):
    return items[k * len(items) // n:(k + 1) * len(items) // n]


def _blend(*lists):
    spots = [((i + 0.5) / len(items), k, item)
             for k, items in enumerate(lists) for i, item in enumerate(items)]
    return [item for *_, item in sorted(spots, key=lambda spot: spot[:2])]


def _witness(values):
    out = None
    for v in values:
        v = pltpu.bitcast(v, U32)
        for r in range(0, v.shape[0], 8):
            for c in range(0, v.shape[1], 128):
                out = v[r:r + 8, c:c + 128] if out is None else out | v[r:r + 8, c:c + 128]
    return out


def _mingle(steps, pieces):
    history = []

    def both(step, mine):
        history.append(step())
        for i, (pace, work, *lag) in enumerate(mine):
            seen = work()
            m = history[max(0, len(history) - 1 - sum(lag))]
            if m is not None:
                r = 8 * (i * (m.shape[0] // 8) // len(mine))
                pace(_witness([m[r:r + 8, :128]] + list(seen)))
        return history[-1]

    return [lambda step=step, mine=_share(pieces, i, len(steps)): both(step, mine)
            for i, step in enumerate(steps)]


def _now(pieces):
    for _, work, *_ in pieces:
        work()


def _pacer(ref, *index):
    def pace(v):
        if ref.dtype == BF16:
            ref[(*index, pl.ds(0, 16), pl.ds(0, 128))] = _bf16(v)
        else:
            ref[(*index, pl.ds(0, 8), pl.ds(0, 128))] = pltpu.bitcast(v, ref.dtype)
    return pace


def _dim_major(src, pace, shuf, dst, page, swap, zero):
    def start(head):
        return ((head % 2) * NH // 2 + head // 2) * PITCH

    def scatter(k, u):
        t = src(k, u)
        for h in range(128 // AD):
            shuf[k, pl.ds(start(4 * u + h), AD), :] = t[h * AD:(h + 1) * AD]
        return [t]

    def gather(d, h):
        x = [[jnp.concatenate([shuf[k, pl.ds(start(h + p) + a * AD // 2 + d, 8, stride=PITCH), :]
                               for p in range(2)], axis=0)
              for k in range(2)] for a in range(2)]
        blocks = ([x[0][0], x[1][0], x[0][1], x[1][1]] if swap
                  else [x[0][0], x[0][1], x[1][0], x[1][1]])
        ops = [_join(v) for v in _operands(blocks, RHS)]
        for i, v in enumerate(ops):
            dst[page, i, pl.ds((d * NH + h) // 2, 8), :] = v
        return ops

    return ([(pace, lambda k=k, u=u: scatter(k, u), _LAG if swap else 0)
             for k in range(2) for u in range(NH * AD // 128)]
            + [(_pacer(shuf, 2 + zero), lambda d=d, h=h: gather(d, h))
               for d in range(AD // 2) for h in range(0, NH, 16)])


def _kernel(ax_hbm, awqkv_hbm, awo_hbm, bx_hbm, c_hbm, wq_hbm, wuk_hbm, wuv_hbm,
            wo_hbm, out_hbm,
            dummy, ctx, wo_raw, woop, awop, xa, awo_raw, shuf,
            sem_x, sem_c, sem_w, sem_aw, sem_a, sem_out):

    def cp_wo(u, s):
        rows = pl.ds(pl.multiple_of((u // 2) * 4 * HD, 4 * HD), 4 * HD)
        return [pltpu.make_async_copy(
            wo_hbm.at[rows, pl.ds(pl.multiple_of(q * 256 + (u % 2) * 128, 128), 128)],
            wo_raw.at[s, q].bitcast(BF16), sem_w.at[6 + s]) for q in range(4)]

    def prep_wo(u, s, zero):
        def piece(r, i):
            outer = {b: [_split(wo_raw[s, 2 * (b % 2) + b2,
                                       pl.ds((2 * a2 + b // 2) * (HD // 2) + r, 8), :])
                         for a2 in range(2) for b2 in range(2)] for b, _ in RHS[i]}
            ops = [_join(v) for v in _operands(_combine(outer, RHS[i]), RHS)]
            row = pl.multiple_of((u // 2) * (HD // 2) + r, 8)
            for k, v in enumerate(ops):
                woop[u % 2, NOPS * i + k, pl.ds(row, 8), :] = v
            return ops
        return [(_pacer(wo_raw, 2 + zero, 0), lambda r=r, i=i: piece(r, i))
                for r in range(0, HD // 2, 8) for i in range(NOPS)]

    def gap(flag, zero):
        if flag in _X:
            @pl.loop(0, 2)
            def _(i):
                _pacer(shuf, 2 + zero * i)(jnp.zeros((8, 128), U32))

    def pad(n, zero):
        if n:
            @pl.when(zero != 0)
            def _():
                v = shuf[0, :128]
                for _ in range(n * 95):
                    v = v * 1.0001 + 0.5
                shuf[0, :128] = v

    dummy[:8] = jnp.zeros((8, 128), F32)
    shuf[0, :8] = dummy[pl.ds(1, 8)]

    def cp_a():
        return ([pltpu.make_async_copy(ax_hbm.at[pl.ds(c * CH, CH)], xa.at[c], sem_a.at[0])
                 for c in range(NC)]
                + [pltpu.make_async_copy(awo_hbm.at[pl.ds(128 * t, 128)], awo_raw.at[t], sem_a.at[1])
                   for t in range(8)])

    def heads(xs, cs, xop, cop, wq_raw, wkv_raw, bwop, q_s, k_s, v_s, aw_raw):
        wq32 = wq_hbm.bitcast(U32)
        wuk32 = wuk_hbm.bitcast(U32)
        wuv32 = wuv_hbm.bitcast(U32)

        def cp_x(c):
            return pltpu.make_async_copy(bx_hbm.at[pl.ds(c * CH, CH)], xs.at[c], sem_x.at[c])

        def cp_c(c):
            return pltpu.make_async_copy(c_hbm.at[pl.ds(c * CH, CH)], cs.at[c], sem_c.at[c])

        def cp_proj_w(j, s):
            return [
                pltpu.make_async_copy(wuk32.at[:, j, :], wkv_raw.at[0, s], sem_w.at[s]),
                pltpu.make_async_copy(wuv32.at[:, j, :], wkv_raw.at[1, s], sem_w.at[2 + s]),
                pltpu.make_async_copy(wq32.at[:, j, :], wq_raw.at[s], sem_w.at[4 + s]),
            ]

        def cp_aw(u, s):
            cols = pl.ds(pl.multiple_of((u // 4) * DM, DM), DM)
            return [pltpu.make_async_copy(
                awqkv_hbm.at[pl.ds(pl.multiple_of((u % 4) * 128 + half * (DM // 2), 128), 128), cols],
                aw_raw.at[s, half], sem_aw.at[2 * s + half]) for half in range(2)]

        def cp_step(j):
            return (cp_proj_w(jnp.minimum(j + 2, NP - 1), j % 2) + cp_wo(j, j % 2)
                    + cp_aw(jnp.minimum(j, N_UNITS - 1), j % 2))

        def prep_x(c):
            for t in range(DM // 256):
                blocks = [_split(pltpu.bitcast(
                    xs[c, pl.ds(k * R, R), pl.ds(h * DM // 2 + 128 * t, 128)], U32))
                    for k in range(2) for h in range(2)]
                for i, v in enumerate(_operands(blocks, LHS)):
                    xop[c, i, :, pl.ds(128 * t, 128)] = _join(v)

        def prep_c(c):
            blocks = [[_split(pltpu.bitcast(
                cs[c, pl.ds(r1 * R + r2 * R // 2, R // 2), pl.ds(a1 * 256 + a2 * 128, 128)], U32))
                for r2 in range(2) for a2 in range(2)] for r1 in range(2) for a1 in range(2)]
            for i, outer in enumerate(_operands(blocks, LHS)):
                for k, v in enumerate(_operands(outer, LHS)):
                    cop[c, NOPS * i + k] = _join(v)

        def both_heads(raw, s, row):
            even, odd = (_halves(raw[s, pl.ds(row + p, 8, stride=2), :]) for p in range(2))
            return [jnp.concatenate([even[h], odd[h]], axis=0) for h in range(2)]

        def prep_q_w(s, slot, zero):
            def piece(r):
                blocks = both_heads(wq_raw, s, r) + both_heads(wq_raw, s, DM // 2 + r)
                ops = [_join(v) for v in _operands(blocks, RHS)]
                for i, v in enumerate(ops):
                    bwop[pl.ds(slot + (i * OPROWS + r // 2), 8), :] = v
                return ops
            return [(_pacer(wq_raw, 2 + zero), lambda r=r: piece(r)) for r in range(0, DM // 2, 16)]

        def prep_kv_w(s, slot, zero):
            def piece(r, i):
                outer = {b: [v for a2 in range(2)
                             for v in both_heads(wkv_raw.at[b % 2], s, (b // 2) * 256 + a2 * 128 + r)]
                         for b, _ in RHS[i]}
                ops = [_join(v) for v in _operands(_combine(outer, RHS[i]), RHS)]
                for k, v in enumerate(ops):
                    bwop[pl.ds(slot + (W_KV + (NOPS * i + k) * KVROWS + r // 2), 8), :] = v
                return ops
            return [(_pacer(wkv_raw, zero, 2), lambda r=r, i=i: piece(r, i))
                    for r in range(0, 128, 16) for i in range(NOPS)]

        def prep_aw(u, s, zero):
            return _dim_major(
                lambda k, t: aw_raw[s, k, :, 128 * t:128 * (t + 1)].astype(F32).T,
                _pacer(xop, NC + zero, 0), shuf, awop, u, True, zero)

        def words(blk):
            return pl.ds(blk * (R // 2), R // 2)

        def q_proj(c, slot):
            def done(o, val):
                _store(q_s, 0, (2 * c + o[0] // 2) * (R // 2), (o[0] % 2) * HD,
                       val * (HD ** -0.5 * LOG2E))
            return _block_product(lambda i: _bf16(xop[c, i]),
                                  lambda i: _bf16(bwop[pl.ds(slot + i * OPROWS, OPROWS), :]), done)

        def kv_proj(c, slot):
            def done(o, val):
                _store((k_s, v_s)[o[0] % 2], 0,
                       (2 * c + o[0] // 2) * (R // 2) + (o[1] // 2) * (R // 4), (o[1] % 2) * HD, val)
            return _group(_block_product(
                lambda i: _bf16(cop[c, i]),
                lambda i: _bf16(bwop[pl.ds(slot + (W_KV + i * KVROWS), KVROWS), :]),
                done, levels=2), _KG)

        def scores(h, blk):
            n = (blk + 1) * R
            s = lax.dot_general(_bf16(q_s[0, words(blk), pl.ds(h * HD, HD)]),
                                _bf16(k_s[0, :n // 2, pl.ds(h * HD, HD)]),
                                NT, preferred_element_type=F32)
            row = lax.broadcasted_iota(jnp.int32, (R, R), 0)
            col = lax.broadcasted_iota(jnp.int32, (R, R), 1)
            diag = jnp.where(col <= row, s[:, n - R:], MASKED)
            return diag if blk == 0 else jnp.concatenate([s[:, :n - R], diag], axis=1)

        def attend(h, blk, s):
            n = (blk + 1) * R
            p = jnp.exp2(s - jnp.max(s, axis=1, keepdims=True))
            if "u" in _X:
                p = p.astype(BF16).astype(F32)
            inv = _recip(jnp.sum(p, axis=1, keepdims=True))
            o = lax.dot_general(p.astype(BF16), _bf16(v_s[0, :n // 2, pl.ds(h * HD, HD)]), NN,
                                preferred_element_type=F32)
            return o * inv

        def pair_attention(j, zero, filler, side=(), depth=1):
            blocks = [(h, 2 * c + u) for c in reversed(range(NC)) for u in (1, 0) for h in (0, 1)]
            tiles = [(b, t) for b in blocks[_Q0:] for t in range(b[1] + 1)]

            def paced_scores(h, blk):
                s = scores(h, blk)
                for n, (b, t) in enumerate(tiles):
                    if b == (h, blk):
                        mine = _share(side, n, len(tiles))
                        for i, (pace, work, *_) in enumerate(mine):
                            r = 8 * (i * (R // 8) // len(mine))
                            pace(_witness([s[r:r + 8, t * R:(t + 1) * R]] + list(work())))
                return s

            todo, done = [], []
            ahead = [paced_scores(*b) for b in blocks[:depth]]
            for n, (h, blk) in enumerate(blocks):
                ahead += [paced_scores(*b) for b in blocks[n + depth:n + depth + 1]]
                cnt = -(-len(todo) // (4 - n % 4))
                _run(todo, cnt - cnt * _SP // 4)
                done.append(attend(h, blk, ahead.pop(0)))
                _store(ctx, j, blk * (R // 2), h * HD, done[-1])
                if len(done) > _CL:
                    q_s[zero, pl.ds(S // 2, 8), :128] = _witness([done.pop(0)])
                _run(todo, cnt * _SP // 4)
                if n % 4 == 3:
                    todo = filler(blk // 2)
            _run(todo)

        w0, w1 = cp_proj_w(0, 0), cp_proj_w(1, 1)
        stages = [w0[:2] + [cp_c(c) for c in (7, 6, 5)],
                  [cp_c(c) for c in (4, 3, 2, 1, 0)] + w0[2:],
                  [cp_x(c) for c in (7, 6, 5, 4)],
                  [cp_x(c) for c in (3, 2, 1)] + w1,
                  [cp_x(0)],
                  cp_step(0)]

        def issue(i, zero):
            for k, stage in enumerate(stages):
                @pl.when(i == k)
                def _(stage=stage):
                    for cp in stage:
                        cp.start()
            return zero + i // NP

        zero = lax.fori_loop(0, len(stages), issue, jnp.int32(0)) if 'pro' in _PARTS else lax.fori_loop(0, 15, lambda i, z: z + i // NP, jnp.int32(0))

        def project(prep, steps, chunks, side):
            for n, c in enumerate(chunks):
                prep(c)
                _run(_mingle(steps(c, SLOT), _share(side, n, len(chunks))))

        if "pro" in _PARTS:
            for cp in stages[0]:
                cp.wait()
            _now(prep_kv_w(0, SLOT, zero))
            project(prep_c, kv_proj, (7, 6, 5), [])
            for cp in stages[1]:
                cp.wait()
            project(prep_c, kv_proj, (4, 3, 2, 1, 0), prep_q_w(0, SLOT, zero))
            for cp in stages[2]:
                cp.wait()
            project(prep_x, q_proj, (7, 6, 5, 4), [])
            for cp in stages[3]:
                cp.wait()
            project(prep_x, q_proj, (3, 2, 1), prep_q_w(1, 0, zero) + prep_kv_w(1, 0, zero))
            for cp in stages[4]:
                cp.wait()
            project(prep_x, q_proj, (0,), [])

        def pair_step(j, zero):
            for cp in cp_step(j):
                cp.wait()
            for cp in cp_step(j + 1):
                cp.start(priority=_PRIO)
            slot = pl.multiple_of((j % RING) * SLOT, KVROWS)
            aw = prep_aw(jnp.minimum(j, N_UNITS - 1), j % 2, zero)
            bw = prep_kv_w(j % 2, slot + SLOT, zero) + prep_q_w(j % 2, slot + SLOT, zero)
            wo = prep_wo(j, j % 2, zero)
            groups = dict(a=aw, o=wo, b=bw)
            side = _blend(*[groups[g] for g in "aob" if g not in _QS])

            def filler(c):
                mine = _share(side, _FIRST - c, _FIRST + 1) if c <= _FIRST else []
                return _mingle(q_proj(c, slot) + kv_proj(c, slot), mine)

            pair_attention(j, zero, filler, _blend(*[groups[g] for g in _QS]))
            return zero + j // NP

        def lap(k, zero):
            @pl.when(k == 0)
            def _():
                for cp in cp_a():
                    cp.start()

            @pl.when(k > 0)
            def _():
                bwop[:SLOT] = bwop[RING * SLOT:]

            return lax.fori_loop(k * RING, (k + 1) * RING, pair_step, zero)

        pad(_PB, zero)
        if "bloop" in _PARTS:
            zero = lax.fori_loop(0, (NP - 1) // RING, lap, zero)
        gap("4", zero)
        if "last" in _PARTS:
            for cp in cp_step(NP - 1) + cp_a():
                cp.wait()
            pair_attention(NP - 1, zero, lambda c: [], depth=_DEPTH)
        else:
            ctx[0, :8, :128] = (q_s[zero, :8, :128] + k_s[zero, :8, :128] + v_s[zero, :8, :128]
                                + bwop[pl.ds(zero, 8), :] + xop[zero, 0, :8, :128] + cop[zero, 0, :8, :])

    def rows(xaop, aoop, aqkv, oop, out_s):
        @pl.loop(0, 2)
        def _(i):
            aqkv[pl.ds(8 + 8 * i, 8), :HALO, :] = jnp.zeros((8, HALO, 128), F32)

        zero = lax.fori_loop(0, NP - 1, lambda i, z: z + i // NP, jnp.int32(0))

        def cp_out(c, half):
            cols = pl.ds(half * DM, DM)
            return pltpu.make_async_copy(
                out_s.at[half, c], out_hbm.at[pl.ds(pl.multiple_of(c * CH, CH), CH), cols],
                sem_out.at[half * NC + c])

        def prep_xa(c, zero, n=_NB):
            def piece(t, r):
                blocks = [_split(pltpu.bitcast(
                    xa[c, pl.ds(k * R + r, n), pl.ds(h * (DM // 2) + 128 * t, 128)], U32))
                    for k in range(2) for h in range(2)]
                ops = [_join(v) for v in _operands(blocks, LHS)]
                for i, v in enumerate(ops):
                    xaop[0, i, pl.ds(r // 2, n // 2), pl.ds(128 * t, 128)] = v
                return ops
            return [(_pacer(xa, NC + zero), lambda t=t, r=r: piece(t, r))
                    for t in range(4) for r in range(0, R, n)]

        def prep_awo(n, zero):
            return _dim_major(
                lambda k, t: awo_raw[t, :, pl.ds(k * (DM // 2) + 128 * n, 128)].astype(F32),
                _pacer(awo_raw, 8 + zero), shuf, awop, N_UNITS + n, False, zero)

        def prep_ctx(c, zero):
            base = pl.multiple_of(c * (CH // 2), CH // 2)

            def piece(m, r, i):
                outer = {b: [_split(ctx[2 * m + a2, pl.ds(base + ((b // 2) * 64 + r2 * 32 + r), 8),
                                        pl.ds((b % 2) * HD, HD)])
                             for r2 in range(2) for a2 in range(2)] for b, _ in LHS[i]}
                ops = [_join(v) for v in _operands(_combine(outer, LHS[i]), LHS)]
                for k, v in enumerate(ops):
                    oop[NOPS * i + k, pl.ds(r, 8), pl.ds(HD * m, HD)] = v
                return ops
            return [(_pacer(ctx, NP + zero), lambda m=m, r=r, i=i: piece(m, r, i))
                    for m in range(NP // 2) for r in range(0, 32, 8) for i in range(NOPS)]

        def o_proj(c):
            steps = []
            for t in range(2):
                def done(o, val, t=t):
                    r0 = (o[0] // 2) * R + (o[1] // 2) * (R // 2)
                    n0 = (o[0] % 2) * 512 + (o[1] % 2) * 256 + 128 * t
                    out_s[1, c, pl.ds(r0, R // 2), pl.ds(n0, 128)] = val.astype(BF16)
                steps += _block_product(lambda i: _bf16(oop[i]),
                                        lambda i, t=t: _bf16(woop[t, i]), done, levels=2)
            return steps + ([lambda: cp_out(c, 1).start(priority=_PRIO)] if 'D' not in _X else [])

        def a_proj(row0):
            steps = []
            for part in range(3):
                for t in range(4):
                    def done(o, val, part=part, t=t):
                        if part == 0:
                            val = val * (AD ** -0.5 * LOG2E)
                        aqkv[8 * part + t + 4 * (o[0] % 2),
                             pl.ds(row0 + (HALO + (o[0] // 2) * R), R), :] = val

                    def rhs(i, part=part, t=t):
                        return _bf16(jnp.concatenate(
                            [awop[4 * part + m, i, pl.ds(64 * t, 64), :] for m in range(4)], axis=1))
                    steps += _block_product(lambda i: _bf16(xaop[0, i]), rhs, done, dims=NT)
            return steps

        def a_attention(c, row0, zero):
            logit, prob, mixed = {}, {}, {}

            def dot(r, w):
                tot = None
                for t in range(8):
                    if (r, t) not in logit:
                        logit[r, t] = aqkv[t, pl.ds(row0 + (HALO + r), 8), :]
                    pr = logit[r, t] * aqkv[8 + t, pl.ds(row0 + (HALO + r - DIL * w), 8), :]
                    tot = pr if tot is None else tot + pr
                logit[r, "w", w] = tot
                if w == WIN - 1:
                    weights(r)
                return [tot]

            def weights(r):
                logits = [logit[r, "w", w] for w in range(WIN)]
                logits = [x + pltpu.roll(x, 64, 1) for x in logits]
                logits = [x + pltpu.roll(x, 32, 1) for x in logits]
                if r < (WIN - 1) * DIL:
                    pos = c * CH + r + lax.broadcasted_iota(jnp.int32, (8, 128), 0)
                    logits = [x if w == 0 else jnp.where(pos >= DIL * w, x, MASKED)
                              for w, x in enumerate(logits)]
                top = logits[0]
                for x in logits[1:]:
                    top = jnp.maximum(top, x)
                e = [jnp.exp2(x - top) for x in logits]
                tot = e[0]
                for x in e[1:]:
                    tot = tot + x
                inv = _recip(tot)
                prob[r] = [x * inv for x in e]

            def mix(r, t, d, h):
                tot = None
                for w in range(WIN):
                    pr = prob[r + d][w] * aqkv[16 + t + 4 * h,
                                               pl.ds(row0 + (HALO + r + d - DIL * w), 8), :]
                    tot = pr if tot is None else tot + pr
                mixed[d, h] = tot
                if (d, h) == (R + 8, 1):
                    ops = _operands([jnp.concatenate([mixed[k, h], mixed[k + 8, h]], axis=0)
                                     for k in (0, R) for h in range(2)], LHS)
                    for i, v in enumerate(ops):
                        _store(aoop, (0, i), r // 2, 128 * t, v)
                    return ops
                return [tot]

            def dots(r):
                return [lambda d=d, w=w: dot(r + d, w) for d in (0, 8, R, R + 8) for w in range(WIN)]

            def mixes(r):
                return [lambda t=t, d=d, h=h: mix(r, t, d, h)
                        for t in range(4) for d in (0, 8, R, R + 8) for h in range(2)]

            work = dots(0)
            for r in range(16, R, 16):
                work += [w for pair in zip(dots(r), mixes(r - 16)) for w in pair]
            work += mixes(R - 16)
            return [(_pacer(aqkv, 24 + zero), lambda g=work[i:i + _NA]: sum((w() for w in g), []))
                    for i in range(0, len(work), _NA)]

        def a_out_proj(c, zero):
            steps = []
            for n in range(4):
                def done(o, val, n=n):
                    out_s[0, c, pl.ds((o[0] // 2) * R, R),
                          pl.ds((o[0] % 2) * (DM // 2) + 128 * n, 128)] = val.astype(BF16)
                steps += _block_product(lambda i: _bf16(aoop[zero, i]),
                                        lambda i, n=n: _bf16(awop[N_UNITS + n, i]), done)
            return steps + ([lambda: cp_out(c, 0).start(priority=_PRIO)] if 'D' not in _X else [])

        if "s0" in _PARTS:
            _now(prep_xa(zero, zero))
            side = _blend(prep_wo(NP - 1, (NP - 1) % 2, zero), prep_ctx(0, zero),
                          sum((prep_awo(n, zero) for n in range(4)), []))
            _run(_mingle(a_proj(0), side))

        def chunk_step(c, zero):
            row0 = pl.multiple_of((c - 1) * CH, CH)
            first, second = o_proj(c - 1), a_proj(row0 + CH)
            att = a_attention(c - 1, row0, zero) if 'A' not in _X else []
            cut = len(att) * _CU // 16
            xap, ctxp = prep_xa(c, zero), prep_ctx(c, zero) if 'C' not in _X else []
            third = a_out_proj(c - 1, zero)
            late = len(ctxp) * _CT // 16
            _run(_mingle(first[:-1], _blend(att[:cut], xap)) + first[-1:])
            _run(_mingle(second[:-_AT], _blend(att[cut:], ctxp[:-late])) + second[-_AT:])
            _run(_mingle(third[:-_AT], ctxp[-late:]) + third[-_AT:])
            return zero + c // NC

        pad(_PA, zero)
        if "aloop" in _PARTS:
            zero = lax.fori_loop(1, NC, chunk_step, zero)
        gap("2", zero)

        if "epi" in _PARTS:
            steps = o_proj(NC - 1)
            _run(_mingle(steps[:-_AT], a_attention(NC - 1, (NC - 1) * CH, zero)) + steps[-_AT:])
            _run(a_out_proj(NC - 1, zero))
            for c in range(NC):
                cp_out(c, 1).wait()
                cp_out(c, 0).wait()
        else:
            out_s[0, 0, :16, :128] = aqkv[3, :16, :].astype(BF16)
            out_s[0, 0, 16:32, :128] = _bf16(awop[0, 0, :8, :] + ctx[0, :8, :128] + woop[0, 0, :8, :]
                                             + oop[0, :8, :128])
            cp_out(0, 0).start()
            cp_out(0, 0).wait()

    vmem = pltpu.VMEM
    pl.run_scoped(
        heads,
        vmem((NC, CH, DM), BF16),
        vmem((NC, CH, DC), BF16),
        vmem((NC + 1, NOPS, R // 2, DM // 2), U32),
        vmem((NC, NOPS * NOPS, R // 4, 128), U32),
        vmem((3, DM, HD), U32),
        vmem((2, 3, DC, HD), U32),
        vmem(((RING + 1) * SLOT, 128), U32),
        vmem((1, S // 2 + _QP, 2 * HD), U32),
        vmem((1, S // 2, 2 * HD), U32),
        vmem((1, S // 2, 2 * HD), U32),
        vmem((3, 2, 128, DM), BF16),
    )
    pl.run_scoped(
        rows,
        vmem((1, NOPS, R // 2, DM // 2), U32),
        vmem((1, NOPS, R // 2, DM // 2), U32),
        vmem((25, HALO + S + _AP, 128), F32),
        vmem((NOPS * NOPS, R // 4, NP * HD // 2), U32),
        vmem((2, NC, CH, DM), BF16),
    )


@jax.jit
def pallas_concat_heads__sliding_local_dilated__compressed_kv_cla__prompt_kernel(
    A_x: jax.Array,
    A_wqkv: jax.Array,
    A_wo: jax.Array,
    B_x: jax.Array,
    B_c_kv: jax.Array,
    B_w_q: jax.Array,
    B_w_uk: jax.Array,
    B_w_uv: jax.Array,
    B_w_o: jax.Array,
):
    vmem = pltpu.VMEM
    dma = pltpu.SemaphoreType.DMA
    scratch = [
        vmem((_DUM, 128), F32),
        vmem((NP + 1, S // 2, 2 * HD), U32),
        vmem((3, 4, 2 * HD, 128), U32),
        vmem((2, NOPS * NOPS, NP * HD // 4, 128), U32),
        vmem((N_UNITS + 4, NOPS, OPROWS, 128), U32),
        vmem((NC + 1, CH, DM), BF16),
        vmem((9, 128, DM), BF16),
        vmem((3, NH * PITCH, 128), F32),
        dma((NC,)), dma((NC,)), dma((8,)), dma((4,)), dma((2,)), dma((2 * NC,)),
    ]
    out = pl.pallas_call(
        _kernel,
        out_shape=jax.ShapeDtypeStruct((S, 2 * DM), BF16),
        in_specs=[pl.BlockSpec(memory_space=pl.ANY)] * 9,
        out_specs=pl.BlockSpec(memory_space=pl.ANY),
        scratch_shapes=scratch,
        compiler_params=pltpu.CompilerParams(vmem_limit_bytes=124 * 2**20),
        name="fused_local_and_latent_attention",
    )(
        A_x.reshape(S, DM), A_wqkv, A_wo,
        B_x.reshape(S, DM), B_c_kv.reshape(S, DC),
        B_w_q, B_w_uk, B_w_uv, B_w_o.reshape(NH * HD, DM),
    )
    return out.reshape(1, S, 2 * DM)
```

```python
import math

import jax
import jax.numpy as jnp
from jax import lax
import jax.experimental.pallas as pl
import jax.experimental.pallas.tpu as pltpu

F32, BF16, U32 = jnp.float32, jnp.bfloat16, jnp.uint32

S = 2048
DM = 1024
DC = 512
NH = 32
HD = 128
AD = 32
WIN, DIL = 8, 2

R = 128
CH = 2 * R
NC = S // CH
NP = NH // 2
HALO = 16
PITCH = 33

_PARTS = ("pro", "bloop", "last", "s0", "aloop", "epi")
_X = ""
_FIRST = 6
_NA = 2
_NB = 16
_LAG = 3
_AT = 3
_PRIO = 0
_QS = 'ob'
_Q0 = 4
_SP = 1
_KG = 2
_CT = 4
_CU = 10
_DUM = 24
_QP = 16
_AP = 16
_PA = 0
_PB = 0
_CL = 4
_DEPTH = 2
LOG2E = math.log2(math.e)
MASKED = -1e9 * LOG2E

NN = (((1,), (0,)), ((), ()))
NT = (((1,), (1,)), ((), ()))

LHS = (((0, 1), (3, 1)), ((2, 1), (3, 1)), ((0, 1),), ((3, 1),),
       ((0, 1), (1, 1)), ((2, 1), (0, -1)), ((1, 1), (3, -1)))
RHS = (((0, 1), (3, 1)), ((0, 1),), ((1, 1), (3, -1)), ((2, 1), (0, -1)),
       ((3, 1),), ((0, 1), (1, 1)), ((2, 1), (3, 1)))
PRODUCTS = ((2, ((1, 1), (3, 1))), (4, ((0, -1), (1, 1))), (3, ((0, 1), (2, 1))),
            (1, ((2, 1), (3, -1))), (5, ((3, 1),)), (0, ((0, 1), (3, 1))),
            (6, ((0, 1),)))
NOPS = len(PRODUCTS)

OPROWS = 256
N_UNITS = 12
W_KV, W_Q = range(2)
RING = 5


def _combine(blocks, terms):
    if isinstance(blocks[terms[0][0]], list):
        return [_combine({b: blocks[b][i] for b, _ in terms}, terms) for i in range(4)]
    out = None
    for i, sign in terms:
        if out is None:
            assert sign > 0
            out = blocks[i]
        else:
            out = out + blocks[i] if sign > 0 else out - blocks[i]
    return out


def _store(words, index, row, col, x):
    matrix = words.bitcast(BF16).at[index]
    matrix[pl.ds(2 * row, x.shape[0]), pl.ds(col, x.shape[1])] = x.astype(BF16)


def _bf16(words):
    return pltpu.bitcast(words, BF16)


def _halves(words):
    lo = pltpu.bitcast(words << 16, F32)
    hi = pltpu.bitcast(words & jnp.uint32(0xFFFF0000), F32)
    return lo, hi


def _split(words):
    return jnp.concatenate(_halves(words), axis=0)


def _join(x):
    n = x.shape[0] // 2
    return pltpu.pack_elementwise([x[:n], x[n:]], packed_dtype=BF16)


def _recip(x):
    r = pltpu.reciprocal(x, approx=True)
    return r * (2.0 - x * r)


def _operands(blocks, side):
    return [_combine(blocks, terms) for terms in side]


def _block_product(lhs, rhs, done, dims=NN, levels=1):
    if levels == 0:
        def step():
            m = lax.dot_general(lhs(0), rhs(0), dims, preferred_element_type=F32)
            done((), m)
            return m
        return [step]

    held, steps = {}, []
    inner = NOPS ** (levels - 1)
    for n, (i, outs) in enumerate(PRODUCTS):
        later = {o for _, others in PRODUCTS[n + 1:] for o, _ in others}

        def add(sub, m, outs=outs, later=later):
            for o, sign in outs:
                if (o, sub) not in held:
                    held[o, sub] = m, sign
                else:
                    c, s = held[o, sub]
                    assert s > 0 or sign > 0
                    held[o, sub] = (m - c if s < 0 else c + m if sign > 0 else c - m), 1
                if o not in later:
                    done((o, *sub), held.pop((o, sub))[0])

        steps += _block_product(lambda k, i=i: lhs(i * inner + k),
                                lambda k, i=i: rhs(i * inner + k), add, dims, levels - 1)
    return steps


def _run(steps, n=None):
    out = None
    for _ in range(len(steps) if n is None else min(n, len(steps))):
        out = steps.pop(0)()
    return out


def _group(steps, n):
    return [lambda g=steps[i:i + n]: _run(g) for i in range(0, len(steps), n)]


def _share(items, k, n):
    return items[k * len(items) // n:(k + 1) * len(items) // n]


def _blend(*lists):
    spots = [((i + 0.5) / len(items), k, item)
             for k, items in enumerate(lists) for i, item in enumerate(items)]
    return [item for *_, item in sorted(spots, key=lambda spot: spot[:2])]


def _witness(values):
    out = None
    for v in values:
        v = pltpu.bitcast(v, U32)
        for r in range(0, v.shape[0], 8):
            for c in range(0, v.shape[1], 128):
                out = v[r:r + 8, c:c + 128] if out is None else out | v[r:r + 8, c:c + 128]
    return out


def _mingle(steps, pieces):
    history = []

    def both(step, mine):
        history.append(step())
        for i, (pace, work, *lag) in enumerate(mine):
            seen = work()
            m = history[max(0, len(history) - 1 - sum(lag))]
            if m is not None:
                r = 8 * (i * (m.shape[0] // 8) // len(mine))
                pace(_witness([m[r:r + 8, :128]] + list(seen)))
        return history[-1]

    return [lambda step=step, mine=_share(pieces, i, len(steps)): both(step, mine)
            for i, step in enumerate(steps)]


def _now(pieces):
    for _, work, *_ in pieces:
        work()


def _pacer(ref, *index):
    def pace(v):
        if ref.dtype == BF16:
            ref[(*index, pl.ds(0, 16), pl.ds(0, 128))] = _bf16(v)
        else:
            ref[(*index, pl.ds(0, 8), pl.ds(0, 128))] = pltpu.bitcast(v, ref.dtype)
    return pace


def _dim_major(src, pace, shuf, dst, page, swap, zero):
    def start(head):
        return ((head % 2) * NH // 2 + head // 2) * PITCH

    def scatter(k, u):
        t = src(k, u)
        for h in range(128 // AD):
            shuf[k, pl.ds(start(4 * u + h), AD), :] = t[h * AD:(h + 1) * AD]
        return [t]

    def gather(d, h):
        x = [[jnp.concatenate([shuf[k, pl.ds(start(h + p) + a * AD // 2 + d, 8, stride=PITCH), :]
                               for p in range(2)], axis=0)
              for k in range(2)] for a in range(2)]
        blocks = ([x[0][0], x[1][0], x[0][1], x[1][1]] if swap
                  else [x[0][0], x[0][1], x[1][0], x[1][1]])
        ops = [_join(v) for v in _operands(blocks, RHS)]
        for i, v in enumerate(ops):
            dst[page, i, pl.ds((d * NH + h) // 2, 8), :] = v
        return ops

    return ([(pace, lambda k=k, u=u: scatter(k, u), _LAG if swap else 0)
             for k in range(2) for u in range(NH * AD // 128)]
            + [(_pacer(shuf, 2 + zero), lambda d=d, h=h: gather(d, h))
               for d in range(AD // 2) for h in range(0, NH, 16)])


def _kernel(ax_hbm, awqkv_hbm, awo_hbm, bx_hbm, c_hbm, wq_hbm, wuk_hbm, wuv_hbm,
            wo_hbm, out_hbm,
            dummy, ctx, wo_raw, woop, awop, xa, awo_raw, shuf,
            sem_x, sem_c, sem_w, sem_aw, sem_a, sem_out):

    def cp_wo(u, s):
        rows = pl.ds(pl.multiple_of((u // 2) * 4 * HD, 4 * HD), 4 * HD)
        return [pltpu.make_async_copy(
            wo_hbm.at[rows, pl.ds(pl.multiple_of(q * 256 + (u % 2) * 128, 128), 128)],
            wo_raw.at[s, q].bitcast(BF16), sem_w.at[6 + s]) for q in range(4)]

    def prep_wo(u, s, zero):
        def piece(r, i):
            outer = {b: [_split(wo_raw[s, 2 * (b % 2) + b2,
                                       pl.ds((2 * a2 + b // 2) * (HD // 2) + r, 8), :])
                         for a2 in range(2) for b2 in range(2)] for b, _ in RHS[i]}
            ops = [_join(v) for v in _operands(_combine(outer, RHS[i]), RHS)]
            row = pl.multiple_of((u // 2) * (HD // 2) + r, 8)
            for k, v in enumerate(ops):
                woop[u % 2, NOPS * i + k, pl.ds(row, 8), :] = v
            return ops
        return [(_pacer(wo_raw, 2 + zero, 0), lambda r=r, i=i: piece(r, i))
                for r in range(0, HD // 2, 8) for i in range(NOPS)]

    def gap(flag, zero):
        if flag in _X:
            @pl.loop(0, 2)
            def _(i):
                _pacer(shuf, 2 + zero * i)(jnp.zeros((8, 128), U32))

    def pad(n, zero):
        if n:
            @pl.when(zero != 0)
            def _():
                v = shuf[0, :128]
                for _ in range(n * 95):
                    v = v * 1.0001 + 0.5
                shuf[0, :128] = v

    dummy[:8] = jnp.zeros((8, 128), F32)
    shuf[0, :8] = dummy[pl.ds(1, 8)]

    def cp_a():
        return ([pltpu.make_async_copy(ax_hbm.at[pl.ds(c * CH, CH)], xa.at[c], sem_a.at[0])
                 for c in range(NC)]
                + [pltpu.make_async_copy(awo_hbm.at[pl.ds(128 * t, 128)], awo_raw.at[t], sem_a.at[1])
                   for t in range(8)])

    def heads(xs, cs, blop, wq_raw, wuk_raw, wuv_raw, bwop, q_s, k_s, v_s, aw_raw):
        wq32 = wq_hbm.bitcast(U32)
        wuk32 = wuk_hbm.bitcast(U32)
        wuv32 = wuv_hbm.bitcast(U32)

        def cp_x(c):
            return pltpu.make_async_copy(bx_hbm.at[pl.ds(c * CH, CH)], xs.at[c], sem_x.at[c])

        def cp_c(c):
            return pltpu.make_async_copy(c_hbm.at[pl.ds(c * CH, CH)], cs.at[c], sem_c.at[c])

        def cp_proj_w(j, s):
            return [
                pltpu.make_async_copy(wuk32.at[:, j, :], wuk_raw.at[s], sem_w.at[s]),
                pltpu.make_async_copy(wuv32.at[:, j, :], wuv_raw.at[s], sem_w.at[2 + s]),
                pltpu.make_async_copy(wq32.at[:, j, :], wq_raw.at[s], sem_w.at[4 + s]),
            ]

        def cp_aw(u, s):
            cols = pl.ds(pl.multiple_of((u // 4) * DM, DM), DM)
            return [pltpu.make_async_copy(
                awqkv_hbm.at[pl.ds(pl.multiple_of((u % 4) * 128 + half * (DM // 2), 128), 128), cols],
                aw_raw.at[s, half], sem_aw.at[2 * s + half]) for half in range(2)]

        def cp_step(j):
            return (cp_proj_w(jnp.minimum(j + 2, NP - 1), j % 2) + cp_wo(j, j % 2)
                    + cp_aw(jnp.minimum(j, N_UNITS - 1), j % 2))

        def prep_rows(src, c, col, zero, n=_NB):
            m = src.shape[2] // 2

            def piece(t, r):
                blocks = [_split(pltpu.bitcast(
                    src[c, pl.ds(k * R + r, n), pl.ds(h * m + 128 * t, 128)], U32))
                    for k in range(2) for h in range(2)]
                ops = [_join(v) for v in _operands(blocks, LHS)]
                for i, v in enumerate(ops):
                    blop[c, i, pl.ds(r // 2, n // 2), pl.ds(col + 128 * t, 128)] = v
                return ops
            return [(_pacer(src, NC + zero), lambda t=t, r=r: piece(t, r))
                    for t in range(m // 128) for r in range(0, R, n)]

        def prep_pair_w(raw, s, page, row0, zero, n=_NB):
            half = raw.shape[1] // 2

            def piece(r):
                blocks = []
                for k in range(2):
                    even, odd = (_halves(raw[s, pl.ds(k * half + r + p, n // 2, stride=2), :])
                                 for p in range(2))
                    blocks += [jnp.concatenate([even[h], odd[h]], axis=0) for h in range(2)]
                ops = [_join(v) for v in _operands(blocks, RHS)]
                for i, v in enumerate(ops):
                    bwop[page, i, pl.ds(row0 + r // 2, n // 2), :] = v
                return ops
            return [(_pacer(raw, 2 + zero), lambda r=r: piece(r)) for r in range(0, half, n)]

        def prep_kv_w(s, page, zero):
            return (prep_pair_w(wuk_raw, s, page + W_KV, 0, zero)
                    + prep_pair_w(wuv_raw, s, page + W_KV, OPROWS // 2, zero))

        def prep_q_w(s, page, zero):
            return prep_pair_w(wq_raw, s, page + W_Q, 0, zero)

        def prep_aw(u, s, zero):
            return _dim_major(
                lambda k, t: aw_raw[s, k, :, 128 * t:128 * (t + 1)].astype(F32).T,
                _pacer(blop, NC + zero, 0), shuf, awop, u, True, zero)

        def words(blk):
            return pl.ds(blk * (R // 2), R // 2)

        def q_proj(c, page):
            def done(o, val):
                _store(q_s, 0, (2 * c + o[0] // 2) * (R // 2), (o[0] % 2) * HD,
                       val * (HD ** -0.5 * LOG2E))
            return _block_product(lambda i: _bf16(blop[c, i, :, :DM // 2]),
                                  lambda i: _bf16(bwop[page + W_Q, i]), done)

        def kv_proj(c, page):
            steps = []
            for n, dst in enumerate((k_s, v_s)):
                def done(o, val, dst=dst):
                    _store(dst, 0, (2 * c + o[0] // 2) * (R // 2), (o[0] % 2) * HD, val)
                steps += _block_product(
                    lambda i: _bf16(blop[c, i, :, DM // 2:]),
                    lambda i, n=n: _bf16(bwop[page + W_KV, i, pl.ds(n * OPROWS // 2, OPROWS // 2), :]),
                    done)
            return _group(steps, _KG)

        def scores(h, blk):
            n = (blk + 1) * R
            s = lax.dot_general(_bf16(q_s[0, words(blk), pl.ds(h * HD, HD)]),
                                _bf16(k_s[0, :n // 2, pl.ds(h * HD, HD)]),
                                NT, preferred_element_type=F32)
            row = lax.broadcasted_iota(jnp.int32, (R, R), 0)
            col = lax.broadcasted_iota(jnp.int32, (R, R), 1)
            diag = jnp.where(col <= row, s[:, n - R:], MASKED)
            return diag if blk == 0 else jnp.concatenate([s[:, :n - R], diag], axis=1)

        def attend(h, blk, s):
            n = (blk + 1) * R
            p = jnp.exp2(s - jnp.max(s, axis=1, keepdims=True))
            if "u" in _X:
                p = p.astype(BF16).astype(F32)
            inv = _recip(jnp.sum(p, axis=1, keepdims=True))
            o = lax.dot_general(p.astype(BF16), _bf16(v_s[0, :n // 2, pl.ds(h * HD, HD)]), NN,
                                preferred_element_type=F32)
            return o * inv

        def pair_attention(j, zero, filler, side=(), depth=1):
            blocks = [(h, 2 * c + u) for c in reversed(range(NC)) for u in (1, 0) for h in (0, 1)]
            tiles = [(b, t) for b in blocks[_Q0:] for t in range(b[1] + 1)]

            def paced_scores(h, blk):
                s = scores(h, blk)
                for n, (b, t) in enumerate(tiles):
                    if b == (h, blk):
                        mine = _share(side, n, len(tiles))
                        for i, (pace, work, *_) in enumerate(mine):
                            r = 8 * (i * (R // 8) // len(mine))
                            pace(_witness([s[r:r + 8, t * R:(t + 1) * R]] + list(work())))
                return s

            todo, done = [], []
            ahead = [paced_scores(*b) for b in blocks[:depth]]
            for n, (h, blk) in enumerate(blocks):
                ahead += [paced_scores(*b) for b in blocks[n + depth:n + depth + 1]]
                cnt = -(-len(todo) // (4 - n % 4))
                _run(todo, cnt - cnt * _SP // 4)
                done.append(attend(h, blk, ahead.pop(0)))
                _store(ctx, j, blk * (R // 2), h * HD, done[-1])
                if len(done) > _CL:
                    q_s[zero, pl.ds(S // 2, 8), :128] = _witness([done.pop(0)])
                _run(todo, cnt * _SP // 4)
                if n % 4 == 3:
                    todo = filler(blk // 2)
            _run(todo)

        w0, w1 = cp_proj_w(0, 0), cp_proj_w(1, 1)
        stages = [w0[:2] + [cp_c(c) for c in (7, 6, 5)],
                  [cp_c(c) for c in (4, 3, 2, 1, 0)] + w0[2:],
                  [cp_x(c) for c in (7, 6, 5, 4)],
                  [cp_x(c) for c in (3, 2, 1)] + w1,
                  [cp_x(0)],
                  cp_step(0)]

        def issue(i, zero):
            for k, stage in enumerate(stages):
                @pl.when(i == k)
                def _(stage=stage):
                    for cp in stage:
                        cp.start()
            return zero + i // NP

        zero = lax.fori_loop(0, len(stages), issue, jnp.int32(0)) if 'pro' in _PARTS else lax.fori_loop(0, 15, lambda i, z: z + i // NP, jnp.int32(0))

        def project(steps, src, col, chunks, side):
            for n, c in enumerate(chunks):
                _now(prep_rows(src, c, col, zero, R))
                _run(_mingle(steps(c, 2), _share(side, n, len(chunks))))

        if "pro" in _PARTS:
            for cp in stages[0]:
                cp.wait()
            _now(prep_kv_w(0, 2, zero))
            project(kv_proj, cs, DM // 2, (7, 6, 5), [])
            for cp in stages[1]:
                cp.wait()
            project(kv_proj, cs, DM // 2, (4, 3, 2, 1, 0), prep_q_w(0, 2, zero))
            for cp in stages[2]:
                cp.wait()
            project(q_proj, xs, 0, (7, 6, 5, 4), [])
            for cp in stages[3]:
                cp.wait()
            project(q_proj, xs, 0, (3, 2, 1), prep_q_w(1, 0, zero) + prep_kv_w(1, 0, zero))
            for cp in stages[4]:
                cp.wait()
            project(q_proj, xs, 0, (0,), [])

        def pair_step(j, zero):
            for cp in cp_step(j):
                cp.wait()
            for cp in cp_step(j + 1):
                cp.start(priority=_PRIO)
            page = 2 * (j % RING)
            aw = prep_aw(jnp.minimum(j, N_UNITS - 1), j % 2, zero)
            bw = prep_kv_w(j % 2, page + 2, zero) + prep_q_w(j % 2, page + 2, zero)
            wo = prep_wo(j, j % 2, zero)
            groups = dict(a=aw, o=wo, b=bw)
            side = _blend(*[groups[g] for g in "aob" if g not in _QS])

            def filler(c):
                mine = _share(side, _FIRST - c, _FIRST + 1) if c <= _FIRST else []
                return _mingle(q_proj(c, page) + kv_proj(c, page), mine)

            pair_attention(j, zero, filler, _blend(*[groups[g] for g in _QS]))
            return zero + j // NP

        def lap(k, zero):
            @pl.when(k == 0)
            def _():
                for cp in cp_a():
                    cp.start()

            @pl.when(k > 0)
            def _():
                bwop[:2] = bwop[2 * RING:]

            return lax.fori_loop(k * RING, (k + 1) * RING, pair_step, zero)

        pad(_PB, zero)
        if "bloop" in _PARTS:
            zero = lax.fori_loop(0, (NP - 1) // RING, lap, zero)
        gap("4", zero)
        if "last" in _PARTS:
            for cp in cp_step(NP - 1) + cp_a():
                cp.wait()
            pair_attention(NP - 1, zero, lambda c: [], depth=_DEPTH)
        else:
            ctx[0, :8, :128] = (q_s[zero, :8, :128] + k_s[zero, :8, :128] + v_s[zero, :8, :128]
                                + bwop[zero, 0, :8, :] + blop[zero, 0, :8, :128])

    def rows(xaop, aoop, aqkv, oop, out_s):
        @pl.loop(0, 2)
        def _(i):
            aqkv[pl.ds(8 + 8 * i, 8), :HALO, :] = jnp.zeros((8, HALO, 128), F32)

        zero = lax.fori_loop(0, NP - 1, lambda i, z: z + i // NP, jnp.int32(0))

        def cp_out(c, half):
            cols = pl.ds(half * DM, DM)
            return pltpu.make_async_copy(
                out_s.at[half, c], out_hbm.at[pl.ds(pl.multiple_of(c * CH, CH), CH), cols],
                sem_out.at[half * NC + c])

        def prep_xa(c, zero, n=_NB):
            def piece(t, r):
                blocks = [_split(pltpu.bitcast(
                    xa[c, pl.ds(k * R + r, n), pl.ds(h * (DM // 2) + 128 * t, 128)], U32))
                    for k in range(2) for h in range(2)]
                ops = [_join(v) for v in _operands(blocks, LHS)]
                for i, v in enumerate(ops):
                    xaop[0, i, pl.ds(r // 2, n // 2), pl.ds(128 * t, 128)] = v
                return ops
            return [(_pacer(xa, NC + zero), lambda t=t, r=r: piece(t, r))
                    for t in range(4) for r in range(0, R, n)]

        def prep_awo(n, zero):
            return _dim_major(
                lambda k, t: awo_raw[t, :, pl.ds(k * (DM // 2) + 128 * n, 128)].astype(F32),
                _pacer(awo_raw, 8 + zero), shuf, awop, N_UNITS + n, False, zero)

        def prep_ctx(c, zero):
            base = pl.multiple_of(c * (CH // 2), CH // 2)

            def piece(m, r, i):
                outer = {b: [_split(ctx[2 * m + a2, pl.ds(base + ((b // 2) * 64 + r2 * 32 + r), 8),
                                        pl.ds((b % 2) * HD, HD)])
                             for r2 in range(2) for a2 in range(2)] for b, _ in LHS[i]}
                ops = [_join(v) for v in _operands(_combine(outer, LHS[i]), LHS)]
                for k, v in enumerate(ops):
                    oop[NOPS * i + k, pl.ds(r, 8), pl.ds(HD * m, HD)] = v
                return ops
            return [(_pacer(ctx, NP + zero), lambda m=m, r=r, i=i: piece(m, r, i))
                    for m in range(NP // 2) for r in range(0, 32, 8) for i in range(NOPS)]

        def o_proj(c):
            steps = []
            for t in range(2):
                def done(o, val, t=t):
                    r0 = (o[0] // 2) * R + (o[1] // 2) * (R // 2)
                    n0 = (o[0] % 2) * 512 + (o[1] % 2) * 256 + 128 * t
                    out_s[1, c, pl.ds(r0, R // 2), pl.ds(n0, 128)] = val.astype(BF16)
                steps += _block_product(lambda i: _bf16(oop[i]),
                                        lambda i, t=t: _bf16(woop[t, i]), done, levels=2)
            return steps + ([lambda: cp_out(c, 1).start(priority=_PRIO)] if 'D' not in _X else [])

        def a_proj(row0):
            steps = []
            for part in range(3):
                for t in range(4):
                    def done(o, val, part=part, t=t):
                        if part == 0:
                            val = val * (AD ** -0.5 * LOG2E)
                        aqkv[8 * part + t + 4 * (o[0] % 2),
                             pl.ds(row0 + (HALO + (o[0] // 2) * R), R), :] = val

                    def rhs(i, part=part, t=t):
                        return _bf16(jnp.concatenate(
                            [awop[4 * part + m, i, pl.ds(64 * t, 64), :] for m in range(4)], axis=1))
                    steps += _block_product(lambda i: _bf16(xaop[0, i]), rhs, done, dims=NT)
            return steps

        def a_attention(c, row0, zero):
            logit, prob, mixed = {}, {}, {}

            def dot(r, w):
                tot = None
                for t in range(8):
                    if (r, t) not in logit:
                        logit[r, t] = aqkv[t, pl.ds(row0 + (HALO + r), 8), :]
                    pr = logit[r, t] * aqkv[8 + t, pl.ds(row0 + (HALO + r - DIL * w), 8), :]
                    tot = pr if tot is None else tot + pr
                logit[r, "w", w] = tot
                if w == WIN - 1:
                    weights(r)
                return [tot]

            def weights(r):
                logits = [logit[r, "w", w] for w in range(WIN)]
                logits = [x + pltpu.roll(x, 64, 1) for x in logits]
                logits = [x + pltpu.roll(x, 32, 1) for x in logits]
                if r < (WIN - 1) * DIL:
                    pos = c * CH + r + lax.broadcasted_iota(jnp.int32, (8, 128), 0)
                    logits = [x if w == 0 else jnp.where(pos >= DIL * w, x, MASKED)
                              for w, x in enumerate(logits)]
                top = logits[0]
                for x in logits[1:]:
                    top = jnp.maximum(top, x)
                e = [jnp.exp2(x - top) for x in logits]
                tot = e[0]
                for x in e[1:]:
                    tot = tot + x
                inv = _recip(tot)
                prob[r] = [x * inv for x in e]

            def mix(r, t, d, h):
                tot = None
                for w in range(WIN):
                    pr = prob[r + d][w] * aqkv[16 + t + 4 * h,
                                               pl.ds(row0 + (HALO + r + d - DIL * w), 8), :]
                    tot = pr if tot is None else tot + pr
                mixed[d, h] = tot
                if (d, h) == (R + 8, 1):
                    ops = _operands([jnp.concatenate([mixed[k, h], mixed[k + 8, h]], axis=0)
                                     for k in (0, R) for h in range(2)], LHS)
                    for i, v in enumerate(ops):
                        _store(aoop, (0, i), r // 2, 128 * t, v)
                    return ops
                return [tot]

            def dots(r):
                return [lambda d=d, w=w: dot(r + d, w) for d in (0, 8, R, R + 8) for w in range(WIN)]

            def mixes(r):
                return [lambda t=t, d=d, h=h: mix(r, t, d, h)
                        for t in range(4) for d in (0, 8, R, R + 8) for h in range(2)]

            work = dots(0)
            for r in range(16, R, 16):
                work += [w for pair in zip(dots(r), mixes(r - 16)) for w in pair]
            work += mixes(R - 16)
            return [(_pacer(aqkv, 24 + zero), lambda g=work[i:i + _NA]: sum((w() for w in g), []))
                    for i in range(0, len(work), _NA)]

        def a_out_proj(c, zero):
            steps = []
            for n in range(4):
                def done(o, val, n=n):
                    out_s[0, c, pl.ds((o[0] // 2) * R, R),
                          pl.ds((o[0] % 2) * (DM // 2) + 128 * n, 128)] = val.astype(BF16)
                steps += _block_product(lambda i: _bf16(aoop[zero, i]),
                                        lambda i, n=n: _bf16(awop[N_UNITS + n, i]), done)
            return steps + ([lambda: cp_out(c, 0).start(priority=_PRIO)] if 'D' not in _X else [])

        if "s0" in _PARTS:
            _now(prep_xa(zero, zero))
            side = _blend(prep_wo(NP - 1, (NP - 1) % 2, zero), prep_ctx(0, zero),
                          sum((prep_awo(n, zero) for n in range(4)), []))
            _run(_mingle(a_proj(0), side))

        def chunk_step(c, zero):
            row0 = pl.multiple_of((c - 1) * CH, CH)
            first, second = o_proj(c - 1), a_proj(row0 + CH)
            att = a_attention(c - 1, row0, zero) if 'A' not in _X else []
            cut = len(att) * _CU // 16
            xap, ctxp = prep_xa(c, zero), prep_ctx(c, zero) if 'C' not in _X else []
            third = a_out_proj(c - 1, zero)
            late = len(ctxp) * _CT // 16
            _run(_mingle(first[:-1], _blend(att[:cut], xap)) + first[-1:])
            _run(_mingle(second[:-_AT], _blend(att[cut:], ctxp[:-late])) + second[-_AT:])
            _run(_mingle(third[:-_AT], ctxp[-late:]) + third[-_AT:])
            return zero + c // NC

        pad(_PA, zero)
        if "aloop" in _PARTS:
            zero = lax.fori_loop(1, NC, chunk_step, zero)
        gap("2", zero)

        if "epi" in _PARTS:
            steps = o_proj(NC - 1)
            _run(_mingle(steps[:-_AT], a_attention(NC - 1, (NC - 1) * CH, zero)) + steps[-_AT:])
            _run(a_out_proj(NC - 1, zero))
            for c in range(NC):
                cp_out(c, 1).wait()
                cp_out(c, 0).wait()
        else:
            out_s[0, 0, :16, :128] = aqkv[3, :16, :].astype(BF16)
            out_s[0, 0, 16:32, :128] = _bf16(awop[0, 0, :8, :] + ctx[0, :8, :128] + woop[0, 0, :8, :]
                                             + oop[0, :8, :128])
            cp_out(0, 0).start()
            cp_out(0, 0).wait()

    vmem = pltpu.VMEM
    pl.run_scoped(
        heads,
        vmem((NC + 1, CH, DM), BF16),
        vmem((NC + 1, CH, DC), BF16),
        vmem((NC + 1, NOPS, R // 2, (DM + DC) // 2), U32),
        vmem((3, DM, HD), U32),
        vmem((3, DC, HD), U32),
        vmem((3, DC, HD), U32),
        vmem((2 * (RING + 1), NOPS, OPROWS, 128), U32),
        vmem((1, S // 2 + _QP, 2 * HD), U32),
        vmem((1, S // 2, 2 * HD), U32),
        vmem((1, S // 2, 2 * HD), U32),
        vmem((3, 2, 128, DM), BF16),
    )
    pl.run_scoped(
        rows,
        vmem((1, NOPS, R // 2, DM // 2), U32),
        vmem((1, NOPS, R // 2, DM // 2), U32),
        vmem((25, HALO + S + _AP, 128), F32),
        vmem((NOPS * NOPS, R // 4, NP * HD // 2), U32),
        vmem((2, NC, CH, DM), BF16),
    )


@jax.jit
def pallas_concat_heads__sliding_local_dilated__compressed_kv_cla__prompt_kernel(
    A_x: jax.Array,
    A_wqkv: jax.Array,
    A_wo: jax.Array,
    B_x: jax.Array,
    B_c_kv: jax.Array,
    B_w_q: jax.Array,
    B_w_uk: jax.Array,
    B_w_uv: jax.Array,
    B_w_o: jax.Array,
):
    vmem = pltpu.VMEM
    dma = pltpu.SemaphoreType.DMA
    scratch = [
        vmem((_DUM, 128), F32),
        vmem((NP + 1, S // 2, 2 * HD), U32),
        vmem((3, 4, 2 * HD, 128), U32),
        vmem((2, NOPS * NOPS, NP * HD // 4, 128), U32),
        vmem((N_UNITS + 4, NOPS, OPROWS, 128), U32),
        vmem((NC + 1, CH, DM), BF16),
        vmem((9, 128, DM), BF16),
        vmem((3, NH * PITCH, 128), F32),
        dma((NC,)), dma((NC,)), dma((8,)), dma((4,)), dma((2,)), dma((2 * NC,)),
    ]
    out = pl.pallas_call(
        _kernel,
        out_shape=jax.ShapeDtypeStruct((S, 2 * DM), BF16),
        in_specs=[pl.BlockSpec(memory_space=pl.ANY)] * 9,
        out_specs=pl.BlockSpec(memory_space=pl.ANY),
        scratch_shapes=scratch,
        compiler_params=pltpu.CompilerParams(vmem_limit_bytes=124 * 2**20),
        name="fused_local_and_latent_attention",
    )(
        A_x.reshape(S, DM), A_wqkv, A_wo,
        B_x.reshape(S, DM), B_c_kv.reshape(S, DC),
        B_w_q, B_w_uk, B_w_uv, B_w_o.reshape(NH * HD, DM),
    )
    return out.reshape(1, S, 2 * DM)
```

```python
import math

import jax
import jax.numpy as jnp
from jax import lax
import jax.experimental.pallas as pl
import jax.experimental.pallas.tpu as pltpu

F32, BF16, U32 = jnp.float32, jnp.bfloat16, jnp.uint32

S = 2048
DM = 1024
DC = 512
NH = 32
HD = 128
AD = 32
WIN, DIL = 8, 2

R = 128
CH = 2 * R
NC = S // CH
NP = NH // 2
HALO = 16
PITCH = 33

_PARTS = ("pro", "bloop", "last", "s0", "aloop", "epi")
_X = ""
_FIRST = 6
_NA = 2
_NB = 16
_LAG = 3
_AT = 3
_PRIO = 0
_D2 = 32
_W = ''
_QE = 0
_AE = 1
_EW = 'w'
_AG = 2
_QS = 'ob'
_Q0 = 4
_SP = 1
_KG = 2
_CT = 4
_CU = 10
_DUM = 24
_QP = 16
_AP = 16
_PA = 0
_PB = 0
_CL = 4
_DEPTH = 2
LOG2E = math.log2(math.e)
MASKED = -1e9 * LOG2E

NN = (((1,), (0,)), ((), ()))
NT = (((1,), (1,)), ((), ()))

LHS = (((0, 1), (3, 1)), ((2, 1), (3, 1)), ((0, 1),), ((3, 1),),
       ((0, 1), (1, 1)), ((2, 1), (0, -1)), ((1, 1), (3, -1)))
RHS = (((0, 1), (3, 1)), ((0, 1),), ((1, 1), (3, -1)), ((2, 1), (0, -1)),
       ((3, 1),), ((0, 1), (1, 1)), ((2, 1), (3, 1)))
PRODUCTS = ((2, ((1, 1), (3, 1))), (4, ((0, -1), (1, 1))), (3, ((0, 1), (2, 1))),
            (1, ((2, 1), (3, -1))), (5, ((3, 1),)), (0, ((0, 1), (3, 1))),
            (6, ((0, 1),)))
NOPS = len(PRODUCTS)

OPROWS = 256
N_UNITS = 12
W_KV, W_Q = range(2)
RING = 5


def _combine(blocks, terms):
    if isinstance(blocks[terms[0][0]], list):
        return [_combine({b: blocks[b][i] for b, _ in terms}, terms) for i in range(4)]
    out = None
    for i, sign in terms:
        if out is None:
            assert sign > 0
            out = blocks[i]
        else:
            out = out + blocks[i] if sign > 0 else out - blocks[i]
    return out


def _store(words, index, row, col, x):
    matrix = words.bitcast(BF16).at[index]
    matrix[pl.ds(2 * row, x.shape[0]), pl.ds(col, x.shape[1])] = x.astype(BF16)


def _bf16(words):
    return pltpu.bitcast(words, BF16)


def _halves(words):
    lo = pltpu.bitcast(words << 16, F32)
    hi = pltpu.bitcast(words & jnp.uint32(0xFFFF0000), F32)
    return lo, hi


def _split(words):
    return jnp.concatenate(_halves(words), axis=0)


def _join(x):
    n = x.shape[0] // 2
    return pltpu.pack_elementwise([x[:n], x[n:]], packed_dtype=BF16)


def _recip(x):
    r = pltpu.reciprocal(x, approx=True)
    return r * (2.0 - x * r)


def _operands(blocks, side):
    return [_combine(blocks, terms) for terms in side]


def _block_product(lhs, rhs, done, dims=NN, levels=1):
    if levels == 0:
        def step():
            m = lax.dot_general(lhs(0), rhs(0), dims, preferred_element_type=F32)
            done((), m)
            return m
        return [step]

    held, steps = {}, []
    inner = NOPS ** (levels - 1)
    for n, (i, outs) in enumerate(PRODUCTS):
        later = {o for _, others in PRODUCTS[n + 1:] for o, _ in others}

        def add(sub, m, outs=outs, later=later):
            for o, sign in outs:
                if (o, sub) not in held:
                    held[o, sub] = m, sign
                else:
                    c, s = held[o, sub]
                    assert s > 0 or sign > 0
                    held[o, sub] = (m - c if s < 0 else c + m if sign > 0 else c - m), 1
                if o not in later:
                    done((o, *sub), held.pop((o, sub))[0])

        steps += _block_product(lambda k, i=i: lhs(i * inner + k),
                                lambda k, i=i: rhs(i * inner + k), add, dims, levels - 1)
    return steps


def _run(steps, n=None):
    out = None
    for _ in range(len(steps) if n is None else min(n, len(steps))):
        out = steps.pop(0)()
    return out


def _group(steps, n):
    return [lambda g=steps[i:i + n]: _run(g) for i in range(0, len(steps), n)]


def _weave(lists, together):
    return [x for xs in zip(*lists) for x in xs] if together else sum(lists, [])


def _share(items, k, n):
    return items[k * len(items) // n:(k + 1) * len(items) // n]


def _blend(*lists):
    spots = [((i + 0.5) / len(items), k, item)
             for k, items in enumerate(lists) for i, item in enumerate(items)]
    return [item for *_, item in sorted(spots, key=lambda spot: spot[:2])]


def _witness(values):
    out = None
    for v in values:
        v = pltpu.bitcast(v, U32)
        for r in range(0, v.shape[0], 8):
            for c in range(0, v.shape[1], 128):
                out = v[r:r + 8, c:c + 128] if out is None else out | v[r:r + 8, c:c + 128]
    return out


def _mingle(steps, pieces):
    history = []

    def both(step, mine):
        history.append(step())
        for i, (pace, work, *lag) in enumerate(mine):
            seen = work()
            m = history[max(0, len(history) - 1 - sum(lag))]
            if m is not None:
                r = 8 * (i * (m.shape[0] // 8) // len(mine))
                pace(_witness([m[r:r + 8, :128]] + list(seen)))
        return history[-1]

    return [lambda step=step, mine=_share(pieces, i, len(steps)): both(step, mine)
            for i, step in enumerate(steps)]


def _now(pieces):
    for _, work, *_ in pieces:
        work()


def _pacer(ref, *index):
    def pace(v):
        if ref.dtype == BF16:
            ref[(*index, pl.ds(0, 16), pl.ds(0, 128))] = _bf16(v)
        else:
            ref[(*index, pl.ds(0, 8), pl.ds(0, 128))] = pltpu.bitcast(v, ref.dtype)
    return pace


def _dim_major(src, pace, shuf, put, swap, zero):
    def start(head):
        return ((head % 2) * 8 + head // 2) * PITCH

    def scatter(k, u):
        t = src(k, u)
        for h in range(128 // AD):
            shuf[k, pl.ds(start(4 * u + h), AD), :] = t[h * AD:(h + 1) * AD]
        return [t]

    def gather(d, i):
        def block(row1, col1, row2, col2):
            quarter, k = 2 * row1 + row2, 2 * col1 + col2
            if swap:
                quarter, k = k, quarter
            return jnp.concatenate(
                [shuf[k, pl.ds(start(p) + quarter * AD // 4 + d, 8, stride=PITCH), :]
                 for p in range(2)], axis=0)
        outer = {b: [block(b // 2, b % 2, s // 2, s % 2) for s in range(4)] for b, _ in RHS[i]}
        ops = [_join(v) for v in _operands(_combine(outer, RHS[i]), RHS)]
        for n, v in enumerate(ops):
            put(NOPS * i + n, d * NH // 2, v)
        return ops

    return ([(pace, lambda k=k, u=u: scatter(k, u), _LAG if swap else 0)
             for k in range(4) for u in range(4)]
            + [(_pacer(shuf, 4 + zero), lambda d=d, i=i: gather(d, i))
               for d in range(AD // 4) for i in range(NOPS)])


def _kernel(ax_hbm, awqkv_hbm, awo_hbm, bx_hbm, c_hbm, wq_hbm, wuk_hbm, wuv_hbm,
            wo_hbm, out_hbm,
            dummy, ctx, wo_raw, woop, awop, awoop, xa, awo_raw, shuf,
            sem_x, sem_c, sem_w, sem_aw, sem_a, sem_out):

    def cp_wo(u, s):
        rows = pl.ds(pl.multiple_of((u // 2) * 4 * HD, 4 * HD), 4 * HD)
        return [pltpu.make_async_copy(
            wo_hbm.at[rows, pl.ds(pl.multiple_of(q * 256 + (u % 2) * 128, 128), 128)],
            wo_raw.at[s, q].bitcast(BF16), sem_w.at[6 + s]) for q in range(4)]

    def prep_wo(u, s, zero):
        def piece(r, i):
            outer = {b: [_split(wo_raw[s, 2 * (b % 2) + b2,
                                       pl.ds((2 * a2 + b // 2) * (HD // 2) + r, 8), :])
                         for a2 in range(2) for b2 in range(2)] for b, _ in RHS[i]}
            ops = [_join(v) for v in _operands(_combine(outer, RHS[i]), RHS)]
            row = pl.multiple_of((u // 2) * (HD // 2) + r, 8)
            for k, v in enumerate(ops):
                woop[u % 2, NOPS * i + k, pl.ds(row, 8), :] = v
            return ops
        return [(_pacer(wo_raw, 2 + zero, 0), lambda r=r, i=i: piece(r, i))
                for r in range(0, HD // 2, 8) for i in range(NOPS)]

    def prep_awo(n, half, zero):
        def put(i, row, v):
            awoop[n, i, pl.ds(8 * half + row, 8), :] = v
        return _dim_major(
            lambda k, t: awo_raw[4 * half + t, :, pl.ds(k * (DM // 4) + 128 * n, 128)].astype(F32),
            _pacer(awo_raw, 8 + zero), shuf, put, False, zero)

    def gap(flag, zero):
        if flag in _X:
            @pl.loop(0, 2)
            def _(i):
                _pacer(shuf, 4 + zero * i)(jnp.zeros((8, 128), U32))

    def pad(n, zero):
        if n:
            @pl.when(zero != 0)
            def _():
                v = shuf[0, :128]
                for _ in range(n * 95):
                    v = v * 1.0001 + 0.5
                shuf[0, :128] = v

    dummy[:8] = jnp.zeros((8, 128), F32)
    shuf[0, :8] = dummy[pl.ds(1, 8)]

    def cp_a():
        return ([pltpu.make_async_copy(ax_hbm.at[pl.ds(c * CH, CH)], xa.at[c], sem_a.at[0])
                 for c in range(NC)]
                + [pltpu.make_async_copy(awo_hbm.at[pl.ds(128 * t, 128)], awo_raw.at[t], sem_a.at[1])
                   for t in range(8)])

    def heads(xs, cs, blop, wq_raw, wuk_raw, wuv_raw, bwop, q_s, k_s, v_s, aw_raw):
        wq32 = wq_hbm.bitcast(U32)
        wuk32 = wuk_hbm.bitcast(U32)
        wuv32 = wuv_hbm.bitcast(U32)

        def cp_x(c):
            return pltpu.make_async_copy(bx_hbm.at[pl.ds(c * CH, CH)], xs.at[c], sem_x.at[c])

        def cp_c(c):
            return pltpu.make_async_copy(c_hbm.at[pl.ds(c * CH, CH)], cs.at[c], sem_c.at[c])

        def cp_proj_w(j, s):
            return [
                pltpu.make_async_copy(wuk32.at[:, j, :], wuk_raw.at[s], sem_w.at[s]),
                pltpu.make_async_copy(wuv32.at[:, j, :], wuv_raw.at[s], sem_w.at[2 + s]),
                pltpu.make_async_copy(wq32.at[:, j, :], wq_raw.at[s], sem_w.at[4 + s]),
            ]

        def cp_aw(u, s):
            cols = pl.ds(pl.multiple_of((u // 4) * DM + (u % 2) * (DM // 2), DM // 2), DM // 2)
            return [pltpu.make_async_copy(
                awqkv_hbm.at[pl.ds(pl.multiple_of((u // 2 % 2) * 128 + k * (DM // 4), 128), 128), cols],
                aw_raw.at[s, k], sem_aw.at[s]) for k in range(4)]

        def cp_step(j):
            return (cp_proj_w(jnp.minimum(j + 2, NP - 1), j % 2) + cp_wo(j, j % 2)
                    + cp_aw(jnp.minimum(j, N_UNITS - 1), j % 2))

        def prep_rows(src, c, col, zero, n=_NB):
            m = src.shape[2] // 2

            def piece(t, r):
                blocks = [_split(pltpu.bitcast(
                    src[c, pl.ds(k * R + r, n), pl.ds(h * m + 128 * t, 128)], U32))
                    for k in range(2) for h in range(2)]
                ops = [_join(v) for v in _operands(blocks, LHS)]
                for i, v in enumerate(ops):
                    blop[c, i, pl.ds(r // 2, n // 2), pl.ds(col + 128 * t, 128)] = v
                return ops
            return [(_pacer(src, NC + zero), lambda t=t, r=r: piece(t, r))
                    for t in range(m // 128) for r in range(0, R, n)]

        def prep_pair_w(raw, s, page, row0, zero, n=_NB):
            half = raw.shape[1] // 2

            def piece(r):
                blocks = []
                for k in range(2):
                    even, odd = (_halves(raw[s, pl.ds(k * half + r + p, n // 2, stride=2), :])
                                 for p in range(2))
                    blocks += [jnp.concatenate([even[h], odd[h]], axis=0) for h in range(2)]
                ops = [_join(v) for v in _operands(blocks, RHS)]
                for i, v in enumerate(ops):
                    bwop[page, i, pl.ds(row0 + r // 2, n // 2), :] = v
                return ops
            return [(_pacer(raw, 2 + zero), lambda r=r: piece(r)) for r in range(0, half, n)]

        def prep_kv_w(s, page, zero):
            return (prep_pair_w(wuk_raw, s, page + W_KV, 0, zero)
                    + prep_pair_w(wuv_raw, s, page + W_KV, OPROWS // 2, zero))

        def prep_q_w(s, page, zero):
            return prep_pair_w(wq_raw, s, page + W_Q, 0, zero)

        def prep_aw(u, s, zero):
            def put(i, row, v):
                awop[u // 2, i, pl.ds(pl.multiple_of(8 * (u % 2), 8) + row, 8), :] = v
            return _dim_major(
                lambda k, t: aw_raw[s, k, :, 128 * t:128 * (t + 1)].astype(F32).T,
                _pacer(blop, NC + zero, 0), shuf, put, True, zero)

        def words(blk):
            return pl.ds(blk * (R // 2), R // 2)

        def q_proj(c, page):
            def done(o, val):
                _store(q_s, 0, (2 * c + o[0] // 2) * (R // 2), (o[0] % 2) * HD,
                       val * (HD ** -0.5 * LOG2E))
            return _block_product(lambda i: _bf16(blop[c, i, :, :DM // 2]),
                                  lambda i: _bf16(bwop[page + W_Q, i]), done)

        def kv_proj(c, page):
            steps = []
            for n, dst in enumerate((k_s, v_s)):
                def done(o, val, dst=dst):
                    _store(dst, 0, (2 * c + o[0] // 2) * (R // 2), (o[0] % 2) * HD, val)
                steps += _block_product(
                    lambda i: _bf16(blop[c, i, :, DM // 2:]),
                    lambda i, n=n: _bf16(bwop[page + W_KV, i, pl.ds(n * OPROWS // 2, OPROWS // 2), :]),
                    done)
            return _group(steps, _KG)

        def scores(h, blk):
            n = (blk + 1) * R
            s = lax.dot_general(_bf16(q_s[0, words(blk), pl.ds(h * HD, HD)]),
                                _bf16(k_s[0, :n // 2, pl.ds(h * HD, HD)]),
                                NT, preferred_element_type=F32)
            row = lax.broadcasted_iota(jnp.int32, (R, R), 0)
            col = lax.broadcasted_iota(jnp.int32, (R, R), 1)
            diag = jnp.where(col <= row, s[:, n - R:], MASKED)
            return diag if blk == 0 else jnp.concatenate([s[:, :n - R], diag], axis=1)

        def attend(h, blk, s):
            n = (blk + 1) * R
            p = jnp.exp2(s - jnp.max(s, axis=1, keepdims=True))
            if "u" in _X:
                p = p.astype(BF16).astype(F32)
            inv = _recip(jnp.sum(p, axis=1, keepdims=True))
            o = lax.dot_general(p.astype(BF16), _bf16(v_s[0, :n // 2, pl.ds(h * HD, HD)]), NN,
                                preferred_element_type=F32)
            return o * inv

        def pair_attention(j, zero, filler, side=(), depth=1, first=None):
            blocks = [(h, 2 * c + u) for c in reversed(range(NC)) for u in (1, 0) for h in (0, 1)]
            tiles = [(b, t) for b in blocks[_Q0 if first is None else first:] for t in range(b[1] + 1)]

            def paced_scores(h, blk):
                s = scores(h, blk)
                for n, (b, t) in enumerate(tiles):
                    if b == (h, blk):
                        mine = _share(side, n, len(tiles))
                        for i, (pace, work, *_) in enumerate(mine):
                            r = 8 * (i * (R // 8) // len(mine))
                            pace(_witness([s[r:r + 8, t * R:(t + 1) * R]] + list(work())))
                return s

            todo, done = [], []
            ahead = [paced_scores(*b) for b in blocks[:depth]]
            for n, (h, blk) in enumerate(blocks):
                ahead += [paced_scores(*b) for b in blocks[n + depth:n + depth + 1]]
                cnt = -(-len(todo) // (4 - n % 4))
                _run(todo, cnt - cnt * _SP // 4)
                done.append(attend(h, blk, ahead.pop(0)))
                _store(ctx, j, blk * (R // 2), h * HD, done[-1])
                if len(done) > _CL:
                    q_s[zero, pl.ds(S // 2, 8), :128] = _witness([done.pop(0)])
                _run(todo, cnt * _SP // 4)
                if n % 4 == 3:
                    todo = filler(blk // 2)
            _run(todo)

        w0, w1 = cp_proj_w(0, 0), cp_proj_w(1, 1)
        stages = [w0[:2] + [cp_c(c) for c in (7, 6, 5)],
                  [cp_c(c) for c in (4, 3, 2, 1, 0)] + w0[2:],
                  [cp_x(c) for c in (7, 6, 5, 4)],
                  [cp_x(c) for c in (3, 2, 1)] + w1,
                  [cp_x(0)],
                  cp_step(0)]

        def issue(i, zero):
            for k, stage in enumerate(stages):
                @pl.when(i == k)
                def _(stage=stage):
                    for cp in stage:
                        cp.start()
            return zero + i // NP

        zero = lax.fori_loop(0, len(stages), issue, jnp.int32(0)) if 'pro' in _PARTS else lax.fori_loop(0, 15, lambda i, z: z + i // NP, jnp.int32(0))

        def project(steps, src, col, chunks, side):
            for n, c in enumerate(chunks):
                _now(prep_rows(src, c, col, zero, R))
                _run(_mingle(steps(c, 2), _share(side, n, len(chunks))))

        if "pro" in _PARTS:
            for cp in stages[0]:
                cp.wait()
            _now(prep_kv_w(0, 2, zero))
            project(kv_proj, cs, DM // 2, (7, 6, 5), [])
            for cp in stages[1]:
                cp.wait()
            project(kv_proj, cs, DM // 2, (4, 3, 2, 1, 0), prep_q_w(0, 2, zero))
            for cp in stages[2]:
                cp.wait()
            project(q_proj, xs, 0, (7, 6, 5, 4), [])
            for cp in stages[3]:
                cp.wait()
            project(q_proj, xs, 0, (3, 2, 1), prep_q_w(1, 0, zero) + prep_kv_w(1, 0, zero))
            for cp in stages[4]:
                cp.wait()
            project(q_proj, xs, 0, (0,), [])

        def pair_step(j, zero):
            for cp in cp_step(j):
                cp.wait()
            for cp in cp_step(j + 1):
                cp.start(priority=_PRIO)
            page = 2 * (j % RING)
            aw = prep_aw(jnp.minimum(j, N_UNITS - 1), j % 2, zero)
            bw = prep_kv_w(j % 2, page + 2, zero) + prep_q_w(j % 2, page + 2, zero)
            wo = prep_wo(j, j % 2, zero)
            groups = dict(a=aw, o=wo, b=bw)
            side = _blend(*[groups[g] for g in "aob" if g not in _QS])

            def filler(c):
                mine = _share(side, _FIRST - c, _FIRST + 1) if c <= _FIRST else []
                return _mingle(q_proj(c, page) + kv_proj(c, page), mine)

            pair_attention(j, zero, filler, _blend(*[groups[g] for g in _QS]))
            return zero + j // NP

        def lap(k, zero):
            @pl.when(k == 0)
            def _():
                for cp in cp_a():
                    cp.start()

            @pl.when(k > 0)
            def _():
                bwop[:2] = bwop[2 * RING:]

            return lax.fori_loop(k * RING, (k + 1) * RING, pair_step, zero)

        pad(_PB, zero)
        if "bloop" in _PARTS:
            zero = lax.fori_loop(0, (NP - 1) // RING, lap, zero)
        gap("4", zero)
        if "last" in _PARTS:
            for cp in cp_step(NP - 1) + cp_a() if 'bloop' in _PARTS else []:
                cp.wait()
            side = sum((prep_awo(n // 2, n % 2, zero) for n in range(_AE)), [])
            if "w" in _EW:
                side = _blend(prep_wo(NP - 1, (NP - 1) % 2, zero), *([side] if side else []))
            pair_attention(NP - 1, zero, lambda c: [], side, _DEPTH, _QE)
        else:
            ctx[0, :8, :128] = (q_s[zero, :8, :128] + k_s[zero, :8, :128] + v_s[zero, :8, :128]
                                + bwop[zero, 0, :8, :] + blop[zero, 0, :8, :128])
        return zero

    def rows(zero, dummy2, xaop, aoop, aqkv, oop, out_s):
        dummy2[:8] = jnp.zeros((8, 128), F32)
        dummy[:8] = dummy2[pl.ds(1, 8)]

        @pl.loop(0, 2)
        def _(i):
            aqkv[pl.ds(8 + 8 * i, 8), :HALO, :] = jnp.zeros((8, HALO, 128), F32)

        def cp_out(c, half):
            cols = pl.ds(half * DM, DM)
            return pltpu.make_async_copy(
                out_s.at[half, c], out_hbm.at[pl.ds(pl.multiple_of(c * CH, CH), CH), cols],
                sem_out.at[half * NC + c])

        def prep_xa(c, zero):
            def piece(t, r, i):
                outer = {b: [_split(pltpu.bitcast(
                    xa[c, pl.ds((b // 2) * R + r2 * R // 2 + r, 16),
                       pl.ds((b % 2) * 512 + a2 * 256 + 128 * t, 128)], U32))
                    for r2 in range(2) for a2 in range(2)] for b, _ in LHS[i]}
                ops = [_join(v) for v in _operands(_combine(outer, LHS[i]), LHS)]
                for k, v in enumerate(ops):
                    xaop[NOPS * i + k, pl.ds(r // 2, 8), pl.ds(128 * t, 128)] = v
                return ops
            return [(_pacer(xa, NC + zero), lambda t=t, r=r, i=i: piece(t, r, i))
                    for t in range(2) for r in range(0, R // 2, 16) for i in range(NOPS)]

        def prep_ctx(c, zero):
            base = pl.multiple_of(c * (CH // 2), CH // 2)

            def piece(m, r, i):
                outer = {b: [_split(ctx[2 * m + a2, pl.ds(base + ((b // 2) * 64 + r2 * 32 + r), 8),
                                        pl.ds((b % 2) * HD, HD)])
                             for r2 in range(2) for a2 in range(2)] for b, _ in LHS[i]}
                ops = [_join(v) for v in _operands(_combine(outer, LHS[i]), LHS)]
                for k, v in enumerate(ops):
                    oop[NOPS * i + k, pl.ds(r, 8), pl.ds(HD * m, HD)] = v
                return ops
            return [(_pacer(ctx, NP + zero), lambda m=m, r=r, i=i: piece(m, r, i))
                    for m in range(NP // 2) for r in range(0, 32, 8) for i in range(NOPS)]

        def o_proj(c):
            steps = []
            for t in range(2):
                def done(o, val, t=t):
                    r0 = (o[0] // 2) * R + (o[1] // 2) * (R // 2)
                    n0 = (o[0] % 2) * 512 + (o[1] % 2) * 256 + 128 * t
                    out_s[1, c, pl.ds(r0, R // 2), pl.ds(n0, 128)] = val.astype(BF16)
                steps.append(_block_product(lambda i: _bf16(oop[i]),
                                            lambda i, t=t: _bf16(woop[t, i]), done, levels=2))
            return _weave(steps, "o" in _W) + ([lambda: cp_out(c, 1).start(priority=_PRIO)] if 'D' not in _X else [])

        def a_proj(row0):
            steps = []
            for part in range(3):
                both = []
                for t in range(2):
                    def done(o, val, part=part, t=t):
                        if part == 0:
                            val = val * (AD ** -0.5 * LOG2E)
                        r0 = (o[0] // 2) * R + (o[1] // 2) * (R // 2)
                        aqkv[8 * part + 4 * (o[0] % 2) + 2 * (o[1] % 2) + t,
                             pl.ds(row0 + (HALO + r0), R // 2), :] = val

                    def rhs(i, part=part, t=t):
                        return _bf16(jnp.concatenate(
                            [awop[2 * part + m, i, pl.ds(64 * t, 64), :] for m in range(2)], axis=1))
                    both.append(_block_product(lambda i: _bf16(xaop[i]), rhs, done, NT, 2))
                steps += _weave(both, "p" in _W)
            return _group(steps, _AG)

        def a_attention(c, row0, zero):
            logit, prob, mixed = {}, {}, {}

            def dot(r, w):
                tot = None
                for t in range(8):
                    if (r, t) not in logit:
                        logit[r, t] = aqkv[t, pl.ds(row0 + (HALO + r), 8), :]
                    pr = logit[r, t] * aqkv[8 + t, pl.ds(row0 + (HALO + r - DIL * w), 8), :]
                    tot = pr if tot is None else tot + pr
                logit[r, "w", w] = tot
                if w == WIN - 1:
                    weights(r)
                return [tot]

            def weights(r):
                logits = [logit[r, "w", w] for w in range(WIN)]
                logits = [x + pltpu.roll(x, 64, 1) for x in logits]
                logits = [x + pltpu.roll(x, 32, 1) for x in logits]
                if r < (WIN - 1) * DIL:
                    pos = c * CH + r + lax.broadcasted_iota(jnp.int32, (8, 128), 0)
                    logits = [x if w == 0 else jnp.where(pos >= DIL * w, x, MASKED)
                              for w, x in enumerate(logits)]
                top = logits[0]
                for x in logits[1:]:
                    top = jnp.maximum(top, x)
                e = [jnp.exp2(x - top) for x in logits]
                tot = e[0]
                for x in e[1:]:
                    tot = tot + x
                inv = _recip(tot)
                prob[r] = [x * inv for x in e]

            def mix(r, t, d, q):
                tot = None
                for w in range(WIN):
                    pr = prob[r + d][w] * aqkv[16 + t + 2 * q,
                                               pl.ds(row0 + (HALO + r + d - DIL * w), 8), :]
                    tot = pr if tot is None else tot + pr
                mixed[r, t, d, q] = tot
                return [tot]

            def operands(r, t, i):
                outer = {b: [jnp.concatenate(
                    [mixed[r, t, (b // 2) * R + r2 * R // 2 + e, 2 * (b % 2) + a2] for e in (0, 8)],
                    axis=0) for r2 in range(2) for a2 in range(2)] for b, _ in LHS[i]}
                ops = _operands(_combine(outer, LHS[i]), LHS)
                for k, v in enumerate(ops):
                    _store(aoop, NOPS * i + k, r // 2, 128 * t, v)
                return ops

            groups = [d + e for d in range(0, CH, R // 2) for e in (0, 8)]

            def dots(r):
                return [lambda d=d, w=w: dot(r + d, w) for d in groups for w in range(WIN)]

            def mixes(r):
                return [work for t in range(2) for work in
                        [lambda t=t, d=d, q=q: mix(r, t, d, q) for d in groups for q in range(4)]
                        + [lambda t=t, i=i: operands(r, t, i) for i in range(NOPS)]]

            work = dots(0)
            for r in range(16, R // 2, 16):
                work += _blend(dots(r), mixes(r - 16))
            work += mixes(R // 2 - 16)
            return [(_pacer(aqkv, 24 + zero), lambda g=work[i:i + _NA]: sum((w() for w in g), []))
                    for i in range(0, len(work), _NA)]

        def a_out_proj(c, zero):
            steps = []
            for n in range(2):
                def done(o, val, n=n):
                    r0 = (o[0] // 2) * R + (o[1] // 2) * (R // 2)
                    n0 = (o[0] % 2) * 512 + (o[1] % 2) * 256 + 128 * n
                    out_s[0, c, pl.ds(r0, R // 2), pl.ds(n0, 128)] = val.astype(BF16)
                steps.append(_block_product(lambda i: _bf16(aoop[zero + i]),
                                            lambda i, n=n: _bf16(awoop[n, i]), done, levels=2))
            return _group(_weave(steps, "a" in _W), _AG) + [lambda: cp_out(c, 0).start()]

        if "s0" in _PARTS:
            _now(prep_xa(zero, zero))
            lists = [prep_ctx(0, zero), sum((prep_awo(n // 2, n % 2, zero) for n in range(_AE, 4)), [])]
            if "w" not in _EW:
                lists.append(prep_wo(NP - 1, (NP - 1) % 2, zero))
            _run(_mingle(a_proj(0), _blend(*[x for x in lists if x])))

        def chunk_step(c, zero):
            row0 = pl.multiple_of((c - 1) * CH, CH)
            first, second = o_proj(c - 1), a_proj(row0 + CH)
            att = a_attention(c - 1, row0, zero) if 'A' not in _X else []
            cut = len(att) * _CU // 16
            xap, ctxp = prep_xa(c, zero), prep_ctx(c, zero) if 'C' not in _X else []
            third = a_out_proj(c - 1, zero)
            late = len(ctxp) * _CT // 16
            _run(_mingle(first[:-1], _blend(att[:cut], xap)) + first[-1:])
            _run(_mingle(second[:-_AT], _blend(att[cut:], ctxp[:-late])) + second[-_AT:])
            _run(_mingle(third[:-_AT], ctxp[-late:]) + third[-_AT:])
            return zero + c // NC

        pad(_PA, zero)
        if "aloop" in _PARTS:
            zero = lax.fori_loop(1, NC, chunk_step, zero)
        gap("2", zero)

        if "epi" in _PARTS:
            steps = o_proj(NC - 1)
            _run(_mingle(steps[:-_AT], a_attention(NC - 1, (NC - 1) * CH, zero)) + steps[-_AT:])
            _run(a_out_proj(NC - 1, zero))
            for c in range(NC):
                cp_out(c, 1).wait()
                cp_out(c, 0).wait()
        else:
            out_s[0, 0, :16, :128] = aqkv[3, :16, :].astype(BF16)
            out_s[0, 0, 16:32, :128] = _bf16(awop[0, 0, :8, :] + ctx[0, :8, :128] + woop[0, 0, :8, :]
                                             + oop[0, :8, :128] + awoop[0, 0, :8, :])
            cp_out(0, 0).start()
            cp_out(0, 0).wait()

    vmem = pltpu.VMEM
    zero = pl.run_scoped(
        heads,
        vmem((NC + 1, CH, DM), BF16),
        vmem((NC + 1, CH, DC), BF16),
        vmem((NC + 1, NOPS, R // 2, (DM + DC) // 2), U32),
        vmem((3, DM, HD), U32),
        vmem((3, DC, HD), U32),
        vmem((3, DC, HD), U32),
        vmem((2 * (RING + 1), NOPS, OPROWS, 128), U32),
        vmem((1, S // 2 + _QP, 2 * HD), U32),
        vmem((1, S // 2, 2 * HD), U32),
        vmem((1, S // 2, 2 * HD), U32),
        vmem((2, 4, 128, DM // 2), BF16),
    )
    pl.run_scoped(
        lambda *refs: rows(zero, *refs),
        vmem((_D2, 128), F32),
        vmem((NOPS * NOPS, R // 4, DM // 4), U32),
        vmem((NOPS * NOPS, R // 4, DM // 4), U32),
        vmem((25, HALO + S + _AP, 128), F32),
        vmem((NOPS * NOPS, R // 4, NP * HD // 2), U32),
        vmem((2, NC, CH, DM), BF16),
    )


@jax.jit
def pallas_concat_heads__sliding_local_dilated__compressed_kv_cla__prompt_kernel(
    A_x: jax.Array,
    A_wqkv: jax.Array,
    A_wo: jax.Array,
    B_x: jax.Array,
    B_c_kv: jax.Array,
    B_w_q: jax.Array,
    B_w_uk: jax.Array,
    B_w_uv: jax.Array,
    B_w_o: jax.Array,
):
    vmem = pltpu.VMEM
    dma = pltpu.SemaphoreType.DMA
    scratch = [
        vmem((_DUM, 128), F32),
        vmem((NP + 1, S // 2, 2 * HD), U32),
        vmem((3, 4, 2 * HD, 128), U32),
        vmem((2, NOPS * NOPS, NP * HD // 4, 128), U32),
        vmem((N_UNITS // 2, NOPS * NOPS, DM // 8, 128), U32),
        vmem((2, NOPS * NOPS, DM // 8, 128), U32),
        vmem((NC + 1, CH, DM), BF16),
        vmem((9, 128, DM), BF16),
        vmem((5, 16 * PITCH + 16, 128), F32),
        dma((NC,)), dma((NC,)), dma((8,)), dma((4,)), dma((2,)), dma((2 * NC,)),
    ]
    out = pl.pallas_call(
        _kernel,
        out_shape=jax.ShapeDtypeStruct((S, 2 * DM), BF16),
        in_specs=[pl.BlockSpec(memory_space=pl.ANY)] * 9,
        out_specs=pl.BlockSpec(memory_space=pl.ANY),
        scratch_shapes=scratch,
        compiler_params=pltpu.CompilerParams(vmem_limit_bytes=124 * 2**20),
        name="fused_local_and_latent_attention",
    )(
        A_x.reshape(S, DM), A_wqkv, A_wo,
        B_x.reshape(S, DM), B_c_kv.reshape(S, DC),
        B_w_q, B_w_uk, B_w_uv, B_w_o.reshape(NH * HD, DM),
    )
    return out.reshape(1, S, 2 * DM)
```

```python
import math

import jax
import jax.numpy as jnp
from jax import lax
import jax.experimental.pallas as pl
import jax.experimental.pallas.tpu as pltpu

F32, BF16, U32 = jnp.float32, jnp.bfloat16, jnp.uint32

S = 2048
DM = 1024
DC = 512
NH = 32
HD = 128
AD = 32
WIN, DIL = 8, 2

R = 128
CH = 2 * R
NC = S // CH
NP = NH // 2
HALO = 16
PITCH = 33

_PARTS = ("pro", "bloop", "last", "s0", "aloop", "epi")
_X = ""
_FIRST = 6
_NA = 2
_NB = 16
_LAG = 5
_AT = 3
_PRIO = 0
_D2 = 32
_W = ''
_QE = 0
_AE = 1
_EW = 'w'
_AG = 2
_QS = 'o'
_Q0 = 8
_SP = 6
_KG = 1
_QK = 0
_K2 = 0
_CT = 4
_CU = 10
_DUM = 24
_QP = 16
_AP = 16
_PA = 0
_PB = 0
_CL = 3
_SC = 2
_DEPTH = 2
LOG2E = math.log2(math.e)
MASKED = -1e9 * LOG2E

NN = (((1,), (0,)), ((), ()))
NT = (((1,), (1,)), ((), ()))

LHS = (((0, 1), (3, 1)), ((2, 1), (3, 1)), ((0, 1),), ((3, 1),),
       ((0, 1), (1, 1)), ((2, 1), (0, -1)), ((1, 1), (3, -1)))
RHS = (((0, 1), (3, 1)), ((0, 1),), ((1, 1), (3, -1)), ((2, 1), (0, -1)),
       ((3, 1),), ((0, 1), (1, 1)), ((2, 1), (3, 1)))
PRODUCTS = ((2, ((1, 1), (3, 1))), (4, ((0, -1), (1, 1))), (3, ((0, 1), (2, 1))),
            (1, ((2, 1), (3, -1))), (5, ((3, 1),)), (0, ((0, 1), (3, 1))),
            (6, ((0, 1),)))
NOPS = len(PRODUCTS)

OPROWS = 256
N_UNITS = 12
KVROWS = 64
W_KV = NOPS * OPROWS
SLOT = W_KV + NOPS * NOPS * KVROWS
RING = 5


def _combine(blocks, terms):
    if isinstance(blocks[terms[0][0]], list):
        return [_combine({b: blocks[b][i] for b, _ in terms}, terms) for i in range(4)]
    out = None
    for i, sign in terms:
        if out is None:
            assert sign > 0
            out = blocks[i]
        else:
            out = out + blocks[i] if sign > 0 else out - blocks[i]
    return out


def _store(words, index, row, col, x):
    matrix = words.bitcast(BF16).at[index]
    matrix[pl.ds(2 * row, x.shape[0]), pl.ds(col, x.shape[1])] = x.astype(BF16)


def _bf16(words):
    return pltpu.bitcast(words, BF16)


def _halves(words):
    lo = pltpu.bitcast(words << 16, F32)
    hi = pltpu.bitcast(words & jnp.uint32(0xFFFF0000), F32)
    return lo, hi


def _split(words):
    return jnp.concatenate(_halves(words), axis=0)


def _join(x):
    n = x.shape[0] // 2
    return pltpu.pack_elementwise([x[:n], x[n:]], packed_dtype=BF16)


def _recip(x):
    r = pltpu.reciprocal(x, approx=True)
    return r * (2.0 - x * r)


def _operands(blocks, side):
    return [_combine(blocks, terms) for terms in side]


def _block_product(lhs, rhs, done, dims=NN, levels=1):
    if levels == 0:
        def step():
            m = lax.dot_general(lhs(0), rhs(0), dims, preferred_element_type=F32)
            done((), m)
            return m
        return [step]

    held, steps = {}, []
    inner = NOPS ** (levels - 1)
    for n, (i, outs) in enumerate(PRODUCTS):
        later = {o for _, others in PRODUCTS[n + 1:] for o, _ in others}

        def add(sub, m, outs=outs, later=later):
            for o, sign in outs:
                if (o, sub) not in held:
                    held[o, sub] = m, sign
                else:
                    c, s = held[o, sub]
                    assert s > 0 or sign > 0
                    held[o, sub] = (m - c if s < 0 else c + m if sign > 0 else c - m), 1
                if o not in later:
                    done((o, *sub), held.pop((o, sub))[0])

        steps += _block_product(lambda k, i=i: lhs(i * inner + k),
                                lambda k, i=i: rhs(i * inner + k), add, dims, levels - 1)
    return steps


def _run(steps, n=None):
    out = None
    for _ in range(len(steps) if n is None else min(n, len(steps))):
        out = steps.pop(0)()
    return out


def _group(steps, n):
    return [lambda g=steps[i:i + n]: _run(g) for i in range(0, len(steps), n)]


def _weave(lists, together):
    return [x for xs in zip(*lists) for x in xs] if together else sum(lists, [])


def _share(items, k, n):
    return items[k * len(items) // n:(k + 1) * len(items) // n]


def _blend(*lists):
    spots = [((i + 0.5) / len(items), k, item)
             for k, items in enumerate(lists) for i, item in enumerate(items)]
    return [item for *_, item in sorted(spots, key=lambda spot: spot[:2])]


def _witness(values):
    out = None
    for v in values:
        v = pltpu.bitcast(v, U32)
        for r in range(0, v.shape[0], 8):
            for c in range(0, v.shape[1], 128):
                out = v[r:r + 8, c:c + 128] if out is None else out | v[r:r + 8, c:c + 128]
    return out


def _mingle(steps, pieces):
    history = []

    def both(step, mine):
        history.append(step())
        mine = [piece for piece in mine if piece]
        for i, (pace, work, *lag) in enumerate(mine):
            seen = work()
            m = history[max(0, len(history) - 1 - sum(lag))]
            if m is not None:
                r = 8 * (i * (m.shape[0] // 8) // len(mine))
                pace(_witness([m[r:r + 8, :128]] + list(seen)))
        return history[-1]

    return [lambda step=step, mine=_share(pieces, i, len(steps)): both(step, mine)
            for i, step in enumerate(steps)]


def _now(pieces):
    for _, work, *_ in pieces:
        work()


def _pacer(ref, *index):
    def pace(v):
        if ref.dtype == BF16:
            ref[(*index, pl.ds(0, 16), pl.ds(0, 128))] = _bf16(v)
        else:
            ref[(*index, pl.ds(0, 8), pl.ds(0, 128))] = pltpu.bitcast(v, ref.dtype)
    return pace


def _dim_major(src, pace, shuf, put, swap, zero):
    def start(head):
        return ((head % 2) * 8 + head // 2) * PITCH

    def scatter(k, u):
        t = src(k, u)
        for h in range(128 // AD):
            shuf[k, pl.ds(start(4 * u + h), AD), :] = t[h * AD:(h + 1) * AD]
        return [t]

    def gather(d, i):
        def block(row1, col1, row2, col2):
            quarter, k = 2 * row1 + row2, 2 * col1 + col2
            if swap:
                quarter, k = k, quarter
            return jnp.concatenate(
                [shuf[k, pl.ds(start(p) + quarter * AD // 4 + d, 8, stride=PITCH), :]
                 for p in range(2)], axis=0)
        outer = {b: [block(b // 2, b % 2, s // 2, s % 2) for s in range(4)] for b, _ in RHS[i]}
        ops = [_join(v) for v in _operands(_combine(outer, RHS[i]), RHS)]
        for n, v in enumerate(ops):
            put(NOPS * i + n, d * NH // 2, v)
        return ops

    return ([x for k in range(4) for u in range(4)
             for x in [(pace, lambda k=k, u=u: scatter(k, u), _LAG if swap else 0)] + [None] * (_SC if swap else 0)]
            + [(_pacer(shuf, 4 + zero), lambda d=d, i=i: gather(d, i))
               for d in range(AD // 4) for i in range(NOPS)])


def _kernel(ax_hbm, awqkv_hbm, awo_hbm, bx_hbm, c_hbm, wq_hbm, wuk_hbm, wuv_hbm,
            wo_hbm, out_hbm,
            dummy, ctx, wo_raw, woop, awop, awoop, xa, awo_raw, shuf,
            sem_x, sem_c, sem_w, sem_aw, sem_a, sem_out):

    def cp_tile(src, row, col, dst, sem):
        def span(i):
            return pl.ds(pl.multiple_of(i * 512, 512), 512)
        return pltpu.make_async_copy(src.at[span(row), span(col)], dst, sem)

    def cp_wo(u, s):
        return [cp_tile(wo_hbm, u // 2, u % 2, wo_raw.at[s].bitcast(BF16), sem_w.at[6 + s])]

    def prep_wo(u, s, zero):
        def piece(r, i):
            outer = {b: [_split(wo_raw[s, pl.ds((2 * a2 + b // 2) * (HD // 2) + r, 8),
                                       pl.ds((2 * (b % 2) + b2) * 128, 128)])
                         for a2 in range(2) for b2 in range(2)] for b, _ in RHS[i]}
            ops = [_join(v) for v in _operands(_combine(outer, RHS[i]), RHS)]
            row = pl.multiple_of((u // 2) * (HD // 2) + r, 8)
            for k, v in enumerate(ops):
                woop[u % 2, NOPS * i + k, pl.ds(row, 8), :] = v
            return ops
        return [(_pacer(wo_raw, 2 + zero), lambda r=r, i=i: piece(r, i))
                for r in range(0, HD // 2, 8) for i in range(NOPS)]

    def prep_awo(n, half, zero):
        def put(i, row, v):
            awoop[n, i, pl.ds(8 * half + row, 8), :] = v
        return _dim_major(
            lambda k, t: awo_raw[4 * half + t, pl.ds(128 * (k // 2), 128),
                                 pl.ds((k % 2) * (DM // 4) + 128 * n, 128)].astype(F32),
            _pacer(awo_raw, 8 + zero), shuf, put, False, zero)

    def gap(flag, zero):
        if flag in _X:
            @pl.loop(0, 2)
            def _(i):
                _pacer(shuf, 4 + zero * i)(jnp.zeros((8, 128), U32))

    def pad(n, zero):
        if n:
            @pl.when(zero != 0)
            def _():
                v = shuf[0, :128]
                for _ in range(n * 95):
                    v = v * 1.0001 + 0.5
                shuf[0, :128] = v

    dummy[:8] = jnp.zeros((8, 128), F32)
    shuf[0, :8] = dummy[pl.ds(1, 8)]

    def cp_a():
        return ([pltpu.make_async_copy(ax_hbm.at[pl.ds(c * CH, CH)], xa.at[c], sem_a.at[0])
                 for c in range(NC)]
                + [pltpu.make_async_copy(awo_hbm.at[pl.ds(128 * t, 128), pl.ds(DC * h, DC)],
                                         awo_raw.at[t, pl.ds(128 * h, 128)], sem_a.at[1])
                   for t in range(8) for h in range(2)])

    def heads(xop, cop, wq_raw, wkv_raw, bwop, q_s, k_s, v_s, aw_raw, unit):
        xs, cs = xa, awo_raw
        wq32 = wq_hbm.bitcast(U32)
        wuk32 = wuk_hbm.bitcast(U32)
        wuv32 = wuv_hbm.bitcast(U32)

        def cp_x(c):
            return pltpu.make_async_copy(bx_hbm.at[pl.ds(c * CH, CH)], xs.at[c], sem_x.at[c])

        def cp_c(c):
            return pltpu.make_async_copy(c_hbm.at[pl.ds(c * CH, CH)], cs.at[c], sem_c.at[c])

        def cp_proj_w(j, s):
            return [
                pltpu.make_async_copy(wuk32.at[:, j, :], wkv_raw.at[0, s], sem_w.at[s]),
                pltpu.make_async_copy(wuv32.at[:, j, :], wkv_raw.at[1, s], sem_w.at[2 + s]),
                pltpu.make_async_copy(wq32.at[:, j, :], wq_raw.at[s], sem_w.at[4 + s]),
            ]

        def cp_aw(u, s):
            return [cp_tile(awqkv_hbm, u // 2 % 2, 2 * (u // 4) + u % 2, aw_raw.at[s], sem_aw.at[s])]

        def cp_step(j):
            return (cp_proj_w(jnp.minimum(j + 2, NP - 1), j % 2) + cp_wo(j, j % 2)
                    + cp_aw(jnp.minimum(j, N_UNITS - 1), j % 2))

        def prep_x(c):
            for t in range(DM // 256):
                blocks = [_split(pltpu.bitcast(
                    xs[c, pl.ds(k * R, R), pl.ds(h * DM // 2 + 128 * t, 128)], U32))
                    for k in range(2) for h in range(2)]
                for i, v in enumerate(_operands(blocks, LHS)):
                    xop[c, i, :, pl.ds(128 * t, 128)] = _join(v)

        def prep_c(c):
            blocks = [[_split(pltpu.bitcast(
                cs[c, pl.ds(r1 * R + r2 * R // 2, R // 2), pl.ds(a1 * 256 + a2 * 128, 128)], U32))
                for r2 in range(2) for a2 in range(2)] for r1 in range(2) for a1 in range(2)]
            for i, outer in enumerate(_operands(blocks, LHS)):
                for k, v in enumerate(_operands(outer, LHS)):
                    cop[c, NOPS * i + k] = _join(v)

        def both_heads(raw, s, row):
            even, odd = (_halves(raw[s, pl.ds(row + p, 8, stride=2), :]) for p in range(2))
            return [jnp.concatenate([even[h], odd[h]], axis=0) for h in range(2)]

        def prep_q_w(s, slot, zero):
            def piece(r):
                blocks = both_heads(wq_raw, s, r) + both_heads(wq_raw, s, DM // 2 + r)
                ops = [_join(v) for v in _operands(blocks, RHS)]
                for i, v in enumerate(ops):
                    bwop[pl.ds(slot + (i * OPROWS + r // 2), 8), :] = v
                return ops
            return [(_pacer(wq_raw, 2 + zero), lambda r=r: piece(r)) for r in range(0, DM // 2, 16)]

        def prep_kv_w(j, s, slot, zero):
            total, inverse = {}, {}

            def measure(n, r):
                w = wkv_raw[n, s, pl.ds(r, 64), :]
                w = jnp.abs(pltpu.bitcast(w, F32)) + jnp.abs(pltpu.bitcast(w << 16, F32))
                w = jnp.sum(w.reshape(8, 8, 128), axis=0)
                total[n] = total[n] + w if r else w
                return [total[n]]

            def size(n):
                both = jnp.sum(jnp.sum(total[n], axis=1, keepdims=True), axis=0, keepdims=True)
                both = jnp.broadcast_to(jnp.clip(both, 2.0 ** -100, 2.0 ** 100), (8, 128))
                power = pltpu.bitcast(both, U32) & jnp.uint32(0x7F800000)
                unit[n, j] = pltpu.bitcast(power, F32)
                inverse[n] = pltpu.bitcast(jnp.uint32(0x7F000000) - power, F32)
                return [power]

            def piece(r, i):
                outer = {b: [v * jnp.concatenate([inverse[b % 2]] * 2, axis=0) for a2 in range(2)
                             for v in both_heads(wkv_raw.at[b % 2], s, (b // 2) * 256 + a2 * 128 + r)]
                         for b, _ in RHS[i]}
                ops = [_join(v) for v in _operands(_combine(outer, RHS[i]), RHS)]
                for k, v in enumerate(ops):
                    bwop[pl.ds(slot + (W_KV + (NOPS * i + k) * KVROWS + r // 2), 8), :] = v
                return ops
            pace = _pacer(wkv_raw, zero, 2)
            return ([(pace, lambda n=n, r=r: measure(n, r)) for n in range(2) for r in range(0, DC, 64)]
                    + [(pace, lambda n=n: size(n)) for n in range(2)],
                    [(_pacer(xop, NC + zero, 0), lambda: list(inverse.values()))]
                    + [(pace, lambda r=r, i=i: piece(r, i))
                       for r in range(0, 128, 16) for i in range(NOPS)])

        def prep_w(j, s, slot, zero):
            sizes, operands = prep_kv_w(j, s, slot, zero)
            return sizes + prep_q_w(s, slot, zero) + operands

        def prep_aw(u, s, zero):
            def put(i, row, v):
                awop[u // 2, i, pl.ds(pl.multiple_of(8 * (u % 2), 8) + row, 8), :] = v
            return _dim_major(
                lambda k, t: aw_raw[s, 128 * k:128 * (k + 1), 128 * t:128 * (t + 1)].astype(F32).T,
                _pacer(xop, NC + zero, 0), shuf, put, True, zero)

        def words(blk):
            return pl.ds(blk * (R // 2), R // 2)

        def q_proj(scale, c, slot):
            def done(o, val):
                _store(q_s, 0, (2 * c + o[0] // 2) * (R // 2), (o[0] % 2) * HD, val * scale)
            return _block_product(lambda i: _bf16(xop[c, i]),
                                  lambda i: _bf16(bwop[pl.ds(slot + i * OPROWS, OPROWS), :]), done)

        def kv_proj(c, slot, n=1):
            def done(o, val):
                for e in range(n):
                    _store((k_s, v_s)[o[0] % 2], 0,
                           (2 * (c + e) + o[0] // 2) * (R // 2) + (o[1] // 2) * (R // 4),
                           (o[1] % 2) * HD, val[e * R // 2:(e + 1) * R // 2])
            return _group(_block_product(
                lambda i: _bf16(jnp.concatenate([cop[c + e, i] for e in range(n)], axis=0)),
                lambda i: _bf16(bwop[pl.ds(slot + (W_KV + i * KVROWS), KVROWS), :]),
                done, levels=2), _KG)

        def scores(h, blk):
            n = (blk + 1) * R
            s = lax.dot_general(_bf16(q_s[0, words(blk), pl.ds(h * HD, HD)]),
                                _bf16(k_s[0, :n // 2, pl.ds(h * HD, HD)]),
                                NT, preferred_element_type=F32)
            row = lax.broadcasted_iota(jnp.int32, (R, R), 0)
            col = lax.broadcasted_iota(jnp.int32, (R, R), 1)
            diag = jnp.where(col <= row, s[:, n - R:], MASKED)
            return diag if blk == 0 else jnp.concatenate([s[:, :n - R], diag], axis=1)

        def attend(scale, h, blk, s):
            n = (blk + 1) * R
            p = jnp.exp2(s - jnp.max(s, axis=1, keepdims=True))
            if "u" in _X:
                p = p.astype(BF16).astype(F32)
            inv = _recip(jnp.sum(p, axis=1, keepdims=True)) * scale
            o = lax.dot_general(p.astype(BF16), _bf16(v_s[0, :n // 2, pl.ds(h * HD, HD)]), NN,
                                preferred_element_type=F32)
            return o * inv

        def pair_attention(j, zero, filler, side=(), depth=1, first=None):
            blocks = [(h, 2 * c + u) for c in reversed(range(NC)) for u in (1, 0) for h in (0, 1)]
            tiles = [(b, t) for b in blocks[_Q0 if first is None else first:] for t in range(b[1] + 1)]

            def paced_scores(h, blk):
                s = scores(h, blk)
                for n, (b, t) in enumerate(tiles):
                    if b == (h, blk):
                        mine = _share(side, n, len(tiles))
                        for i, (pace, work, *_) in enumerate(mine):
                            r = 8 * (i * (R // 8) // len(mine))
                            pace(_witness([s[r:r + 8, t * R:(t + 1) * R]] + list(work())))
                return s

            todo, done = [[]] * 8, []
            v_scale = unit[1, j, :1]
            ahead = [paced_scores(*b) for b in blocks[:depth]]
            for n, (h, blk) in enumerate(blocks):
                ahead += [paced_scores(*b) for b in blocks[n + depth:n + depth + 1]]
                _run(todo[2 * (n % 4)])
                done.append(attend(v_scale, h, blk, ahead.pop(0)))
                _store(ctx, j, blk * (R // 2), h * HD, done[-1])
                if len(done) > _CL:
                    q_s[zero, pl.ds(S // 2, 8), :128] = _witness([done.pop(0)])
                _run(todo[2 * (n % 4) + 1])
                if n % 4 == 3:
                    todo = filler(blk // 2)
            _run(sum(todo, []))

        w0, w1 = cp_proj_w(0, 0), cp_proj_w(1, 1)
        stages = [w0[:2] + [cp_c(c) for c in (7, 6, 5)],
                  [cp_c(c) for c in (4, 3, 2, 1, 0)] + w0[2:],
                  [cp_x(c) for c in (7, 6, 5, 4)],
                  [cp_x(c) for c in (3, 2, 1)] + w1,
                  [cp_x(0)],
                  cp_step(0)]

        def issue(i, zero):
            for k, stage in enumerate(stages):
                @pl.when(i == k)
                def _(stage=stage):
                    for cp in stage:
                        cp.start()
            return zero + i // NP

        zero = lax.fori_loop(0, len(stages), issue, jnp.int32(0)) if 'pro' in _PARTS else lax.fori_loop(0, 15, lambda i, z: z + i // NP, jnp.int32(0))

        def project(prep, steps, chunks, side):
            for n, c in enumerate(chunks):
                prep(c)
                _run(_mingle(steps(c, SLOT), _share(side, n, len(chunks))))

        if "pro" in _PARTS:
            for cp in stages[0]:
                cp.wait()
            _now(sum(prep_kv_w(0, 0, SLOT, zero), []))
            project(prep_c, kv_proj, (7, 6, 5), [])
            for cp in stages[1]:
                cp.wait()
            project(prep_c, kv_proj, (4, 3, 2, 1, 0), prep_q_w(0, SLOT, zero))
            for cp in stages[2]:
                cp.wait()
            scale = unit[0, 0, :1] * (HD ** -0.5 * LOG2E)
            q_proj0 = lambda c, slot: q_proj(scale, c, slot)
            project(prep_x, q_proj0, (7, 6, 5, 4), [])
            for cp in stages[3]:
                cp.wait()
            project(prep_x, q_proj0, (3, 2, 1), prep_w(1, 1, 0, zero))
            for cp in stages[4]:
                cp.wait()
            project(prep_x, q_proj0, (0,), [])

        def pair_step(j, zero):
            for cp in cp_step(j):
                cp.wait()
            for cp in cp_step(j + 1):
                cp.start(priority=_PRIO)
            slot = pl.multiple_of((j % RING) * SLOT, KVROWS)
            scale = unit[0, j + 1, :1] * (HD ** -0.5 * LOG2E)
            aw = prep_aw(jnp.minimum(j, N_UNITS - 1), j % 2, zero)
            bw = prep_w(j + 2, j % 2, slot + SLOT, zero)
            wo = prep_wo(j, j % 2, zero)
            groups = dict(a=aw, o=wo, b=bw)
            side = _blend(*[groups[g] for g in "aob" if g not in _QS])

            def filler(c):
                mine = _share(side, _FIRST - c, _FIRST + 1) if c <= _FIRST else []
                q, kv = q_proj(scale, c, slot), kv_proj(c, slot)
                slots = []
                for n in range(4):
                    qn, kvn = _share(q, n, 4), _share(kv, n, 4)
                    k = len(kvn) * _SP // 8
                    slots += {0: [kvn[k:] + qn, kvn[:k]][::1], 1: [qn + kvn[k:], kvn[:k]], 2: [kvn[k:], qn + kvn[:k]]}[_QK]
                order = iter(q), iter(kv)
                slots = [[next(order[0]) if step in q else next(order[1]) for step in slot] for slot in slots]
                steps = iter(_mingle(sum(slots, []), mine))
                return [[next(steps) for _ in slot] for slot in slots]

            pair_attention(j, zero, filler, _blend(*[groups[g] for g in _QS]))
            return zero + j // NP

        def lap(k, zero):
            @pl.when(k == 0)
            def _():
                for cp in cp_a():
                    cp.start()

            @pl.when(k > 0)
            def _():
                bwop[:SLOT] = bwop[RING * SLOT:]

            return lax.fori_loop(k * RING, (k + 1) * RING, pair_step, zero)

        pad(_PB, zero)
        if "bloop" in _PARTS:
            zero = lax.fori_loop(0, (NP - 1) // RING, lap, zero)
        gap("4", zero)
        if "last" in _PARTS:
            for cp in cp_step(NP - 1) + cp_a() if 'bloop' in _PARTS else []:
                cp.wait()
            side = sum((prep_awo(n // 2, n % 2, zero) for n in range(_AE)), [])
            if "w" in _EW:
                side = _blend(prep_wo(NP - 1, (NP - 1) % 2, zero), *([side] if side else []))
            pair_attention(NP - 1, zero, lambda c: [[]] * 8, side, _DEPTH, _QE)
        else:
            ctx[0, :8, :128] = (q_s[zero, :8, :128] + k_s[zero, :8, :128] + v_s[zero, :8, :128]
                                + bwop[pl.ds(zero, 8), :] + xop[zero, 0, :8, :128] + cop[zero, 0, :8, :])
        return zero

    def rows(zero, dummy2, xaop, aoop, aqkv, oop, out_s):
        dummy2[:8] = jnp.zeros((8, 128), F32)
        dummy[:8] = dummy2[pl.ds(1, 8)]

        @pl.loop(0, 2)
        def _(i):
            aqkv[pl.ds(8 + 8 * i, 8), :HALO, :] = jnp.zeros((8, HALO, 128), F32)

        def cp_out(c, half):
            cols = pl.ds(half * DM, DM)
            return pltpu.make_async_copy(
                out_s.at[half, c], out_hbm.at[pl.ds(pl.multiple_of(c * CH, CH), CH), cols],
                sem_out.at[half * NC + c])

        def prep_xa(c, zero):
            def piece(t, r, i):
                outer = {b: [_split(pltpu.bitcast(
                    xa[c, pl.ds((b // 2) * R + r2 * R // 2 + r, 16),
                       pl.ds(512 * t + (b % 2) * 256 + a2 * 128, 128)], U32))
                    for r2 in range(2) for a2 in range(2)] for b, _ in LHS[i]}
                ops = [_join(v) for v in _operands(_combine(outer, LHS[i]), LHS)]
                for k, v in enumerate(ops):
                    xaop[NOPS * i + k, pl.ds(r // 2, 8), pl.ds(128 * t, 128)] = v
                return ops
            return [(_pacer(xa, NC + zero), lambda t=t, r=r, i=i: piece(t, r, i))
                    for t in range(2) for r in range(0, R // 2, 16) for i in range(NOPS)]

        def prep_ctx(c, zero):
            base = pl.multiple_of(c * (CH // 2), CH // 2)

            def piece(m, r, i):
                outer = {b: [_split(ctx[2 * m + a2, pl.ds(base + ((b // 2) * 64 + r2 * 32 + r), 8),
                                        pl.ds((b % 2) * HD, HD)])
                             for r2 in range(2) for a2 in range(2)] for b, _ in LHS[i]}
                ops = [_join(v) for v in _operands(_combine(outer, LHS[i]), LHS)]
                for k, v in enumerate(ops):
                    oop[NOPS * i + k, pl.ds(r, 8), pl.ds(HD * m, HD)] = v
                return ops
            return [(_pacer(ctx, NP + zero), lambda m=m, r=r, i=i: piece(m, r, i))
                    for m in range(NP // 2) for r in range(0, 32, 8) for i in range(NOPS)]

        def o_proj(c):
            steps = []
            for t in range(2):
                def done(o, val, t=t):
                    r0 = (o[0] // 2) * R + (o[1] // 2) * (R // 2)
                    n0 = 512 * t + (o[0] % 2) * 256 + (o[1] % 2) * 128
                    out_s[1, c, pl.ds(r0, R // 2), pl.ds(n0, 128)] = val.astype(BF16)
                steps.append(_block_product(lambda i: _bf16(oop[i]),
                                            lambda i, t=t: _bf16(woop[t, i]), done, levels=2))
            return _weave(steps, "o" in _W) + ([lambda: cp_out(c, 1).start(priority=_PRIO)] if 'D' not in _X else [])

        def a_proj(row0):
            steps = []
            for part in range(3):
                both = []
                for t in range(2):
                    def done(o, val, part=part, t=t):
                        if part == 0:
                            val = val * (AD ** -0.5 * LOG2E)
                        r0 = (o[0] // 2) * R + (o[1] // 2) * (R // 2)
                        aqkv[8 * part + 4 * (o[0] % 2) + 2 * (o[1] % 2) + t,
                             pl.ds(row0 + (HALO + r0), R // 2), :] = val

                    def rhs(i, part=part, t=t):
                        return _bf16(jnp.concatenate(
                            [awop[2 * part + m, i, pl.ds(64 * t, 64), :] for m in range(2)], axis=1))
                    both.append(_block_product(lambda i: _bf16(xaop[i]), rhs, done, NT, 2))
                steps += _weave(both, "p" in _W)
            return _group(steps, _AG)

        def a_attention(c, row0, zero):
            logit, prob, mixed = {}, {}, {}

            def dot(r, w):
                tot = None
                for t in range(8):
                    if (r, t) not in logit:
                        logit[r, t] = aqkv[t, pl.ds(row0 + (HALO + r), 8), :]
                    pr = logit[r, t] * aqkv[8 + t, pl.ds(row0 + (HALO + r - DIL * w), 8), :]
                    tot = pr if tot is None else tot + pr
                logit[r, "w", w] = tot
                if w == WIN - 1:
                    weights(r)
                return [tot]

            def weights(r):
                logits = [logit[r, "w", w] for w in range(WIN)]
                logits = [x + pltpu.roll(x, 64, 1) for x in logits]
                logits = [x + pltpu.roll(x, 32, 1) for x in logits]
                if r < (WIN - 1) * DIL:
                    pos = c * CH + r + lax.broadcasted_iota(jnp.int32, (8, 128), 0)
                    logits = [x if w == 0 else jnp.where(pos >= DIL * w, x, MASKED)
                              for w, x in enumerate(logits)]
                top = logits[0]
                for x in logits[1:]:
                    top = jnp.maximum(top, x)
                e = [jnp.exp2(x - top) for x in logits]
                tot = e[0]
                for x in e[1:]:
                    tot = tot + x
                inv = _recip(tot)
                prob[r] = [x * inv for x in e]

            def mix(r, t, d, q):
                tot = None
                for w in range(WIN):
                    pr = prob[r + d][w] * aqkv[16 + t + 2 * q,
                                               pl.ds(row0 + (HALO + r + d - DIL * w), 8), :]
                    tot = pr if tot is None else tot + pr
                mixed[r, t, d, q] = tot
                return [tot]

            def operands(r, t, i):
                outer = {b: [jnp.concatenate(
                    [mixed[r, t, (b // 2) * R + r2 * R // 2 + e, 2 * (b % 2) + a2] for e in (0, 8)],
                    axis=0) for r2 in range(2) for a2 in range(2)] for b, _ in LHS[i]}
                ops = _operands(_combine(outer, LHS[i]), LHS)
                for k, v in enumerate(ops):
                    _store(aoop, NOPS * i + k, r // 2, 128 * t, v)
                return ops

            groups = [d + e for d in range(0, CH, R // 2) for e in (0, 8)]

            def dots(r):
                return [lambda d=d, w=w: dot(r + d, w) for d in groups for w in range(WIN)]

            def mixes(r):
                return [work for t in range(2) for work in
                        [lambda t=t, d=d, q=q: mix(r, t, d, q) for d in groups for q in range(4)]
                        + [lambda t=t, i=i: operands(r, t, i) for i in range(NOPS)]]

            work = dots(0)
            for r in range(16, R // 2, 16):
                work += _blend(dots(r), mixes(r - 16))
            work += mixes(R // 2 - 16)
            return [(_pacer(aqkv, 24 + zero), lambda g=work[i:i + _NA]: sum((w() for w in g), []))
                    for i in range(0, len(work), _NA)]

        def a_out_proj(c, zero):
            steps = []
            for n in range(2):
                def done(o, val, n=n):
                    r0 = (o[0] // 2) * R + (o[1] // 2) * (R // 2)
                    n0 = (o[0] % 2) * 512 + (o[1] % 2) * 256 + 128 * n
                    out_s[0, c, pl.ds(r0, R // 2), pl.ds(n0, 128)] = val.astype(BF16)
                steps.append(_block_product(lambda i: _bf16(aoop[zero + i]),
                                            lambda i, n=n: _bf16(awoop[n, i]), done, levels=2))
            return _group(_weave(steps, "a" in _W), _AG) + [lambda: cp_out(c, 0).start()]

        if "s0" in _PARTS:
            _now(prep_xa(zero, zero))
            lists = [prep_ctx(0, zero), sum((prep_awo(n // 2, n % 2, zero) for n in range(_AE, 4)), [])]
            if "w" not in _EW:
                lists.append(prep_wo(NP - 1, (NP - 1) % 2, zero))
            _run(_mingle(a_proj(0), _blend(*[x for x in lists if x])))

        def chunk_step(c, zero):
            row0 = pl.multiple_of((c - 1) * CH, CH)
            first, second = o_proj(c - 1), a_proj(row0 + CH)
            att = a_attention(c - 1, row0, zero) if 'A' not in _X else []
            cut = len(att) * _CU // 16
            xap, ctxp = prep_xa(c, zero), prep_ctx(c, zero) if 'C' not in _X else []
            third = a_out_proj(c - 1, zero)
            late = len(ctxp) * _CT // 16
            _run(_mingle(first[:-1], _blend(att[:cut], xap)) + first[-1:])
            _run(_mingle(second[:-_AT], _blend(att[cut:], ctxp[:-late])) + second[-_AT:])
            _run(_mingle(third[:-_AT], ctxp[-late:]) + third[-_AT:])
            return zero + c // NC

        pad(_PA, zero)
        if "aloop" in _PARTS:
            zero = lax.fori_loop(1, NC, chunk_step, zero)
        gap("2", zero)

        if "epi" in _PARTS:
            steps = o_proj(NC - 1)
            _run(_mingle(steps[:-_AT], a_attention(NC - 1, (NC - 1) * CH, zero)) + steps[-_AT:])
            _run(a_out_proj(NC - 1, zero))
            for c in range(NC):
                cp_out(c, 1).wait()
                cp_out(c, 0).wait()
        else:
            out_s[0, 0, :16, :128] = aqkv[3, :16, :].astype(BF16)
            out_s[0, 0, 16:32, :128] = _bf16(awop[0, 0, :8, :] + ctx[0, :8, :128] + woop[0, 0, :8, :]
                                             + oop[0, :8, :128] + awoop[0, 0, :8, :])
            cp_out(0, 0).start()
            cp_out(0, 0).wait()

    vmem = pltpu.VMEM
    zero = pl.run_scoped(
        heads,
        vmem((NC + 1, NOPS, R // 2, DM // 2), U32),
        vmem((NC, NOPS * NOPS, R // 4, 128), U32),
        vmem((3, DM, HD), U32),
        vmem((2, 3, DC, HD), U32),
        vmem(((RING + 1) * SLOT, 128), U32),
        vmem((1, S // 2 + _QP, 2 * HD), U32),
        vmem((1, S // 2, 2 * HD), U32),
        vmem((1, S // 2, 2 * HD), U32),
        vmem((2, 512, 512), BF16),
        vmem((2, NP + 2, 8, 128), F32),
    )
    pl.run_scoped(
        lambda *refs: rows(zero, *refs),
        vmem((_D2, 128), F32),
        vmem((NOPS * NOPS, R // 4, DM // 4), U32),
        vmem((NOPS * NOPS, R // 4, DM // 4), U32),
        vmem((25, HALO + S + _AP, 128), F32),
        vmem((NOPS * NOPS, R // 4, NP * HD // 2), U32),
        vmem((2, NC, CH, DM), BF16),
    )


@jax.jit
def pallas_concat_heads__sliding_local_dilated__compressed_kv_cla__prompt_kernel(
    A_x: jax.Array,
    A_wqkv: jax.Array,
    A_wo: jax.Array,
    B_x: jax.Array,
    B_c_kv: jax.Array,
    B_w_q: jax.Array,
    B_w_uk: jax.Array,
    B_w_uv: jax.Array,
    B_w_o: jax.Array,
):
    vmem = pltpu.VMEM
    dma = pltpu.SemaphoreType.DMA
    scratch = [
        vmem((_DUM, 128), F32),
        vmem((NP + 1, S // 2, 2 * HD), U32),
        vmem((3, 2 * HD, 512), U32),
        vmem((2, NOPS * NOPS, NP * HD // 4, 128), U32),
        vmem((N_UNITS // 2, NOPS * NOPS, DM // 8, 128), U32),
        vmem((2, NOPS * NOPS, DM // 8, 128), U32),
        vmem((NC + 1, CH, DM), BF16),
        vmem((9, CH, DC), BF16),
        vmem((5, 16 * PITCH + 16, 128), F32),
        dma((NC,)), dma((NC,)), dma((8,)), dma((4,)), dma((2,)), dma((2 * NC,)),
    ]
    out = pl.pallas_call(
        _kernel,
        out_shape=jax.ShapeDtypeStruct((S, 2 * DM), BF16),
        in_specs=[pl.BlockSpec(memory_space=pl.ANY)] * 9,
        out_specs=pl.BlockSpec(memory_space=pl.ANY),
        scratch_shapes=scratch,
        compiler_params=pltpu.CompilerParams(vmem_limit_bytes=124 * 2**20),
        name="fused_local_and_latent_attention",
    )(
        A_x.reshape(S, DM), A_wqkv, A_wo,
        B_x.reshape(S, DM), B_c_kv.reshape(S, DC),
        B_w_q, B_w_uk, B_w_uv, B_w_o.reshape(NH * HD, DM),
    )
    return out.reshape(1, S, 2 * DM)
```

```python
import math

import jax
import jax.numpy as jnp
from jax import lax
import jax.experimental.pallas as pl
import jax.experimental.pallas.tpu as pltpu

F32, BF16, U32 = jnp.float32, jnp.bfloat16, jnp.uint32

S = 2048
DM = 1024
DC = 512
NH = 32
HD = 128
AD = 32
WIN, DIL = 8, 2

R = 128
CH = 2 * R
NC = S // CH
NP = NH // 2
HALO = 16
PITCH = 33

_PARTS = ("pro", "bloop", "last", "s0", "aloop", "epi")
_X = ""
_FIRST = 6
_NA = 1
_NB = 16
_LAG = 5
_AT = 6
_PRIO = 0
_D2 = 32
_W = ''
_QE = 0
_AE = 1
_EW = 'w'
_AG = 2
_QS = 'o'
_Q0 = 8
_SP = 6
_KG = 1
_QK = 0
_K2 = 0
_CT = 4
_CU = 10
_DUM = 24
_QP = 16
_AP = 16
_PA = 0
_PB = 0
_CL = 3
_SC = 2
_KA = 5
_XS = tuple((c,) for c in range(7, -1, -1))
_XW = 0
_CS = ((7, 6), (5, 4), (3, 2), (1, 0))
_CW = 3
_AL = 0
_HI = 1
_S0 = 16
_EN = 2
_ET = 3
_SG = 16
_E0 = 0
_E1 = 2
_DEPTH = 2
LOG2E = math.log2(math.e)
MASKED = -1e9 * LOG2E

NN = (((1,), (0,)), ((), ()))
NT = (((1,), (1,)), ((), ()))

LHS = (((0, 1), (3, 1)), ((2, 1), (3, 1)), ((0, 1),), ((3, 1),),
       ((0, 1), (1, 1)), ((2, 1), (0, -1)), ((1, 1), (3, -1)))
RHS = (((0, 1), (3, 1)), ((0, 1),), ((1, 1), (3, -1)), ((2, 1), (0, -1)),
       ((3, 1),), ((0, 1), (1, 1)), ((2, 1), (3, 1)))
PRODUCTS = ((2, ((1, 1), (3, 1))), (4, ((0, -1), (1, 1))), (3, ((0, 1), (2, 1))),
            (1, ((2, 1), (3, -1))), (5, ((3, 1),)), (0, ((0, 1), (3, 1))),
            (6, ((0, 1),)))
NOPS = len(PRODUCTS)

OPROWS = 256
RING = 8
N_UNITS = 12
KVROWS = 64
SLOT = NOPS * NOPS * KVROWS


def _combine(blocks, terms):
    if isinstance(blocks[terms[0][0]], list):
        return [_combine({b: blocks[b][i] for b, _ in terms}, terms) for i in range(4)]
    out = None
    for i, sign in terms:
        if out is None:
            assert sign > 0
            out = blocks[i]
        else:
            out = out + blocks[i] if sign > 0 else out - blocks[i]
    return out


def _store(words, index, row, col, x):
    matrix = words.bitcast(BF16).at[index]
    matrix[pl.ds(pl.multiple_of(2 * row, 16), x.shape[0]), pl.ds(col, x.shape[1])] = x.astype(BF16)


def _bf16(words):
    return pltpu.bitcast(words, BF16)


def _halves(words):
    lo = pltpu.bitcast(words << 16, F32)
    hi = pltpu.bitcast(words & jnp.uint32(0xFFFF0000), F32)
    return lo, hi


def _split(words):
    return jnp.concatenate(_halves(words), axis=0)


def _join(x):
    n = x.shape[0] // 2
    return pltpu.pack_elementwise([x[:n], x[n:]], packed_dtype=BF16)


def _recip(x):
    r = pltpu.reciprocal(x, approx=True)
    return r * (2.0 - x * r)


def _operands(blocks, side):
    return [_combine(blocks, terms) for terms in side]


def _block_product(lhs, rhs, done, dims=NN, levels=1):
    if levels == 0:
        def step():
            m = lax.dot_general(lhs(0), rhs(0), dims, preferred_element_type=F32)
            done((), m)
            return m
        return [step]

    held, steps = {}, []
    inner = NOPS ** (levels - 1)
    for n, (i, outs) in enumerate(PRODUCTS):
        later = {o for _, others in PRODUCTS[n + 1:] for o, _ in others}

        def add(sub, m, outs=outs, later=later):
            for o, sign in outs:
                if (o, sub) not in held:
                    held[o, sub] = m, sign
                else:
                    c, s = held[o, sub]
                    assert s > 0 or sign > 0
                    held[o, sub] = (m - c if s < 0 else c + m if sign > 0 else c - m), 1
                if o not in later:
                    done((o, *sub), held.pop((o, sub))[0])

        steps += _block_product(lambda k, i=i: lhs(i * inner + k),
                                lambda k, i=i: rhs(i * inner + k), add, dims, levels - 1)
    return steps


def _run(steps, n=None):
    out = None
    for _ in range(len(steps) if n is None else min(n, len(steps))):
        out = steps.pop(0)()
    return out


def _group(steps, n):
    return [lambda g=steps[i:i + n]: _run(g) for i in range(0, len(steps), n)]


def _weave(lists, together):
    return [x for xs in zip(*lists) for x in xs] if together else sum(lists, [])


def _share(items, k, n):
    return items[k * len(items) // n:(k + 1) * len(items) // n]


def _blend(*lists):
    spots = [((i + 0.5) / len(items), k, item)
             for k, items in enumerate(lists) for i, item in enumerate(items)]
    return [item for *_, item in sorted(spots, key=lambda spot: spot[:2])]


def _witness(values):
    out = None
    for v in values:
        v = pltpu.bitcast(v, U32)
        for r in range(0, v.shape[0], 8):
            for c in range(0, v.shape[1], 128):
                out = v[r:r + 8, c:c + 128] if out is None else out | v[r:r + 8, c:c + 128]
    return out


def _mingle(steps, pieces, history=None):
    history = [] if history is None else history

    def both(step, mine):
        history.append(step())
        mine = [piece for piece in mine if piece]
        for i, (pace, work, *lag) in enumerate(mine):
            seen = work()
            m = history[max(0, len(history) - 1 - sum(lag))]
            if m is not None:
                r = 8 * (i * (m.shape[0] // 8) // len(mine))
                pace(_witness([m[r:r + 8, :128]] + list(seen)))
        return history[-1]

    return [lambda step=step, mine=_share(pieces, i, len(steps)): both(step, mine)
            for i, step in enumerate(steps)]


def _now(pieces):
    for _, work, *_ in pieces:
        work()


def _pacer(ref, *index):
    def pace(v):
        if ref.dtype == BF16:
            ref[(*index, pl.ds(0, 16), pl.ds(0, 128))] = _bf16(v)
        else:
            ref[(*index, pl.ds(0, 8), pl.ds(0, 128))] = pltpu.bitcast(v, ref.dtype)
    return pace


def _dim_major(src, pace, shuf, put, swap, zero):
    def start(head):
        return ((head % 2) * 8 + head // 2) * PITCH

    def scatter(k, u):
        t = src(k, u)
        for h in range(128 // AD):
            shuf[k, pl.ds(start(4 * u + h), AD), :] = t[h * AD:(h + 1) * AD]
        return [t]

    def gather(d, i):
        def block(row1, col1, row2, col2):
            quarter, k = 2 * row1 + row2, 2 * col1 + col2
            if swap:
                quarter, k = k, quarter
            return jnp.concatenate(
                [shuf[k, pl.ds(start(p) + quarter * AD // 4 + d, 8, stride=PITCH), :]
                 for p in range(2)], axis=0)
        outer = {b: [block(b // 2, b % 2, s // 2, s % 2) for s in range(4)] for b, _ in RHS[i]}
        ops = [_join(v) for v in _operands(_combine(outer, RHS[i]), RHS)]
        for n, v in enumerate(ops):
            put(NOPS * i + n, d * NH // 2, v)
        return ops

    return ([x for k in range(4) for u in range(4)
             for x in [(pace, lambda k=k, u=u: scatter(k, u), _LAG if swap else 0)] + [None] * (_SC if swap else 0)]
            + [(_pacer(shuf, 4 + zero), lambda d=d, i=i: gather(d, i))
               for d in range(AD // 4) for i in range(NOPS)])


def _kernel(ax_hbm, awqkv_hbm, awo_hbm, bx_hbm, c_hbm, wq_hbm, wuk_hbm, wuv_hbm,
            wo_hbm, out_hbm,
            dummy, ctx, wo_raw, woop, awop, awoop, xa, awo_raw, shuf,
            sem_x, sem_c, sem_w, sem_aw, sem_a, sem_out):

    def cp_tile(src, row, col, dst, sem):
        def span(i):
            return pl.ds(pl.multiple_of(i * 512, 512), 512)
        return pltpu.make_async_copy(src.at[span(row), span(col)], dst, sem)

    def cp_wo(u, s):
        return [cp_tile(wo_hbm, u // 2, u % 2, wo_raw.at[s].bitcast(BF16), sem_w.at[6 + s])]

    def prep_wo(u, s, zero):
        def piece(r, i):
            outer = {b: [_split(wo_raw[s, pl.ds((2 * a2 + b // 2) * (HD // 2) + r, 8),
                                       pl.ds((2 * (b % 2) + b2) * 128, 128)])
                         for a2 in range(2) for b2 in range(2)] for b, _ in RHS[i]}
            ops = [_join(v) for v in _operands(_combine(outer, RHS[i]), RHS)]
            row = pl.multiple_of((u // 2) * (HD // 2) + r, 8)
            for k, v in enumerate(ops):
                woop[u % 2, NOPS * i + k, pl.ds(row, 8), :] = v
            return ops
        return [(_pacer(wo_raw, 2 + zero), lambda r=r, i=i: piece(r, i))
                for r in range(0, HD // 2, 8) for i in range(NOPS)]

    def prep_awo(n, half, zero):
        def put(i, row, v):
            awoop[n, i, pl.ds(8 * half + row, 8), :] = v
        return _dim_major(
            lambda k, t: awo_raw[4 * half + t, pl.ds(128 * (k // 2), 128),
                                 pl.ds((k % 2) * (DM // 4) + 128 * n, 128)].astype(F32),
            _pacer(awo_raw, 8 + zero), shuf, put, False, zero)

    def gap(flag, zero):
        if flag in _X:
            @pl.loop(0, 2)
            def _(i):
                _pacer(shuf, 4 + zero * i)(jnp.zeros((8, 128), U32))

    def pad(n, zero):
        if n:
            @pl.when(zero != 0)
            def _():
                v = shuf[0, :128]
                for _ in range(n * 95):
                    v = v * 1.0001 + 0.5
                shuf[0, :128] = v

    dummy[:8] = jnp.zeros((8, 128), F32)
    shuf[0, :8] = dummy[pl.ds(1, 8)]

    def cp_a():
        return ([pltpu.make_async_copy(ax_hbm.at[pl.ds(c * CH, CH)], xa.at[c], sem_a.at[0])
                 for c in range(NC)]
                + [pltpu.make_async_copy(awo_hbm.at[pl.ds(128 * t, 128), pl.ds(DC * h, DC)],
                                         awo_raw.at[t, pl.ds(128 * h, 128)], sem_a.at[1])
                   for t in range(8) for h in range(2)])

    def heads(xop, cop, wq_raw, wkv_raw, qwop, bwop, q_s, k_s, v_s, aw_raw, unit):
        xs, cs = xa, awo_raw
        wq32 = wq_hbm.bitcast(U32)
        wuk32 = wuk_hbm.bitcast(U32)
        wuv32 = wuv_hbm.bitcast(U32)

        def cp_x(c):
            return pltpu.make_async_copy(bx_hbm.at[pl.ds(c * CH, CH)], xs.at[c], sem_x.at[c])

        def cp_c(c):
            return pltpu.make_async_copy(c_hbm.at[pl.ds(c * CH, CH)], cs.at[c], sem_c.at[c])

        def cp_proj_w(j, s, jq):
            return [
                pltpu.make_async_copy(wuk32.at[:, j, :], wkv_raw.at[s], sem_w.at[s]),
                pltpu.make_async_copy(wuv32.at[:, j, :], wkv_raw.at[2 + s], sem_w.at[2 + s]),
                pltpu.make_async_copy(wq32.at[:, jq, :], wq_raw.at[s], sem_w.at[4 + s]),
            ]

        def cp_aw(u, s):
            return [cp_tile(awqkv_hbm, u // 2 % 2, 2 * (u // 4) + u % 2, aw_raw.at[s], sem_aw.at[s])]

        def aw_unit(j):
            return jnp.clip(j - 1, 0, N_UNITS - 1)

        def cp_step(j):
            return (cp_proj_w(jnp.minimum(j + 2, NP - 1), j % 2, jnp.minimum(j + 1, NP - 1)) + cp_wo(j, j % 2)
                    + cp_aw(aw_unit(j), j % 2))

        def prep_x(c):
            for t in range(DM // 256):
                blocks = [_split(pltpu.bitcast(
                    xs[c, pl.ds(k * R, R), pl.ds(h * DM // 2 + 128 * t, 128)], U32))
                    for k in range(2) for h in range(2)]
                for i, v in enumerate(_operands(blocks, LHS)):
                    xop[NOPS * c + i, :, pl.ds(128 * t, 128)] = _join(v)

        def prep_c(c):
            blocks = [[_split(pltpu.bitcast(
                cs[c, pl.ds(r1 * R + r2 * R // 2, R // 2), pl.ds(a1 * 256 + a2 * 128, 128)], U32))
                for r2 in range(2) for a2 in range(2)] for r1 in range(2) for a1 in range(2)]
            for i, outer in enumerate(_operands(blocks, LHS)):
                for k, v in enumerate(_operands(outer, LHS)):
                    cop[c, NOPS * i + k] = _join(v)

        def both_heads(raw, s, row):
            even, odd = (_halves(raw[s, pl.ds(row + p, 8, stride=2), :]) for p in range(2))
            return [jnp.concatenate([even[h], odd[h]], axis=0) for h in range(2)]

        def prep_q_w(s, zero):
            def piece(r):
                blocks = both_heads(wq_raw, s, r) + both_heads(wq_raw, s, DM // 2 + r)
                ops = [_join(v) for v in _operands(blocks, RHS)]
                for i, v in enumerate(ops):
                    qwop[i, pl.ds(r // 2, 8), :] = v
                return ops
            return [(_pacer(wq_raw, 2 + zero), lambda r=r: piece(r)) for r in range(0, DM // 2, 16)]

        def prep_kv_w(j, s, slot, zero):
            total, inverse = {}, {}

            def measure(n, r):
                w = wkv_raw[2 * n + s, pl.ds(r, 64), :]
                w = jnp.abs(pltpu.bitcast(w, F32)) + jnp.abs(pltpu.bitcast(w << 16, F32))
                w = jnp.sum(w.reshape(8, 8, 128), axis=0)
                total[n] = total[n] + w if r else w
                return [total[n]]

            def size(n):
                both = jnp.sum(jnp.sum(total[n], axis=1, keepdims=True), axis=0, keepdims=True)
                both = jnp.broadcast_to(jnp.clip(both, 2.0 ** -100, 2.0 ** 100), (8, 128))
                power = pltpu.bitcast(both, U32) & jnp.uint32(0x7F800000)
                unit[n, j] = pltpu.bitcast(power, F32)
                inverse[n] = pltpu.bitcast(jnp.uint32(0x7F000000) - power, F32)
                return [power]

            def piece(r, i):
                outer = {b: [v * jnp.concatenate([inverse[b % 2]] * 2, axis=0) for a2 in range(2)
                             for v in both_heads(wkv_raw, 2 * (b % 2) + s, (b // 2) * 256 + a2 * 128 + r)]
                         for b, _ in RHS[i]}
                ops = [_join(v) for v in _operands(_combine(outer, RHS[i]), RHS)]
                for k, v in enumerate(ops):
                    bwop[pl.ds(slot + ((NOPS * i + k) * KVROWS + r // 2), 8), :] = v
                return ops
            pace = _pacer(wkv_raw, 4 + zero)
            return ([(pace, lambda n=n, r=r: measure(n, r)) for n in range(2) for r in range(0, DC, 64)]
                    + [(pace, lambda n=n: size(n)) for n in range(2)],
                    [(_pacer(xop, NOPS * NC + zero), lambda: list(inverse.values()))]
                    + [(pace, lambda r=r, i=i: piece(r, i))
                       for r in range(0, 128, 16) for i in range(NOPS)])

        def prep_aw(u, s, zero):
            def put(i, row, v):
                awop[u // 2, i, pl.ds(pl.multiple_of(8 * (u % 2), 8) + row, 8), :] = v
            return _dim_major(
                lambda k, t: aw_raw[s, 128 * k:128 * (k + 1), 128 * t:128 * (t + 1)].astype(F32).T,
                _pacer(xop, NOPS * NC + zero), shuf, put, True, zero)

        def words(blk):
            return pl.ds(blk * (R // 2), R // 2)

        def q_proj(scale, c):
            def done(o, val):
                _store(q_s, 0, (2 * c + o[0] // 2) * (R // 2), (o[0] % 2) * HD, val * scale)
            return _block_product(lambda i: _bf16(xop[NOPS * c + i]),
                                  lambda i: _bf16(qwop[i]), done)

        def kv_proj(c, slot, n=1):
            def done(o, val):
                for e in range(n):
                    _store((k_s, v_s)[o[0] % 2], 0,
                           (2 * (c + e) + o[0] // 2) * (R // 2) + (o[1] // 2) * (R // 4),
                           (o[1] % 2) * HD, val[e * R // 2:(e + 1) * R // 2])
            return _group(_block_product(
                lambda i: _bf16(jnp.concatenate([cop[c + e, i] for e in range(n)], axis=0)),
                lambda i: _bf16(bwop[pl.ds(slot + i * KVROWS, KVROWS), :]),
                done, levels=2), _KG)

        def scores(h, blk):
            n = (blk + 1) * R
            s = lax.dot_general(_bf16(q_s[0, words(blk), pl.ds(h * HD, HD)]),
                                _bf16(k_s[0, :n // 2, pl.ds(h * HD, HD)]),
                                NT, preferred_element_type=F32)
            row = lax.broadcasted_iota(jnp.int32, (R, R), 0)
            col = lax.broadcasted_iota(jnp.int32, (R, R), 1)
            diag = jnp.where(col <= row, s[:, n - R:], MASKED)
            return diag if blk == 0 else jnp.concatenate([s[:, :n - R], diag], axis=1)

        def attend(scale, h, blk, s):
            n = (blk + 1) * R
            p = jnp.exp2(s - jnp.max(s, axis=1, keepdims=True))
            if "u" in _X:
                p = p.astype(BF16).astype(F32)
            inv = _recip(jnp.sum(p, axis=1, keepdims=True)) * scale
            o = lax.dot_general(p.astype(BF16), _bf16(v_s[0, :n // 2, pl.ds(h * HD, HD)]), NN,
                                preferred_element_type=F32)
            return o * inv

        def pair_attention(j, zero, filler, side=(), depth=1, first=None, early=()):
            blocks = [(h, 2 * c + u) for c in reversed(range(NC)) for u in (1, 0) for h in (0, 1)]
            plan = {}
            for pieces, span in ((side, blocks[_Q0 if first is None else first:]), (early, blocks[_E0:_E1])):
                tiles = [(b, t) for b in span for t in range(b[1] + 1)]
                for n, tile in enumerate(tiles):
                    plan.setdefault(tile, []).extend(_share(pieces, n, len(tiles)))

            def paced_scores(h, blk):
                s = scores(h, blk)
                for t in range(blk + 1):
                    mine = plan.get(((h, blk), t), [])
                    for i, (pace, work, *_) in enumerate(mine):
                        r = 8 * (i * (R // 8) // len(mine))
                        pace(_witness([s[r:r + 8, t * R:(t + 1) * R]] + list(work())))
                return s

            todo, done = [[]] * 8, []
            v_scale = unit[1, j, :1]
            ahead = [paced_scores(*b) for b in blocks[:depth]]
            for n, (h, blk) in enumerate(blocks):
                ahead += [paced_scores(*b) for b in blocks[n + depth:n + depth + 1]]
                _run(todo[2 * (n % 4)])
                done.append(attend(v_scale, h, blk, ahead.pop(0)))
                _store(ctx, 0, pl.multiple_of(j * (S // 2), S // 2) + blk * (R // 2), h * HD, done[-1])
                if len(done) > _CL:
                    q_s[zero, pl.ds(S // 2, 8), :128] = _witness([done.pop(0)])
                _run(todo[2 * (n % 4) + 1])
                if n % 4 == 3:
                    todo = filler(blk // 2)
            _run(sum(todo, []))

        w0, w1 = cp_proj_w(0, 0, 0), cp_proj_w(1, 1, 0)
        stages = ([w0[:2]]
                  + [[cp_c(c) for c in part] + (w1[2:] if n == _CW else []) for n, part in enumerate(_CS)]
                  + [[cp_x(c) for c in part] + (w1[:2] if n == _XW else []) for n, part in enumerate(_XS)]
                  + [cp_step(0)[2:4]])

        def issue(i, zero):
            for k, stage in enumerate(stages):
                @pl.when(i == k)
                def _(stage=stage):
                    for cp in stage:
                        cp.start()
            return zero + i // NP

        zero = lax.fori_loop(0, len(stages), issue, jnp.int32(0)) if 'pro' in _PARTS else lax.fori_loop(0, 15, lambda i, z: z + i // NP, jnp.int32(0))

        def project(prep, steps, chunks, side):
            for n, c in enumerate(chunks):
                prep(c)
                _run(_mingle(steps(c, SLOT), _share(side, n, len(chunks))))

        if "pro" in _PARTS:
            aw_raw[0] = jnp.zeros(aw_raw.shape[1:], BF16)
            for cp in stages[0]:
                cp.wait()
            _now(sum(prep_kv_w(0, 0, SLOT, zero), []))
            side = prep_q_w(1, zero)
            for n, chunks in enumerate(_CS):
                for cp in stages[1 + n]:
                    cp.wait()
                if n == 0:
                    for cp in cp_step(0)[:2]:
                        cp.start()
                project(prep_c, kv_proj, chunks, _share(side, n - _CW, len(_CS) - _CW) if n >= _CW else [])
            scale = unit[0, 0, :1] * (HD ** -0.5 * LOG2E)
            side = sum(prep_kv_w(1, 1, 0, zero), [])
            for n, chunks in enumerate(_XS):
                for cp in stages[1 + len(_CS) + n]:
                    cp.wait()
                project(prep_x, lambda c, slot: q_proj(scale, c), chunks,
                        _share(side, n - _XW, len(_XS) - _XW) if n >= _XW else [])

        def pair_step(j, zero):
            for cp in cp_step(j)[:4]:
                cp.wait()

            @pl.when(j > 0)
            def _():
                cp_step(j)[4].wait()


            @pl.when(j == RING)
            def _():
                bwop[:SLOT] = bwop[RING * SLOT:]
                for cp in cp_a():
                    cp.start()

            for cp in cp_step(j + 1):
                cp.start()
            slot = pl.multiple_of((j % RING) * SLOT, KVROWS)
            scale = unit[0, j + 1, :1] * (HD ** -0.5 * LOG2E)
            aw = prep_aw(aw_unit(j), j % 2, zero)
            sizes, bw = prep_kv_w(j + 2, j % 2, slot + SLOT, zero)
            bw = sizes + [None] * _SG + bw
            wo = prep_wo(j, j % 2, zero)
            groups = dict(a=aw, o=wo, b=bw)
            side = [None] * _S0 + _blend(*[groups[g] for g in "aob" if g not in _QS])

            history = []

            def filler(c):
                mine = _share(side, _FIRST - c, _FIRST + 1) if c <= _FIRST else []
                q, kv = q_proj(scale, c), kv_proj(c, slot)
                slots = []
                for n in range(4):
                    qn, kvn = _share(q, n, 4), _share(kv, n, 4)
                    k = len(kvn) * _SP // 8
                    slots += {0: [kvn[k:] + qn, kvn[:k]][::1], 1: [qn + kvn[k:], kvn[:k]], 2: [kvn[k:], qn + kvn[:k]]}[_QK]
                order = iter(q), iter(kv)
                slots = [[next(order[0]) if step in q else next(order[1]) for step in slot] for slot in slots]
                steps = iter(_mingle(sum(slots, []), mine, history if _HI else None))
                return [[next(steps) for _ in slot] for slot in slots]

            pair_attention(j, zero, filler, _blend(*[groups[g] for g in _QS]), early=prep_q_w(j % 2, zero))
            return zero + j // NP

        if "bloop" in _PARTS:
            zero = lax.fori_loop(0, NP - 1, pair_step, zero)
        gap("4", zero)
        if "last" in _PARTS:
            for cp in cp_step(NP - 1) + cp_a() if 'bloop' in _PARTS else []:
                cp.wait()
            side = sum((prep_awo(n // 2, n % 2, zero) for n in range(_AE)), [])
            if "w" in _EW:
                side = _blend(prep_wo(NP - 1, (NP - 1) % 2, zero), *([side] if side else []))
            pair_attention(NP - 1, zero, lambda c: [[]] * 8, side, _DEPTH, _QE)
        else:
            ctx[0, :8, :128] = (q_s[zero, :8, :128] + k_s[zero, :8, :128] + v_s[zero, :8, :128]
                                + bwop[pl.ds(zero, 8), :] + qwop[zero, :8, :] + xop[zero, :8, :128] + cop[zero, 0, :8, :])
        return zero

    def rows(zero, dummy2, xaop, aoop, aqkv, oop, out_s):
        dummy2[:8] = jnp.zeros((8, 128), F32)
        dummy[:8] = dummy2[pl.ds(1, 8)]

        @pl.loop(0, 2)
        def _(i):
            aqkv[pl.ds(8 + 8 * i, 8), :HALO, :] = jnp.zeros((8, HALO, 128), F32)

        def cp_out(c, half):
            cols = pl.ds(half * DM, DM)
            return pltpu.make_async_copy(
                out_s.at[half, c], out_hbm.at[pl.ds(pl.multiple_of(c * CH, CH), CH), cols],
                sem_out.at[half * NC + c])

        def prep_xa(c, zero):
            def piece(t, r, i):
                outer = {b: [_split(pltpu.bitcast(
                    xa[c, pl.ds((b // 2) * R + r2 * R // 2 + r, 16),
                       pl.ds(512 * t + (b % 2) * 256 + a2 * 128, 128)], U32))
                    for r2 in range(2) for a2 in range(2)] for b, _ in LHS[i]}
                ops = [_join(v) for v in _operands(_combine(outer, LHS[i]), LHS)]
                for k, v in enumerate(ops):
                    xaop[NOPS * i + k, pl.ds(r // 2, 8), pl.ds(128 * t, 128)] = v
                return ops
            return [(_pacer(xa, NC + zero), lambda t=t, r=r, i=i: piece(t, r, i))
                    for t in range(2) for r in range(0, R // 2, 16) for i in range(NOPS)]

        def prep_ctx(c, zero):
            base = pl.multiple_of(c * (CH // 2), CH // 2)

            def piece(m, r, i):
                outer = {b: [_split(ctx[0, pl.ds(base + ((2 * m + a2) * (S // 2) + (b // 2) * 64 + r2 * 32 + r), 8),
                                        pl.ds((b % 2) * HD, HD)])
                             for r2 in range(2) for a2 in range(2)] for b, _ in LHS[i]}
                ops = [_join(v) for v in _operands(_combine(outer, LHS[i]), LHS)]
                for k, v in enumerate(ops):
                    oop[NOPS * i + k, pl.ds(r, 8), pl.ds(HD * m, HD)] = v
                return ops
            def pace(v):
                ctx[zero, pl.ds(NP * S // 2, 8), :128] = v
            return [(pace, lambda m=m, r=r, i=i: piece(m, r, i))
                    for m in range(NP // 2) for r in range(0, 32, 8) for i in range(NOPS)]

        def o_proj(c):
            steps = []
            for t in range(2):
                def done(o, val, t=t):
                    r0 = (o[0] // 2) * R + (o[1] // 2) * (R // 2)
                    n0 = 512 * t + (o[0] % 2) * 256 + (o[1] % 2) * 128
                    out_s[1, c, pl.ds(r0, R // 2), pl.ds(n0, 128)] = val.astype(BF16)
                steps.append(_block_product(lambda i: _bf16(oop[i]),
                                            lambda i, t=t: _bf16(woop[t, i]), done, levels=2))
            return _weave(steps, "o" in _W) + ([lambda: cp_out(c, 1).start(priority=_PRIO)] if 'D' not in _X else [])

        def a_proj(row0):
            steps = []
            for part in range(3):
                both = []
                for t in range(2):
                    def done(o, val, part=part, t=t):
                        if part == 0:
                            val = val * (AD ** -0.5 * LOG2E)
                        r0 = (o[0] // 2) * R + (o[1] // 2) * (R // 2)
                        aqkv[8 * part + 4 * (o[0] % 2) + 2 * (o[1] % 2) + t,
                             pl.ds(row0 + (HALO + r0), R // 2), :] = val

                    def rhs(i, part=part, t=t):
                        return _bf16(jnp.concatenate(
                            [awop[2 * part + m, i, pl.ds(64 * t, 64), :] for m in range(2)], axis=1))
                    both.append(_block_product(lambda i: _bf16(xaop[i]), rhs, done, NT, 2))
                steps += _weave(both, "p" in _W)
            return _group(steps, _AG)

        def a_attention(c, row0, zero, n):
            logit, prob, mixed = {}, {}, {}

            def dot(r, w):
                tot = None
                for t in range(8):
                    if (r, t) not in logit:
                        logit[r, t] = aqkv[t, pl.ds(row0 + (HALO + r), 8), :]
                    pr = logit[r, t] * aqkv[8 + t, pl.ds(row0 + (HALO + r - DIL * w if not _AL else r + 8 * w), 8), :]
                    tot = pr if tot is None else tot + pr
                logit[r, "w", w] = tot
                if w == WIN - 1:
                    weights(r)
                return [tot]

            def weights(r):
                logits = [logit[r, "w", w] for w in range(WIN)]
                logits = [x + pltpu.roll(x, 64, 1) for x in logits]
                logits = [x + pltpu.roll(x, 32, 1) for x in logits]
                if r < (WIN - 1) * DIL:
                    pos = c * CH + r + lax.broadcasted_iota(jnp.int32, (8, 128), 0)
                    logits = [x if w == 0 else jnp.where(pos >= DIL * w, x, MASKED)
                              for w, x in enumerate(logits)]
                top = logits[0]
                for x in logits[1:]:
                    top = jnp.maximum(top, x)
                e = [jnp.exp2(x - top) for x in logits]
                tot = e[0]
                for x in e[1:]:
                    tot = tot + x
                inv = _recip(tot)
                prob[r] = [x * inv for x in e]

            def mix(r, t, d, q):
                tot = None
                for w in range(WIN):
                    pr = prob[r + d][w] * aqkv[16 + t + 2 * q,
                                               pl.ds(row0 + (HALO + r + d - DIL * w if not _AL else r + d + 8 * w), 8), :]
                    tot = pr if tot is None else tot + pr
                mixed[r, t, d, q] = tot
                return [tot]

            def operands(r, t, i):
                outer = {b: [jnp.concatenate(
                    [mixed[r, t, (b // 2) * R + r2 * R // 2 + e, 2 * (b % 2) + a2] for e in (0, 8)],
                    axis=0) for r2 in range(2) for a2 in range(2)] for b, _ in LHS[i]}
                ops = _operands(_combine(outer, LHS[i]), LHS)
                for k, v in enumerate(ops):
                    _store(aoop, NOPS * i + k, r // 2, 128 * t, v)
                return ops

            groups = [d + e for d in range(0, CH, R // 2) for e in (0, 8)]

            def dots(r):
                return [lambda d=d, w=w: dot(r + d, w) for d in groups for w in range(WIN)]

            def mixes(r):
                return [work for t in range(2) for work in
                        [lambda t=t, d=d, q=q: mix(r, t, d, q) for d in groups for q in range(4)]
                        + [lambda t=t, i=i: operands(r, t, i) for i in range(NOPS)]]

            work = dots(0)
            for r in range(16, R // 2, 16):
                work += _blend(dots(r), mixes(r - 16))
            work += mixes(R // 2 - 16)
            return [(_pacer(aqkv, 24 + zero), lambda g=work[i:i + n]: sum((w() for w in g), []))
                    for i in range(0, len(work), n)]

        def a_out_proj(c, zero):
            steps = []
            for n in range(2):
                def done(o, val, n=n):
                    r0 = (o[0] // 2) * R + (o[1] // 2) * (R // 2)
                    n0 = (o[0] % 2) * 512 + (o[1] % 2) * 256 + 128 * n
                    out_s[0, c, pl.ds(r0, R // 2), pl.ds(n0, 128)] = val.astype(BF16)
                steps.append(_block_product(lambda i: _bf16(aoop[zero + i]),
                                            lambda i, n=n: _bf16(awoop[n, i]), done, levels=2))
            return _group(_weave(steps, "a" in _W), _AG) + ([lambda: cp_out(c, 0).start()] if 'D' not in _X else [])

        if "s0" in _PARTS:
            _now(prep_xa(zero, zero))
            lists = [prep_ctx(0, zero), sum((prep_awo(n // 2, n % 2, zero) for n in range(_AE, 4)), [])]
            if "w" not in _EW:
                lists.append(prep_wo(NP - 1, (NP - 1) % 2, zero))
            _run(_mingle(a_proj(0), _blend(*[x for x in lists if x])))

        def chunk_step(c, zero):
            row0 = pl.multiple_of((c - 1) * CH, CH)
            first, second = o_proj(c - 1), a_proj(row0 + CH)
            att = a_attention(c - 1, row0, zero, _NA) if 'A' not in _X else []
            cut = len(att) * _CU // 16
            xap, ctxp = prep_xa(c, zero), prep_ctx(c, zero) if 'C' not in _X else []
            third = a_out_proj(c - 1, zero)
            late = len(ctxp) * _CT // 16
            _run((_mingle(first[:-1], _blend(att[:cut], xap)) if '1' not in _X else []) + first[-1:])
            if '2' not in _X:
                _run(_mingle(second[:-_AT], _blend(att[cut:], ctxp[:-late])) + second[-_AT:])
            _run((_mingle(third[:-_AT], ctxp[-late:]) + third[-_AT:-1] if '3' not in _X else []) + third[-1:])
            return zero + c // NC

        pad(_PA, zero)
        if "aloop" in _PARTS:
            zero = lax.fori_loop(1, NC, chunk_step, zero)

        if "epi" in _PARTS:
            steps = o_proj(NC - 1)
            _run(_mingle(steps[:-_ET], a_attention(NC - 1, (NC - 1) * CH, zero, _EN)) + steps[-_ET:])
            _run(a_out_proj(NC - 1, zero))
            for c in range(NC if 'D' in _X else 0):
                cp_out(c, 1).start()
                cp_out(c, 0).start()
            for c in range(NC):
                cp_out(c, 1).wait()
                cp_out(c, 0).wait()
        else:
            out_s[0, 0, :16, :128] = aqkv[3, :16, :].astype(BF16)
            out_s[0, 0, 16:32, :128] = _bf16(awop[0, 0, :8, :] + ctx[0, :8, :128] + woop[0, 0, :8, :]
                                             + oop[0, :8, :128] + awoop[0, 0, :8, :])
            cp_out(0, 0).start()
            cp_out(0, 0).wait()

    vmem = pltpu.VMEM
    zero = pl.run_scoped(
        heads,
        vmem((NOPS * NC + 1, R // 2, DM // 2), U32),
        vmem((NC, NOPS * NOPS, R // 4, 128), U32),
        vmem((3, DM, HD), U32),
        vmem((5, DC, HD), U32),
        vmem((NOPS, OPROWS, 128), U32),
        vmem(((RING + 1) * SLOT, 128), U32),
        vmem((1, S // 2 + _QP, 2 * HD), U32),
        vmem((1, S // 2, 2 * HD), U32),
        vmem((1, S // 2, 2 * HD), U32),
        vmem((2, 512, 512), BF16),
        vmem((2, NP + 2, 8, 128), F32),
    )
    pl.run_scoped(
        lambda *refs: rows(zero, *refs),
        vmem((_D2, 128), F32),
        vmem((NOPS * NOPS, R // 4, DM // 4), U32),
        vmem((NOPS * NOPS, R // 4, DM // 4), U32),
        vmem((25, HALO + S + _AP + 64 * _AL, 128), F32),
        vmem((NOPS * NOPS, R // 4, NP * HD // 2), U32),
        vmem((2, NC, CH, DM), BF16),
    )


@jax.jit
def pallas_concat_heads__sliding_local_dilated__compressed_kv_cla__prompt_kernel(
    A_x: jax.Array,
    A_wqkv: jax.Array,
    A_wo: jax.Array,
    B_x: jax.Array,
    B_c_kv: jax.Array,
    B_w_q: jax.Array,
    B_w_uk: jax.Array,
    B_w_uv: jax.Array,
    B_w_o: jax.Array,
):
    vmem = pltpu.VMEM
    dma = pltpu.SemaphoreType.DMA
    scratch = [
        vmem((_DUM, 128), F32),
        vmem((1, NP * S // 2 + 16, 2 * HD), U32),
        vmem((3, 2 * HD, 512), U32),
        vmem((2, NOPS * NOPS, NP * HD // 4, 128), U32),
        vmem((N_UNITS // 2, NOPS * NOPS, DM // 8, 128), U32),
        vmem((2, NOPS * NOPS, DM // 8, 128), U32),
        vmem((NC + 1, CH, DM), BF16),
        vmem((9, CH, DC), BF16),
        vmem((5, 16 * PITCH + 16, 128), F32),
        dma((NC,)), dma((NC,)), dma((8,)), dma((4,)), dma((2,)), dma((2 * NC,)),
    ]
    out = pl.pallas_call(
        _kernel,
        out_shape=jax.ShapeDtypeStruct((S, 2 * DM), BF16),
        in_specs=[pl.BlockSpec(memory_space=pl.ANY)] * 9,
        out_specs=pl.BlockSpec(memory_space=pl.ANY),
        scratch_shapes=scratch,
        compiler_params=pltpu.CompilerParams(vmem_limit_bytes=124 * 2**20),
        name="fused_local_and_latent_attention",
    )(
        A_x.reshape(S, DM), A_wqkv, A_wo,
        B_x.reshape(S, DM), B_c_kv.reshape(S, DC),
        B_w_q, B_w_uk, B_w_uv, B_w_o.reshape(NH * HD, DM),
    )
    return out.reshape(1, S, 2 * DM)
```

```python
import math

import jax
import jax.numpy as jnp
from jax import lax
import jax.experimental.pallas as pl
import jax.experimental.pallas.tpu as pltpu

F32, BF16, U32 = jnp.float32, jnp.bfloat16, jnp.uint32

S = 2048
DM = 1024
DC = 512
NH = 32
HD = 128
AD = 32
WIN, DIL = 8, 2

R = 128
CH = 2 * R
NC = S // CH
NP = NH // 2
HALO = 16
PITCH = 33

_PARTS = ("pro", "bloop", "last", "s0", "aloop", "epi")
_X = ""
_FIRST = 7
_NA = 1
_NB = 16
_LAG = 5
_AT = 6
_PRIO = 0
_D2 = 32
_W = ''
_QE = 2
_AE = 1
_EW = 'x'
_WS = 1
_AG = 2
_QS = 'o'
_Q0 = 6
_SP = 6
_KG = 1
_QK = 0
_K2 = 0
_CT = 4
_CU = 10
_DUM = 24
_QP = 16
_AP = 16
_PA = 0
_PB = 0
_CL = 3
_CZ = 4
_SC = 2
_QD = 2
_QC = (0, 6, 10)
_KA = 5
_XS = tuple((c,) for c in range(7, -1, -1))
_XW = 0
_CS = ((7, 6), (5, 4), (3, 2), (1, 0))
_CW = 3
_AL = 0
_HI = 1
_S0 = 16
_EN = 2
_ET = 3
_SG = 16
_E0 = 2
_E1 = 12
_DEPTH = 1
LOG2E = math.log2(math.e)
MASKED = -1e9 * LOG2E

NN = (((1,), (0,)), ((), ()))
NT = (((1,), (1,)), ((), ()))

LHS = (((0, 1), (3, 1)), ((2, 1), (3, 1)), ((0, 1),), ((3, 1),),
       ((0, 1), (1, 1)), ((2, 1), (0, -1)), ((1, 1), (3, -1)))
RHS = (((0, 1), (3, 1)), ((0, 1),), ((1, 1), (3, -1)), ((2, 1), (0, -1)),
       ((3, 1),), ((0, 1), (1, 1)), ((2, 1), (3, 1)))
PRODUCTS = ((2, ((1, 1), (3, 1))), (4, ((0, -1), (1, 1))), (3, ((0, 1), (2, 1))),
            (1, ((2, 1), (3, -1))), (5, ((3, 1),)), (0, ((0, 1), (3, 1))),
            (6, ((0, 1),)))
NOPS = len(PRODUCTS)

SLOPE = (-1.5, -0.5, 0.5, 1.5)
COUPLES = tuple((i, j) for j in range(4) for i in range(j, -1, -1))
NQ = sum(2 if i == j else 3 for i, j in COUPLES)


def _couple_left(x, i, j):
    if i == j:
        p = q = x(i, i)
        for k in range(4):
            if k != i:
                p, q = p - x(k, i), q + x(i, k)
        return [p, q]
    return [x(i, j) + x(j, i), x(i, j), x(j, i)]


def _couple_right(w, i, j):
    (a0, a1), (b0, b1) = w(i), w(j)
    if i == j:
        return [a0, SLOPE[i] * a0 + a1]
    return [(SLOPE[i] * a0 + a1) - (SLOPE[j] * b0 + b1),
            SLOPE[i] * (b0 - a0) + (b1 - a1), SLOPE[j] * (b0 - a0) + (b1 - a1)]


def _couple_product(lhs, rhs, done):
    first, second, steps = {}, {}, []

    def add(i, j, m):
        if i == j:
            first[i], second[i] = m
        else:
            t = m[0] + m[1] + m[2]
            gap = SLOPE[j] - SLOPE[i]
            t = t if gap == 1 else t * (1 / gap)
            first[i], first[j] = first[i] - t, first[j] - t
            second[i], second[j] = second[i] + m[1], second[j] - m[2]
        if j == 3 and i < j:
            for r in (i,) if i else (0, 3):
                done(r, first[r], second[r] - SLOPE[r] * first[r])

    for i, j in COUPLES:
        got, n = [], 2 if i == j else 3
        for _ in range(n):
            def step(i=i, j=j, got=got, n=n, k=len(steps)):
                got.append(lax.dot_general(lhs(k), rhs(k), NN, preferred_element_type=F32))
                if len(got) == n:
                    add(i, j, got)
                return got[-1]
            steps.append(step)
    return steps


RING = 8
N_UNITS = 12
KVROWS = 64
SLOT = NOPS * NOPS * KVROWS


def _combine(blocks, terms):
    if isinstance(blocks[terms[0][0]], list):
        return [_combine({b: blocks[b][i] for b, _ in terms}, terms) for i in range(4)]
    out = None
    for i, sign in terms:
        if out is None:
            assert sign > 0
            out = blocks[i]
        else:
            out = out + blocks[i] if sign > 0 else out - blocks[i]
    return out


def _store(words, index, row, col, x):
    matrix = words.bitcast(BF16).at[index]
    matrix[pl.ds(pl.multiple_of(2 * row, 16), x.shape[0]), pl.ds(col, x.shape[1])] = x.astype(BF16)


def _bf16(words):
    return pltpu.bitcast(words, BF16)


def _halves(words):
    lo = pltpu.bitcast(words << 16, F32)
    hi = pltpu.bitcast(words & jnp.uint32(0xFFFF0000), F32)
    return lo, hi


def _split(words):
    return jnp.concatenate(_halves(words), axis=0)


def _join(x):
    n = x.shape[0] // 2
    return pltpu.pack_elementwise([x[:n], x[n:]], packed_dtype=BF16)


def _recip(x):
    r = pltpu.reciprocal(x, approx=True)
    return r * (2.0 - x * r)


def _operands(blocks, side):
    return [_combine(blocks, terms) for terms in side]


def _block_product(lhs, rhs, done, dims=NN, levels=1):
    if levels == 0:
        def step():
            m = lax.dot_general(lhs(0), rhs(0), dims, preferred_element_type=F32)
            done((), m)
            return m
        return [step]

    held, steps = {}, []
    inner = NOPS ** (levels - 1)
    for n, (i, outs) in enumerate(PRODUCTS):
        later = {o for _, others in PRODUCTS[n + 1:] for o, _ in others}

        def add(sub, m, outs=outs, later=later):
            for o, sign in outs:
                if (o, sub) not in held:
                    held[o, sub] = m, sign
                else:
                    c, s = held[o, sub]
                    assert s > 0 or sign > 0
                    held[o, sub] = (m - c if s < 0 else c + m if sign > 0 else c - m), 1
                if o not in later:
                    done((o, *sub), held.pop((o, sub))[0])

        steps += _block_product(lambda k, i=i: lhs(i * inner + k),
                                lambda k, i=i: rhs(i * inner + k), add, dims, levels - 1)
    return steps


def _run(steps, n=None):
    out = None
    for _ in range(len(steps) if n is None else min(n, len(steps))):
        out = steps.pop(0)()
    return out


def _group(steps, n):
    return [lambda g=steps[i:i + n]: _run(g) for i in range(0, len(steps), n)]


def _weave(lists, together):
    return [x for xs in zip(*lists) for x in xs] if together else sum(lists, [])


def _share(items, k, n):
    return items[k * len(items) // n:(k + 1) * len(items) // n]


def _blend(*lists):
    spots = [((i + 0.5) / len(items), k, item)
             for k, items in enumerate(lists) for i, item in enumerate(items)]
    return [item for *_, item in sorted(spots, key=lambda spot: spot[:2])]


def _witness(values):
    out = None
    for v in values:
        v = pltpu.bitcast(v, U32)
        for r in range(0, v.shape[0], 8):
            for c in range(0, v.shape[1], 128):
                out = v[r:r + 8, c:c + 128] if out is None else out | v[r:r + 8, c:c + 128]
    return out


def _mingle(steps, pieces, history=None):
    history = [] if history is None else history

    def both(step, mine):
        history.append(step())
        mine = [piece for piece in mine if piece]
        for i, (pace, work, *lag) in enumerate(mine):
            seen = work()
            m = history[max(0, len(history) - 1 - sum(lag))]
            if m is not None:
                r = 8 * (i * (m.shape[0] // 8) // len(mine))
                pace(_witness([m[r:r + 8, :128]] + list(seen)))
        return history[-1]

    return [lambda step=step, mine=_share(pieces, i, len(steps)): both(step, mine)
            for i, step in enumerate(steps)]


def _now(pieces):
    for _, work, *_ in pieces:
        work()


def _pacer(ref, *index):
    def pace(v):
        if ref.dtype == BF16:
            ref[(*index, pl.ds(0, 16), pl.ds(0, 128))] = _bf16(v)
        else:
            ref[(*index, pl.ds(0, 8), pl.ds(0, 128))] = pltpu.bitcast(v, ref.dtype)
    return pace


def _dim_major(src, pace, shuf, put, swap, zero):
    def start(head):
        return ((head % 2) * 8 + head // 2) * PITCH

    def scatter(k, u):
        t = src(k, u)
        for h in range(128 // AD):
            shuf[k, pl.ds(start(4 * u + h), AD), :] = t[h * AD:(h + 1) * AD]
        return [t]

    def gather(d, i):
        def block(row1, col1, row2, col2):
            quarter, k = 2 * row1 + row2, 2 * col1 + col2
            if swap:
                quarter, k = k, quarter
            return jnp.concatenate(
                [shuf[k, pl.ds(start(p) + quarter * AD // 4 + d, 8, stride=PITCH), :]
                 for p in range(2)], axis=0)
        outer = {b: [block(b // 2, b % 2, s // 2, s % 2) for s in range(4)] for b, _ in RHS[i]}
        ops = [_join(v) for v in _operands(_combine(outer, RHS[i]), RHS)]
        for n, v in enumerate(ops):
            put(NOPS * i + n, d * NH // 2, v)
        return ops

    return ([x for k in range(4) for u in range(4)
             for x in [(pace, lambda k=k, u=u: scatter(k, u), _LAG if swap else 0)] + [None] * (_SC if swap else 0)]
            + [(_pacer(shuf, 4 + zero), lambda d=d, i=i: gather(d, i))
               for d in range(AD // 4) for i in range(NOPS)])


def _kernel(ax_hbm, awqkv_hbm, awo_hbm, bx_hbm, c_hbm, wq_hbm, wuk_hbm, wuv_hbm,
            wo_hbm, out_hbm,
            dummy, ctx, wo_raw, woop, awop, awoop, xa, xaop, awo_raw, shuf,
            sem_x, sem_c, sem_w, sem_aw, sem_a, sem_out):

    def cp_tile(src, row, col, dst, sem):
        def span(i):
            return pl.ds(pl.multiple_of(i * 512, 512), 512)
        return pltpu.make_async_copy(src.at[span(row), span(col)], dst, sem)

    def cp_wo(u, s):
        return [cp_tile(wo_hbm, u // 2, u % 2, wo_raw.at[s].bitcast(BF16), sem_w.at[6 + s])]

    def prep_wo(u, s, zero):
        def piece(r, i):
            outer = {b: [_split(wo_raw[s, pl.ds((2 * a2 + b // 2) * (HD // 2) + r, 8),
                                       pl.ds((2 * (b % 2) + b2) * 128, 128)])
                         for a2 in range(2) for b2 in range(2)] for b, _ in RHS[i]}
            ops = [_join(v) for v in _operands(_combine(outer, RHS[i]), RHS)]
            row = pl.multiple_of((u // 2) * (HD // 2) + r, 8)
            for k, v in enumerate(ops):
                woop[u % 2, NOPS * i + k, pl.ds(row, 8), :] = v
            return ops
        return [(_pacer(wo_raw, 2 + zero), lambda r=r, i=i: piece(r, i))
                for r in range(0, HD // 2, 8) for i in range(NOPS)]

    def prep_awo(n, half, zero):
        def put(i, row, v):
            awoop[n, i, pl.ds(8 * half + row, 8), :] = v
        return _dim_major(
            lambda k, t: awo_raw[4 * half + t, pl.ds(128 * (k // 2), 128),
                                 pl.ds((k % 2) * (DM // 4) + 128 * n, 128)].astype(F32),
            _pacer(awo_raw, 8 + zero), shuf, put, False, zero)

    def prep_xa(c, zero):
        def piece(t, r, i):
            outer = {b: [_split(pltpu.bitcast(
                xa[c, pl.ds((b // 2) * R + r2 * R // 2 + r, 16),
                   pl.ds(512 * t + (b % 2) * 256 + a2 * 128, 128)], U32))
                for r2 in range(2) for a2 in range(2)] for b, _ in LHS[i]}
            ops = [_join(v) for v in _operands(_combine(outer, LHS[i]), LHS)]
            for k, v in enumerate(ops):
                xaop[NOPS * i + k, pl.ds(r // 2, 8), pl.ds(128 * t, 128)] = v
            return ops
        return [(_pacer(xa, NC + zero), lambda t=t, r=r, i=i: piece(t, r, i))
                for t in range(2) for r in range(0, R // 2, 16) for i in range(NOPS)]

    def gap(flag, zero):
        if flag in _X:
            @pl.loop(0, 2)
            def _(i):
                _pacer(shuf, 4 + zero * i)(jnp.zeros((8, 128), U32))

    def pad(n, zero):
        if n:
            @pl.when(zero != 0)
            def _():
                v = shuf[0, :128]
                for _ in range(n * 95):
                    v = v * 1.0001 + 0.5
                shuf[0, :128] = v

    dummy[:8] = jnp.zeros((8, 128), F32)
    shuf[0, :8] = dummy[pl.ds(1, 8)]

    def cp_a():
        return ([pltpu.make_async_copy(ax_hbm.at[pl.ds(c * CH, CH)], xa.at[c], sem_a.at[0])
                 for c in range(NC)]
                + [pltpu.make_async_copy(awo_hbm.at[pl.ds(128 * t, 128), pl.ds(DC * h, DC)],
                                         awo_raw.at[t, pl.ds(128 * h, 128)], sem_a.at[1])
                   for t in range(8) for h in range(2)])

    def heads(xop, cop, wq_raw, wkv_raw, qwop, bwop, q_s, k_s, v_s, aw_raw, unit):
        xs, cs = xa, awo_raw
        wq32 = wq_hbm.bitcast(U32)
        wuk32 = wuk_hbm.bitcast(U32)
        wuv32 = wuv_hbm.bitcast(U32)

        def cp_x(c):
            return pltpu.make_async_copy(bx_hbm.at[pl.ds(c * CH, CH)], xs.at[c], sem_x.at[c])

        def cp_c(c):
            return pltpu.make_async_copy(c_hbm.at[pl.ds(c * CH, CH)], cs.at[c], sem_c.at[c])

        def cp_proj_w(j, s, jq):
            return [
                pltpu.make_async_copy(wuk32.at[:, j, :], wkv_raw.at[s], sem_w.at[s]),
                pltpu.make_async_copy(wuv32.at[:, j, :], wkv_raw.at[2 + s], sem_w.at[2 + s]),
                pltpu.make_async_copy(wq32.at[:, jq, :], wq_raw.at[s], sem_w.at[4 + s]),
            ]

        def cp_aw(u, s):
            return [cp_tile(awqkv_hbm, u // 2 % 2, 2 * (u // 4) + u % 2, aw_raw.at[s], sem_aw.at[s])]

        def aw_unit(j):
            return jnp.clip(j - 1, 0, N_UNITS - 1)

        def cp_step(j):
            return (cp_proj_w(jnp.minimum(j + 2, NP - 1), j % 2, jnp.minimum(j + 1, NP - 1)) + cp_wo(jnp.maximum(j - _WS, 0), j % 2)
                    + cp_aw(aw_unit(j), j % 2))

        def prep_x(c):
            for t in range(2):
                blocks = [[_split(pltpu.bitcast(
                    xs[c, pl.ds(r * R // 2, R // 2), pl.ds(k * DM // 4 + 128 * t, 128)], U32))
                    for k in range(4)] for r in range(4)]
                ops = [v for i, j in COUPLES for v in _couple_left(lambda r, k: blocks[r][k], i, j)]
                for n, v in enumerate(ops):
                    xop[NQ * c + n, :, pl.ds(128 * t, 128)] = _join(v)

        def prep_c(c):
            blocks = [[_split(pltpu.bitcast(
                cs[c, pl.ds(r1 * R + r2 * R // 2, R // 2), pl.ds(a1 * 256 + a2 * 128, 128)], U32))
                for r2 in range(2) for a2 in range(2)] for r1 in range(2) for a1 in range(2)]
            for i, outer in enumerate(_operands(blocks, LHS)):
                for k, v in enumerate(_operands(outer, LHS)):
                    cop[c, NOPS * i + k] = _join(v)

        def both_heads(raw, s, row):
            even, odd = (_halves(raw[s, pl.ds(row + p, 8, stride=2), :]) for p in range(2))
            return [jnp.concatenate([even[h], odd[h]], axis=0) for h in range(2)]

        def prep_q_w(s, zero):
            def piece(r, couples, n):
                w = {k: both_heads(wq_raw, s, k * DM // 4 + r) for couple in couples for k in couple}
                ops = [_join(v) for i, j in couples for v in _couple_right(w.get, i, j)]
                for k, v in enumerate(ops):
                    qwop[n + k, pl.ds(r // 2, 8), :] = v
                return ops
            parts = [COUPLES[a:b] for a, b in zip(_QC, _QC[1:])]
            starts = [sum(2 if i == j else 3 for i, j in COUPLES[:a]) for a in _QC]
            return [(_pacer(wq_raw, 2 + zero), lambda r=r, part=part, n=n: piece(r, part, n))
                    for r in range(0, DM // 4, 16) for part, n in zip(parts, starts)]

        def prep_kv_w(j, s, slot, zero):
            total, inverse = {}, {}

            def measure(n, r):
                w = wkv_raw[2 * n + s, pl.ds(r, 64), :]
                w = jnp.abs(pltpu.bitcast(w, F32)) + jnp.abs(pltpu.bitcast(w << 16, F32))
                w = jnp.sum(w.reshape(8, 8, 128), axis=0)
                total[n] = total[n] + w if r else w
                return [total[n]]

            def size(n):
                both = jnp.sum(jnp.sum(total[n], axis=1, keepdims=True), axis=0, keepdims=True)
                both = jnp.broadcast_to(jnp.clip(both, 2.0 ** -100, 2.0 ** 100), (8, 128))
                power = pltpu.bitcast(both, U32) & jnp.uint32(0x7F800000)
                unit[n, j] = pltpu.bitcast(power, F32)
                inverse[n] = pltpu.bitcast(jnp.uint32(0x7F000000) - power, F32)
                return [power]

            def piece(r, i):
                outer = {b: [v * jnp.concatenate([inverse[b % 2]] * 2, axis=0) for a2 in range(2)
                             for v in both_heads(wkv_raw, 2 * (b % 2) + s, (b // 2) * 256 + a2 * 128 + r)]
                         for b, _ in RHS[i]}
                ops = [_join(v) for v in _operands(_combine(outer, RHS[i]), RHS)]
                for k, v in enumerate(ops):
                    bwop[pl.ds(slot + ((NOPS * i + k) * KVROWS + r // 2), 8), :] = v
                return ops
            pace = _pacer(wkv_raw, 4 + zero)
            return ([(pace, lambda n=n, r=r: measure(n, r)) for n in range(2) for r in range(0, DC, 64)]
                    + [(pace, lambda n=n: size(n)) for n in range(2)],
                    [(_pacer(xop, NQ * NC + zero), lambda: list(inverse.values()))]
                    + [(pace, lambda r=r, i=i: piece(r, i))
                       for r in range(0, 128, 16) for i in range(NOPS)])

        def prep_aw(u, s, zero):
            def put(i, row, v):
                awop[u // 2, i, pl.ds(pl.multiple_of(8 * (u % 2), 8) + row, 8), :] = v
            return _dim_major(
                lambda k, t: aw_raw[s, 128 * k:128 * (k + 1), 128 * t:128 * (t + 1)].astype(F32).T,
                _pacer(xop, NQ * NC + zero), shuf, put, True, zero)

        def words(blk):
            return pl.ds(blk * (R // 2), R // 2)

        def q_proj(scale, c):
            def done(r, *heads):
                for h, val in enumerate(heads):
                    _store(q_s, 0, c * R + r * (R // 4), h * HD, val * scale)
            return _couple_product(lambda i: _bf16(xop[NQ * c + i]), lambda i: _bf16(qwop[i]), done)

        def kv_proj(c, slot, n=1):
            def done(o, val):
                for e in range(n):
                    _store((k_s, v_s)[o[0] % 2], 0,
                           (2 * (c + e) + o[0] // 2) * (R // 2) + (o[1] // 2) * (R // 4),
                           (o[1] % 2) * HD, val[e * R // 2:(e + 1) * R // 2])
            return _group(_block_product(
                lambda i: _bf16(jnp.concatenate([cop[c + e, i] for e in range(n)], axis=0)),
                lambda i: _bf16(bwop[pl.ds(slot + i * KVROWS, KVROWS), :]),
                done, levels=2), _KG)

        def scores(h, blk):
            n = (blk + 1) * R
            s = lax.dot_general(_bf16(q_s[0, words(blk), pl.ds(h * HD, HD)]),
                                _bf16(k_s[0, :n // 2, pl.ds(h * HD, HD)]),
                                NT, preferred_element_type=F32)
            row = lax.broadcasted_iota(jnp.int32, (R, R), 0)
            col = lax.broadcasted_iota(jnp.int32, (R, R), 1)
            diag = jnp.where(col <= row, s[:, n - R:], MASKED)
            return diag if blk == 0 else jnp.concatenate([s[:, :n - R], diag], axis=1)

        def attend(scale, h, blk, s):
            n = (blk + 1) * R
            p = jnp.exp2(s - jnp.max(s, axis=1, keepdims=True))
            if "u" in _X:
                p = p.astype(BF16).astype(F32)
            inv = _recip(jnp.sum(p, axis=1, keepdims=True)) * scale
            o = lax.dot_general(p.astype(BF16), _bf16(v_s[0, :n // 2, pl.ds(h * HD, HD)]), NN,
                                preferred_element_type=F32)
            return o * inv

        def pair_attention(j, zero, filler, side=(), depth=1, first=None, early=()):
            blocks = [(h, 2 * c + u) for c in reversed(range(NC)) for u in (1, 0) for h in (0, 1)]
            plan = {}
            for pieces, span in ((side, blocks[_Q0 if first is None else first:]), (early, blocks[_E0:_E1])):
                tiles = [(b, t) for b in span for t in range(b[1] + 1)]
                for n, tile in enumerate(tiles):
                    plan.setdefault(tile, []).extend(_share(pieces, n, len(tiles)))

            def paced_scores(h, blk):
                s = scores(h, blk)
                for t in range(blk + 1):
                    mine = plan.get(((h, blk), t), [])
                    for i, (pace, work, *_) in enumerate(mine):
                        r = 8 * (i * (R // 8) // len(mine))
                        pace(_witness([s[r:r + 8, t * R:(t + 1) * R]] + list(work())))
                return s

            todo, done = [[]] * 8, []
            v_scale = unit[1, j, :1]
            ahead = [paced_scores(*b) for b in blocks[:depth]]
            for n, (h, blk) in enumerate(blocks):
                ahead += [paced_scores(*b) for b in blocks[n + depth:n + depth + 1]]
                _run(todo[2 * (n % 4)])
                done.append(attend(v_scale, h, blk, ahead.pop(0)))
                _store(ctx, 0, pl.multiple_of(j * (S // 2), S // 2) + blk * (R // 2), h * HD, done[-1])
                if len(done) > (_CL if early else _CZ):
                    q_s[zero, pl.ds(S // 2, 8), :128] = _witness([done.pop(0)])
                _run(todo[2 * (n % 4) + 1])
                if n % 4 == 3:
                    todo = filler(blk // 2)
            _run(sum(todo, []))

        w0, w1 = cp_proj_w(0, 0, 0), cp_proj_w(1, 1, 0)
        stages = ([w0[:2]]
                  + [[cp_c(c) for c in part] + (w1[2:] if n == _CW else []) for n, part in enumerate(_CS)]
                  + [[cp_x(c) for c in part] + (w1[:2] if n == _XW else []) for n, part in enumerate(_XS)]
                  + [cp_step(0)[2:4 - _WS]])

        def issue(i, zero):
            for k, stage in enumerate(stages):
                @pl.when(i == k)
                def _(stage=stage):
                    for cp in stage:
                        cp.start()
            return zero + i // NP

        zero = lax.fori_loop(0, len(stages), issue, jnp.int32(0)) if 'pro' in _PARTS else lax.fori_loop(0, 15, lambda i, z: z + i // NP, jnp.int32(0))

        def project(prep, steps, chunks, side):
            for n, c in enumerate(chunks):
                prep(c)
                _run(_mingle(steps(c, SLOT), _share(side, n, len(chunks))))

        if "pro" in _PARTS:
            aw_raw[0] = jnp.zeros(aw_raw.shape[1:], BF16)
            if _WS:
                wo_raw[0] = jnp.zeros(wo_raw.shape[1:], U32)
            for cp in stages[0]:
                cp.wait()
            _now(sum(prep_kv_w(0, 0, SLOT, zero), []))
            side = prep_q_w(1, zero)
            for n, chunks in enumerate(_CS):
                for cp in stages[1 + n]:
                    cp.wait()
                if n == 0:
                    for cp in cp_step(0)[:2]:
                        cp.start()
                project(prep_c, kv_proj, chunks, _share(side, n - _CW, len(_CS) - _CW) if n >= _CW else [])
            scale = unit[0, 0, :1] * (HD ** -0.5 * LOG2E)
            side = sum(prep_kv_w(1, 1, 0, zero), [])
            for n, chunks in enumerate(_XS):
                for cp in stages[1 + len(_CS) + n]:
                    cp.wait()
                project(prep_x, lambda c, slot: q_proj(scale, c), chunks,
                        _share(side, n - _XW, len(_XS) - _XW) if n >= _XW else [])

        def pair_step(j, zero):
            for cp in cp_step(j)[:4 - _WS]:
                cp.wait()

            @pl.when(j > 0)
            def _():
                for cp in cp_step(j)[4 - _WS:]:
                    cp.wait()

            @pl.when(j == RING)
            def _():
                bwop[:SLOT] = bwop[RING * SLOT:]
                for cp in cp_a():
                    cp.start()

            for cp in cp_step(j + 1):
                cp.start()
            slot = pl.multiple_of((j % RING) * SLOT, KVROWS)
            scale = unit[0, j + 1, :1] * (HD ** -0.5 * LOG2E)
            aw = prep_aw(aw_unit(j), j % 2, zero)
            sizes, bw = prep_kv_w(j + 2, j % 2, slot + SLOT, zero)
            bw = sizes + [None] * _SG + bw
            wo = prep_wo(jnp.maximum(j - _WS, 0), j % 2, zero)
            groups = dict(a=aw, o=wo, b=bw)
            side = [None] * _S0 + _blend(*[groups[g] for g in "aob" if g not in _QS])

            history = []
            qs = sum((q_proj(scale, c) for c in reversed(range(NC))), [])

            def filler(c):
                mine = _share(side, _FIRST - c, _FIRST + 1) if c <= _FIRST else []
                q = _share(qs, NC - 1 - _QD - c, NC - _QD) if c < NC - _QD else []
                kv = kv_proj(c, slot)
                slots = []
                for n in range(4):
                    qn, kvn = _share(q, n, 4), _share(kv, n, 4)
                    k = len(kvn) * _SP // 8
                    slots += {0: [kvn[k:] + qn, kvn[:k]][::1], 1: [qn + kvn[k:], kvn[:k]], 2: [kvn[k:], qn + kvn[:k]]}[_QK]
                order = iter(q), iter(kv)
                slots = [[next(order[0]) if step in q else next(order[1]) for step in slot] for slot in slots]
                steps = iter(_mingle(sum(slots, []), mine, history if _HI else None))
                return [[next(steps) for _ in slot] for slot in slots]

            pair_attention(j, zero, filler, _blend(*[groups[g] for g in _QS]), early=prep_q_w(j % 2, zero))
            return zero + j // NP

        if "bloop" in _PARTS:
            zero = lax.fori_loop(0, NP - 1, pair_step, zero)
        gap("4", zero)
        if "last" in _PARTS:
            for cp in cp_step(NP - 1) + cp_a() if 'bloop' in _PARTS else []:
                cp.wait()
            if _WS:
                cp_wo(NP - 1, 0)[0].start()
            side = sum((prep_awo(n // 2, n % 2, zero) for n in range(_AE)), [])
            lists = [prep_wo(NP - 1 - _WS, (NP - 1) % 2, zero), side] + ([prep_xa(zero, zero)] if "x" in _EW else [])
            side = _blend(*[x for x in lists if x])
            pair_attention(NP - 1, zero, lambda c: [[]] * 8, side, _DEPTH, _QE)
        else:
            ctx[0, :8, :128] = (q_s[zero, :8, :128] + k_s[zero, :8, :128] + v_s[zero, :8, :128]
                                + bwop[pl.ds(zero, 8), :] + qwop[zero, :8, :] + xop[zero, :8, :128] + cop[zero, 0, :8, :])
        return zero

    def rows(zero, dummy2, aoop, aqkv, oop, out_s):
        dummy2[:8] = jnp.zeros((8, 128), F32)
        dummy[:8] = dummy2[pl.ds(1, 8)]

        @pl.loop(0, 2)
        def _(i):
            aqkv[pl.ds(8 + 8 * i, 8), :HALO, :] = jnp.zeros((8, HALO, 128), F32)

        def cp_out(c, half):
            cols = pl.ds(half * DM, DM)
            return pltpu.make_async_copy(
                out_s.at[half, c], out_hbm.at[pl.ds(pl.multiple_of(c * CH, CH), CH), cols],
                sem_out.at[half * NC + c])

        def prep_ctx(c, zero):
            base = pl.multiple_of(c * (CH // 2), CH // 2)

            def piece(m, r, i):
                outer = {b: [_split(ctx[0, pl.ds(base + ((2 * m + a2) * (S // 2) + (b // 2) * 64 + r2 * 32 + r), 8),
                                        pl.ds((b % 2) * HD, HD)])
                             for r2 in range(2) for a2 in range(2)] for b, _ in LHS[i]}
                ops = [_join(v) for v in _operands(_combine(outer, LHS[i]), LHS)]
                for k, v in enumerate(ops):
                    oop[NOPS * i + k, pl.ds(r, 8), pl.ds(HD * m, HD)] = v
                return ops
            def pace(v):
                ctx[zero, pl.ds(NP * S // 2, 8), :128] = v
            return [(pace, lambda m=m, r=r, i=i: piece(m, r, i))
                    for m in range(NP // 2) for r in range(0, 32, 8) for i in range(NOPS)]

        def o_proj(c):
            steps = []
            for t in range(2):
                def done(o, val, t=t):
                    r0 = (o[0] // 2) * R + (o[1] // 2) * (R // 2)
                    n0 = 512 * t + (o[0] % 2) * 256 + (o[1] % 2) * 128
                    out_s[1, c, pl.ds(r0, R // 2), pl.ds(n0, 128)] = val.astype(BF16)
                steps.append(_block_product(lambda i: _bf16(oop[i]),
                                            lambda i, t=t: _bf16(woop[t, i]), done, levels=2))
            return _weave(steps, "o" in _W) + ([lambda: cp_out(c, 1).start(priority=_PRIO)] if 'D' not in _X else [])

        def a_proj(row0):
            steps = []
            for part in range(3):
                both = []
                for t in range(2):
                    def done(o, val, part=part, t=t):
                        if part == 0:
                            val = val * (AD ** -0.5 * LOG2E)
                        r0 = (o[0] // 2) * R + (o[1] // 2) * (R // 2)
                        aqkv[8 * part + 4 * (o[0] % 2) + 2 * (o[1] % 2) + t,
                             pl.ds(row0 + (HALO + r0), R // 2), :] = val

                    def rhs(i, part=part, t=t):
                        return _bf16(jnp.concatenate(
                            [awop[2 * part + m, i, pl.ds(64 * t, 64), :] for m in range(2)], axis=1))
                    both.append(_block_product(lambda i: _bf16(xaop[i]), rhs, done, NT, 2))
                steps += _weave(both, "p" in _W)
            return _group(steps, _AG)

        def a_attention(c, row0, zero, n):
            logit, prob, mixed = {}, {}, {}

            def dot(r, w):
                tot = None
                for t in range(8):
                    if (r, t) not in logit:
                        logit[r, t] = aqkv[t, pl.ds(row0 + (HALO + r), 8), :]
                    pr = logit[r, t] * aqkv[8 + t, pl.ds(row0 + (HALO + r - DIL * w if not _AL else r + 8 * w), 8), :]
                    tot = pr if tot is None else tot + pr
                logit[r, "w", w] = tot
                if w == WIN - 1:
                    weights(r)
                return [tot]

            def weights(r):
                logits = [logit[r, "w", w] for w in range(WIN)]
                logits = [x + pltpu.roll(x, 64, 1) for x in logits]
                logits = [x + pltpu.roll(x, 32, 1) for x in logits]
                if r < (WIN - 1) * DIL:
                    pos = c * CH + r + lax.broadcasted_iota(jnp.int32, (8, 128), 0)
                    logits = [x if w == 0 else jnp.where(pos >= DIL * w, x, MASKED)
                              for w, x in enumerate(logits)]
                top = logits[0]
                for x in logits[1:]:
                    top = jnp.maximum(top, x)
                e = [jnp.exp2(x - top) for x in logits]
                tot = e[0]
                for x in e[1:]:
                    tot = tot + x
                inv = _recip(tot)
                prob[r] = [x * inv for x in e]

            def mix(r, t, d, q):
                tot = None
                for w in range(WIN):
                    pr = prob[r + d][w] * aqkv[16 + t + 2 * q,
                                               pl.ds(row0 + (HALO + r + d - DIL * w if not _AL else r + d + 8 * w), 8), :]
                    tot = pr if tot is None else tot + pr
                mixed[r, t, d, q] = tot
                return [tot]

            def operands(r, t, i):
                outer = {b: [jnp.concatenate(
                    [mixed[r, t, (b // 2) * R + r2 * R // 2 + e, 2 * (b % 2) + a2] for e in (0, 8)],
                    axis=0) for r2 in range(2) for a2 in range(2)] for b, _ in LHS[i]}
                ops = _operands(_combine(outer, LHS[i]), LHS)
                for k, v in enumerate(ops):
                    _store(aoop, NOPS * i + k, r // 2, 128 * t, v)
                return ops

            groups = [d + e for d in range(0, CH, R // 2) for e in (0, 8)]

            def dots(r):
                return [lambda d=d, w=w: dot(r + d, w) for d in groups for w in range(WIN)]

            def mixes(r):
                return [work for t in range(2) for work in
                        [lambda t=t, d=d, q=q: mix(r, t, d, q) for d in groups for q in range(4)]
                        + [lambda t=t, i=i: operands(r, t, i) for i in range(NOPS)]]

            work = dots(0)
            for r in range(16, R // 2, 16):
                work += _blend(dots(r), mixes(r - 16))
            work += mixes(R // 2 - 16)
            return [(_pacer(aqkv, 24 + zero), lambda g=work[i:i + n]: sum((w() for w in g), []))
                    for i in range(0, len(work), n)]

        def a_out_proj(c, zero):
            steps = []
            for n in range(2):
                def done(o, val, n=n):
                    r0 = (o[0] // 2) * R + (o[1] // 2) * (R // 2)
                    n0 = (o[0] % 2) * 512 + (o[1] % 2) * 256 + 128 * n
                    out_s[0, c, pl.ds(r0, R // 2), pl.ds(n0, 128)] = val.astype(BF16)
                steps.append(_block_product(lambda i: _bf16(aoop[zero + i]),
                                            lambda i, n=n: _bf16(awoop[n, i]), done, levels=2))
            return _group(_weave(steps, "a" in _W), _AG) + ([lambda: cp_out(c, 0).start()] if 'D' not in _X else [])

        if "s0" in _PARTS:
            if "x" not in _EW:
                _now(prep_xa(zero, zero))
            lists = [prep_ctx(0, zero), sum((prep_awo(n // 2, n % 2, zero) for n in range(_AE, 4)), [])]
            if _WS:
                cp_wo(NP - 1, 0)[0].wait()
                lists.append(prep_wo(NP - 1, 0, zero))
            _run(_mingle(a_proj(0), _blend(*[x for x in lists if x])))

        def chunk_step(c, zero):
            row0 = pl.multiple_of((c - 1) * CH, CH)
            first, second = o_proj(c - 1), a_proj(row0 + CH)
            att = a_attention(c - 1, row0, zero, _NA) if 'A' not in _X else []
            cut = len(att) * _CU // 16
            xap, ctxp = prep_xa(c, zero), prep_ctx(c, zero) if 'C' not in _X else []
            third = a_out_proj(c - 1, zero)
            late = len(ctxp) * _CT // 16
            _run((_mingle(first[:-1], _blend(att[:cut], xap)) if '1' not in _X else []) + first[-1:])
            if '2' not in _X:
                _run(_mingle(second[:-_AT], _blend(att[cut:], ctxp[:-late])) + second[-_AT:])
            _run((_mingle(third[:-_AT], ctxp[-late:]) + third[-_AT:-1] if '3' not in _X else []) + third[-1:])
            return zero + c // NC

        pad(_PA, zero)
        if "aloop" in _PARTS:
            zero = lax.fori_loop(1, NC, chunk_step, zero)

        if "epi" in _PARTS:
            steps = o_proj(NC - 1)
            _run(_mingle(steps[:-_ET], a_attention(NC - 1, (NC - 1) * CH, zero, _EN)) + steps[-_ET:])
            _run(a_out_proj(NC - 1, zero))
            for c in range(NC if 'D' in _X else 0):
                cp_out(c, 1).start()
                cp_out(c, 0).start()
            for c in range(NC):
                cp_out(c, 1).wait()
                cp_out(c, 0).wait()
        else:
            out_s[0, 0, :16, :128] = aqkv[3, :16, :].astype(BF16)
            out_s[0, 0, 16:32, :128] = _bf16(awop[0, 0, :8, :] + ctx[0, :8, :128] + woop[0, 0, :8, :]
                                             + oop[0, :8, :128] + awoop[0, 0, :8, :])
            cp_out(0, 0).start()
            cp_out(0, 0).wait()

    vmem = pltpu.VMEM
    zero = pl.run_scoped(
        heads,
        vmem((NQ * NC + 1, R // 4, DM // 4), U32),
        vmem((NC, NOPS * NOPS, R // 4, 128), U32),
        vmem((3, DM, HD), U32),
        vmem((5, DC, HD), U32),
        vmem((NQ, DM // 8, 128), U32),
        vmem(((RING + 1) * SLOT, 128), U32),
        vmem((1, S // 2 + _QP, 2 * HD), U32),
        vmem((1, S // 2, 2 * HD), U32),
        vmem((1, S // 2, 2 * HD), U32),
        vmem((2, 512, 512), BF16),
        vmem((2, NP + 2, 8, 128), F32),
    )
    pl.run_scoped(
        lambda *refs: rows(zero, *refs),
        vmem((_D2, 128), F32),
        vmem((NOPS * NOPS, R // 4, DM // 4), U32),
        vmem((25, HALO + S + _AP + 64 * _AL, 128), F32),
        vmem((NOPS * NOPS, R // 4, NP * HD // 2), U32),
        vmem((2, NC, CH, DM), BF16),
    )


@jax.jit
def pallas_concat_heads__sliding_local_dilated__compressed_kv_cla__prompt_kernel(
    A_x: jax.Array,
    A_wqkv: jax.Array,
    A_wo: jax.Array,
    B_x: jax.Array,
    B_c_kv: jax.Array,
    B_w_q: jax.Array,
    B_w_uk: jax.Array,
    B_w_uv: jax.Array,
    B_w_o: jax.Array,
):
    vmem = pltpu.VMEM
    dma = pltpu.SemaphoreType.DMA
    scratch = [
        vmem((_DUM, 128), F32),
        vmem((1, NP * S // 2 + 16, 2 * HD), U32),
        vmem((3, 2 * HD, 512), U32),
        vmem((2, NOPS * NOPS, NP * HD // 4, 128), U32),
        vmem((N_UNITS // 2, NOPS * NOPS, DM // 8, 128), U32),
        vmem((2, NOPS * NOPS, DM // 8, 128), U32),
        vmem((NC + 1, CH, DM), BF16),
        vmem((NOPS * NOPS, R // 4, DM // 4), U32),
        vmem((9, CH, DC), BF16),
        vmem((5, 16 * PITCH + 16, 128), F32),
        dma((NC,)), dma((NC,)), dma((8,)), dma((4,)), dma((2,)), dma((2 * NC,)),
    ]
    out = pl.pallas_call(
        _kernel,
        out_shape=jax.ShapeDtypeStruct((S, 2 * DM), BF16),
        in_specs=[pl.BlockSpec(memory_space=pl.ANY)] * 9,
        out_specs=pl.BlockSpec(memory_space=pl.ANY),
        scratch_shapes=scratch,
        compiler_params=pltpu.CompilerParams(vmem_limit_bytes=124 * 2**20),
        name="fused_local_and_latent_attention",
    )(
        A_x.reshape(S, DM), A_wqkv, A_wo,
        B_x.reshape(S, DM), B_c_kv.reshape(S, DC),
        B_w_q, B_w_uk, B_w_uv, B_w_o.reshape(NH * HD, DM),
    )
    return out.reshape(1, S, 2 * DM)
```

```python
import math

import jax
import jax.numpy as jnp
from jax import lax
import jax.experimental.pallas as pl
import jax.experimental.pallas.tpu as pltpu

F32, BF16, U32 = jnp.float32, jnp.bfloat16, jnp.uint32

S = 2048
DM = 1024
DC = 512
NH = 32
HD = 128
AD = 32
WIN, DIL = 8, 2

R = 128
CH = 2 * R
NC = S // CH
NP = NH // 2
HALO = 16
PITCH = 33
TILE = 512
LOG2E = math.log2(math.e)
MASKED = -1e9 * LOG2E

NN = (((1,), (0,)), ((), ()))
NT = (((1,), (1,)), ((), ()))

LHS = (((0, 1), (3, 1)), ((2, 1), (3, 1)), ((0, 1),), ((3, 1),),
       ((0, 1), (1, 1)), ((2, 1), (0, -1)), ((1, 1), (3, -1)))
RHS = (((0, 1), (3, 1)), ((0, 1),), ((1, 1), (3, -1)), ((2, 1), (0, -1)),
       ((3, 1),), ((0, 1), (1, 1)), ((2, 1), (3, 1)))
PRODUCTS = ((2, ((1, 1), (3, 1))), (4, ((0, -1), (1, 1))), (3, ((0, 1), (2, 1))),
            (1, ((2, 1), (3, -1))), (5, ((3, 1),)), (0, ((0, 1), (3, 1))),
            (6, ((0, 1),)))
NOPS = len(PRODUCTS)

SLOPE = (-1.5, -0.5, 0.5, 1.5)
COUPLES = tuple((i, j) for j in range(4) for i in range(j, -1, -1))
NQ = sum(2 if i == j else 3 for i, j in COUPLES)

KVROWS = 64
SLOT = NOPS * NOPS * KVROWS
RING = 8


def _square_forms(x, i, j):
    if i == j:
        p = q = x(i, i)
        for k in range(4):
            if k != i:
                p, q = p - x(k, i), q + x(i, k)
        return [p, q]
    return [x(i, j) + x(j, i), x(i, j), x(j, i)]


def _pair_forms(w, i, j):
    (a0, a1), (b0, b1) = w(i), w(j)
    if i == j:
        return [a0, SLOPE[i] * a0 + a1]
    return [(SLOPE[i] * a0 + a1) - (SLOPE[j] * b0 + b1),
            SLOPE[i] * (b0 - a0) + (b1 - a1), SLOPE[j] * (b0 - a0) + (b1 - a1)]


def _couple_product(lhs, rhs, done):
    first, second, steps = {}, {}, []

    def add(i, j, m):
        if i == j:
            first[i], second[i] = m
            return
        t, gap = m[0] + m[1] + m[2], SLOPE[j] - SLOPE[i]
        t = t if gap == 1 else t * (1 / gap)
        first[i], first[j] = first[i] - t, first[j] - t
        second[i], second[j] = second[i] + m[1], second[j] - m[2]
        if j == 3:
            for r in (i,) if i else (0, 3):
                done(r, first[r], second[r] - SLOPE[r] * first[r])

    for i, j in COUPLES:
        got, n = [], 2 if i == j else 3
        for _ in range(n):
            def step(i=i, j=j, got=got, n=n, k=len(steps)):
                got.append(lax.dot_general(lhs(k), rhs(k), NN, preferred_element_type=F32))
                if len(got) == n:
                    add(i, j, got)
                return got[-1]
            steps.append(step)
    return steps


def _combine(blocks, terms):
    if isinstance(blocks[terms[0][0]], list):
        return [_combine({b: blocks[b][i] for b, _ in terms}, terms) for i in range(4)]
    out = blocks[terms[0][0]]
    for i, sign in terms[1:]:
        out = out + blocks[i] if sign > 0 else out - blocks[i]
    return out


def _operands(blocks, side):
    return [_combine(blocks, terms) for terms in side]


def _block_product(lhs, rhs, done, dims=NN, levels=2):
    if levels == 0:
        def step():
            m = lax.dot_general(lhs(0), rhs(0), dims, preferred_element_type=F32)
            done((), m)
            return m
        return [step]

    held, steps = {}, []
    inner = NOPS ** (levels - 1)
    for n, (i, outs) in enumerate(PRODUCTS):
        later = {o for _, others in PRODUCTS[n + 1:] for o, _ in others}

        def add(sub, m, outs=outs, later=later):
            for o, sign in outs:
                if (o, sub) not in held:
                    held[o, sub] = m, sign
                else:
                    c, s = held[o, sub]
                    held[o, sub] = (m - c if s < 0 else c + m if sign > 0 else c - m), 1
                if o not in later:
                    done((o, *sub), held.pop((o, sub))[0])

        steps += _block_product(lambda k, i=i: lhs(i * inner + k),
                                lambda k, i=i: rhs(i * inner + k), add, dims, levels - 1)
    return steps


def _corner(o, rows, cols):
    return (2 * (o[0] // 2) + o[1] // 2) * rows, (2 * (o[0] % 2) + o[1] % 2) * cols


def _bf16(words):
    return pltpu.bitcast(words, BF16)


def _halves(words):
    lo = pltpu.bitcast(words << 16, F32)
    hi = pltpu.bitcast(words & jnp.uint32(0xFFFF0000), F32)
    return lo, hi


def _split(words):
    return jnp.concatenate(_halves(words), axis=0)


def _join(x):
    n = x.shape[0] // 2
    return pltpu.pack_elementwise([x[:n], x[n:]], packed_dtype=BF16)


def _store(words, index, row, col, x):
    matrix = words.bitcast(BF16).at[index]
    matrix[pl.ds(pl.multiple_of(2 * row, 16), x.shape[0]), pl.ds(col, x.shape[1])] = x.astype(BF16)


def _recip(x):
    r = pltpu.reciprocal(x, approx=True)
    return r * (2.0 - x * r)


def _run(steps):
    out = None
    for step in steps:
        out = step()
    return out


def _group(steps, n):
    return [lambda g=steps[i:i + n]: _run(g) for i in range(0, len(steps), n)]


def _share(items, k, n):
    return items[k * len(items) // n:(k + 1) * len(items) // n]


def _blend(*lists):
    spots = [((i + 0.5) / len(items), k, item)
             for k, items in enumerate(lists) for i, item in enumerate(items)]
    return [item for *_, item in sorted(spots, key=lambda spot: spot[:2])]


def _witness(values):
    out = None
    for v in values:
        v = pltpu.bitcast(v, U32)
        for r in range(0, v.shape[0], 8):
            for c in range(0, v.shape[1], 128):
                out = v[r:r + 8, c:c + 128] if out is None else out | v[r:r + 8, c:c + 128]
    return out


def _pacer(ref, index, row=0):
    def pace(v):
        if ref.dtype == BF16:
            ref[index, pl.ds(row, 16), pl.ds(0, 128)] = _bf16(v)
        else:
            ref[index, pl.ds(row, 8), pl.ds(0, 128)] = pltpu.bitcast(v, ref.dtype)
    return pace


def _tie(pieces, result):
    for i, (pace, work, *lag) in enumerate(pieces):
        seen, m = work(), result(sum(lag))
        r = 8 * (i * (m.shape[0] // 8) // len(pieces))
        pace(_witness([m[r:r + 8]] + list(seen)))


def _mingle(steps, pieces, history=None):
    history = [] if history is None else history

    def both(step, mine):
        history.append(step())
        _tie([piece for piece in mine if piece],
             lambda lag: history[max(0, len(history) - 1 - lag)][:, :128])

    return [lambda step=step, mine=_share(pieces, i, len(steps)): both(step, mine)
            for i, step in enumerate(steps)]


def _now(pieces):
    for _, work, *_ in pieces:
        work()


def _dim_major(src, pace, shuf, put, swap, zero, lag=0, gap=0):
    def start(head):
        return ((head % 2) * 8 + head // 2) * PITCH

    def scatter(k, u):
        t = src(k, u)
        for h in range(128 // AD):
            shuf[k, pl.ds(start(4 * u + h), AD), :] = t[h * AD:(h + 1) * AD]
        return [t]

    def gather(d, i):
        def block(row1, col1, row2, col2):
            quarter, k = 2 * row1 + row2, 2 * col1 + col2
            if swap:
                quarter, k = k, quarter
            return jnp.concatenate(
                [shuf[k, pl.ds(start(p) + quarter * AD // 4 + d, 8, stride=PITCH), :]
                 for p in range(2)], axis=0)
        outer = {b: [block(b // 2, b % 2, s // 2, s % 2) for s in range(4)] for b, _ in RHS[i]}
        ops = [_join(v) for v in _operands(_combine(outer, RHS[i]), RHS)]
        for n, v in enumerate(ops):
            put(NOPS * i + n, d * NH // 2, v)
        return ops

    return ([x for k in range(4) for u in range(4)
             for x in [(pace, lambda k=k, u=u: scatter(k, u), lag)] + [None] * gap]
            + [(_pacer(shuf, 4 + zero), lambda d=d, i=i: gather(d, i))
               for d in range(AD // 4) for i in range(NOPS)])


def _kernel(ax_hbm, awqkv_hbm, awo_hbm, bx_hbm, c_hbm, wq_hbm, wuk_hbm, wuv_hbm,
            wo_hbm, out_hbm,
            offset, ctx, wo_raw, woop, awop, awoop, xa, xaop, awo_raw, shuf,
            sem_x, sem_c, sem_w, sem_a, sem_out):

    def cp_tile(src, row, col, dst, sem):
        def span(i):
            return pl.ds(pl.multiple_of(i * TILE, TILE), TILE)
        return pltpu.make_async_copy(src.at[span(row), span(col)], dst, sem)

    def cp_wo(u, s):
        return cp_tile(wo_hbm, u // 2, u % 2, wo_raw.at[s].bitcast(BF16), sem_w.at[6 + s])

    def cp_a():
        return ([pltpu.make_async_copy(ax_hbm.at[pl.ds(c * CH, CH)], xa.at[c], sem_a.at[0])
                 for c in range(NC)]
                + [pltpu.make_async_copy(awo_hbm.at[pl.ds(128 * t, 128), pl.ds(DC * h, DC)],
                                         awo_raw.at[t, pl.ds(128 * h, 128)], sem_a.at[1])
                   for t in range(8) for h in range(2)])

    def prep_wo(u, s, zero):
        def piece(r, i):
            outer = {b: [_split(wo_raw[s, pl.ds((2 * a2 + b // 2) * (HD // 2) + r, 8),
                                       pl.ds((2 * (b % 2) + b2) * 128, 128)])
                         for a2 in range(2) for b2 in range(2)] for b, _ in RHS[i]}
            ops = [_join(v) for v in _operands(_combine(outer, RHS[i]), RHS)]
            row = pl.multiple_of((u // 2) * (HD // 2) + r, 8)
            for k, v in enumerate(ops):
                woop[u % 2, NOPS * i + k, pl.ds(row, 8), :] = v
            return ops
        return [(_pacer(wo_raw, 2 + zero), lambda r=r, i=i: piece(r, i))
                for r in range(0, HD // 2, 8) for i in range(NOPS)]

    def prep_awo(u, zero):
        n, half = u // 2, u % 2

        def put(i, row, v):
            awoop[n, i, pl.ds(8 * half + row, 8), :] = v
        return _dim_major(
            lambda k, t: awo_raw[4 * half + t, pl.ds(128 * n, 128), pl.ds(128 * k, 128)].astype(F32),
            _pacer(awo_raw, 8 + zero), shuf, put, False, zero)

    def prep_xa(c, zero):
        def piece(t, r, i):
            outer = {b: [_split(pltpu.bitcast(
                xa[c, pl.ds((b // 2) * R + r2 * R // 2 + r, 16),
                   pl.ds(512 * t + (b % 2) * 256 + a2 * 128, 128)], U32))
                for r2 in range(2) for a2 in range(2)] for b, _ in LHS[i]}
            ops = [_join(v) for v in _operands(_combine(outer, LHS[i]), LHS)]
            for k, v in enumerate(ops):
                xaop[NOPS * i + k, pl.ds(r // 2, 8), pl.ds(128 * t, 128)] = v
            return ops
        return [(_pacer(xa, NC + zero), lambda t=t, r=r, i=i: piece(t, r, i))
                for t in range(2) for r in range(0, R // 2, 16) for i in range(NOPS)]

    offset[:16] = jnp.zeros((16, 128), F32)
    shuf[0, :8] = offset[pl.ds(1, 8)]

    def heads(xop, cop, wq_raw, wkv_raw, qwop, kvwop, q_s, k_s, v_s, aw_raw, unit):
        xs, cs = xa, awo_raw
        wq32 = wq_hbm.bitcast(U32)
        wuk32 = wuk_hbm.bitcast(U32)
        wuv32 = wuv_hbm.bitcast(U32)

        def cp_x(c):
            return pltpu.make_async_copy(bx_hbm.at[pl.ds(c * CH, CH)], xs.at[c], sem_x.at[c])

        def cp_c(c):
            return pltpu.make_async_copy(c_hbm.at[pl.ds(c * CH, CH)], cs.at[c], sem_c.at[c])

        def cp_wkv(j, s):
            return [pltpu.make_async_copy(wuk32.at[:, j, :], wkv_raw.at[s], sem_w.at[s]),
                    pltpu.make_async_copy(wuv32.at[:, j, :], wkv_raw.at[2 + s], sem_w.at[2 + s])]

        def cp_wq(j, s):
            return [pltpu.make_async_copy(wq32.at[:, j, :], wq_raw.at[s], sem_w.at[4 + s])]

        def wo_unit(j):
            return jnp.maximum(j - 1, 0)

        def aw_unit(j):
            return jnp.clip(j - 1, 0, 3 * DM * DM // TILE ** 2 - 1)

        def cp_heads(j):
            return (cp_wkv(jnp.minimum(j + 2, NP - 1), j % 2)
                    + cp_wq(jnp.minimum(j + 1, NP - 1), j % 2))

        def cp_tiles(j):
            u = aw_unit(j)
            return [cp_wo(wo_unit(j), j % 2),
                    cp_tile(awqkv_hbm, u // 2 % 2, 2 * (u // 4) + u % 2, aw_raw.at[j % 2],
                            sem_w.at[8 + j % 2])]

        def prep_x(c):
            for t in range(2):
                blocks = [[_split(pltpu.bitcast(
                    xs[c, pl.ds(r * R // 2, R // 2), pl.ds(k * DM // 4 + 128 * t, 128)], U32))
                    for k in range(4)] for r in range(4)]
                ops = [v for i, j in COUPLES
                       for v in _square_forms(lambda r, k: blocks[r][k], i, j)]
                for n, v in enumerate(ops):
                    xop[NQ * c + n, :, pl.ds(128 * t, 128)] = _join(v)

        def prep_c(c):
            blocks = [[_split(pltpu.bitcast(
                cs[c, pl.ds(r1 * R + r2 * R // 2, R // 2), pl.ds(a1 * 256 + a2 * 128, 128)], U32))
                for r2 in range(2) for a2 in range(2)] for r1 in range(2) for a1 in range(2)]
            for i, outer in enumerate(_operands(blocks, LHS)):
                for k, v in enumerate(_operands(outer, LHS)):
                    cop[c, NOPS * i + k] = _join(v)

        def both_heads(raw, s, row):
            even, odd = (_halves(raw[s, pl.ds(row + p, 8, stride=2), :]) for p in range(2))
            return [jnp.concatenate([even[h], odd[h]], axis=0) for h in range(2)]

        def prep_wq(s, zero):
            def piece(r, couples, n):
                w = {k: both_heads(wq_raw, s, k * DM // 4 + r) for couple in couples for k in couple}
                ops = [_join(v) for i, j in couples for v in _pair_forms(w.get, i, j)]
                for k, v in enumerate(ops):
                    qwop[n + k, pl.ds(r // 2, 8), :] = v
                return ops
            parts = (COUPLES[:6], 0), (COUPLES[6:], 15)
            return [(_pacer(wq_raw, 2 + zero), lambda r=r, part=part: piece(r, *part))
                    for r in range(0, DM // 4, 16) for part in parts]

        def prep_wkv(j, s, slot, zero):
            total, inverse = {}, {}

            def measure(n, r):
                w = wkv_raw[2 * n + s, pl.ds(r, 64), :]
                w = jnp.abs(pltpu.bitcast(w, F32)) + jnp.abs(pltpu.bitcast(w << 16, F32))
                w = jnp.sum(w.reshape(8, 8, 128), axis=0)
                total[n] = total[n] + w if r else w
                return [total[n]]

            def size(n):
                both = jnp.sum(jnp.sum(total[n], axis=1, keepdims=True), axis=0, keepdims=True)
                both = jnp.broadcast_to(jnp.clip(both, 2.0 ** -100, 2.0 ** 100), (8, 128))
                power = pltpu.bitcast(both, U32) & jnp.uint32(0x7F800000)
                unit[n, j] = pltpu.bitcast(power, F32)
                inverse[n] = pltpu.bitcast(jnp.uint32(0x7F000000) - power, F32)
                return [power]

            def piece(r, i):
                outer = {b: [v * jnp.concatenate([inverse[b % 2]] * 2, axis=0) for a2 in range(2)
                             for v in both_heads(wkv_raw, 2 * (b % 2) + s,
                                                 (b // 2) * 256 + a2 * 128 + r)]
                         for b, _ in RHS[i]}
                ops = [_join(v) for v in _operands(_combine(outer, RHS[i]), RHS)]
                for k, v in enumerate(ops):
                    kvwop[pl.ds(slot + ((NOPS * i + k) * KVROWS + r // 2), 8), :] = v
                return ops

            pace = _pacer(wkv_raw, 4 + zero)
            return ([(pace, lambda n=n, r=r: measure(n, r))
                     for n in range(2) for r in range(0, DC, 64)]
                    + [(pace, lambda n=n: size(n)) for n in range(2)],
                    [(_pacer(xop, NQ * NC + zero), lambda: list(inverse.values()))]
                    + [(pace, lambda r=r, i=i: piece(r, i))
                       for r in range(0, 128, 16) for i in range(NOPS)])

        def prep_aw(u, s, zero):
            def put(i, row, v):
                awop[u // 2, i, pl.ds(pl.multiple_of(8 * (u % 2), 8) + row, 8), :] = v
            return _dim_major(
                lambda k, t: aw_raw[s, pl.ds(128 * k, 128), pl.ds(128 * t, 128)].astype(F32).T,
                _pacer(xop, NQ * NC + zero), shuf, put, True, zero, lag=5, gap=2)

        def q_proj(scale, c):
            def done(r, *both):
                for h, val in enumerate(both):
                    _store(q_s, 0, c * R + r * (R // 4), h * HD, val * scale)
            return _couple_product(lambda i: _bf16(xop[NQ * c + i]), lambda i: _bf16(qwop[i]), done)

        def kv_proj(c, slot):
            def done(o, val):
                row, col = _corner(o, R // 4, HD)
                _store((k_s, v_s)[col // (2 * HD)], 0, c * R + row, col % (2 * HD), val)
            return _block_product(
                lambda i: _bf16(cop[c, i]),
                lambda i: _bf16(kvwop[pl.ds(slot + i * KVROWS, KVROWS), :]), done)

        def q_scale(j):
            return unit[0, j, :1] * (HD ** -0.5 * LOG2E)

        def scores(h, blk):
            n = (blk + 1) * R
            s = lax.dot_general(_bf16(q_s[0, pl.ds(blk * R // 2, R // 2), pl.ds(h * HD, HD)]),
                                _bf16(k_s[0, :n // 2, pl.ds(h * HD, HD)]),
                                NT, preferred_element_type=F32)
            row = lax.broadcasted_iota(jnp.int32, (R, R), 0)
            col = lax.broadcasted_iota(jnp.int32, (R, R), 1)
            diag = jnp.where(col <= row, s[:, n - R:], MASKED)
            return diag if blk == 0 else jnp.concatenate([s[:, :n - R], diag], axis=1)

        def attend(scale, h, blk, s):
            n = (blk + 1) * R
            p = jnp.exp2(s - jnp.max(s, axis=1, keepdims=True))
            inv = _recip(jnp.sum(p, axis=1, keepdims=True)) * scale
            o = lax.dot_general(p.astype(BF16), _bf16(v_s[0, :n // 2, pl.ds(h * HD, HD)]), NN,
                                preferred_element_type=F32)
            return o * inv

        def pair_attention(j, zero, filler, sides, slack):
            blocks = [(h, 2 * c + u) for c in reversed(range(NC)) for u in (1, 0) for h in (0, 1)]
            plan = {}
            for pieces, span in sides:
                tiles = [(b, t) for b in blocks[span] for t in range(b[1] + 1)]
                for n, tile in enumerate(tiles):
                    plan.setdefault(tile, []).extend(_share(pieces, n, len(tiles)))

            def paced_scores(h, blk):
                s = scores(h, blk)
                for t in range(blk + 1):
                    _tie(plan.get(((h, blk), t), []), lambda lag: s[:, t * R:(t + 1) * R])
                return s

            todo, done = [[]] * 8, []
            v_scale = unit[1, j, :1]
            ahead = [paced_scores(*blocks[0])]
            for n, (h, blk) in enumerate(blocks):
                ahead += [paced_scores(*b) for b in blocks[n + 1:n + 2]]
                _run(todo[2 * (n % 4)])
                done.append(attend(v_scale, h, blk, ahead.pop(0)))
                _store(ctx, 0, pl.multiple_of(j * (S // 2), S // 2) + blk * (R // 2), h * HD, done[-1])
                if len(done) > slack:
                    _pacer(q_s, zero, S // 2)(_witness([done.pop(0)]))
                _run(todo[2 * (n % 4) + 1])
                if n % 4 == 3:
                    todo = filler(blk // 2)
            _run(sum(todo, []))

        c_parts = ((7, 6), (5, 4), (3, 2), (1, 0))
        x_parts = tuple(reversed(range(NC)))
        stages = ([cp_wkv(0, 0)] + [[cp_c(c) for c in part] for part in c_parts]
                  + [[cp_x(c)] for c in x_parts] + [cp_wq(1, 0)])
        stages[len(c_parts)] += cp_wq(0, 1)
        stages[len(c_parts) + 1] += cp_wkv(1, 1)

        def issue(i, zero):
            for k, stage in enumerate(stages):
                @pl.when(i == k)
                def _(stage=stage):
                    for cp in stage:
                        cp.start()
            return zero + i // NP

        zero = lax.fori_loop(0, len(stages), issue, jnp.int32(0))

        aw_raw[0] = jnp.zeros(aw_raw.shape[1:], BF16)
        wo_raw[0] = jnp.zeros(wo_raw.shape[1:], U32)
        for cp in stages[0]:
            cp.wait()
        _now(sum(prep_wkv(0, 0, SLOT, zero), []))
        for n, part in enumerate(c_parts):
            for cp in stages[1 + n]:
                cp.wait()
            if n == 0:
                for cp in cp_wkv(2, 0):
                    cp.start()
            side = prep_wq(1, zero) if n == len(c_parts) - 1 else []
            for k, c in enumerate(part):
                prep_c(c)
                _run(_mingle(kv_proj(c, SLOT), _share(side, k, len(part))))
        scale, side = q_scale(0), sum(prep_wkv(1, 1, 0, zero), [])
        for n, c in enumerate(x_parts):
            for cp in stages[1 + len(c_parts) + n]:
                cp.wait()
            prep_x(c)
            _run(_mingle(q_proj(scale, c), _share(side, n, NC)))

        def pair_step(j, zero):
            for cp in cp_heads(j):
                cp.wait()

            @pl.when(j > 0)
            def _():
                for cp in cp_tiles(j):
                    cp.wait()

            @pl.when(j == RING)
            def _():
                kvwop[:SLOT] = kvwop[RING * SLOT:]
                for cp in cp_a():
                    cp.start()

            for cp in cp_heads(j + 1) + cp_tiles(j + 1):
                cp.start()
            slot = pl.multiple_of((j % RING) * SLOT, KVROWS)
            scale = q_scale(j + 1)
            sizes, operands = prep_wkv(j + 2, j % 2, slot + SLOT, zero)
            side = [None] * 16 + _blend(prep_aw(aw_unit(j), j % 2, zero),
                                        sizes + [None] * 16 + operands)
            q_steps = sum((q_proj(scale, c) for c in reversed(range(NC))), [])
            history = []

            def filler(c):
                q = _share(q_steps, NC - 3 - c, NC - 2) if c < NC - 2 else []
                kv = kv_proj(c, slot)
                slots = []
                for n in range(4):
                    mine = _share(kv, n, 4)
                    early = len(mine) - len(mine) * 3 // 4
                    slots += [mine[:early] + _share(q, n, 4), mine[early:]]
                steps = iter(_mingle(sum(slots, []), _share(side, NC - 1 - c, NC), history))
                return [[next(steps) for _ in slot] for slot in slots]

            pair_attention(j, zero, filler, [(prep_wo(wo_unit(j), j % 2, zero), slice(6, None)),
                                             (prep_wq(j % 2, zero), slice(2, 12))], 3)
            return zero + j // NP

        zero = lax.fori_loop(0, NP - 1, pair_step, zero)

        @pl.loop(0, 2)
        def _(i):
            _pacer(shuf, 4 + zero * i)(jnp.zeros((8, 128), U32))

        for cp in cp_heads(NP - 1) + cp_tiles(NP - 1) + cp_a():
            cp.wait()
        cp_wo(NP - 1, 0).start()
        side = _blend(prep_wo(NP - 2, 1, zero), prep_awo(0, zero), prep_xa(zero, zero))
        pair_attention(NP - 1, zero, lambda c: [[]] * 8, [(side, slice(2, None))], 4)
        return zero

    def rows(zero, aoop, aqkv, oop, out_s):
        @pl.loop(0, 2)
        def _(i):
            aqkv[pl.ds(8 + 8 * i, 8), :HALO, :] = jnp.zeros((8, HALO, 128), F32)

        def cp_out(c, half):
            return pltpu.make_async_copy(
                out_s.at[half, c],
                out_hbm.at[pl.ds(pl.multiple_of(c * CH, CH), CH), pl.ds(half * DM, DM)],
                sem_out.at[half * NC + c])

        def cp_last(row, col, n, sem):
            return pltpu.make_async_copy(
                out_s.at[0, NC - 1, pl.ds(row, n), pl.ds(col, DM // 2)],
                out_hbm.at[pl.ds((NC - 1) * CH + row, n), pl.ds(col, DM // 2)], sem_x.at[sem])

        def prep_ctx(c, zero):
            base = pl.multiple_of(c * R, R)

            def piece(m, r, i):
                outer = {b: [_split(ctx[0, pl.ds(base + ((2 * m + a2) * (S // 2) + (b // 2) * 64
                                                         + r2 * 32 + r), 8),
                                        pl.ds((b % 2) * HD, HD)])
                             for r2 in range(2) for a2 in range(2)] for b, _ in LHS[i]}
                ops = [_join(v) for v in _operands(_combine(outer, LHS[i]), LHS)]
                for k, v in enumerate(ops):
                    oop[NOPS * i + k, pl.ds(r, 8), pl.ds(HD * m, HD)] = v
                return ops
            return [(_pacer(ctx, zero, NP * S // 2), lambda m=m, r=r, i=i: piece(m, r, i))
                    for m in range(NP // 2) for r in range(0, 32, 8) for i in range(NOPS)]

        def out_proj(half, c, lhs, rhs):
            steps = []
            for t in range(2):
                def done(o, val, t=t):
                    row, col = _corner(o, R // 2, 128)
                    out_s[half, c, pl.ds(row, R // 2), pl.ds(512 * t + col, 128)] = val.astype(BF16)
                steps += _block_product(lhs, lambda i, t=t: _bf16(rhs[t, i]), done)
            return steps

        def b_out_proj(c):
            return out_proj(1, c, lambda i: _bf16(oop[i]), woop)

        def a_out_proj(c, zero):
            return out_proj(0, c, lambda i: _bf16(aoop[zero + i]), awoop)

        def a_proj(row0):
            steps = []
            for part in range(3):
                for t in range(2):
                    def done(o, val, part=part, t=t):
                        if part == 0:
                            val = val * (AD ** -0.5 * LOG2E)
                        row, plane = _corner(o, R // 2, 2)
                        aqkv[8 * part + plane + t, pl.ds(row0 + (HALO + row), R // 2), :] = val

                    def rhs(i, part=part, t=t):
                        return _bf16(jnp.concatenate(
                            [awop[2 * part + m, i, pl.ds(64 * t, 64), :] for m in range(2)], axis=1))
                    steps += _block_product(lambda i: _bf16(xaop[i]), rhs, done, NT)
            return _group(steps, 2)

        def a_attention(c, row0, zero, n):
            query, logit, prob, mixed = {}, {}, {}, {}

            def dot(r, w):
                tot = None
                for t in range(8):
                    if (r, t) not in query:
                        query[r, t] = aqkv[t, pl.ds(row0 + (HALO + r), 8), :]
                    pr = query[r, t] * aqkv[8 + t, pl.ds(row0 + (HALO + r - DIL * w), 8), :]
                    tot = pr if tot is None else tot + pr
                logit[r, w] = tot
                if w == WIN - 1:
                    weights(r)
                return [tot]

            def weights(r):
                logits = [logit[r, w] for w in range(WIN)]
                logits = [x + pltpu.roll(x, 64, 1) for x in logits]
                logits = [x + pltpu.roll(x, 32, 1) for x in logits]
                if r < (WIN - 1) * DIL:
                    pos = c * CH + r + lax.broadcasted_iota(jnp.int32, (8, 128), 0)
                    logits = [x if w == 0 else jnp.where(pos >= DIL * w, x, MASKED)
                              for w, x in enumerate(logits)]
                top = logits[0]
                for x in logits[1:]:
                    top = jnp.maximum(top, x)
                e = [jnp.exp2(x - top) for x in logits]
                tot = e[0]
                for x in e[1:]:
                    tot = tot + x
                inv = _recip(tot)
                prob[r] = [x * inv for x in e]

            def mix(r, t, d, q):
                tot = None
                for w in range(WIN):
                    pr = prob[r + d][w] * aqkv[16 + t + 2 * q,
                                               pl.ds(row0 + (HALO + r + d - DIL * w), 8), :]
                    tot = pr if tot is None else tot + pr
                mixed[r, t, d, q] = tot
                return [tot]

            def operands(r, t, i):
                outer = {b: [jnp.concatenate(
                    [mixed[r, t, (b // 2) * R + r2 * R // 2 + e, 2 * (b % 2) + a2] for e in (0, 8)],
                    axis=0) for r2 in range(2) for a2 in range(2)] for b, _ in LHS[i]}
                ops = _operands(_combine(outer, LHS[i]), LHS)
                for k, v in enumerate(ops):
                    _store(aoop, NOPS * i + k, r // 2, 128 * t, v)
                return ops

            groups = [d + e for d in range(0, CH, R // 2) for e in (0, 8)]

            def dots(r):
                return [lambda d=d, w=w: dot(r + d, w) for d in groups for w in range(WIN)]

            def mixes(r):
                return [work for t in range(2) for work in
                        [lambda t=t, d=d, q=q: mix(r, t, d, q) for d in groups for q in range(4)]
                        + [lambda t=t, i=i: operands(r, t, i) for i in range(NOPS)]]

            work = dots(0)
            for r in range(16, R // 2, 16):
                work += _blend(dots(r), mixes(r - 16))
            work += mixes(R // 2 - 16)
            return [(_pacer(aqkv, zero, HALO + S), lambda g=work[i:i + n]: sum((w() for w in g), []))
                    for i in range(0, len(work), n)]

        cp_wo(NP - 1, 0).wait()
        _run(_mingle(a_proj(0), _blend(prep_ctx(0, zero),
                                       sum((prep_awo(u, zero) for u in range(1, 4)), []),
                                       prep_wo(NP - 1, 0, zero))))

        def chunk_step(c, zero):
            row0 = pl.multiple_of((c - 1) * CH, CH)
            first, second, third = b_out_proj(c - 1), a_proj(row0 + CH), a_out_proj(c - 1, zero)
            att, ctxp = a_attention(c - 1, row0, zero, 1), prep_ctx(c, zero)
            cut, late, tail = len(att) * 5 // 8, len(ctxp) // 4, 6
            _run(_mingle(first, _blend(att[:cut], prep_xa(c, zero))))
            cp_out(c - 1, 1).start()
            _run(_mingle(second[:-tail], _blend(att[cut:], ctxp[:-late])) + second[-tail:])
            third = _group(third, 2)
            _run(_mingle(third[:1 - tail], ctxp[-late:]) + third[1 - tail:])
            cp_out(c - 1, 0).start()
            return zero + c // NC

        zero = lax.fori_loop(1, NC, chunk_step, zero)

        steps = b_out_proj(NC - 1)
        _run(_mingle(steps[:-2], a_attention(NC - 1, (NC - 1) * CH, zero, 2)) + steps[-2:])
        cp_out(NC - 1, 1).start()
        steps = a_out_proj(NC - 1, zero)
        parts = [cp_last(0, 0, CH, 0), cp_last(R, DM // 2, R, 1), cp_last(0, DM // 2, R, 2)]
        for cp, part in zip(parts, (steps[:NOPS * NOPS], steps[NOPS * NOPS:-NOPS], steps[-NOPS:])):
            _run(part)
            cp.start()
        for cp in ([cp_out(c, 1) for c in range(NC)] + [cp_out(c, 0) for c in range(NC - 1)] + parts):
            cp.wait()

    vmem = pltpu.VMEM
    zero = pl.run_scoped(
        heads,
        vmem((NQ * NC + 1, R // 4, DM // 4), U32),
        vmem((NC, NOPS * NOPS, R // 4, 128), U32),
        vmem((3, DM, HD), U32),
        vmem((5, DC, HD), U32),
        vmem((NQ, DM // 8, 128), U32),
        vmem(((RING + 1) * SLOT, 128), U32),
        vmem((1, S // 2 + 16, 2 * HD), U32),
        vmem((1, S // 2, 2 * HD), U32),
        vmem((1, S // 2, 2 * HD), U32),
        vmem((2, TILE, TILE), BF16),
        vmem((2, NP + 2, 8, 128), F32),
    )
    pl.run_scoped(
        lambda *refs: rows(zero, *refs),
        vmem((NOPS * NOPS, R // 4, DM // 4), U32),
        vmem((24, HALO + S + 16, 128), F32),
        vmem((NOPS * NOPS, R // 4, NP * HD // 2), U32),
        vmem((2, NC, CH, DM), BF16),
    )


@jax.jit
def pallas_concat_heads__sliding_local_dilated__compressed_kv_cla__prompt_kernel(
    A_x: jax.Array,
    A_wqkv: jax.Array,
    A_wo: jax.Array,
    B_x: jax.Array,
    B_c_kv: jax.Array,
    B_w_q: jax.Array,
    B_w_uk: jax.Array,
    B_w_uv: jax.Array,
    B_w_o: jax.Array,
):
    vmem = pltpu.VMEM
    dma = pltpu.SemaphoreType.DMA
    scratch = [
        vmem((24, 128), F32),
        vmem((1, NP * S // 2 + 16, 2 * HD), U32),
        vmem((3, TILE // 2, TILE), U32),
        vmem((2, NOPS * NOPS, NP * HD // 4, 128), U32),
        vmem((6, NOPS * NOPS, DM // 8, 128), U32),
        vmem((2, NOPS * NOPS, DM // 8, 128), U32),
        vmem((NC + 1, CH, DM), BF16),
        vmem((NOPS * NOPS, R // 4, DM // 4), U32),
        vmem((NC + 1, CH, DC), BF16),
        vmem((5, 16 * PITCH + 16, 128), F32),
        dma((NC,)), dma((NC,)), dma((10,)), dma((2,)), dma((2 * NC,)),
    ]
    out = pl.pallas_call(
        _kernel,
        out_shape=jax.ShapeDtypeStruct((S, 2 * DM), BF16),
        in_specs=[pl.BlockSpec(memory_space=pl.ANY)] * 9,
        out_specs=pl.BlockSpec(memory_space=pl.ANY),
        scratch_shapes=scratch,
        compiler_params=pltpu.CompilerParams(vmem_limit_bytes=124 * 2**20),
        name="fused_local_and_latent_attention",
    )(
        A_x.reshape(S, DM), A_wqkv, A_wo,
        B_x.reshape(S, DM), B_c_kv.reshape(S, DC),
        B_w_q, B_w_uk, B_w_uv, B_w_o.reshape(NH * HD, DM),
    )
    return out.reshape(1, S, 2 * DM)
```

```python
import math

import jax
import jax.numpy as jnp
from jax import lax
import jax.experimental.pallas as pl
import jax.experimental.pallas.tpu as pltpu

F32, BF16, U32 = jnp.float32, jnp.bfloat16, jnp.uint32

S = 2048
DM = 1024
DC = 512
NH = 32
HD = 128
AD = 32
WIN, DIL = 8, 2

R = 128
CH = 2 * R
NC = S // CH
NP = NH // 2
HALO = 16
PITCH = 33
TILE = 512
LOG2E = math.log2(math.e)
MASKED = -1e9 * LOG2E

NN = (((1,), (0,)), ((), ()))
NT = (((1,), (1,)), ((), ()))

LHS = (((0, 1), (3, 1)), ((2, 1), (3, 1)), ((0, 1),), ((3, 1),),
       ((0, 1), (1, 1)), ((2, 1), (0, -1)), ((1, 1), (3, -1)))
RHS = (((0, 1), (3, 1)), ((0, 1),), ((1, 1), (3, -1)), ((2, 1), (0, -1)),
       ((3, 1),), ((0, 1), (1, 1)), ((2, 1), (3, 1)))
PRODUCTS = ((2, ((1, 1), (3, 1))), (4, ((0, -1), (1, 1))), (3, ((0, 1), (2, 1))),
            (1, ((2, 1), (3, -1))), (5, ((3, 1),)), (0, ((0, 1), (3, 1))),
            (6, ((0, 1),)))
NOPS = len(PRODUCTS)

SLOPE = (-1.5, -0.5, 0.5, 1.5)
COUPLES = tuple((i, j) for j in range(4) for i in range(j, -1, -1))
NQ = sum(2 if i == j else 3 for i, j in COUPLES)

SLOT = NOPS * NOPS
RING = 8


def _square_forms(x, i, j):
    if i == j:
        p = q = x(i, i)
        for k in range(4):
            if k != i:
                p, q = p - x(k, i), q + x(i, k)
        return [p, q]
    return [x(i, j) + x(j, i), x(i, j), x(j, i)]


def _pair_forms(w, i, j):
    (a0, a1), (b0, b1) = w(i), w(j)
    if i == j:
        return [a0, SLOPE[i] * a0 + a1]
    return [(SLOPE[i] * a0 + a1) - (SLOPE[j] * b0 + b1),
            SLOPE[i] * (b0 - a0) + (b1 - a1), SLOPE[j] * (b0 - a0) + (b1 - a1)]


def _couple_product(lhs, rhs, done):
    first, second, steps = {}, {}, []

    def add(i, j, m):
        if i == j:
            first[i], second[i] = m
            return
        t, gap = m[0] + m[1] + m[2], SLOPE[j] - SLOPE[i]
        t = t if gap == 1 else t * (1 / gap)
        first[i], first[j] = first[i] - t, first[j] - t
        second[i], second[j] = second[i] + m[1], second[j] - m[2]
        if j == 3:
            for r in (i,) if i else (0, 3):
                done(r, first[r], second[r] - SLOPE[r] * first[r])

    for i, j in COUPLES:
        got, n = [], 2 if i == j else 3
        for _ in range(n):
            def step(i=i, j=j, got=got, n=n, k=len(steps)):
                got.append(lax.dot_general(lhs(k), rhs(k), NN, preferred_element_type=F32))
                if len(got) == n:
                    add(i, j, got)
                return got[-1]
            steps.append(step)
    return steps


def _combine(blocks, terms):
    if isinstance(blocks[terms[0][0]], list):
        return [_combine({b: blocks[b][i] for b, _ in terms}, terms) for i in range(4)]
    out = blocks[terms[0][0]]
    for i, sign in terms[1:]:
        out = out + blocks[i] if sign > 0 else out - blocks[i]
    return out


def _operands(blocks, side):
    return [_combine(blocks, terms) for terms in side]


def _block_product(lhs, rhs, done, dims=NN, levels=2):
    if levels == 0:
        def step():
            m = lax.dot_general(lhs(0), rhs(0), dims, preferred_element_type=F32)
            done((), m)
            return m
        return [step]

    held, steps = {}, []
    inner = NOPS ** (levels - 1)
    for n, (i, outs) in enumerate(PRODUCTS):
        later = {o for _, others in PRODUCTS[n + 1:] for o, _ in others}

        def add(sub, m, outs=outs, later=later):
            for o, sign in outs:
                if (o, sub) not in held:
                    held[o, sub] = m, sign
                else:
                    c, s = held[o, sub]
                    held[o, sub] = (m - c if s < 0 else c + m if sign > 0 else c - m), 1
                if o not in later:
                    done((o, *sub), held.pop((o, sub))[0])

        steps += _block_product(lambda k, i=i: lhs(i * inner + k),
                                lambda k, i=i: rhs(i * inner + k), add, dims, levels - 1)
    return steps


def _corner(o, rows, cols):
    return (2 * (o[0] // 2) + o[1] // 2) * rows, (2 * (o[0] % 2) + o[1] % 2) * cols


def _bf16(words):
    return pltpu.bitcast(words, BF16)


def _halves(words):
    lo = pltpu.bitcast(words << 16, F32)
    hi = pltpu.bitcast(words & jnp.uint32(0xFFFF0000), F32)
    return lo, hi


def _f32(words):
    return _bf16(words).astype(F32)


def _load(ref, *index):
    return _bf16(ref.bitcast(U32)[index])


def _beside(tiles):
    return jnp.concatenate(list(tiles), axis=1)


def _put(ref, index, row, values):
    for k, v in enumerate(values):
        ref[(*index(k), pl.ds(row, v.shape[0]), slice(None))] = v.astype(BF16)
    return [v[:8] for v in values]


def _store(words, index, row, col, x):
    matrix = words.bitcast(BF16).at[index]
    matrix[pl.ds(pl.multiple_of(2 * row, 16), x.shape[0]), pl.ds(col, x.shape[1])] = x.astype(BF16)


def _recip(x):
    r = pltpu.reciprocal(x, approx=True)
    return r * (2.0 - x * r)


def _run(steps):
    out = None
    for step in steps:
        out = step()
    return out


def _group(steps, n):
    return [lambda g=steps[i:i + n]: _run(g) for i in range(0, len(steps), n)]


def _share(items, k, n):
    return items[k * len(items) // n:(k + 1) * len(items) // n]


def _blend(*lists):
    spots = [((i + 0.5) / len(items), k, item)
             for k, items in enumerate(lists) for i, item in enumerate(items)]
    return [item for *_, item in sorted(spots, key=lambda spot: spot[:2])]


def _witness(values):
    out = None
    for v in values:
        v = pltpu.bitcast(v, U32)
        for r in range(0, v.shape[0], 8):
            for c in range(0, v.shape[1], 128):
                out = v[r:r + 8, c:c + 128] if out is None else out | v[r:r + 8, c:c + 128]
    return out


def _pacer(ref, index, row=0):
    def pace(v):
        if ref.dtype == BF16 and ref.shape[-1] == 128:
            ref.bitcast(U32)[index, pl.ds(row, 8), :] = v
        elif ref.dtype == BF16:
            ref[index, pl.ds(row, 16), pl.ds(0, 128)] = _bf16(v)
        else:
            ref[index, pl.ds(row, 8), pl.ds(0, 128)] = pltpu.bitcast(v, ref.dtype)
    return pace


def _tie(pieces, result):
    for i, (pace, work, *lag) in enumerate(pieces):
        seen, m = work(), result(sum(lag))
        r = 8 * (i * (m.shape[0] // 8) // len(pieces))
        pace(_witness([m[r:r + 8]] + list(seen)))


def _mingle(steps, pieces, history=None):
    history = [] if history is None else history

    def both(step, mine):
        history.append(step())
        _tie([piece for piece in mine if piece],
             lambda lag: history[max(0, len(history) - 1 - lag)][:, :128])

    return [lambda step=step, mine=_share(pieces, i, len(steps)): both(step, mine)
            for i, step in enumerate(steps)]


def _now(pieces):
    for _, work, *_ in pieces:
        work()


def _dim_major(src, pace, shuf, put, swap, zero, lag=0, gap=0):
    def scatter(k, u):
        t = src(k, u)
        for h in range(128 // AD):
            shuf[k, pl.ds((4 * u + h) * PITCH, AD), :] = t[h * AD:(h + 1) * AD]
        return [t]

    def gather(d, i):
        def block(row1, col1, row2, col2):
            quarter, k = 2 * row1 + row2, 2 * col1 + col2
            if swap:
                quarter, k = k, quarter
            return jnp.concatenate(
                [shuf[k, pl.ds(8 * p * PITCH + quarter * AD // 4 + d, 8, stride=PITCH), :]
                 for p in range(2)], axis=0)
        outer = {b: [block(b // 2, b % 2, s // 2, s % 2) for s in range(4)] for b, _ in RHS[i]}
        return put(NOPS * i, d * NH, _operands(_combine(outer, RHS[i]), RHS))

    return ([x for k in range(4) for u in range(4)
             for x in [(pace, lambda k=k, u=u: scatter(k, u), lag)] + [None] * gap]
            + [(_pacer(shuf, 4 + zero), lambda d=d, i=i: gather(d, i))
               for d in range(AD // 4) for i in range(NOPS)])


def _kernel(ax_hbm, awqkv_hbm, awo_hbm, bx_hbm, c_hbm, wq_hbm, wuk_hbm, wuv_hbm,
            wo_hbm, out_hbm,
            offset, ctx, wo_raw, woop, awop, awoop, xa, xaop, awo_raw, shuf,
            sem_x, sem_c, sem_w, sem_a, sem_out):

    def cp_tile(src, row, col, dst, sem):
        def span(i):
            return pl.ds(pl.multiple_of(i * TILE, TILE), TILE)
        return pltpu.make_async_copy(src.at[span(row), span(col)], dst, sem)

    def cp_wo(u, s):
        return cp_tile(wo_hbm, u // 2, u % 2, wo_raw.at[s].bitcast(BF16), sem_w.at[6 + s])

    def cp_a():
        return ([pltpu.make_async_copy(ax_hbm.at[pl.ds(c * CH, CH)], xa.at[c], sem_a.at[0])
                 for c in range(NC)]
                + [pltpu.make_async_copy(awo_hbm.at[pl.ds(128 * t, 128), pl.ds(DC * h, DC)],
                                         awo_raw.at[t, pl.ds(128 * h, 128)], sem_a.at[1])
                   for t in range(8) for h in range(2)])

    def prep_wo(u, s, zero):
        def piece(r, i):
            outer = {b: [_f32(wo_raw[s, pl.ds((2 * a2 + b // 2) * (HD // 2) + r, 8),
                                       pl.ds((2 * (b % 2) + b2) * 128, 128)])
                         for a2 in range(2) for b2 in range(2)] for b, _ in RHS[i]}
            return _put(woop, lambda k: (u % 2, NOPS * i + k), pl.multiple_of(u // 2 * HD + 2 * r, 16),
                        _operands(_combine(outer, RHS[i]), RHS))
        return [(_pacer(wo_raw, 2 + zero), lambda r=r, i=i: piece(r, i))
                for r in range(0, HD // 2, 8) for i in range(NOPS)]

    def prep_awo(u, zero):
        n, half = u // 2, u % 2

        def put(i, row, values):
            return _put(awoop, lambda k: (n, i + k), 16 * half + row, values)
        return _dim_major(
            lambda k, t: awo_raw[4 * half + t, pl.ds(128 * n, 128), pl.ds(128 * k, 128)].astype(F32),
            _pacer(awo_raw, 8 + zero), shuf, put, False, zero)

    def prep_xa(c, zero):
        def piece(t, r, i):
            outer = {b: [xa[c, pl.ds((b // 2) * R + r2 * R // 2 + r, 16),
                            pl.ds(512 * t + (b % 2) * 256 + a2 * 128, 128)].astype(F32)
                for r2 in range(2) for a2 in range(2)] for b, _ in LHS[i]}
            return _put(xaop, lambda k: (NOPS * i + k, t), r, _operands(_combine(outer, LHS[i]), LHS))
        return [(_pacer(xa, NC + zero), lambda t=t, r=r, i=i: piece(t, r, i))
                for t in range(2) for r in range(0, R // 2, 16) for i in range(NOPS)]

    offset[:16] = jnp.zeros((16, 128), F32)
    shuf[0, :8] = offset[pl.ds(1, 8)]

    def heads(xop, cop, wq_raw, wkv_raw, qwop, kvwop, q_s, k_s, v_s, aw_raw, unit):
        xs, cs = xa, awo_raw
        wq32 = wq_hbm.bitcast(U32)
        wuk32 = wuk_hbm.bitcast(U32)
        wuv32 = wuv_hbm.bitcast(U32)

        def cp_x(c):
            return pltpu.make_async_copy(bx_hbm.at[pl.ds(c * CH, CH)], xs.at[c], sem_x.at[c])

        def cp_c(c):
            return pltpu.make_async_copy(c_hbm.at[pl.ds(c * CH, CH)], cs.at[c], sem_c.at[c])

        def cp_wkv(j, s):
            return [pltpu.make_async_copy(wuk32.at[:, j, :], wkv_raw.at[s], sem_w.at[s]),
                    pltpu.make_async_copy(wuv32.at[:, j, :], wkv_raw.at[2 + s], sem_w.at[2 + s])]

        def cp_wq(j, s):
            return [pltpu.make_async_copy(wq32.at[:, j, :], wq_raw.at[s], sem_w.at[4 + s])]

        def wo_unit(j):
            return jnp.maximum(j - 1, 0)

        def aw_unit(j):
            return jnp.clip(j - 1, 0, 3 * DM * DM // TILE ** 2 - 1)

        def cp_heads(j):
            return (cp_wkv(jnp.minimum(j + 2, NP - 1), j % 2)
                    + cp_wq(jnp.minimum(j + 1, NP - 1), j % 2))

        def cp_tiles(j):
            u = aw_unit(j)
            return [cp_wo(wo_unit(j), j % 2),
                    cp_tile(awqkv_hbm, u // 2 % 2, 2 * (u // 4) + u % 2, aw_raw.at[j % 2],
                            sem_w.at[8 + j % 2])]

        def prep_x(c):
            for t in range(2):
                blocks = [[
                    xs[c, pl.ds(r * R // 2, R // 2), pl.ds(k * DM // 4 + 128 * t, 128)].astype(F32)
                    for k in range(4)] for r in range(4)]
                ops = [v for i, j in COUPLES
                       for v in _square_forms(lambda r, k: blocks[r][k], i, j)]
                _put(xop, lambda n: (2 * (NQ * c + n) + t,), 0, ops)

        def prep_c(c):
            blocks = [[
                cs[c, pl.ds(r1 * R + r2 * R // 2, R // 2), pl.ds(a1 * 256 + a2 * 128, 128)].astype(F32)
                for r2 in range(2) for a2 in range(2)] for r1 in range(2) for a1 in range(2)]
            for i, outer in enumerate(_operands(blocks, LHS)):
                _put(cop, lambda k: (c, NOPS * i + k), 0, _operands(outer, LHS))

        def both_heads(raw, s, row):
            return _halves(raw[s, pl.ds(row, 16), :])

        def prep_wq(s, zero):
            def piece(r, couples, n):
                w = {k: both_heads(wq_raw, s, k * DM // 4 + r) for couple in couples for k in couple}
                return _put(qwop, lambda k: (n + k,), r,
                            [v for i, j in couples for v in _pair_forms(w.get, i, j)])
            parts = (COUPLES[:6], 0), (COUPLES[6:], 15)
            return [(_pacer(wq_raw, 2 + zero), lambda r=r, part=part: piece(r, *part))
                    for r in range(0, DM // 4, 16) for part in parts]

        def prep_wkv(j, s, slot, zero):
            total, inverse = {}, {}

            def measure(n, r):
                w = wkv_raw[2 * n + s, pl.ds(r, 64), :]
                w = jnp.abs(pltpu.bitcast(w, F32)) + jnp.abs(pltpu.bitcast(w << 16, F32))
                w = jnp.sum(w.reshape(8, 8, 128), axis=0)
                total[n] = total[n] + w if r else w
                return [total[n]]

            def size(n):
                both = jnp.sum(jnp.sum(total[n], axis=1, keepdims=True), axis=0, keepdims=True)
                both = jnp.broadcast_to(jnp.clip(both, 2.0 ** -100, 2.0 ** 100), (8, 128))
                power = pltpu.bitcast(both, U32) & jnp.uint32(0x7F800000)
                unit[n, j] = pltpu.bitcast(power, F32)
                inverse[n] = pltpu.bitcast(jnp.uint32(0x7F000000) - power, F32)
                return [power]

            def piece(r, i):
                outer = {b: [v * jnp.concatenate([inverse[b % 2]] * 2, axis=0) for a2 in range(2)
                             for v in both_heads(wkv_raw, 2 * (b % 2) + s,
                                                 (b // 2) * 256 + a2 * 128 + r)]
                         for b, _ in RHS[i]}
                return _put(kvwop, lambda k: (slot + (NOPS * i + k),), r,
                            _operands(_combine(outer, RHS[i]), RHS))

            pace = _pacer(wkv_raw, 4 + zero)
            return ([(pace, lambda n=n, r=r: measure(n, r))
                     for n in range(2) for r in range(0, DC, 64)]
                    + [(pace, lambda n=n: size(n)) for n in range(2)],
                    [(_pacer(xop, 2 * NQ * NC + zero), lambda: list(inverse.values()))]
                    + [(pace, lambda r=r, i=i: piece(r, i))
                       for r in range(0, 128, 16) for i in range(NOPS)])

        def prep_aw(u, s, zero):
            def put(i, row, values):
                return _put(awop, lambda k: (u // 2, i + k), pl.multiple_of(16 * (u % 2), 16) + row,
                            values)
            return _dim_major(
                lambda k, t: aw_raw[s, pl.ds(128 * k, 128), pl.ds(128 * t, 128)].astype(F32).T,
                _pacer(xop, 2 * NQ * NC + zero), shuf, put, True, zero, lag=5, gap=2)

        def q_proj(scale, c):
            def done(r, *both):
                for h, val in enumerate(both):
                    _store(q_s, 0, c * R + r * (R // 4), h * HD, val * scale)
            return _couple_product(lambda i: _beside(_load(xop, 2 * (NQ * c + i) + t) for t in range(2)),
                                   lambda i: _load(qwop, i), done)

        def kv_proj(c, slot):
            def done(o, val):
                row, col = _corner(o, R // 4, HD)
                _store((k_s, v_s)[col // (2 * HD)], 0, c * R + row, col % (2 * HD), val)
            return _block_product(lambda i: _load(cop, c, i), lambda i: _load(kvwop, slot + i), done)

        def q_scale(j):
            return unit[0, j, :1] * (HD ** -0.5 * LOG2E)

        def scores(h, blk):
            n = (blk + 1) * R
            s = lax.dot_general(_bf16(q_s[0, pl.ds(blk * R // 2, R // 2), pl.ds(h * HD, HD)]),
                                _bf16(k_s[0, :n // 2, pl.ds(h * HD, HD)]),
                                NT, preferred_element_type=F32)
            row = lax.broadcasted_iota(jnp.int32, (R, R), 0)
            col = lax.broadcasted_iota(jnp.int32, (R, R), 1)
            diag = jnp.where(col <= row, s[:, n - R:], MASKED)
            return diag if blk == 0 else jnp.concatenate([s[:, :n - R], diag], axis=1)

        def attend(scale, h, blk, s):
            n = (blk + 1) * R
            p = jnp.exp2(s - jnp.max(s, axis=1, keepdims=True))
            inv = _recip(jnp.sum(p, axis=1, keepdims=True)) * scale
            o = lax.dot_general(p.astype(BF16), _bf16(v_s[0, :n // 2, pl.ds(h * HD, HD)]), NN,
                                preferred_element_type=F32)
            return o * inv

        def pair_attention(j, zero, filler, sides, slack):
            blocks = [(h, 2 * c + u) for c in reversed(range(NC)) for u in (1, 0) for h in (0, 1)]
            plan = {}
            for pieces, span in sides:
                tiles = [(b, t) for b in blocks[span] for t in range(b[1] + 1)]
                for n, tile in enumerate(tiles):
                    plan.setdefault(tile, []).extend(_share(pieces, n, len(tiles)))

            def paced_scores(h, blk):
                s = scores(h, blk)
                for t in range(blk + 1):
                    _tie(plan.get(((h, blk), t), []), lambda lag: s[:, t * R:(t + 1) * R])
                return s

            todo, done = [[]] * 8, []
            v_scale = unit[1, j, :1]
            ahead = [paced_scores(*blocks[0])]
            for n, (h, blk) in enumerate(blocks):
                ahead += [paced_scores(*b) for b in blocks[n + 1:n + 2]]
                _run(todo[2 * (n % 4)])
                done.append(attend(v_scale, h, blk, ahead.pop(0)))
                _store(ctx, 0, pl.multiple_of(j * (S // 2), S // 2) + blk * (R // 2), h * HD, done[-1])
                if len(done) > slack:
                    _pacer(q_s, zero, S // 2)(_witness([done.pop(0)]))
                _run(todo[2 * (n % 4) + 1])
                if n % 4 == 3:
                    todo = filler(blk // 2)
            _run(sum(todo, []))

        c_parts = ((7, 6), (5, 4), (3, 2), (1, 0))
        x_parts = tuple(reversed(range(NC)))
        stages = ([cp_wkv(0, 0)] + [[cp_c(c) for c in part] for part in c_parts]
                  + [[cp_x(c)] for c in x_parts] + [cp_wq(1, 0)])
        stages[len(c_parts)] += cp_wq(0, 1)
        stages[len(c_parts) + 1] += cp_wkv(1, 1)

        def issue(i, zero):
            for k, stage in enumerate(stages):
                @pl.when(i == k)
                def _(stage=stage):
                    for cp in stage:
                        cp.start()
            return zero + i // NP

        zero = lax.fori_loop(0, len(stages), issue, jnp.int32(0))

        aw_raw[0] = jnp.zeros(aw_raw.shape[1:], BF16)
        wo_raw[0] = jnp.zeros(wo_raw.shape[1:], U32)
        for cp in stages[0]:
            cp.wait()
        _now(sum(prep_wkv(0, 0, SLOT, zero), []))
        for n, part in enumerate(c_parts):
            for cp in stages[1 + n]:
                cp.wait()
            if n == 0:
                for cp in cp_wkv(2, 0):
                    cp.start()
            side = prep_wq(1, zero) if n == len(c_parts) - 1 else []
            for k, c in enumerate(part):
                prep_c(c)
                _run(_mingle(kv_proj(c, SLOT), _share(side, k, len(part))))
        scale, side = q_scale(0), sum(prep_wkv(1, 1, 0, zero), [])
        for n, c in enumerate(x_parts):
            for cp in stages[1 + len(c_parts) + n]:
                cp.wait()
            prep_x(c)
            _run(_mingle(q_proj(scale, c), _share(side, n, NC)))

        def pair_step(j, zero):
            for cp in cp_heads(j):
                cp.wait()

            @pl.when(j > 0)
            def _():
                for cp in cp_tiles(j):
                    cp.wait()

            @pl.when(j == RING)
            def _():
                words = kvwop.bitcast(U32)
                words[:SLOT] = words[RING * SLOT:]
                for cp in cp_a():
                    cp.start()

            for cp in cp_heads(j + 1) + cp_tiles(j + 1):
                cp.start()
            slot = (j % RING) * SLOT
            scale = q_scale(j + 1)
            sizes, operands = prep_wkv(j + 2, j % 2, slot + SLOT, zero)
            side = [None] * 24 + _blend(prep_aw(aw_unit(j), j % 2, zero),
                                        sizes + [None] * 12 + operands)
            q_steps = sum((q_proj(scale, c) for c in reversed(range(NC))), [])
            history = []

            def filler(c):
                q = _share(q_steps, NC - 3 - c, NC - 2) if c < NC - 2 else []
                kv = kv_proj(c, slot)
                slots = []
                for n in range(4):
                    mine = _share(kv, n, 4)
                    early = len(mine) - len(mine) * 3 // 4
                    slots += [mine[:early] + _share(q, n, 4), mine[early:]]
                along = _share(side, NC - 2 - c, NC - 1) if c < NC - 1 else []
                steps = iter(_mingle(sum(slots, []), along, history))
                return [[next(steps) for _ in slot] for slot in slots]

            pair_attention(j, zero, filler, [(prep_wo(wo_unit(j), j % 2, zero), slice(10, None)),
                                             (prep_wq(j % 2, zero), slice(2, 12))], 3)
            return zero + j // NP

        zero = lax.fori_loop(0, NP - 1, pair_step, zero)

        @pl.loop(0, 2)
        def _(i):
            _pacer(shuf, 4 + zero * i)(jnp.zeros((8, 128), U32))

        for cp in cp_heads(NP - 1) + cp_tiles(NP - 1) + cp_a():
            cp.wait()
        cp_wo(NP - 1, 0).start()
        side = _blend(prep_wo(NP - 2, 1, zero), prep_awo(0, zero), prep_xa(zero, zero))
        pair_attention(NP - 1, zero, lambda c: [[]] * 8, [(side, slice(2, None))], 5)
        return zero

    def rows(zero, aoop, aqkv, oop, out_s):
        @pl.loop(0, 2)
        def _(i):
            aqkv[pl.ds(8 + 8 * i, 8), :HALO, :] = jnp.zeros((8, HALO, 128), F32)

        def cp_out(c, half):
            return pltpu.make_async_copy(
                out_s.at[half, c],
                out_hbm.at[pl.ds(pl.multiple_of(c * CH, CH), CH), pl.ds(half * DM, DM)],
                sem_out.at[half * NC + c])

        def cp_last(row, col, n, sem):
            return pltpu.make_async_copy(
                out_s.at[0, NC - 1, pl.ds(row, n), pl.ds(col, DM // 2)],
                out_hbm.at[pl.ds((NC - 1) * CH + row, n), pl.ds(col, DM // 2)], sem_x.at[sem])

        def prep_ctx(c, zero):
            base = pl.multiple_of(c * R, R)

            def piece(m, r, i):
                outer = {b: [_f32(ctx[0, pl.ds(base + ((2 * m + a2) * (S // 2) + (b // 2) * 64
                                                         + r2 * 32 + r), 8),
                                        pl.ds((b % 2) * HD, HD)])
                             for r2 in range(2) for a2 in range(2)] for b, _ in LHS[i]}
                return _put(oop, lambda k: (NOPS * i + k, m), 2 * r,
                            _operands(_combine(outer, LHS[i]), LHS))
            return [(_pacer(ctx, zero, NP * S // 2), lambda m=m, r=r, i=i: piece(m, r, i))
                    for m in range(NP // 2) for r in range(0, 32, 8) for i in range(NOPS)]

        def out_proj(half, c, lhs, rhs):
            steps = []
            for t in range(2):
                def done(o, val, t=t):
                    row, col = _corner(o, R // 2, 128)
                    out_s[half, c, pl.ds(row, R // 2), pl.ds(512 * t + col, 128)] = val.astype(BF16)
                steps += _block_product(lhs, lambda i, t=t: _load(rhs, t, i), done)
            return steps

        def b_out_proj(c):
            return out_proj(1, c, lambda i: _beside(_load(oop, i, m) for m in range(NP // 2)), woop)

        def a_out_proj(c, zero):
            return out_proj(0, c, lambda i: _bf16(aoop[zero + i]), awoop)

        def a_proj(row0):
            steps = []
            for part in range(3):
                for t in range(2):
                    def done(o, val, part=part, t=t):
                        if part == 0:
                            val = val * (AD ** -0.5 * LOG2E)
                        row, plane = _corner(o, R // 2, 2)
                        aqkv[8 * part + plane + t, pl.ds(row0 + (HALO + row), R // 2), :] = val

                    def rhs(i, part=part, t=t):
                        return _beside(_load(awop, 2 * part + m, i, pl.ds(64 * t, 64)) for m in range(2))
                    steps += _block_product(lambda i: _beside(_load(xaop, i, m) for m in range(2)),
                                            rhs, done, NT)
            return steps

        def a_attention(c, row0, zero, n):
            query, logit, prob, mixed = {}, {}, {}, {}

            def dot(r, w):
                tot = None
                for t in range(8):
                    if (r, t) not in query:
                        query[r, t] = aqkv[t, pl.ds(row0 + (HALO + r), 8), :]
                    pr = query[r, t] * aqkv[8 + t, pl.ds(row0 + (HALO + r - DIL * w), 8), :]
                    tot = pr if tot is None else tot + pr
                logit[r, w] = tot
                if w == WIN - 1:
                    weights(r)
                return [tot]

            def weights(r):
                logits = [logit[r, w] for w in range(WIN)]
                logits = [x + pltpu.roll(x, 64, 1) for x in logits]
                logits = [x + pltpu.roll(x, 32, 1) for x in logits]
                if r < (WIN - 1) * DIL:
                    pos = c * CH + r + lax.broadcasted_iota(jnp.int32, (8, 128), 0)
                    logits = [x if w == 0 else jnp.where(pos >= DIL * w, x, MASKED)
                              for w, x in enumerate(logits)]
                top = logits[0]
                for x in logits[1:]:
                    top = jnp.maximum(top, x)
                e = [jnp.exp2(x - top) for x in logits]
                tot = e[0]
                for x in e[1:]:
                    tot = tot + x
                inv = _recip(tot)
                prob[r] = [x * inv for x in e]

            def mix(r, t, d, q):
                tot = None
                for w in range(WIN):
                    pr = prob[r + d][w] * aqkv[16 + t + 2 * q,
                                               pl.ds(row0 + (HALO + r + d - DIL * w), 8), :]
                    tot = pr if tot is None else tot + pr
                mixed[r, t, d, q] = tot
                return [tot]

            def operands(r, t, i):
                outer = {b: [jnp.concatenate(
                    [mixed[r, t, (b // 2) * R + r2 * R // 2 + e, 2 * (b % 2) + a2] for e in (0, 8)],
                    axis=0) for r2 in range(2) for a2 in range(2)] for b, _ in LHS[i]}
                ops = _operands(_combine(outer, LHS[i]), LHS)
                for k, v in enumerate(ops):
                    _store(aoop, NOPS * i + k, r // 2, 128 * t, v)
                return ops

            groups = [d + e for d in range(0, CH, R // 2) for e in (0, 8)]

            def dots(r):
                return [lambda d=d, w=w: dot(r + d, w) for d in groups for w in range(WIN)]

            def mixes(r):
                return [work for t in range(2) for work in
                        [lambda t=t, d=d, q=q: mix(r, t, d, q) for d in groups for q in range(4)]
                        + [lambda t=t, i=i: operands(r, t, i) for i in range(NOPS)]]

            work = dots(0)
            for r in range(16, R // 2, 16):
                work += _blend(dots(r), mixes(r - 16))
            work += mixes(R // 2 - 16)
            return [(_pacer(aqkv, zero, HALO + S), lambda g=work[i:i + n]: sum((w() for w in g), []))
                    for i in range(0, len(work), n)]

        cp_wo(NP - 1, 0).wait()
        _run(_mingle(_group(a_proj(0), 2),
                     _blend(prep_ctx(0, zero), sum((prep_awo(u, zero) for u in range(1, 4)), []),
                            prep_wo(NP - 1, 0, zero))))

        def chunk_step(c, zero):
            row0 = pl.multiple_of((c - 1) * CH, CH)
            first, second, third = b_out_proj(c - 1), a_proj(row0 + CH), a_out_proj(c - 1, zero)
            att, ctxp = a_attention(c - 1, row0, zero, 1), prep_ctx(c, zero)
            cut, late = len(att) * 9 // 16, len(ctxp) * 5 // 16
            _run(_mingle(first, _blend(att[:cut], prep_xa(c, zero))))
            cp_out(c - 1, 1).start()
            _run(_mingle(second[:-4], _blend(att[cut:], ctxp[:-late])) + second[-4:])
            third = _group(third, 2)
            _run(_mingle(third[:-3], ctxp[-late:]) + third[-3:])
            cp_out(c - 1, 0).start()
            return zero + c // NC

        zero = lax.fori_loop(1, NC, chunk_step, zero)

        steps = b_out_proj(NC - 1)
        _run(_mingle(steps[:-2], a_attention(NC - 1, (NC - 1) * CH, zero, 2)) + steps[-2:])
        cp_out(NC - 1, 1).start()
        steps = a_out_proj(NC - 1, zero)
        parts = [cp_last(0, 0, CH, 0), cp_last(R, DM // 2, R, 1), cp_last(0, DM // 2, R, 2)]
        for cp, part in zip(parts, (steps[:NOPS * NOPS], steps[NOPS * NOPS:-NOPS], steps[-NOPS:])):
            _run(part)
            cp.start()
        for cp in ([cp_out(c, 1) for c in range(NC)] + [cp_out(c, 0) for c in range(NC - 1)] + parts):
            cp.wait()

    vmem = pltpu.VMEM
    zero = pl.run_scoped(
        heads,
        vmem((2 * NQ * NC + 1, R // 2, 128), BF16),
        vmem((NC, NOPS * NOPS, R // 2, 128), BF16),
        vmem((3, DM, HD), U32),
        vmem((5, DC, HD), U32),
        vmem((NQ, DM // 4, 128), BF16),
        vmem(((RING + 1) * SLOT, 128, 128), BF16),
        vmem((1, S // 2 + 16, 2 * HD), U32),
        vmem((1, S // 2, 2 * HD), U32),
        vmem((1, S // 2, 2 * HD), U32),
        vmem((2, TILE, TILE), BF16),
        vmem((2, NP + 2, 8, 128), F32),
    )
    pl.run_scoped(
        lambda *refs: rows(zero, *refs),
        vmem((NOPS * NOPS, R // 4, DM // 4), U32),
        vmem((24, HALO + S + 16, 128), F32),
        vmem((NOPS * NOPS, NP // 2, R // 2, HD), BF16),
        vmem((2, NC, CH, DM), BF16),
    )


@jax.jit
def pallas_concat_heads__sliding_local_dilated__compressed_kv_cla__prompt_kernel(
    A_x: jax.Array,
    A_wqkv: jax.Array,
    A_wo: jax.Array,
    B_x: jax.Array,
    B_c_kv: jax.Array,
    B_w_q: jax.Array,
    B_w_uk: jax.Array,
    B_w_uv: jax.Array,
    B_w_o: jax.Array,
):
    vmem = pltpu.VMEM
    dma = pltpu.SemaphoreType.DMA
    scratch = [
        vmem((24, 128), F32),
        vmem((1, NP * S // 2 + 16, 2 * HD), U32),
        vmem((3, TILE // 2, TILE), U32),
        vmem((2, NOPS * NOPS, NP * HD // 2, 128), BF16),
        vmem((6, NOPS * NOPS, DM // 4, 128), BF16),
        vmem((2, NOPS * NOPS, DM // 4, 128), BF16),
        vmem((NC + 1, CH, DM), BF16),
        vmem((NOPS * NOPS, 2, R // 2, 128), BF16),
        vmem((NC + 1, CH, DC), BF16),
        vmem((5, 16 * PITCH + 16, 128), F32),
        dma((NC,)), dma((NC,)), dma((10,)), dma((2,)), dma((2 * NC,)),
    ]
    out = pl.pallas_call(
        _kernel,
        out_shape=jax.ShapeDtypeStruct((S, 2 * DM), BF16),
        in_specs=[pl.BlockSpec(memory_space=pl.ANY)] * 9,
        out_specs=pl.BlockSpec(memory_space=pl.ANY),
        scratch_shapes=scratch,
        compiler_params=pltpu.CompilerParams(vmem_limit_bytes=124 * 2**20),
        name="fused_local_and_latent_attention",
    )(
        A_x.reshape(S, DM), A_wqkv, A_wo,
        B_x.reshape(S, DM), B_c_kv.reshape(S, DC),
        B_w_q, B_w_uk, B_w_uv, B_w_o.reshape(NH * HD, DM),
    )
    return out.reshape(1, S, 2 * DM)
```

```python
import math

import jax
import jax.numpy as jnp
from jax import lax
import jax.experimental.pallas as pl
import jax.experimental.pallas.tpu as pltpu

F32, BF16, U32 = jnp.float32, jnp.bfloat16, jnp.uint32

S = 2048
DM = 1024
DC = 512
NH = 32
HD = 128
AD = 32
WIN, DIL = 8, 2

R = 128
CH = 2 * R
NC = S // CH
NP = NH // 2
HALO = 16
PITCH = 33
TILE = 512
LOG2E = math.log2(math.e)
MASKED = -1e9 * LOG2E

NN = (((1,), (0,)), ((), ()))
NT = (((1,), (1,)), ((), ()))

LHS = (((0, 1), (3, 1)), ((2, 1), (3, 1)), ((0, 1),), ((3, 1),),
       ((0, 1), (1, 1)), ((2, 1), (0, -1)), ((1, 1), (3, -1)))
RHS = (((0, 1), (3, 1)), ((0, 1),), ((1, 1), (3, -1)), ((2, 1), (0, -1)),
       ((3, 1),), ((0, 1), (1, 1)), ((2, 1), (3, 1)))
PRODUCTS = ((2, ((1, 1), (3, 1))), (4, ((0, -1), (1, 1))), (3, ((0, 1), (2, 1))),
            (1, ((2, 1), (3, -1))), (5, ((3, 1),)), (0, ((0, 1), (3, 1))),
            (6, ((0, 1),)))
NOPS = len(PRODUCTS)

SLOPE = (-1.5, -0.5, 0.5, 1.5)
COUPLES = tuple((i, j) for j in range(4) for i in range(j, -1, -1))
NQ = sum(2 if i == j else 3 for i, j in COUPLES)

SLOT = NOPS * NOPS
RING = 8


def _square_forms(x, i, j):
    if i == j:
        p = q = x(i, i)
        for k in range(4):
            if k != i:
                p, q = p - x(k, i), q + x(i, k)
        return [p, q]
    return [x(i, j) + x(j, i), x(i, j), x(j, i)]


def _pair_forms(w, i, j):
    (a0, a1), (b0, b1) = w(i), w(j)
    if i == j:
        return [a0, SLOPE[i] * a0 + a1]
    return [(SLOPE[i] * a0 + a1) - (SLOPE[j] * b0 + b1),
            SLOPE[i] * (b0 - a0) + (b1 - a1), SLOPE[j] * (b0 - a0) + (b1 - a1)]


def _couple_product(lhs, rhs, done):
    first, second, steps = {}, {}, []

    def add(i, j, m):
        if i == j:
            first[i], second[i] = m
            return
        t, gap = m[0] + m[1] + m[2], SLOPE[j] - SLOPE[i]
        t = t if gap == 1 else t * (1 / gap)
        first[i], first[j] = first[i] - t, first[j] - t
        second[i], second[j] = second[i] + m[1], second[j] - m[2]
        if j == 3:
            for r in (i,) if i else (0, 3):
                done(r, first[r], second[r] - SLOPE[r] * first[r])

    for i, j in COUPLES:
        got, n = [], 2 if i == j else 3
        for _ in range(n):
            def step(i=i, j=j, got=got, n=n, k=len(steps)):
                got.append(lax.dot_general(lhs(k), rhs(k), NN, preferred_element_type=F32))
                if len(got) == n:
                    add(i, j, got)
                return got[-1]
            steps.append(step)
    return steps


def _combine(blocks, terms):
    if isinstance(blocks[terms[0][0]], list):
        return [_combine({b: blocks[b][i] for b, _ in terms}, terms) for i in range(4)]
    out = blocks[terms[0][0]]
    for i, sign in terms[1:]:
        out = out + blocks[i] if sign > 0 else out - blocks[i]
    return out


def _operands(blocks, side):
    return [_combine(blocks, terms) for terms in side]


def _block_product(lhs, rhs, done, dims=NN, levels=2):
    if levels == 0:
        def step():
            m = lax.dot_general(lhs(0), rhs(0), dims, preferred_element_type=F32)
            done((), m)
            return m
        return [step]

    held, steps = {}, []
    inner = NOPS ** (levels - 1)
    for n, (i, outs) in enumerate(PRODUCTS):
        later = {o for _, others in PRODUCTS[n + 1:] for o, _ in others}

        def add(sub, m, outs=outs, later=later):
            for o, sign in outs:
                if (o, sub) not in held:
                    held[o, sub] = m, sign
                else:
                    c, s = held[o, sub]
                    held[o, sub] = (m - c if s < 0 else c + m if sign > 0 else c - m), 1
                if o not in later:
                    done((o, *sub), held.pop((o, sub))[0])

        steps += _block_product(lambda k, i=i: lhs(i * inner + k),
                                lambda k, i=i: rhs(i * inner + k), add, dims, levels - 1)
    return steps


def _corner(o, rows, cols):
    return (2 * (o[0] // 2) + o[1] // 2) * rows, (2 * (o[0] % 2) + o[1] % 2) * cols


def _bf16(words):
    return pltpu.bitcast(words, BF16)


def _halves(words):
    lo = pltpu.bitcast(words << 16, F32)
    hi = pltpu.bitcast(words & jnp.uint32(0xFFFF0000), F32)
    return lo, hi


def _f32(words):
    return _bf16(words).astype(F32)


def _load(ref, *index):
    return _bf16(ref.bitcast(U32)[index])


def _beside(tiles):
    return jnp.concatenate(list(tiles), axis=1)


def _put(ref, index, row, values):
    for k, v in enumerate(values):
        ref[(*index(k), pl.ds(row, v.shape[0]), slice(None))] = v.astype(BF16)
    return [v[:8] for v in values]


def _store(words, index, row, col, x):
    matrix = words.bitcast(BF16).at[index]
    matrix[pl.ds(pl.multiple_of(2 * row, 16), x.shape[0]), pl.ds(col, x.shape[1])] = x.astype(BF16)


def _recip(x):
    r = pltpu.reciprocal(x, approx=True)
    return r * (2.0 - x * r)


def _run(steps):
    out = None
    for step in steps:
        out = step()
    return out


def _group(steps, n):
    return [lambda g=steps[i:i + n]: _run(g) for i in range(0, len(steps), n)]


def _share(items, k, n):
    return items[k * len(items) // n:(k + 1) * len(items) // n]


def _blend(*lists):
    spots = [((i + 0.5) / len(items), k, item)
             for k, items in enumerate(lists) for i, item in enumerate(items)]
    return [item for *_, item in sorted(spots, key=lambda spot: spot[:2])]


def _witness(values):
    out = None
    for v in values:
        v = pltpu.bitcast(v, U32)
        for r in range(0, v.shape[0], 8):
            for c in range(0, v.shape[1], 128):
                out = v[r:r + 8, c:c + 128] if out is None else out | v[r:r + 8, c:c + 128]
    return out


def _pacer(ref, index, row=0):
    def pace(v):
        if ref.dtype == BF16 and ref.shape[-1] == 128:
            ref.bitcast(U32)[index, pl.ds(row, 8), :] = v
        elif ref.dtype == BF16:
            ref[index, pl.ds(row, 16), pl.ds(0, 128)] = _bf16(v)
        else:
            ref[index, pl.ds(row, 8), pl.ds(0, 128)] = pltpu.bitcast(v, ref.dtype)
    return pace


def _tie(pieces, result):
    for i, (pace, work, *lag) in enumerate(pieces):
        seen, m = work(), result(sum(lag))
        r = 8 * (i * (m.shape[0] // 8) // len(pieces))
        pace(_witness([m[r:r + 8]] + list(seen)))


def _mingle(steps, pieces, history=None):
    history = [] if history is None else history

    def both(step, mine):
        history.append(step())
        _tie([piece for piece in mine if piece],
             lambda lag: history[max(0, len(history) - 1 - lag)][:, :128])

    return [lambda step=step, mine=_share(pieces, i, len(steps)): both(step, mine)
            for i, step in enumerate(steps)]


def _now(pieces):
    for _, work, *_ in pieces:
        work()


def _dim_major(src, pace, shuf, put, swap, zero, lag=0, gap=0):
    def scatter(k, u):
        t = src(k, u)
        for h in range(128 // AD):
            shuf[k, pl.ds((4 * u + h) * PITCH, AD), :] = t[h * AD:(h + 1) * AD]
        return [t]

    def gather(d, i):
        def block(row1, col1, row2, col2):
            quarter, k = 2 * row1 + row2, 2 * col1 + col2
            if swap:
                quarter, k = k, quarter
            return jnp.concatenate(
                [shuf[k, pl.ds(8 * p * PITCH + quarter * AD // 4 + d, 8, stride=PITCH), :]
                 for p in range(2)], axis=0)
        outer = {b: [block(b // 2, b % 2, s // 2, s % 2) for s in range(4)] for b, _ in RHS[i]}
        return put(NOPS * i, d * NH, _operands(_combine(outer, RHS[i]), RHS))

    return ([x for k in range(4) for u in range(4)
             for x in [(pace, lambda k=k, u=u: scatter(k, u), lag)] + [None] * gap]
            + [(_pacer(shuf, 4 + zero), lambda d=d, i=i: gather(d, i))
               for d in range(AD // 4) for i in range(NOPS)])


def _kernel(ax_hbm, awqkv_hbm, awo_hbm, bx_hbm, c_hbm, wq_hbm, wuk_hbm, wuv_hbm,
            wo_hbm, out_hbm,
            offset, ctx, wo_raw, woop, awop, awoop, xa, xaop, awo_raw, shuf,
            sem_x, sem_c, sem_w, sem_a, sem_out):

    def cp_tile(src, row, col, dst, sem):
        def span(i):
            return pl.ds(pl.multiple_of(i * TILE, TILE), TILE)
        return pltpu.make_async_copy(src.at[span(row), span(col)], dst, sem)

    def cp_wo(u, s):
        return cp_tile(wo_hbm, u // 2, u % 2, wo_raw.at[s].bitcast(BF16), sem_w.at[6 + s])

    def cp_a():
        return ([pltpu.make_async_copy(ax_hbm.at[pl.ds(c * CH, CH)], xa.at[c], sem_a.at[0])
                 for c in range(NC)]
                + [pltpu.make_async_copy(awo_hbm.at[pl.ds(128 * t, 128), pl.ds(DC * h, DC)],
                                         awo_raw.at[t, pl.ds(128 * h, 128)], sem_a.at[1])
                   for t in range(8) for h in range(2)])

    def prep_wo(u, s, zero):
        def piece(r, i):
            outer = {b: [_f32(wo_raw[s, pl.ds((2 * a2 + b // 2) * (HD // 2) + r, 8),
                                       pl.ds((2 * (b % 2) + b2) * 128, 128)])
                         for a2 in range(2) for b2 in range(2)] for b, _ in RHS[i]}
            return _put(woop, lambda k: (u % 2, NOPS * i + k), pl.multiple_of(u // 2 * HD + 2 * r, 16),
                        _operands(_combine(outer, RHS[i]), RHS))
        return [(_pacer(wo_raw, 2 + zero), lambda r=r, i=i: piece(r, i))
                for r in range(0, HD // 2, 8) for i in range(NOPS)]

    def prep_awo(u, zero):
        n, half = u // 2, u % 2

        def put(i, row, values):
            return _put(awoop, lambda k: (n, i + k), 16 * half + row, values)
        return _dim_major(
            lambda k, t: awo_raw[4 * half + t, pl.ds(128 * n, 128), pl.ds(128 * k, 128)].astype(F32),
            _pacer(awo_raw, 8 + zero), shuf, put, False, zero)

    def prep_xa(c, zero):
        def piece(t, r, i):
            outer = {b: [xa[c, pl.ds((b // 2) * R + r2 * R // 2 + r, 16),
                            pl.ds(512 * t + (b % 2) * 256 + a2 * 128, 128)].astype(F32)
                for r2 in range(2) for a2 in range(2)] for b, _ in LHS[i]}
            return _put(xaop, lambda k: (NOPS * i + k, t), r, _operands(_combine(outer, LHS[i]), LHS))
        return [(_pacer(xa, NC + zero), lambda t=t, r=r, i=i: piece(t, r, i))
                for t in range(2) for r in range(0, R // 2, 16) for i in range(NOPS)]

    offset[:16] = jnp.zeros((16, 128), F32)
    shuf[0, :8] = offset[pl.ds(1, 8)]

    def heads(xop, cop, wq_raw, wkv_raw, qwop, kvwop, q_s, k_s, v_s, aw_raw, unit):
        xs, cs = xa, awo_raw
        wq32 = wq_hbm.bitcast(U32)
        wuk32 = wuk_hbm.bitcast(U32)
        wuv32 = wuv_hbm.bitcast(U32)

        def cp_x(c):
            return pltpu.make_async_copy(bx_hbm.at[pl.ds(c * CH, CH)], xs.at[c], sem_x.at[c])

        def cp_c(c):
            return pltpu.make_async_copy(c_hbm.at[pl.ds(c * CH, CH)], cs.at[c], sem_c.at[c])

        def cp_wkv(j, s):
            return [pltpu.make_async_copy(wuk32.at[:, j, :], wkv_raw.at[s], sem_w.at[s]),
                    pltpu.make_async_copy(wuv32.at[:, j, :], wkv_raw.at[2 + s], sem_w.at[2 + s])]

        def cp_wq(j, s):
            return [pltpu.make_async_copy(wq32.at[:, j, :], wq_raw.at[s], sem_w.at[4 + s])]

        def wo_unit(j):
            return jnp.maximum(j - 1, 0)

        def aw_unit(j):
            return jnp.clip(j - 1, 0, 3 * DM * DM // TILE ** 2 - 1)

        def cp_heads(j):
            return (cp_wkv(jnp.minimum(j + 2, NP - 1), j % 2)
                    + cp_wq(jnp.minimum(j + 1, NP - 1), j % 2))

        def cp_tiles(j):
            u = aw_unit(j)
            return [cp_wo(wo_unit(j), j % 2),
                    cp_tile(awqkv_hbm, u // 2 % 2, 2 * (u // 4) + u % 2, aw_raw.at[j % 2],
                            sem_w.at[8 + j % 2])]

        def prep_x(c):
            for t in range(2):
                blocks = [[
                    xs[c, pl.ds(r * R // 2, R // 2), pl.ds(k * DM // 4 + 128 * t, 128)].astype(F32)
                    for k in range(4)] for r in range(4)]
                ops = [v for i, j in COUPLES
                       for v in _square_forms(lambda r, k: blocks[r][k], i, j)]
                _put(xop, lambda n: (2 * (NQ * c + n) + t,), 0, ops)

        def prep_c(c):
            blocks = [[
                cs[c, pl.ds(r1 * R + r2 * R // 2, R // 2), pl.ds(a1 * 256 + a2 * 128, 128)].astype(F32)
                for r2 in range(2) for a2 in range(2)] for r1 in range(2) for a1 in range(2)]
            for i, outer in enumerate(_operands(blocks, LHS)):
                _put(cop, lambda k: (c, NOPS * i + k), 0, _operands(outer, LHS))

        def both_heads(raw, s, row):
            return _halves(raw[s, pl.ds(row, 16), :])

        def prep_wq(s, zero):
            def piece(r, couples, n):
                w = {k: both_heads(wq_raw, s, k * DM // 4 + r) for couple in couples for k in couple}
                return _put(qwop, lambda k: (n + k,), r,
                            [v for i, j in couples for v in _pair_forms(w.get, i, j)])
            parts = (COUPLES[:6], 0), (COUPLES[6:], 15)
            return [(_pacer(wq_raw, 2 + zero), lambda r=r, part=part: piece(r, *part))
                    for r in range(0, DM // 4, 16) for part in parts]

        def prep_wkv(j, s, slot, zero):
            total, inverse = {}, {}

            def measure(n, r):
                w = wkv_raw[2 * n + s, pl.ds(r, 64), :]
                w = jnp.abs(pltpu.bitcast(w, F32)) + jnp.abs(pltpu.bitcast(w << 16, F32))
                w = jnp.sum(w.reshape(8, 8, 128), axis=0)
                total[n] = total[n] + w if r else w
                return [total[n]]

            def size(n):
                both = jnp.sum(jnp.sum(total[n], axis=1, keepdims=True), axis=0, keepdims=True)
                both = jnp.broadcast_to(jnp.clip(both, 2.0 ** -100, 2.0 ** 100), (8, 128))
                power = pltpu.bitcast(both, U32) & jnp.uint32(0x7F800000)
                unit[n, j] = pltpu.bitcast(power, F32)
                inverse[n] = pltpu.bitcast(jnp.uint32(0x7F000000) - power, F32)
                return [power]

            def piece(r, i):
                outer = {b: [v * jnp.concatenate([inverse[b % 2]] * 2, axis=0) for a2 in range(2)
                             for v in both_heads(wkv_raw, 2 * (b % 2) + s,
                                                 (b // 2) * 256 + a2 * 128 + r)]
                         for b, _ in RHS[i]}
                return _put(kvwop, lambda k: (slot + (NOPS * i + k),), r,
                            _operands(_combine(outer, RHS[i]), RHS))

            pace = _pacer(wkv_raw, 4 + zero)
            return ([(pace, lambda n=n, r=r: measure(n, r))
                     for n in range(2) for r in range(0, DC, 64)]
                    + [(pace, lambda n=n: size(n)) for n in range(2)],
                    [(_pacer(xop, 2 * NQ * NC + zero), lambda: list(inverse.values()))]
                    + [(pace, lambda r=r, i=i: piece(r, i))
                       for r in range(0, 128, 16) for i in range(NOPS)])

        def prep_aw(u, s, zero):
            def put(i, row, values):
                return _put(awop, lambda k: (u // 2, i + k), pl.multiple_of(16 * (u % 2), 16) + row,
                            values)
            return _dim_major(
                lambda k, t: aw_raw[s, pl.ds(128 * k, 128), pl.ds(128 * t, 128)].astype(F32).T,
                _pacer(xop, 2 * NQ * NC + zero), shuf, put, True, zero, lag=5, gap=2)

        def q_proj(scale, c):
            def done(r, *both):
                for h, val in enumerate(both):
                    _store(q_s, 0, c * R + r * (R // 4), h * HD, val * scale)
            return _couple_product(lambda i: _beside(_load(xop, 2 * (NQ * c + i) + t) for t in range(2)),
                                   lambda i: _load(qwop, i), done)

        def kv_proj(c, slot):
            def done(o, val):
                row, col = _corner(o, R // 4, HD)
                _store((k_s, v_s)[col // (2 * HD)], 0, c * R + row, col % (2 * HD), val)
            return _block_product(lambda i: _load(cop, c, i), lambda i: _load(kvwop, slot + i), done)

        def q_scale(j):
            return unit[0, j, :1] * (HD ** -0.5 * LOG2E)

        def scores(h, blk):
            n = (blk + 1) * R
            s = lax.dot_general(_bf16(q_s[0, pl.ds(blk * R // 2, R // 2), pl.ds(h * HD, HD)]),
                                _bf16(k_s[0, :n // 2, pl.ds(h * HD, HD)]),
                                NT, preferred_element_type=F32)
            row = lax.broadcasted_iota(jnp.int32, (R, R), 0)
            col = lax.broadcasted_iota(jnp.int32, (R, R), 1)
            diag = jnp.where(col <= row, s[:, n - R:], MASKED)
            return diag if blk == 0 else jnp.concatenate([s[:, :n - R], diag], axis=1)

        def attend(scale, h, blk, s):
            n = (blk + 1) * R
            p = jnp.exp2(s - jnp.max(s, axis=1, keepdims=True))
            inv = _recip(jnp.sum(p, axis=1, keepdims=True)) * scale
            o = lax.dot_general(p.astype(BF16), _bf16(v_s[0, :n // 2, pl.ds(h * HD, HD)]), NN,
                                preferred_element_type=F32)
            return o * inv

        def pair_attention(j, zero, filler, sides, slack):
            blocks = [(h, 2 * c + u) for c in reversed(range(NC)) for u in (1, 0) for h in (0, 1)]
            plan = {}
            for pieces, span in sides:
                tiles = [(b, t) for b in blocks[span] for t in range(b[1] + 1)]
                for n, tile in enumerate(tiles):
                    plan.setdefault(tile, []).extend(_share(pieces, n, len(tiles)))

            def paced_scores(h, blk):
                s = scores(h, blk)
                for t in range(blk + 1):
                    _tie(plan.get(((h, blk), t), []), lambda lag: s[:, t * R:(t + 1) * R])
                return s

            todo, done = [[]] * 8, []
            v_scale = unit[1, j, :1]
            ahead = [paced_scores(*blocks[0])]
            for n, (h, blk) in enumerate(blocks):
                ahead += [paced_scores(*b) for b in blocks[n + 1:n + 2]]
                _run(todo[2 * (n % 4)])
                done.append(attend(v_scale, h, blk, ahead.pop(0)))
                _store(ctx, 0, pl.multiple_of(j * (S // 2), S // 2) + blk * (R // 2), h * HD, done[-1])
                if len(done) > slack:
                    _pacer(q_s, zero, S // 2)(_witness([done.pop(0)]))
                _run(todo[2 * (n % 4) + 1])
                if n % 4 == 3:
                    todo = filler(blk // 2)
            _run(sum(todo, []))

        c_parts = ((7, 6), (5, 4), (3, 2), (1, 0))
        x_parts = tuple(reversed(range(NC)))
        stages = ([cp_wkv(0, 0)] + [[cp_c(c) for c in part] for part in c_parts]
                  + [[cp_x(c)] for c in x_parts] + [cp_wq(1, 0)])
        stages[len(c_parts)] += cp_wq(0, 1)
        stages[len(c_parts) + 1] += cp_wkv(1, 1)

        def issue(i, zero):
            for k, stage in enumerate(stages):
                @pl.when(i == k)
                def _(stage=stage):
                    for cp in stage:
                        cp.start()
            return zero + i // NP

        zero = lax.fori_loop(0, len(stages), issue, jnp.int32(0))

        aw_raw[0] = jnp.zeros(aw_raw.shape[1:], BF16)
        wo_raw[0] = jnp.zeros(wo_raw.shape[1:], U32)
        for cp in stages[0]:
            cp.wait()
        _now(sum(prep_wkv(0, 0, SLOT, zero), []))
        for n, part in enumerate(c_parts):
            for cp in stages[1 + n]:
                cp.wait()
            if n == 0:
                for cp in cp_wkv(2, 0):
                    cp.start()
            side = prep_wq(1, zero) if n == len(c_parts) - 1 else []
            for k, c in enumerate(part):
                prep_c(c)
                _run(_mingle(kv_proj(c, SLOT), _share(side, k, len(part))))
        scale, side = q_scale(0), sum(prep_wkv(1, 1, 0, zero), [])
        for n, c in enumerate(x_parts):
            for cp in stages[1 + len(c_parts) + n]:
                cp.wait()
            prep_x(c)
            _run(_mingle(q_proj(scale, c), _share(side, n, NC)))

        def pair_step(j, zero):
            for cp in cp_heads(j):
                cp.wait()

            @pl.when(j > 0)
            def _():
                for cp in cp_tiles(j):
                    cp.wait()

            @pl.when(j == RING)
            def _():
                words = kvwop.bitcast(U32)
                words[:SLOT] = words[RING * SLOT:]
                for cp in cp_a():
                    cp.start()

            for cp in cp_heads(j + 1) + cp_tiles(j + 1):
                cp.start()
            slot = (j % RING) * SLOT
            scale = q_scale(j + 1)
            sizes, operands = prep_wkv(j + 2, j % 2, slot + SLOT, zero)
            side = [None] * 24 + _blend(prep_aw(aw_unit(j), j % 2, zero),
                                        sizes + [None] * 12 + operands)
            q_steps = sum((q_proj(scale, c) for c in reversed(range(NC))), [])
            history = []

            def filler(c):
                q = _share(q_steps, NC - 3 - c, NC - 2) if c < NC - 2 else []
                kv = kv_proj(c, slot)
                slots = []
                for n in range(4):
                    mine = _share(kv, n, 4)
                    early = len(mine) - len(mine) * 3 // 4
                    slots += [mine[:early] + _share(q, n, 4), mine[early:]]
                along = _share(side, NC - 2 - c, NC - 1) if c < NC - 1 else []
                steps = iter(_mingle(sum(slots, []), along, history))
                return [[next(steps) for _ in slot] for slot in slots]

            pair_attention(j, zero, filler, [(prep_wo(wo_unit(j), j % 2, zero), slice(10, None)),
                                             (prep_wq(j % 2, zero), slice(2, 12))], 3)
            return zero + j // NP

        zero = lax.fori_loop(0, NP - 1, pair_step, zero)

        @pl.loop(0, 2)
        def _(i):
            _pacer(shuf, 4 + zero * i)(jnp.zeros((8, 128), U32))

        for cp in cp_heads(NP - 1) + cp_tiles(NP - 1) + cp_a():
            cp.wait()
        cp_wo(NP - 1, 0).start()
        side = _blend(prep_wo(NP - 2, 1, zero), prep_awo(0, zero), prep_xa(zero, zero))
        pair_attention(NP - 1, zero, lambda c: [[]] * 8, [(side, slice(2, None))], 5)
        return zero

    def rows(zero, aoop, aqkv, oop, out_s):
        @pl.loop(0, 2)
        def _(i):
            aqkv[pl.ds(8 + 8 * i, 8), :HALO, :] = jnp.zeros((8, HALO, 128), F32)

        def cp_out(c, half):
            return pltpu.make_async_copy(
                out_s.at[half, c],
                out_hbm.at[pl.ds(pl.multiple_of(c * CH, CH), CH), pl.ds(half * DM, DM)],
                sem_out.at[half * NC + c])

        def cp_last(row, col, n, sem):
            return pltpu.make_async_copy(
                out_s.at[0, NC - 1, pl.ds(row, n), pl.ds(col, DM // 2)],
                out_hbm.at[pl.ds((NC - 1) * CH + row, n), pl.ds(col, DM // 2)], sem_x.at[sem])

        def prep_ctx(c, zero):
            base = pl.multiple_of(c * R, R)

            def piece(m, r, i):
                outer = {b: [_f32(ctx[0, pl.ds(base + ((2 * m + a2) * (S // 2) + (b // 2) * 64
                                                         + r2 * 32 + r), 8),
                                        pl.ds((b % 2) * HD, HD)])
                             for r2 in range(2) for a2 in range(2)] for b, _ in LHS[i]}
                return _put(oop, lambda k: (NOPS * i + k, m), 2 * r,
                            _operands(_combine(outer, LHS[i]), LHS))
            return [(_pacer(ctx, zero, NP * S // 2), lambda m=m, r=r, i=i: piece(m, r, i))
                    for m in range(NP // 2) for r in range(0, 32, 8) for i in range(NOPS)]

        def out_proj(half, c, lhs, rhs):
            steps = []
            for t in range(2):
                def done(o, val, t=t):
                    row, col = _corner(o, R // 2, 128)
                    out_s[half, c, pl.ds(row, R // 2), pl.ds(512 * t + col, 128)] = val.astype(BF16)
                steps += _block_product(lhs, lambda i, t=t: _load(rhs, t, i), done)
            return steps

        def b_out_proj(c):
            return out_proj(1, c, lambda i: _beside(_load(oop, i, m) for m in range(NP // 2)), woop)

        def a_out_proj(c, zero):
            return out_proj(0, c, lambda i: _bf16(aoop[zero + i]), awoop)

        def a_proj():
            steps = []
            for part in range(3):
                for t in range(2):
                    def done(o, val, part=part, t=t):
                        if part == 0:
                            val = val * (AD ** -0.5 * LOG2E)
                        row, plane = _corner(o, R // 2, 2)
                        aqkv[8 * part + plane + t, pl.ds(HALO + row, R // 2), :] = val

                    def rhs(i, part=part, t=t):
                        return _beside(_load(awop, 2 * part + m, i, pl.ds(64 * t, 64)) for m in range(2))
                    steps += _block_product(lambda i: _beside(_load(xaop, i, m) for m in range(2)),
                                            rhs, done, NT)
            return steps

        def a_attention(c, zero):
            query, logit, prob, mixed = {}, {}, {}, {}

            def dot(r, w):
                tot = None
                for t in range(8):
                    if (r, t) not in query:
                        query[r, t] = aqkv[t, pl.ds(HALO + r, 8), :]
                    pr = query[r, t] * aqkv[8 + t, pl.ds(HALO + r - DIL * w, 8), :]
                    tot = pr if tot is None else tot + pr
                logit[r, w] = tot
                if w == WIN - 1:
                    weights(r)
                return [tot]

            def weights(r):
                logits = [logit[r, w] for w in range(WIN)]
                logits = [x + pltpu.roll(x, 64, 1) for x in logits]
                logits = [x + pltpu.roll(x, 32, 1) for x in logits]
                if r < (WIN - 1) * DIL:
                    pos = c * CH + r + lax.broadcasted_iota(jnp.int32, (8, 128), 0)
                    logits = [x if w == 0 else jnp.where(pos >= DIL * w, x, MASKED)
                              for w, x in enumerate(logits)]
                top = logits[0]
                for x in logits[1:]:
                    top = jnp.maximum(top, x)
                e = [jnp.exp2(x - top) for x in logits]
                tot = e[0]
                for x in e[1:]:
                    tot = tot + x
                inv = _recip(tot)
                prob[r] = [x * inv for x in e]

            def mix(r, t, d, q):
                tot = None
                for w in range(WIN):
                    pr = prob[r + d][w] * aqkv[16 + t + 2 * q, pl.ds(HALO + r + d - DIL * w, 8), :]
                    tot = pr if tot is None else tot + pr
                mixed[r, t, d, q] = tot
                return [tot]

            def operands(r, t, i):
                outer = {b: [jnp.concatenate(
                    [mixed[r, t, (b // 2) * R + r2 * R // 2 + e, 2 * (b % 2) + a2] for e in (0, 8)],
                    axis=0) for r2 in range(2) for a2 in range(2)] for b, _ in LHS[i]}
                ops = _operands(_combine(outer, LHS[i]), LHS)
                for k, v in enumerate(ops):
                    _store(aoop, NOPS * i + k, r // 2, 128 * t, v)
                return ops

            groups = [d + e for d in range(0, CH, R // 2) for e in (0, 8)]

            def dots(r):
                return [lambda d=d, w=w: dot(r + d, w) for d in groups for w in range(WIN)]

            def mixes(r):
                return [work for t in range(2) for work in
                        [lambda t=t, d=d, q=q: mix(r, t, d, q) for d in groups for q in range(4)]
                        + [lambda t=t, i=i: operands(r, t, i) for i in range(NOPS)]]

            work = dots(0)
            for r in range(16, R // 2, 16):
                work += _blend(dots(r), mixes(r - 16))
            work += mixes(R // 2 - 16)
            return [(_pacer(aqkv, zero, HALO + CH), lambda g=work[i:i + 2]: sum((w() for w in g), []))
                    for i in range(0, len(work), 2)]

        cp_wo(NP - 1, 0).wait()
        _run(_mingle(_group(a_proj(), 2),
                     _blend(prep_ctx(0, zero), sum((prep_awo(u, zero) for u in range(1, 4)), []),
                            prep_wo(NP - 1, 0, zero))))

        def attention_step(c, zero):
            steps = b_out_proj(c)
            _run(_mingle(steps[:-2], a_attention(c, zero)) + steps[-2:])
            cp_out(c, 1).start()

        def chunk_step(c, zero):
            attention_step(c, zero)
            aqkv[8:, :HALO, :] = aqkv[8:, CH:CH + HALO, :]
            side = prep_ctx(c + 1, zero)
            early = len(side) // 4
            steps = _group(a_out_proj(c, zero), 2)
            _run(_mingle(steps[:-3], _blend(prep_xa(c + 1, zero), side[:early])) + steps[-3:])
            cp_out(c, 0).start()
            steps = _group(a_proj(), 2)
            _run(_mingle(steps[:-4], side[early:]) + steps[-4:])
            return zero + c // NC

        zero = lax.fori_loop(0, NC - 1, chunk_step, zero)

        attention_step(NC - 1, zero)
        steps = a_out_proj(NC - 1, zero)
        parts = [cp_last(0, 0, CH, 0), cp_last(R, DM // 2, R, 1), cp_last(0, DM // 2, R, 2)]
        for cp, part in zip(parts, (steps[:NOPS * NOPS], steps[NOPS * NOPS:-NOPS], steps[-NOPS:])):
            _run(part)
            cp.start()
        for cp in ([cp_out(c, 1) for c in range(NC)] + [cp_out(c, 0) for c in range(NC - 1)] + parts):
            cp.wait()

    vmem = pltpu.VMEM
    zero = pl.run_scoped(
        heads,
        vmem((2 * NQ * NC + 1, R // 2, 128), BF16),
        vmem((NC, NOPS * NOPS, R // 2, 128), BF16),
        vmem((3, DM, HD), U32),
        vmem((5, DC, HD), U32),
        vmem((NQ, DM // 4, 128), BF16),
        vmem(((RING + 1) * SLOT, 128, 128), BF16),
        vmem((1, S // 2 + 16, 2 * HD), U32),
        vmem((1, S // 2, 2 * HD), U32),
        vmem((1, S // 2, 2 * HD), U32),
        vmem((2, TILE, TILE), BF16),
        vmem((2, NP + 2, 8, 128), F32),
    )
    pl.run_scoped(
        lambda *refs: rows(zero, *refs),
        vmem((NOPS * NOPS, R // 4, DM // 4), U32),
        vmem((24, HALO + CH + 16, 128), F32),
        vmem((NOPS * NOPS, NP // 2, R // 2, HD), BF16),
        vmem((2, NC, CH, DM), BF16),
    )


@jax.jit
def pallas_concat_heads__sliding_local_dilated__compressed_kv_cla__prompt_kernel(
    A_x: jax.Array,
    A_wqkv: jax.Array,
    A_wo: jax.Array,
    B_x: jax.Array,
    B_c_kv: jax.Array,
    B_w_q: jax.Array,
    B_w_uk: jax.Array,
    B_w_uv: jax.Array,
    B_w_o: jax.Array,
):
    vmem = pltpu.VMEM
    dma = pltpu.SemaphoreType.DMA
    scratch = [
        vmem((24, 128), F32),
        vmem((1, NP * S // 2 + 16, 2 * HD), U32),
        vmem((3, TILE // 2, TILE), U32),
        vmem((2, NOPS * NOPS, NP * HD // 2, 128), BF16),
        vmem((6, NOPS * NOPS, DM // 4, 128), BF16),
        vmem((2, NOPS * NOPS, DM // 4, 128), BF16),
        vmem((NC + 1, CH, DM), BF16),
        vmem((NOPS * NOPS, 2, R // 2, 128), BF16),
        vmem((NC + 1, CH, DC), BF16),
        vmem((5, 16 * PITCH + 16, 128), F32),
        dma((NC,)), dma((NC,)), dma((10,)), dma((2,)), dma((2 * NC,)),
    ]
    out = pl.pallas_call(
        _kernel,
        out_shape=jax.ShapeDtypeStruct((S, 2 * DM), BF16),
        in_specs=[pl.BlockSpec(memory_space=pl.ANY)] * 9,
        out_specs=pl.BlockSpec(memory_space=pl.ANY),
        scratch_shapes=scratch,
        compiler_params=pltpu.CompilerParams(vmem_limit_bytes=124 * 2**20),
        name="fused_local_and_latent_attention",
    )(
        A_x.reshape(S, DM), A_wqkv, A_wo,
        B_x.reshape(S, DM), B_c_kv.reshape(S, DC),
        B_w_q, B_w_uk, B_w_uv, B_w_o.reshape(NH * HD, DM),
    )
    return out.reshape(1, S, 2 * DM)
```

```python
import math

import jax
import jax.numpy as jnp
from jax import lax
import jax.experimental.pallas as pl
import jax.experimental.pallas.tpu as pltpu

F32, BF16, U32 = jnp.float32, jnp.bfloat16, jnp.uint32

S = 2048
DM = 1024
DC = 512
NH = 32
HD = 128
AD = 32
WIN, DIL = 8, 2

R = 128
CH = 2 * R
NC = S // CH
NP = NH // 2
HALO = 16
PITCH = 33
TILE = 512
LOG2E = math.log2(math.e)
MASKED = -1e9 * LOG2E

NN = (((1,), (0,)), ((), ()))
NT = (((1,), (1,)), ((), ()))

LHS = (((0, 1), (3, 1)), ((2, 1), (3, 1)), ((0, 1),), ((3, 1),),
       ((0, 1), (1, 1)), ((2, 1), (0, -1)), ((1, 1), (3, -1)))
RHS = (((0, 1), (3, 1)), ((0, 1),), ((1, 1), (3, -1)), ((2, 1), (0, -1)),
       ((3, 1),), ((0, 1), (1, 1)), ((2, 1), (3, 1)))
PRODUCTS = ((2, ((1, 1), (3, 1))), (4, ((0, -1), (1, 1))), (3, ((0, 1), (2, 1))),
            (1, ((2, 1), (3, -1))), (5, ((3, 1),)), (0, ((0, 1), (3, 1))),
            (6, ((0, 1),)))
NOPS = len(PRODUCTS)

SLOPE = (-1.5, -0.5, 0.5, 1.5)
COUPLES = tuple((i, j) for j in range(4) for i in range(j, -1, -1))
NQ = sum(2 if i == j else 3 for i, j in COUPLES)

SLOT = NOPS * NOPS


def _square_forms(x, i, j):
    if i == j:
        p = q = x(i, i)
        for k in range(4):
            if k != i:
                p, q = p - x(k, i), q + x(i, k)
        return [p, q]
    return [x(i, j) + x(j, i), x(i, j), x(j, i)]


def _pair_forms(w, i, j):
    (a0, a1), (b0, b1) = w(i), w(j)
    if i == j:
        return [a0, SLOPE[i] * a0 + a1]
    return [(SLOPE[i] * a0 + a1) - (SLOPE[j] * b0 + b1),
            SLOPE[i] * (b0 - a0) + (b1 - a1), SLOPE[j] * (b0 - a0) + (b1 - a1)]


def _couple_product(lhs, rhs, done):
    first, second, steps = {}, {}, []

    def add(i, j, m):
        if i == j:
            first[i], second[i] = m
            return
        t, gap = m[0] + m[1] + m[2], SLOPE[j] - SLOPE[i]
        t = t if gap == 1 else t * (1 / gap)
        first[i], first[j] = first[i] - t, first[j] - t
        second[i], second[j] = second[i] + m[1], second[j] - m[2]
        if j == 3:
            for r in (i,) if i else (0, 3):
                done(r, first[r], second[r] - SLOPE[r] * first[r])

    for i, j in COUPLES:
        got, n = [], 2 if i == j else 3
        for _ in range(n):
            def step(i=i, j=j, got=got, n=n, k=len(steps)):
                got.append(lax.dot_general(lhs(k), rhs(k), NN, preferred_element_type=F32))
                if len(got) == n:
                    add(i, j, got)
                return got[-1]
            steps.append(step)
    return steps


def _combine(blocks, terms):
    if isinstance(blocks[terms[0][0]], list):
        return [_combine({b: blocks[b][i] for b, _ in terms}, terms) for i in range(4)]
    out = blocks[terms[0][0]]
    for i, sign in terms[1:]:
        out = out + blocks[i] if sign > 0 else out - blocks[i]
    return out


def _operands(blocks, side):
    return [_combine(blocks, terms) for terms in side]


def _block_product(lhs, rhs, done, dims=NN, levels=2):
    if levels == 0:
        def step():
            m = lax.dot_general(lhs(0), rhs(0), dims, preferred_element_type=F32)
            done((), m)
            return m
        return [step]

    held, steps = {}, []
    inner = NOPS ** (levels - 1)
    for n, (i, outs) in enumerate(PRODUCTS):
        later = {o for _, others in PRODUCTS[n + 1:] for o, _ in others}

        def add(sub, m, outs=outs, later=later):
            for o, sign in outs:
                if (o, sub) not in held:
                    held[o, sub] = m, sign
                else:
                    c, s = held[o, sub]
                    held[o, sub] = (m - c if s < 0 else c + m if sign > 0 else c - m), 1
                if o not in later:
                    done((o, *sub), held.pop((o, sub))[0])

        steps += _block_product(lambda k, i=i: lhs(i * inner + k),
                                lambda k, i=i: rhs(i * inner + k), add, dims, levels - 1)
    return steps


def _corner(o, rows, cols):
    return (2 * (o[0] // 2) + o[1] // 2) * rows, (2 * (o[0] % 2) + o[1] % 2) * cols


def _bf16(words):
    return pltpu.bitcast(words, BF16)


def _halves(words):
    lo = pltpu.bitcast(words << 16, F32)
    hi = pltpu.bitcast(words & jnp.uint32(0xFFFF0000), F32)
    return lo, hi


def _f32(words):
    return _bf16(words).astype(F32)


def _load(ref, *index):
    return _bf16(ref.bitcast(U32)[index])


def _beside(tiles):
    return jnp.concatenate(list(tiles), axis=1)


def _put(ref, index, row, values):
    for k, v in enumerate(values):
        ref[(*index(k), pl.ds(row, v.shape[0]), slice(None))] = v.astype(BF16)
    return [v[:8] for v in values]


def _store(words, index, row, col, x):
    matrix = words.bitcast(BF16).at[index]
    matrix[pl.ds(pl.multiple_of(2 * row, 16), x.shape[0]), pl.ds(col, x.shape[1])] = x.astype(BF16)


def _part(i, size, row=0, n=None):
    return pl.ds(pl.multiple_of(i * size + row, 8), size if n is None else n)


def _recip(x):
    r = pltpu.reciprocal(x, approx=True)
    return r * (2.0 - x * r)


def _run(steps):
    out = None
    for step in steps:
        out = step()
    return out


def _group(steps, n):
    return [lambda g=steps[i:i + n]: _run(g) for i in range(0, len(steps), n)]


def _share(items, k, n):
    return items[k * len(items) // n:(k + 1) * len(items) // n]


def _blend(*lists):
    spots = [((i + 0.5) / len(items), k, item)
             for k, items in enumerate(lists) for i, item in enumerate(items)]
    return [item for *_, item in sorted(spots, key=lambda spot: spot[:2])]


def _witness(values):
    out = None
    for v in values:
        v = pltpu.bitcast(v, U32)
        for r in range(0, v.shape[0], 8):
            for c in range(0, v.shape[1], 128):
                out = v[r:r + 8, c:c + 128] if out is None else out | v[r:r + 8, c:c + 128]
    return out


def _pacer(ref, index, row=0):
    def pace(v):
        if ref.dtype == BF16 and ref.shape[-1] == 128:
            ref.bitcast(U32)[index, pl.ds(row, 8), :] = v
        elif ref.dtype == BF16:
            ref[index, pl.ds(row, 16), pl.ds(0, 128)] = _bf16(v)
        else:
            ref[index, pl.ds(row, 8), pl.ds(0, 128)] = pltpu.bitcast(v, ref.dtype)
    return pace


def _tie(pieces, result):
    for i, (pace, work, *lag) in enumerate(pieces):
        seen, m = work(), result(sum(lag))
        r = 8 * (i * (m.shape[0] // 8) // len(pieces))
        pace(_witness([m[r:r + 8]] + list(seen)))


def _mingle(steps, pieces, history=None):
    history = [] if history is None else history

    def both(step, mine):
        history.append(step())
        _tie([piece for piece in mine if piece],
             lambda lag: history[max(0, len(history) - 1 - lag)][:, :128])

    return [lambda step=step, mine=_share(pieces, i, len(steps)): both(step, mine)
            for i, step in enumerate(steps)]


def _now(pieces):
    for _, work, *_ in pieces:
        work()


def _dim_major(src, pace, shuf, put, swap, zero, lag=0, gap=0):
    def scatter(k, u):
        t = src(k, u)
        for h in range(128 // AD):
            shuf[k, pl.ds((4 * u + h) * PITCH, AD), :] = t[h * AD:(h + 1) * AD]
        return [t]

    def gather(d, i):
        def block(row1, col1, row2, col2):
            quarter, k = 2 * row1 + row2, 2 * col1 + col2
            if swap:
                quarter, k = k, quarter
            return jnp.concatenate(
                [shuf[k, pl.ds(8 * p * PITCH + quarter * AD // 4 + d, 8, stride=PITCH), :]
                 for p in range(2)], axis=0)
        outer = {b: [block(b // 2, b % 2, s // 2, s % 2) for s in range(4)] for b, _ in RHS[i]}
        return put(NOPS * i, d * NH, _operands(_combine(outer, RHS[i]), RHS))

    return ([x for k in range(4) for u in range(4)
             for x in [(pace, lambda k=k, u=u: scatter(k, u), lag)] + [None] * gap]
            + [(_pacer(shuf, 4 + zero), lambda d=d, i=i: gather(d, i))
               for d in range(AD // 4) for i in range(NOPS)])


def _kernel(ax_hbm, awqkv_hbm, awo_hbm, bx_hbm, c_hbm, wq_hbm, wuk_hbm, wuv_hbm,
            wo_hbm, out_hbm,
            offset, ctx, wo_raw, woop, awop, awoop0, xa, xaop, awo_raw, shuf,
            sem_x, sem_c, sem_w, sem_a, sem_out):

    def cp_tile(src, row, col, dst, sem):
        def span(i):
            return pl.ds(pl.multiple_of(i * TILE, TILE), TILE)
        return pltpu.make_async_copy(src.at[span(row), span(col)], dst, sem)

    def cp_wo(u, s):
        return cp_tile(wo_hbm, u // 2, u % 2, wo_raw.at[0, _part(s, TILE // 2)].bitcast(BF16), sem_w.at[6 + s])

    def cp_a():
        return ([pltpu.make_async_copy(ax_hbm.at[pl.ds(c * CH, CH)], xa.at[c], sem_a.at[0])
                 for c in range(NC)]
                + [pltpu.make_async_copy(awo_hbm.at[pl.ds(128 * t, 128), pl.ds(DC * h, DC)],
                                         awo_raw.at[t, pl.ds(128 * h, 128)], sem_a.at[1])
                   for t in range(8) for h in range(2)])

    def prep_wo(u, s, zero):
        def piece(r, i):
            outer = {b: [_f32(wo_raw[0, _part(s, TILE // 2, (2 * a2 + b // 2) * (HD // 2) + r, 8),
                                       pl.ds((2 * (b % 2) + b2) * 128, 128)])
                         for a2 in range(2) for b2 in range(2)] for b, _ in RHS[i]}
            return _put(woop, lambda k: (u % 2, NOPS * i + k), pl.multiple_of(u // 2 * HD + 2 * r, 16),
                        _operands(_combine(outer, RHS[i]), RHS))
        return [(_pacer(wo_raw, zero, TILE), lambda r=r, i=i: piece(r, i))
                for r in range(0, HD // 2, 8) for i in range(NOPS)]

    def prep_awo(dst, n, half, zero):
        def put(i, row, values):
            return _put(dst, lambda k: (i + k,), 16 * half + row, values)
        return _dim_major(
            lambda k, t: awo_raw[4 * half + t, pl.ds(128 * n, 128), pl.ds(128 * k, 128)].astype(F32),
            _pacer(awo_raw, 8 + zero), shuf, put, False, zero)

    def prep_xa(c, zero):
        def piece(t, r, i):
            outer = {b: [xa[c, pl.ds((b // 2) * R + r2 * R // 2 + r, 16),
                            pl.ds(512 * t + (b % 2) * 256 + a2 * 128, 128)].astype(F32)
                for r2 in range(2) for a2 in range(2)] for b, _ in LHS[i]}
            return _put(xaop, lambda k: (NOPS * i + k, t), r, _operands(_combine(outer, LHS[i]), LHS))
        return [(_pacer(xa, NC + zero), lambda t=t, r=r, i=i: piece(t, r, i))
                for t in range(2) for r in range(0, R // 2, 16) for i in range(NOPS)]

    offset[:16] = jnp.zeros((16, 128), F32)
    shuf[0, :8] = offset[pl.ds(1, 8)]

    def heads(xop, cop, wq_raw, wkv_raw, qwop, kvwop, q_s, k_s, v_s, aw_raw, unit):
        xs, cs = xa, awo_raw
        wq32 = wq_hbm.bitcast(U32)
        wuk32 = wuk_hbm.bitcast(U32)
        wuv32 = wuv_hbm.bitcast(U32)

        def cp_x(c):
            return pltpu.make_async_copy(bx_hbm.at[pl.ds(c * CH, CH)], xs.at[c], sem_x.at[c])

        def cp_c(c):
            return pltpu.make_async_copy(c_hbm.at[pl.ds(c * CH, CH)], cs.at[c], sem_c.at[c])

        def cp_wkv(j, s):
            return [pltpu.make_async_copy(w.at[:, j, :], wkv_raw.at[0, _part(2 * n + s, DC)],
                                          sem_w.at[2 * n + s]) for n, w in enumerate((wuk32, wuv32))]

        def cp_wq(j, s):
            return [pltpu.make_async_copy(wq32.at[:, j, :], wq_raw.at[0, _part(s, DM)], sem_w.at[4 + s])]

        def wo_unit(j):
            return jnp.maximum(j - 1, 0)

        def aw_unit(j):
            return jnp.clip(j - 1, 0, 3 * DM * DM // TILE ** 2 - 1)

        def cp_heads(j):
            return (cp_wkv(jnp.minimum(j + 2, NP - 1), j % 2)
                    + cp_wq(jnp.minimum(j + 1, NP - 1), j % 2))

        def cp_tiles(j):
            u = aw_unit(j)
            return [cp_wo(wo_unit(j), j % 2),
                    cp_tile(awqkv_hbm, u // 2 % 2, 2 * (u // 4) + u % 2, aw_raw.at[j % 2],
                            sem_w.at[8 + j % 2])]

        def prep_x(c):
            for t in range(2):
                blocks = [[
                    xs[c, pl.ds(r * R // 2, R // 2), pl.ds(k * DM // 4 + 128 * t, 128)].astype(F32)
                    for k in range(4)] for r in range(4)]
                ops = [v for i, j in COUPLES
                       for v in _square_forms(lambda r, k: blocks[r][k], i, j)]
                _put(xop, lambda n: (2 * (NQ * c + n) + t,), 0, ops)

        def prep_c(c):
            blocks = [[
                cs[c, pl.ds(r1 * R + r2 * R // 2, R // 2), pl.ds(a1 * 256 + a2 * 128, 128)].astype(F32)
                for r2 in range(2) for a2 in range(2)] for r1 in range(2) for a1 in range(2)]
            for i, outer in enumerate(_operands(blocks, LHS)):
                _put(cop, lambda k: (c, NOPS * i + k), 0, _operands(outer, LHS))

        def both_heads(raw, rows):
            return _halves(raw[0, rows, :])

        def prep_wq(s, zero):
            def piece(r, couples, n):
                w = {k: both_heads(wq_raw, _part(s, DM, k * DM // 4 + r, 16))
                     for couple in couples for k in couple}
                return _put(qwop, lambda k: (n + k,), r,
                            [v for i, j in couples for v in _pair_forms(w.get, i, j)])
            parts = (COUPLES[:6], 0), (COUPLES[6:], 15)
            return [(_pacer(wq_raw, zero, 2 * DM), lambda r=r, part=part: piece(r, *part))
                    for r in range(0, DM // 4, 16) for part in parts]

        def prep_wkv(j, s, slot, zero):
            total, inverse = {}, {}

            def measure(n, r):
                w = wkv_raw[0, _part(2 * n + s, DC, r, 64), :]
                w = jnp.abs(pltpu.bitcast(w, F32)) + jnp.abs(pltpu.bitcast(w << 16, F32))
                w = jnp.sum(w.reshape(8, 8, 128), axis=0)
                total[n] = total[n] + w if r else w
                return [total[n]]

            def size(n):
                both = jnp.sum(jnp.sum(total[n], axis=1, keepdims=True), axis=0, keepdims=True)
                both = jnp.broadcast_to(jnp.clip(both, 2.0 ** -100, 2.0 ** 100), (8, 128))
                power = pltpu.bitcast(both, U32) & jnp.uint32(0x7F800000)
                unit[n, j] = pltpu.bitcast(power, F32)
                inverse[n] = pltpu.bitcast(jnp.uint32(0x7F000000) - power, F32)
                return [power]

            def piece(r, i):
                outer = {b: [v * jnp.concatenate([inverse[b % 2]] * 2, axis=0) for a2 in range(2)
                             for v in both_heads(wkv_raw, _part(2 * (b % 2) + s, DC,
                                                                (b // 2) * 256 + a2 * 128 + r, 16))]
                         for b, _ in RHS[i]}
                return _put(kvwop, lambda k: (slot + (NOPS * i + k),), r,
                            _operands(_combine(outer, RHS[i]), RHS))

            pace = _pacer(wkv_raw, zero, 4 * DC)
            return ([(pace, lambda n=n, r=r: measure(n, r))
                     for n in range(2) for r in range(0, DC, 64)]
                    + [(pace, lambda n=n: size(n)) for n in range(2)],
                    [(_pacer(xop, 2 * NQ * NC + zero), lambda: list(inverse.values()))]
                    + [(pace, lambda r=r, i=i: piece(r, i))
                       for r in range(0, 128, 16) for i in range(NOPS)])

        def prep_aw(u, s, zero):
            def put(i, row, values):
                return _put(awop, lambda k: (u // 2, i + k), pl.multiple_of(16 * (u % 2), 16) + row,
                            values)
            return _dim_major(
                lambda k, t: aw_raw[s, pl.ds(128 * k, 128), pl.ds(128 * t, 128)].astype(F32).T,
                _pacer(xop, 2 * NQ * NC + zero), shuf, put, True, zero, lag=5, gap=2)

        def q_proj(scale, c):
            def done(r, *both):
                for h, val in enumerate(both):
                    _store(q_s, 0, c * R + r * (R // 4), h * HD, val * scale)
            return _couple_product(lambda i: _beside(_load(xop, 2 * (NQ * c + i) + t) for t in range(2)),
                                   lambda i: _load(qwop, i), done)

        def kv_proj(c, slot):
            def done(o, val):
                row, col = _corner(o, R // 4, HD)
                _store((k_s, v_s)[col // (2 * HD)], 0, c * R + row, col % (2 * HD), val)
            return _block_product(lambda i: _load(cop, c, i), lambda i: _load(kvwop, slot + i), done)

        def q_scale(j):
            return unit[0, j, :1] * (HD ** -0.5 * LOG2E)

        def scores(h, blk):
            n = (blk + 1) * R
            s = lax.dot_general(_bf16(q_s[0, pl.ds(blk * R // 2, R // 2), pl.ds(h * HD, HD)]),
                                _bf16(k_s[0, :n // 2, pl.ds(h * HD, HD)]),
                                NT, preferred_element_type=F32)
            row = lax.broadcasted_iota(jnp.int32, (R, R), 0)
            col = lax.broadcasted_iota(jnp.int32, (R, R), 1)
            diag = jnp.where(col <= row, s[:, n - R:], MASKED)
            return diag if blk == 0 else jnp.concatenate([s[:, :n - R], diag], axis=1)

        def attend(scale, h, blk, s):
            n = (blk + 1) * R
            p = jnp.exp2(s - jnp.max(s, axis=1, keepdims=True))
            inv = _recip(jnp.sum(p, axis=1, keepdims=True)) * scale
            o = lax.dot_general(p.astype(BF16), _bf16(v_s[0, :n // 2, pl.ds(h * HD, HD)]), NN,
                                preferred_element_type=F32)
            return o * inv

        def pair_attention(j, zero, filler, sides, slack):
            blocks = [(h, 2 * c + u) for c in reversed(range(NC)) for u in (1, 0) for h in (0, 1)]
            plan = {}
            for pieces, span in sides:
                tiles = [(b, t) for b in blocks[span] for t in range(b[1] + 1)]
                for n, tile in enumerate(tiles):
                    plan.setdefault(tile, []).extend(_share(pieces, n, len(tiles)))

            def paced_scores(h, blk):
                s = scores(h, blk)
                for t in range(blk + 1):
                    _tie(plan.get(((h, blk), t), []), lambda lag: s[:, t * R:(t + 1) * R])
                return s

            todo, done = [[]] * 8, []
            v_scale = unit[1, j, :1]
            ahead = [paced_scores(*blocks[0])]
            for n, (h, blk) in enumerate(blocks):
                ahead += [paced_scores(*b) for b in blocks[n + 1:n + 2]]
                _run(todo[2 * (n % 4)])
                done.append(attend(v_scale, h, blk, ahead.pop(0)))
                _store(ctx, 0, pl.multiple_of(j * (S // 2), S // 2) + blk * (R // 2), h * HD, done[-1])
                if len(done) > slack:
                    _pacer(q_s, zero, S // 2)(_witness([done.pop(0)]))
                _run(todo[2 * (n % 4) + 1])
                if n % 4 == 3:
                    todo = filler(blk // 2)
            _run(sum(todo, []))

        c_parts = ((7, 6), (5, 4), (3, 2), (1, 0))
        x_parts = tuple(reversed(range(NC)))
        stages = ([cp_wkv(0, 0)] + [[cp_c(c) for c in part] for part in c_parts]
                  + [[cp_x(c)] for c in x_parts] + [cp_wq(1, 0)])
        stages[len(c_parts)] += cp_wq(0, 1)
        stages[len(c_parts) + 1] += cp_wkv(1, 1)

        def issue(i, zero):
            for k, stage in enumerate(stages):
                @pl.when(i == k)
                def _(stage=stage):
                    for cp in stage:
                        cp.start()
            return zero + i // NP

        zero = lax.fori_loop(0, len(stages), issue, jnp.int32(0))

        aw_raw[0] = jnp.zeros(aw_raw.shape[1:], BF16)
        wo_raw[0, :TILE // 2] = jnp.zeros((TILE // 2, TILE), U32)
        for cp in stages[0]:
            cp.wait()
        _now(sum(prep_wkv(0, 0, SLOT, zero), []))
        for n, part in enumerate(c_parts):
            for cp in stages[1 + n]:
                cp.wait()
            if n == 0:
                for cp in cp_wkv(2, 0):
                    cp.start()
            side = prep_wq(1, zero) if n == len(c_parts) - 1 else []
            for k, c in enumerate(part):
                prep_c(c)
                _run(_mingle(kv_proj(c, SLOT), _share(side, k, len(part))))
        scale, side = q_scale(0), sum(prep_wkv(1, 1, 0, zero), [])
        for n, c in enumerate(x_parts):
            for cp in stages[1 + len(c_parts) + n]:
                cp.wait()
            prep_x(c)
            _run(_mingle(q_proj(scale, c), _share(side, n, NC)))

        def pair_step(j, zero):
            for cp in cp_heads(j):
                cp.wait()

            @pl.when(j > 0)
            def _():
                for cp in cp_tiles(j):
                    cp.wait()

            @pl.when(j == NP // 2)
            def _():
                for cp in cp_a():
                    cp.start()

            for cp in cp_heads(j + 1) + cp_tiles(j + 1):
                cp.start()
            slot = j * SLOT
            scale = q_scale(j + 1)
            sizes, operands = prep_wkv(j + 2, j % 2, slot + SLOT, zero)
            side = [None] * 24 + _blend(prep_aw(aw_unit(j), j % 2, zero),
                                        sizes + [None] * 12 + operands)
            q_steps = sum((q_proj(scale, c) for c in reversed(range(NC))), [])
            history = []

            def filler(c):
                q = _share(q_steps, NC - 3 - c, NC - 2) if c < NC - 2 else []
                kv = kv_proj(c, slot)
                slots = []
                for n in range(4):
                    mine = _share(kv, n, 4)
                    early = len(mine) - len(mine) * 3 // 4
                    slots += [mine[:early] + _share(q, n, 4), mine[early:]]
                along = _share(side, NC - 2 - c, NC - 1) if c < NC - 1 else []
                steps = iter(_mingle(sum(slots, []), along, history))
                return [[next(steps) for _ in slot] for slot in slots]

            pair_attention(j, zero, filler, [(prep_wo(wo_unit(j), j % 2, zero), slice(10, None)),
                                             (prep_wq(j % 2, zero), slice(2, 12))], 3)
            return zero + j // NP

        zero = lax.fori_loop(0, NP - 1, pair_step, zero)

        @pl.loop(0, 2)
        def _(i):
            _pacer(shuf, 4 + zero * i)(jnp.zeros((8, 128), U32))

        for cp in cp_heads(NP - 1) + cp_tiles(NP - 1) + cp_a():
            cp.wait()
        cp_wo(NP - 1, 0).start()
        side = _blend(prep_wo(NP - 2, 1, zero), prep_awo(awoop0, 0, 0, zero), prep_xa(zero, zero))
        pair_attention(NP - 1, zero, lambda c: [[]] * 8, [(side, slice(2, None))], 4)
        return zero

    def rows(zero, awoop1, aoop, aqkv, oop, out_s):
        @pl.loop(0, 2)
        def _(i):
            aqkv[pl.ds(8 + 8 * i, 8), :HALO, :] = jnp.zeros((8, HALO, 128), F32)

        def cp_out(c, half):
            return pltpu.make_async_copy(
                out_s.at[half, c],
                out_hbm.at[pl.ds(pl.multiple_of(c * CH, CH), CH), pl.ds(half * DM, DM)],
                sem_out.at[half * NC + c])

        def cp_last(row, col, n, sem):
            return pltpu.make_async_copy(
                out_s.at[0, NC - 1, pl.ds(row, n), pl.ds(col, DM // 2)],
                out_hbm.at[pl.ds((NC - 1) * CH + row, n), pl.ds(col, DM // 2)], sem_x.at[sem])

        def prep_ctx(c, zero):
            base = pl.multiple_of(c * R, R)

            def piece(m, r, i):
                outer = {b: [_f32(ctx[0, pl.ds(base + ((2 * m + a2) * (S // 2) + (b // 2) * 64
                                                         + r2 * 32 + r), 8),
                                        pl.ds((b % 2) * HD, HD)])
                             for r2 in range(2) for a2 in range(2)] for b, _ in LHS[i]}
                return _put(oop, lambda k: (NOPS * i + k, m), 2 * r,
                            _operands(_combine(outer, LHS[i]), LHS))
            return [(_pacer(ctx, zero, NP * S // 2), lambda m=m, r=r, i=i: piece(m, r, i))
                    for m in range(NP // 2) for r in range(0, 32, 8) for i in range(NOPS)]

        def out_proj(half, c, lhs, rhs):
            steps = []
            for t in range(2):
                def done(o, val, t=t):
                    row, col = _corner(o, R // 2, 128)
                    out_s[half, c, pl.ds(row, R // 2), pl.ds(512 * t + col, 128)] = val.astype(BF16)
                steps += _block_product(lhs, lambda i, t=t: rhs(t, i), done)
            return steps

        def b_out_proj(c):
            return out_proj(1, c, lambda i: _beside(_load(oop, i, m) for m in range(NP // 2)),
                            lambda t, i: _load(woop, t, i))

        def a_out_proj(c, zero):
            return out_proj(0, c, lambda i: _bf16(aoop[zero + i]),
                            lambda t, i: _load((awoop0, awoop1)[t], i))

        def a_proj():
            steps = []
            for part in range(3):
                for t in range(2):
                    def done(o, val, part=part, t=t):
                        if part == 0:
                            val = val * (AD ** -0.5 * LOG2E)
                        row, plane = _corner(o, R // 2, 2)
                        aqkv[8 * part + plane + t, pl.ds(HALO + row, R // 2), :] = val

                    def rhs(i, part=part, t=t):
                        return _beside(_load(awop, 2 * part + m, i, pl.ds(64 * t, 64)) for m in range(2))
                    steps += _block_product(lambda i: _beside(_load(xaop, i, m) for m in range(2)),
                                            rhs, done, NT)
            return steps

        def a_attention(c, zero):
            query, logit, prob, mixed = {}, {}, {}, {}

            def dot(r, w):
                tot = None
                for t in range(8):
                    if (r, t) not in query:
                        query[r, t] = aqkv[t, pl.ds(HALO + r, 8), :]
                    pr = query[r, t] * aqkv[8 + t, pl.ds(HALO + r - DIL * w, 8), :]
                    tot = pr if tot is None else tot + pr
                logit[r, w] = tot
                if w == WIN - 1:
                    weights(r)
                return [tot]

            def weights(r):
                logits = [logit[r, w] for w in range(WIN)]
                logits = [x + pltpu.roll(x, 64, 1) for x in logits]
                logits = [x + pltpu.roll(x, 32, 1) for x in logits]
                if r < (WIN - 1) * DIL:
                    pos = c * CH + r + lax.broadcasted_iota(jnp.int32, (8, 128), 0)
                    logits = [x if w == 0 else jnp.where(pos >= DIL * w, x, MASKED)
                              for w, x in enumerate(logits)]
                top = logits[0]
                for x in logits[1:]:
                    top = jnp.maximum(top, x)
                e = [jnp.exp2(x - top) for x in logits]
                tot = e[0]
                for x in e[1:]:
                    tot = tot + x
                inv = _recip(tot)
                prob[r] = [x * inv for x in e]

            def mix(r, t, d, q):
                tot = None
                for w in range(WIN):
                    pr = prob[r + d][w] * aqkv[16 + t + 2 * q, pl.ds(HALO + r + d - DIL * w, 8), :]
                    tot = pr if tot is None else tot + pr
                mixed[r, t, d, q] = tot
                return [tot]

            def operands(r, t, i):
                outer = {b: [jnp.concatenate(
                    [mixed[r, t, (b // 2) * R + r2 * R // 2 + e, 2 * (b % 2) + a2] for e in (0, 8)],
                    axis=0) for r2 in range(2) for a2 in range(2)] for b, _ in LHS[i]}
                ops = _operands(_combine(outer, LHS[i]), LHS)
                for k, v in enumerate(ops):
                    _store(aoop, NOPS * i + k, r // 2, 128 * t, v)
                return ops

            groups = [d + e for d in range(0, CH, R // 2) for e in (0, 8)]

            def dots(r):
                return [lambda d=d, w=w: dot(r + d, w) for d in groups for w in range(WIN)]

            def mixes(r):
                return [work for t in range(2) for work in
                        [lambda t=t, d=d, q=q: mix(r, t, d, q) for d in groups for q in range(4)]
                        + [lambda t=t, i=i: operands(r, t, i) for i in range(NOPS)]]

            work = dots(0)
            for r in range(16, R // 2, 16):
                work += _blend(dots(r), mixes(r - 16))
            work += mixes(R // 2 - 16)
            return [(_pacer(aqkv, zero, HALO + CH), lambda g=work[i:i + 2]: sum((w() for w in g), []))
                    for i in range(0, len(work), 2)]

        cp_wo(NP - 1, 0).wait()
        _run(_mingle(_group(a_proj(), 2),
                     _blend(prep_ctx(0, zero),
                            prep_awo(awoop0, 0, 1, zero) + prep_awo(awoop1, 1, 0, zero)
                            + prep_awo(awoop1, 1, 1, zero),
                            prep_wo(NP - 1, 0, zero))))

        def attention_step(c, zero):
            steps = b_out_proj(c)
            _run(_mingle(steps[:-2], a_attention(c, zero)) + steps[-2:])
            cp_out(c, 1).start()

        def chunk_step(c, zero):
            attention_step(c, zero)
            aqkv[8:, :HALO, :] = aqkv[8:, CH:CH + HALO, :]
            side = prep_ctx(c + 1, zero)
            early = len(side) // 4
            steps = _group(a_out_proj(c, zero), 2)
            _run(_mingle(steps[:-3], _blend(prep_xa(c + 1, zero), side[:early])) + steps[-3:])
            cp_out(c, 0).start()
            steps = _group(a_proj(), 2)
            _run(_mingle(steps[:-4], side[early:]) + steps[-4:])
            return zero + c // NC

        zero = lax.fori_loop(0, NC - 1, chunk_step, zero)

        attention_step(NC - 1, zero)
        steps = a_out_proj(NC - 1, zero)
        parts = [cp_last(0, 0, CH, 0), cp_last(R, DM // 2, R, 1), cp_last(0, DM // 2, R, 2)]
        for cp, part in zip(parts, (steps[:NOPS * NOPS], steps[NOPS * NOPS:-NOPS], steps[-NOPS:])):
            _run(part)
            cp.start()
        for cp in ([cp_out(c, 1) for c in range(NC)] + [cp_out(c, 0) for c in range(NC - 1)] + parts):
            cp.wait()

    vmem = pltpu.VMEM
    zero = pl.run_scoped(
        heads,
        vmem((2 * NQ * NC + 1, R // 2, 128), BF16),
        vmem((NC, NOPS * NOPS, R // 2, 128), BF16),
        vmem((1, 2 * DM + 32, HD), U32),
        vmem((1, 4 * DC + 32, HD), U32),
        vmem((NQ, DM // 4, 128), BF16),
        vmem((NP * SLOT, 128, 128), BF16),
        vmem((1, S // 2 + 16, 2 * HD), U32),
        vmem((1, S // 2, 2 * HD), U32),
        vmem((1, S // 2, 2 * HD), U32),
        vmem((2, TILE, TILE), BF16),
        vmem((2, NP + 2, 8, 128), F32),
    )
    pl.run_scoped(
        lambda *refs: rows(zero, *refs),
        vmem((NOPS * NOPS, DM // 4, 128), BF16),
        vmem((NOPS * NOPS, R // 4, DM // 4), U32),
        vmem((24, HALO + CH + 16, 128), F32),
        vmem((NOPS * NOPS, NP // 2, R // 2, HD), BF16),
        vmem((2, NC, CH, DM), BF16),
    )


@jax.jit
def pallas_concat_heads__sliding_local_dilated__compressed_kv_cla__prompt_kernel(
    A_x: jax.Array,
    A_wqkv: jax.Array,
    A_wo: jax.Array,
    B_x: jax.Array,
    B_c_kv: jax.Array,
    B_w_q: jax.Array,
    B_w_uk: jax.Array,
    B_w_uv: jax.Array,
    B_w_o: jax.Array,
):
    vmem = pltpu.VMEM
    dma = pltpu.SemaphoreType.DMA
    scratch = [
        vmem((24, 128), F32),
        vmem((1, NP * S // 2 + 16, 2 * HD), U32),
        vmem((1, TILE + 8, TILE), U32),
        vmem((2, NOPS * NOPS, NP * HD // 2, 128), BF16),
        vmem((6, NOPS * NOPS, DM // 4, 128), BF16),
        vmem((NOPS * NOPS, DM // 4, 128), BF16),
        vmem((NC + 1, CH, DM), BF16),
        vmem((NOPS * NOPS, 2, R // 2, 128), BF16),
        vmem((NC + 1, CH, DC), BF16),
        vmem((5, 16 * PITCH + 48, 128), F32),
        dma((NC,)), dma((NC,)), dma((10,)), dma((2,)), dma((2 * NC,)),
    ]
    out = pl.pallas_call(
        _kernel,
        out_shape=jax.ShapeDtypeStruct((S, 2 * DM), BF16),
        in_specs=[pl.BlockSpec(memory_space=pl.ANY)] * 9,
        out_specs=pl.BlockSpec(memory_space=pl.ANY),
        scratch_shapes=scratch,
        compiler_params=pltpu.CompilerParams(vmem_limit_bytes=127 * 2**20),
        name="fused_local_and_latent_attention",
    )(
        A_x.reshape(S, DM), A_wqkv, A_wo,
        B_x.reshape(S, DM), B_c_kv.reshape(S, DC),
        B_w_q, B_w_uk, B_w_uv, B_w_o.reshape(NH * HD, DM),
    )
    return out.reshape(1, S, 2 * DM)
```
